```python
import jax
import jax.numpy as jnp

def _softmax(x, axis=-1):
    return jax.nn.softmax(x, axis=axis)
def _gelu(x):
    return jax.nn.gelu(x, approximate=True)
def _silu(x):
    return jax.nn.silu(x)
def _sigmoid(x):
    return jax.nn.sigmoid(x)
def _layernorm(x, axis=-1, eps=1e-5):
    m = jnp.mean(x, axis=axis, keepdims=True)
    v = jnp.var(x, axis=axis, keepdims=True)
    return (x - m) / jnp.sqrt(v + eps)
def _scatter_add(tgt, idx, src, axis=0):
    return tgt.at[idx].add(src)
def _segment_sum(src, seg, n):
    return jax.ops.segment_sum(src, seg, n)
class _Rng:
    def __init__(self, key):
        self._k = key
    def _next(self):
        self._k, sub = jax.random.split(self._k)
        return sub
    def normal(self, shape):
        return jax.random.normal(self._next(), shape, dtype=jnp.bfloat16)
    def randint(self, lo, hi, shape):
        return jax.random.randint(self._next(), shape, lo, hi, dtype=jnp.int32)
    def uniform(self, shape, lo=0.0, hi=1.0):
        return jax.random.uniform(self._next(), shape, jnp.bfloat16, lo, hi)
    def permutation(self, n):
        return jax.random.permutation(self._next(), n)


kernel_name = 'interleave_layers__compressed_kv_cla__moe_arch_mod__decode'

def setup_inputs():
    _rng = _Rng(jax.random.key(int.from_bytes(__import__("os").urandom(4), "little")))
    _w = (lambda a: (lambda t: t.astype(jnp.bfloat16) if jnp.issubdtype(t.dtype, jnp.floating) else t)(jnp.asarray(a)))
    def _A_setup():
        B, H, Sq, Sk, D, M = 1, 32, 1, 4096, 128, 640
        Dc = 4 * D
        return {
            "x": _w((lambda *s: _rng.normal(s) * 0.05)(B, Sq, M)),
            "c_kv": _w((lambda *s: _rng.normal(s) * 0.05)(B, Sk, Dc)),
            "w_q": _w((lambda *s: _rng.normal(s) * 0.05)(M, H, D) * (M ** -0.5)),
            "w_uk": _w((lambda *s: _rng.normal(s) * 0.05)(Dc, H, D) * (Dc ** -0.5)),
            "w_uv": _w((lambda *s: _rng.normal(s) * 0.05)(Dc, H, D) * (Dc ** -0.5)),
            "w_o": _w((lambda *s: _rng.normal(s) * 0.05)(H, D, M) * ((H * D) ** -0.5)),
        }
    _A_in = _A_setup()

    def _B_setup():
        B, S, D, F, C = 1, 1, 640, 1728, 1
        return {
            "x": _w((lambda *s: _rng.normal(s) * 0.05)(B, S, D)),
            "w_r": _w((lambda *s: _rng.normal(s) * 0.05)(D)),
            "w_gate": _w((lambda *s: _rng.normal(s) * 0.05)(D, F)),
            "w_up": _w((lambda *s: _rng.normal(s) * 0.05)(D, F)),
            "w_down": _w((lambda *s: _rng.normal(s) * 0.05)(F, D)),
        }
    _B_in = _B_setup()

    return {
        "A_x": _A_in["x"],
        "A_c_kv": _A_in["c_kv"],
        "A_w_q": _A_in["w_q"],
        "A_w_uk": _A_in["w_uk"],
        "A_w_uv": _A_in["w_uv"],
        "A_w_o": _A_in["w_o"],
        "B_x": _B_in["x"],
        "B_w_r": _B_in["w_r"],
        "B_w_gate": _B_in["w_gate"],
        "B_w_up": _B_in["w_up"],
        "B_w_down": _B_in["w_down"],
    }

def reference(A_x, A_c_kv, A_w_q, A_w_uk, A_w_uv, A_w_o, B_x, B_w_r, B_w_gate, B_w_up, B_w_down):
    def _A_ref(x, c_kv, w_q, w_uk, w_uv, w_o):
        B, Sq, M = x.shape[0], x.shape[1], x.shape[2]
        Sk = c_kv.shape[1]
        H, D = w_q.shape[1], w_q.shape[2]
        q = jnp.einsum("bqm,mhd->bhqd", x, w_q)
        k = jnp.einsum("bkc,chd->bhkd", c_kv, w_uk)
        v = jnp.einsum("bkc,chd->bhkd", c_kv, w_uv)
        scores = jnp.einsum("bhqd,bhkd->bhqk", q, k) * (D ** -0.5)
        off = Sk - Sq
        qi = jnp.arange(Sq)[:, None]
        kj = jnp.arange(Sk)[None, :]
        cmask = kj <= (qi + off)
        scores = jnp.where(cmask[None, None], scores, -1e9)
        p = _softmax(scores, axis=-1)
        ctx = jnp.einsum("bhqk,bhkd->bhqd", p, v)
        return jnp.einsum("bhqd,hdm->bqm", ctx, w_o)

    def _B_ref(x, w_r, w_gate, w_up, w_down):
        B, S, D = x.shape
        C = 1
        r = x @ w_r
        idx = jnp.argsort(-r, axis=-1)[:, :C]
        idx_e = jnp.repeat(idx.reshape(B, C, 1), D, axis=2)
        x_sel = jnp.take_along_axis(x, idx_e, axis=1)
        g = _silu(x_sel @ w_gate)
        u = x_sel @ w_up
        y = (g * u) @ w_down
        r_sel = _sigmoid(jnp.take_along_axis(r, idx, axis=1))
        y = y * r_sel.reshape(B, C, 1)
        b_off = (jnp.arange(B) * S).reshape(B, 1)
        flat_idx = (idx + b_off).reshape(B * C)
        zero = (x * 0.0).reshape(B * S, D)
        upd = _scatter_add(zero, flat_idx, y.reshape(B * C, D), axis=0)
        return x + upd.reshape(B, S, D)

    x = A_x
    x = x + _A_ref(_layernorm(x, axis=-1), A_c_kv, A_w_q, A_w_uk, A_w_uv, A_w_o)
    x = x + _B_ref(_layernorm(x, axis=-1), B_w_r, B_w_gate, B_w_up, B_w_down)
    x = x + _A_ref(_layernorm(x, axis=-1), A_c_kv, A_w_q, A_w_uk, A_w_uv, A_w_o)
    x = x + _B_ref(_layernorm(x, axis=-1), B_w_r, B_w_gate, B_w_up, B_w_down)
    return x
```

```python
import functools

import jax
import jax.numpy as jnp
from jax import lax
import jax.experimental.pallas as pl
import jax.experimental.pallas.tpu as pltpu

f32 = jnp.float32
bf16 = jnp.bfloat16
u32 = jnp.uint32
i32 = jnp.int32

M = 640
H = 32
D = 128
DC = 512
SK = 4096
F = 1728
NM = M // 128
NC = DC // 128
NK = SK // 128
NF = 14
EPS = 1e-5
SCALE = float(D) ** -0.5
KB = 8
NB = NK // KB


def _dot(a, b):
    return jnp.dot(a, b, preferred_element_type=f32)


def _rbf(x):
    return x.astype(bf16).astype(f32)


def _tile(ref, *idx):
    return pltpu.bitcast(ref[idx], bf16)


def _stats(xs):
    s = xs[0] + xs[1] + xs[2] + xs[3] + xs[4]
    mean = jnp.sum(s, axis=1, keepdims=True) * (1.0 / M)
    ds = [x - mean for x in xs]
    q = ds[0] * ds[0] + ds[1] * ds[1] + ds[2] * ds[2] + ds[3] * ds[3] + ds[4] * ds[4]
    var = jnp.sum(q, axis=1, keepdims=True) * (1.0 / M)
    rstd = 1.0 / jnp.sqrt(var + EPS)
    return mean, rstd


def _router(lns, wr):
    s = lns[0] * wr[0] + lns[1] * wr[1] + lns[2] * wr[2] + lns[3] * wr[3] + lns[4] * wr[4]
    r = jnp.sum(s, axis=1, keepdims=True)
    return jax.nn.sigmoid(r)


def _rowsum(x):
    return jnp.broadcast_to(jnp.sum(x, axis=0, keepdims=True), x.shape)


def _silu(g):
    return g * jax.nn.sigmoid(g)


def _kernel(x_hbm, ckv_hbm, wq_hbm, wuk_hbm, wuv_hbm, wo_hbm, wr_hbm, wg_hbm, wu_hbm, wd_hbm,
            o_ref,
            x_v, wr_v, lq, luk, luv, lckv, lo, lg, lu, ld,
            wq, wukt, wuv, ckvt, gt, ut,
            csq, csg, csu, qa_s, cc_s, ctx_s, hh_s, x_s,
            sems):
    row8 = lax.broadcasted_iota(i32, (8, 128), 0)
    masks = [row8 == r for r in range(8)]

    copies = {}
    order = []

    def add(name, pairs):
        sem = sems.at[len(copies)]
        cs = [pltpu.make_async_copy(s, d, sem) for s, d in pairs]
        copies[name] = cs
        order.append(name)

    add("x", [(x_hbm, x_v)])
    add("wr", [(wr_hbm, wr_v)])
    for i in range(NM):
        add(("q", i), [(wq_hbm.at[pl.ds(i * 128, 128)], lq.at[pl.ds(i * 128, 128)])])
    for i in range(NC):
        add(("uk", i), [(wuk_hbm.at[pl.ds(i * 128, 128)], luk.at[pl.ds(i * 128, 128)])])
    ckv32 = ckv_hbm.at[0].bitcast(u32)
    for b in range(NB):
        add(("ckv", b), [(ckv32.at[pl.ds(b * 512, 512), pl.ds(ct * 128, 128)],
                          lckv.at[ct, pl.ds(b * 512, 512)]) for ct in range(NC)])
    FS = [(0, 896), (896, F - 896)]
    for i, (s, n) in enumerate(FS):
        add(("g", i), [(wg_hbm.at[pl.ds(s, n)], lg.at[pl.ds(s, n)])])
    for i, (s, n) in enumerate(FS):
        add(("u", i), [(wu_hbm.at[pl.ds(s, n)], lu.at[pl.ds(s, n)])])
    for i in range(NC):
        add(("uv", i), [(wuv_hbm.at[pl.ds(i * 128, 128)], luv.at[pl.ds(i * 128, 128)])])
    for g in range(4):
        add(("o", g), [(wo_hbm.at[pl.ds(g * 8, 8)], lo.at[pl.ds(g * 8, 8)])])
    DS = [(0, 512), (512, 512), (1024, 512), (1536, F - 1536)]
    for i, (s, n) in enumerate(DS):
        add(("d", i), [(wd_hbm.at[pl.ds(s, n)], ld.at[pl.ds(s, n)])])

    for name in order:
        for c in copies[name]:
            c.start()

    def wait(name):
        for c in copies[name]:
            c.wait()

    names = list(copies)

    def wait_dyn(first_name, i, pairs_fn):
        base = names.index(first_name)
        for s, d in pairs_fn(i):
            pltpu.make_async_copy(s, d, sems.at[base + i]).wait()

    wait("x")
    wait("wr")
    xr = x_v[0].astype(f32)
    x0 = [jnp.broadcast_to(xr[:, n * 128:(n + 1) * 128], (8, 128)) for n in range(NM)]
    wrf = wr_v[...].astype(f32)
    wr = [jnp.broadcast_to(wrf[n:n + 1, :], (8, 128)) for n in range(NM)]
    for n in range(NM):
        x_s[n] = x0[n]
    mean0, rstd0 = _stats(x0)
    ones8 = jnp.ones((8, 128), f32)
    zero8 = jnp.zeros((8, 128), f32)

    def a_body(kt, carry):
        raw, cs = carry
        s = pl.multiple_of(kt * 128, 128)
        wait_dyn(("q", 0), kt, lambda i: [(wq_hbm.at[pl.ds(s, 128)], lq.at[pl.ds(s, 128)])])
        t = jnp.swapaxes(lq[pl.ds(s, 128)], 0, 1)
        s2 = pl.multiple_of(kt * 64, 64)
        for h in range(H):
            wq[h, pl.ds(s2, 64), :] = pltpu.bitcast(t[h], u32)
        lhs = jnp.concatenate([x_s[kt], ones8], axis=0)
        raw, cs = list(raw), list(cs)
        for h in range(H):
            g, r = divmod(h, 8)
            out = _dot(lhs, pltpu.bitcast(wq[h, pl.ds(s2, 64), :], bf16))
            raw[g] = jnp.where(masks[r], raw[g] + out[0:8], raw[g])
            cs[g] = jnp.where(masks[r], cs[g] + out[8:16], cs[g])
        return tuple(raw), tuple(cs)

    raw, cs = lax.fori_loop(0, NM, a_body, ((zero8,) * 4, (zero8,) * 4))
    for g in range(4):
        csq[g] = cs[g]
    q = [rstd0 * (raw[g] - mean0 * cs[g]) for g in range(4)]

    def b_body(ct, _):
        s = pl.multiple_of(ct * 128, 128)
        wait_dyn(("uk", 0), ct, lambda i: [(wuk_hbm.at[pl.ds(s, 128)], luk.at[pl.ds(s, 128)])])
        t = jnp.swapaxes(luk[pl.ds(s, 128)], 0, 1)
        for h in range(H):
            wukt[h, ct] = pltpu.bitcast(t[h].T, u32)
        qa = [zero8] * 4
        for h in range(H):
            g, r = divmod(h, 8)
            out = _dot(q[g], pltpu.bitcast(wukt[h, ct], bf16))
            qa[g] = jnp.where(masks[r], out, qa[g])
        qa_s[ct] = jnp.concatenate(qa, axis=0)
        return _

    lax.fori_loop(0, NC, b_body, 0)

    def cd_body(b, carry):
        m, l, acc = carry
        s = pl.multiple_of(b * 512, 512)
        wait_dyn(("ckv", 0), b, lambda i: [(ckv32.at[pl.ds(s, 512), pl.ds(ct * 128, 128)],
                                            lckv.at[ct, pl.ds(s, 512)]) for ct in range(NC)])
        ss = []
        for j in range(KB):
            kt = b * KB + j
            sk = pl.multiple_of(s + j * 64, 64)
            sc = None
            for ct in range(NC):
                t = pltpu.bitcast(lckv[ct, pl.ds(sk, 64), :], bf16).T
                ckvt[kt, ct] = pltpu.bitcast(t, u32)
                o = _dot(qa_s[ct], t)
                sc = o if sc is None else sc + o
            ss.append(sc * SCALE)
        mb = ss[0]
        for j in range(1, KB):
            mb = jnp.maximum(mb, ss[j])
        m_new = jnp.maximum(m, jnp.max(mb, axis=1, keepdims=True))
        alpha = jnp.exp(m - m_new)
        ps = [jnp.exp(sj - m_new) for sj in ss]
        lb = ps[0]
        for j in range(1, KB):
            lb = lb + ps[j]
        l = l * alpha + lb
        acc = [a * alpha for a in acc]
        for j in range(KB):
            sk = pl.multiple_of(s + j * 64, 64)
            for ct in range(NC):
                acc[ct] = acc[ct] + _dot(ps[j], pltpu.bitcast(lckv[ct, pl.ds(sk, 64), :], bf16))
        return m_new, l, acc

    m_init = jnp.full((H, 128), -jnp.inf, f32)
    _, l, acc = lax.fori_loop(0, NB, cd_body,
                              (m_init, jnp.zeros((H, 128), f32),
                               [jnp.zeros((H, 128), f32)] * NC))
    linv = 1.0 / jnp.sum(l, axis=1, keepdims=True)
    for ct in range(NC):
        cc_s[ct] = acc[ct]

    def transpose_ffn(land, dst, fam):
        def body(ft, _):
            s = pl.multiple_of(ft * 128, 128)
            for kt in range(NM):
                dst[ft, kt] = pltpu.bitcast(land[pl.ds(s, 128), pl.ds(kt * 128, 128)].T, u32)
            return _
        wait((fam, 0))
        lax.fori_loop(0, 7, body, 0)
        wait((fam, 1))
        lax.fori_loop(7, 13, body, 0)
        for kt in range(NM):
            t = land[pl.ds(13 * 128, 64), pl.ds(kt * 128, 128)]
            t = jnp.concatenate([t, jnp.zeros((64, 128), bf16)], axis=0)
            dst[13, kt] = pltpu.bitcast(t.T, u32)

    transpose_ffn(lg, gt, "g")
    transpose_ffn(lu, ut, "u")

    def e_body(ct, ctx):
        s = pl.multiple_of(ct * 128, 128)
        wait_dyn(("uv", 0), ct, lambda i: [(wuv_hbm.at[pl.ds(s, 128)], luv.at[pl.ds(s, 128)])])
        t = jnp.swapaxes(luv[pl.ds(s, 128)], 0, 1)
        s2 = pl.multiple_of(ct * 64, 64)
        for h in range(H):
            wuv[h, pl.ds(s2, 64), :] = pltpu.bitcast(t[h], u32)
        ctx = list(ctx)
        cc = cc_s[ct]
        for h in range(H):
            g, r = divmod(h, 8)
            out = _dot(cc[g * 8:(g + 1) * 8], pltpu.bitcast(wuv[h, pl.ds(s2, 64), :], bf16))
            ctx[g] = jnp.where(masks[r], ctx[g] + out, ctx[g])
        return tuple(ctx)

    ctx = lax.fori_loop(0, NC, e_body, (zero8,) * 4)
    for g in range(4):
        ctx_s[g] = ctx[g] * linv[g * 8:(g + 1) * 8]

    def f_body(g, acc):
        s = pl.multiple_of(g * 8, 8)
        wait_dyn(("o", 0), g, lambda i: [(wo_hbm.at[pl.ds(s, 8)], lo.at[pl.ds(s, 8)])])
        acc = list(acc)
        cg = ctx_s[g]
        for r in range(8):
            lhs = jnp.where(masks[r], cg, 0.0)
            for n in range(NM):
                acc[n] = acc[n] + _dot(lhs, lo[g * 8 + r, :, pl.ds(n * 128, 128)])
        return tuple(acc)

    acc = lax.fori_loop(0, 4, f_body, (zero8,) * NM)
    x1 = [_rbf(x0[n] + _rbf(_rowsum(acc[n]))) for n in range(NM)]

    mean1, rstd1 = _stats(x1)
    ln1 = [(x - mean1) * rstd1 for x in x1]
    sig1 = _router(ln1, wr)
    lhs1 = [jnp.concatenate([x1[kt], ones8], axis=0) for kt in range(NM)]

    def g_body(ft, _):
        og = ou = None
        for kt in range(NM):
            a = _dot(lhs1[kt], pltpu.bitcast(gt[ft, kt], bf16))
            b = _dot(lhs1[kt], pltpu.bitcast(ut[ft, kt], bf16))
            og = a if og is None else og + a
            ou = b if ou is None else ou + b
        csg[ft] = og[8:16]
        csu[ft] = ou[8:16]
        g = rstd1 * (og[0:8] - mean1 * og[8:16])
        u = rstd1 * (ou[0:8] - mean1 * ou[8:16])
        hh_s[ft] = _silu(g) * u
        return _

    lax.fori_loop(0, NF, g_body, 0)

    def down(ft, n, hh):
        if ft < 13:
            return _dot(hh, ld[pl.ds(ft * 128, 128), pl.ds(n * 128, 128)])
        return _dot(hh[:, :64], ld[pl.ds(13 * 128, 64), pl.ds(n * 128, 128)])

    y = [None] * NM
    for i, (s, nrows) in enumerate(DS):
        wait(("d", i))
        for ft in range(s // 128, (s + nrows + 127) // 128):
            hh = hh_s[ft]
            for n in range(NM):
                o = down(ft, n, hh)
                y[n] = o if y[n] is None else y[n] + o
    x2 = [_rbf(x1[n] + _rbf(ln1[n] + _rbf(y[n] * sig1))) for n in range(NM)]

    mean2, rstd2 = _stats(x2)
    q = []
    for g in range(4):
        rawg = zero8
        for r in range(8):
            h = g * 8 + r
            o = None
            for kt in range(NM):
                t = _dot(x2[kt], _tile(wq, h, pl.ds(kt * 64, 64)))
                o = t if o is None else o + t
            rawg = jnp.where(masks[r], o, rawg)
        q.append(rstd2 * (rawg - mean2 * csq[g]))
    qa = []
    for ct in range(NC):
        qg = [zero8] * 4
        for h in range(H):
            g, r = divmod(h, 8)
            qg[g] = jnp.where(masks[r], _dot(q[g], _tile(wukt, h, ct)), qg[g])
        qa.append(jnp.concatenate(qg, axis=0))

    def scores(b):
        ss = []
        for j in range(KB):
            kt = b * KB + j
            sc = None
            for ct in range(NC):
                o = _dot(qa[ct], _tile(ckvt, kt, ct))
                sc = o if sc is None else sc + o
            ss.append(sc * SCALE)
        return ss

    def soft(ss, m, l):
        mb = ss[0]
        for j in range(1, KB):
            mb = jnp.maximum(mb, ss[j])
        mb = jnp.max(mb, axis=1, keepdims=True)
        m_new = mb if m is None else jnp.maximum(m, mb)
        ps = [jnp.exp(sj - m_new) for sj in ss]
        lb = ps[0]
        for j in range(1, KB):
            lb = lb + ps[j]
        if m is None:
            return ps, m_new, lb, None
        alpha = jnp.exp(m - m_new)
        return ps, m_new, l * alpha + lb, alpha

    def ctxc(b, ps, alpha, acc):
        if acc is not None:
            acc = [a * alpha for a in acc]
        else:
            acc = [None] * NC
        acc = list(acc)
        last = b == NB - 1
        seq = ([(j, ct) for ct in range(NC) for j in range(KB)] if last
               else [(j, ct) for j in range(KB) for ct in range(NC)])
        for j, ct in seq:
            kt = b * KB + j
            o = _dot(ps[j], _tile(lckv, ct, pl.ds(kt * 64, 64)))
            acc[ct] = o if acc[ct] is None else acc[ct] + o
        return acc

    s0 = scores(0)
    s1 = scores(1)
    p0, m, l, al0 = soft(s0, None, None)
    acc = ctxc(0, p0, None, None)
    s2 = scores(2)
    p1, m, l, al1 = soft(s1, m, l)
    acc = ctxc(1, p1, al1, acc)
    s3 = scores(3)
    p2, m, l, al2 = soft(s2, m, l)
    acc = ctxc(2, p2, al2, acc)
    p3, m, l, al3 = soft(s3, m, l)
    acc = ctxc(3, p3, al3, acc)
    linv = 1.0 / jnp.sum(l, axis=1, keepdims=True)

    ctx = [zero8] * 4
    for ct in range(NC):
        for h in range(H):
            g, r = divmod(h, 8)
            o = _dot(acc[ct][g * 8:(g + 1) * 8], _tile(wuv, h, pl.ds(ct * 64, 64)))
            ctx[g] = jnp.where(masks[r], ctx[g] + o, ctx[g])
    ctx = [ctx[g] * linv[g * 8:(g + 1) * 8] for g in range(4)]
    x3 = []
    for n in range(NM):
        a = None
        for h in range(H):
            g, r = divmod(h, 8)
            o = _dot(jnp.where(masks[r], ctx[g], 0.0), lo[h, :, pl.ds(n * 128, 128)])
            a = o if a is None else a + o
        x3.append(_rbf(x2[n] + _rbf(_rowsum(a))))
    mean3, rstd3 = _stats(x3)
    ln3 = [(x - mean3) * rstd3 for x in x3]
    sig3 = _router(ln3, wr)
    hh = []
    for ft in range(NF):
        og = ou = None
        for kt in range(NM):
            a = _dot(x3[kt], _tile(gt, ft, kt))
            b = _dot(x3[kt], _tile(ut, ft, kt))
            og = a if og is None else og + a
            ou = b if ou is None else ou + b
        g = rstd3 * (og - mean3 * csg[ft])
        u = rstd3 * (ou - mean3 * csu[ft])
        hh.append(_silu(g) * u)
    y = [None] * NM
    for ft in range(NF):
        for n in range(NM):
            o = down(ft, n, hh[ft])
            y[n] = o if y[n] is None else y[n] + o
    x4 = [x3[n] + _rbf(ln3[n] + _rbf(y[n] * sig3)) for n in range(NM)]
    out = jnp.concatenate([x[0:1, :] for x in x4], axis=1)
    o_ref[0] = out.astype(bf16)


@jax.jit
def pallas_interleave_layers__compressed_kv_cla__moe_arch_mod__decode_kernel(
    A_x: jax.Array,
    A_c_kv: jax.Array,
    A_w_q: jax.Array,
    A_w_uk: jax.Array,
    A_w_uv: jax.Array,
    A_w_o: jax.Array,
    B_x: jax.Array,
    B_w_r: jax.Array,
    B_w_gate: jax.Array,
    B_w_up: jax.Array,
    B_w_down: jax.Array,
):
    del B_x
    any_spec = pl.BlockSpec(memory_space=pl.ANY)
    V = pltpu.VMEM
    scratch = [
        V((1, 1, M), bf16),
        V((NM, 128), bf16),
        V((M, H, D), bf16),
        V((DC, H, D), bf16),
        V((DC, H, D), bf16),
        V((NC, SK // 2, 128), u32),
        V((H, D, M), bf16),
        V((F, M), bf16),
        V((F, M), bf16),
        V((F, M), bf16),
        V((H, M // 2, D), u32),
        V((H, NC, D // 2, 128), u32),
        V((H, DC // 2, D), u32),
        V((NK, NC, 64, 128), u32),
        V((NF, NM, 64, 128), u32),
        V((NF, NM, 64, 128), u32),
        V((4, 8, 128), f32),
        V((NF, 8, 128), f32),
        V((NF, 8, 128), f32),
        V((NC, H, 128), f32),
        V((NC, H, 128), f32),
        V((4, 8, 128), f32),
        V((NF, 8, 128), f32),
        V((NM, 8, 128), f32),
        pltpu.SemaphoreType.DMA((32,)),
    ]
    return pl.pallas_call(
        _kernel,
        out_shape=jax.ShapeDtypeStruct((1, 1, M), bf16),
        in_specs=[any_spec] * 10,
        out_specs=pl.BlockSpec(memory_space=pltpu.VMEM),
        scratch_shapes=scratch,
        compiler_params=pltpu.CompilerParams(
            vmem_limit_bytes=100 * 1024 * 1024,
            disable_semaphore_checks=True,
        ),
    )(A_x, A_c_kv, A_w_q, A_w_uk, A_w_uv, A_w_o, B_w_r.reshape(NM, 128),
      B_w_gate.T, B_w_up.T, B_w_down)
```

```python
import functools

import jax
import jax.numpy as jnp
from jax import lax
import jax.experimental.pallas as pl
import jax.experimental.pallas.tpu as pltpu

f32 = jnp.float32
bf16 = jnp.bfloat16
u32 = jnp.uint32
i32 = jnp.int32

M = 640
H = 32
D = 128
DC = 512
SK = 4096
F = 1728
NM = M // 128
NC = DC // 128
NK = SK // 128
NF = 14
EPS = 1e-5
SCALE = float(D) ** -0.5
KB = 8
NB = NK // KB


def _dot(a, b):
    return jnp.dot(a, b, preferred_element_type=f32)


def _rbf(x):
    return x.astype(bf16).astype(f32)


def _tile(ref, *idx):
    return pltpu.bitcast(ref[idx], bf16)


def _stats(xs):
    s = xs[0] + xs[1] + xs[2] + xs[3] + xs[4]
    mean = jnp.sum(s, axis=1, keepdims=True) * (1.0 / M)
    ds = [x - mean for x in xs]
    q = ds[0] * ds[0] + ds[1] * ds[1] + ds[2] * ds[2] + ds[3] * ds[3] + ds[4] * ds[4]
    var = jnp.sum(q, axis=1, keepdims=True) * (1.0 / M)
    rstd = 1.0 / jnp.sqrt(var + EPS)
    return mean, rstd


def _router(lns, wr):
    s = lns[0] * wr[0] + lns[1] * wr[1] + lns[2] * wr[2] + lns[3] * wr[3] + lns[4] * wr[4]
    r = jnp.sum(s, axis=1, keepdims=True)
    return jax.nn.sigmoid(r)


def _rowsum(x):
    return jnp.broadcast_to(jnp.sum(x, axis=0, keepdims=True), x.shape)


def _silu(g):
    return g * jax.nn.sigmoid(g)


def _kernel(x_hbm, ckv_hbm, wq_hbm, wuk_hbm, wuv_hbm, wo_hbm, wr_hbm, wg_hbm, wu_hbm, wd_hbm,
            o_ref,
            x_v, wr_v, lq, luk, luv, lckv, lo, lg, lu, ld,
            wq, wukt, wuv, ckvt, gt, ut,
            csq, csg, csu, qa_s, cc_s, ctx_s, hh_s, x_s,
            sems):
    row8 = lax.broadcasted_iota(i32, (8, 128), 0)
    masks = [row8 == r for r in range(8)]

    copies = {}
    order = []

    def add(name, pairs):
        sem = sems.at[len(copies)]
        cs = [pltpu.make_async_copy(s, d, sem) for s, d in pairs]
        copies[name] = cs
        order.append(name)

    add("x", [(x_hbm, x_v)])
    add("wr", [(wr_hbm, wr_v)])
    for i in range(NM):
        add(("q", i), [(wq_hbm.at[pl.ds(i * 128, 128)], lq.at[pl.ds(i * 128, 128)])])
    for i in range(NC):
        add(("uk", i), [(wuk_hbm.at[pl.ds(i * 128, 128)], luk.at[pl.ds(i * 128, 128)])])
    ckv32 = ckv_hbm.at[0].bitcast(u32)
    for b in range(NB):
        add(("ckv", b), [(ckv32.at[pl.ds(b * 512, 512), pl.ds(ct * 128, 128)],
                          lckv.at[ct, pl.ds(b * 512, 512)]) for ct in range(NC)])
    FS = [(0, 896), (896, F - 896)]
    for i, (s, n) in enumerate(FS):
        add(("g", i), [(wg_hbm.at[pl.ds(s, n)], lg.at[pl.ds(s, n)])])
    for i, (s, n) in enumerate(FS):
        add(("u", i), [(wu_hbm.at[pl.ds(s, n)], lu.at[pl.ds(s, n)])])
    for i in range(NC):
        add(("uv", i), [(wuv_hbm.at[pl.ds(i * 128, 128)], luv.at[pl.ds(i * 128, 128)])])
    for g in range(4):
        add(("o", g), [(wo_hbm.at[pl.ds(g * 8, 8)], lo.at[pl.ds(g * 8, 8)])])
    DS = [(0, 512), (512, 512), (1024, 512), (1536, F - 1536)]
    for i, (s, n) in enumerate(DS):
        add(("d", i), [(wd_hbm.at[pl.ds(s, n)], ld.at[pl.ds(s, n)])])

    for name in order:
        for c in copies[name]:
            c.start()

    def wait(name):
        for c in copies[name]:
            c.wait()

    names = list(copies)

    def wait_dyn(first_name, i, pairs_fn):
        base = names.index(first_name)
        for s, d in pairs_fn(i):
            pltpu.make_async_copy(s, d, sems.at[base + i]).wait()

    wait("x")
    wait("wr")
    xr = x_v[0].astype(f32)
    x0 = [jnp.broadcast_to(xr[:, n * 128:(n + 1) * 128], (8, 128)) for n in range(NM)]
    wrf = wr_v[...].astype(f32)
    wr = [jnp.broadcast_to(wrf[n:n + 1, :], (8, 128)) for n in range(NM)]
    for n in range(NM):
        x_s[n] = x0[n]
    mean0, rstd0 = _stats(x0)
    ones8 = jnp.ones((8, 128), f32)
    zero8 = jnp.zeros((8, 128), f32)

    def a_body(kt, carry):
        raw, cs = carry
        s = pl.multiple_of(kt * 128, 128)
        wait_dyn(("q", 0), kt, lambda i: [(wq_hbm.at[pl.ds(s, 128)], lq.at[pl.ds(s, 128)])])
        t = jnp.swapaxes(lq[pl.ds(s, 128)], 0, 1)
        s2 = pl.multiple_of(kt * 64, 64)
        for h in range(H):
            wq[h, pl.ds(s2, 64), :] = pltpu.bitcast(t[h], u32)
        lhs = jnp.concatenate([x_s[kt], ones8], axis=0)
        raw, cs = list(raw), list(cs)
        for h in range(H):
            g, r = divmod(h, 8)
            out = _dot(lhs, pltpu.bitcast(wq[h, pl.ds(s2, 64), :], bf16))
            raw[g] = jnp.where(masks[r], raw[g] + out[0:8], raw[g])
            cs[g] = jnp.where(masks[r], cs[g] + out[8:16], cs[g])
        return tuple(raw), tuple(cs)

    raw, cs = lax.fori_loop(0, NM, a_body, ((zero8,) * 4, (zero8,) * 4))
    for g in range(4):
        csq[g] = cs[g]
    q = [rstd0 * (raw[g] - mean0 * cs[g]) for g in range(4)]

    def b_body(ct, _):
        s = pl.multiple_of(ct * 128, 128)
        wait_dyn(("uk", 0), ct, lambda i: [(wuk_hbm.at[pl.ds(s, 128)], luk.at[pl.ds(s, 128)])])
        t = jnp.swapaxes(luk[pl.ds(s, 128)], 0, 1)
        for h in range(H):
            wukt[h, ct] = pltpu.bitcast(t[h].T, u32)
        qa = [zero8] * 4
        for h in range(H):
            g, r = divmod(h, 8)
            out = _dot(q[g], pltpu.bitcast(wukt[h, ct], bf16))
            qa[g] = jnp.where(masks[r], out, qa[g])
        qa_s[ct] = jnp.concatenate(qa, axis=0)
        return _

    lax.fori_loop(0, NC, b_body, 0)

    def cd_body(b, carry):
        m, l, acc = carry
        s = pl.multiple_of(b * 512, 512)
        wait_dyn(("ckv", 0), b, lambda i: [(ckv32.at[pl.ds(s, 512), pl.ds(ct * 128, 128)],
                                            lckv.at[ct, pl.ds(s, 512)]) for ct in range(NC)])
        ss = []
        for j in range(KB):
            kt = b * KB + j
            sk = pl.multiple_of(s + j * 64, 64)
            sc = None
            for ct in range(NC):
                t = pltpu.bitcast(lckv[ct, pl.ds(sk, 64), :], bf16).T
                ckvt[kt, ct] = pltpu.bitcast(t, u32)
                o = _dot(qa_s[ct], t)
                sc = o if sc is None else sc + o
            ss.append(sc * SCALE)
        mb = ss[0]
        for j in range(1, KB):
            mb = jnp.maximum(mb, ss[j])
        m_new = jnp.maximum(m, jnp.max(mb, axis=1, keepdims=True))
        alpha = jnp.exp(m - m_new)
        ps = [jnp.exp(sj - m_new) for sj in ss]
        lb = ps[0]
        for j in range(1, KB):
            lb = lb + ps[j]
        l = l * alpha + lb
        acc = [a * alpha for a in acc]
        for j in range(KB):
            sk = pl.multiple_of(s + j * 64, 64)
            for ct in range(NC):
                acc[ct] = acc[ct] + _dot(ps[j], pltpu.bitcast(lckv[ct, pl.ds(sk, 64), :], bf16))
        return m_new, l, acc

    m_init = jnp.full((H, 128), -jnp.inf, f32)
    _, l, acc = lax.fori_loop(0, NB, cd_body,
                              (m_init, jnp.zeros((H, 128), f32),
                               [jnp.zeros((H, 128), f32)] * NC))
    linv = 1.0 / jnp.sum(l, axis=1, keepdims=True)
    for ct in range(NC):
        cc_s[ct] = acc[ct]

    def transpose_ffn(land, dst, fam):
        def body(ft, _):
            s = pl.multiple_of(ft * 128, 128)
            for kt in range(NM):
                dst[ft, kt] = pltpu.bitcast(land[pl.ds(s, 128), pl.ds(kt * 128, 128)].T, u32)
            return _
        wait((fam, 0))
        lax.fori_loop(0, 7, body, 0)
        wait((fam, 1))
        lax.fori_loop(7, 13, body, 0)
        for kt in range(NM):
            t = land[pl.ds(13 * 128, 64), pl.ds(kt * 128, 128)]
            t = jnp.concatenate([t, jnp.zeros((64, 128), bf16)], axis=0)
            dst[13, kt] = pltpu.bitcast(t.T, u32)

    transpose_ffn(lg, gt, "g")
    transpose_ffn(lu, ut, "u")

    def e_body(ct, ctx):
        s = pl.multiple_of(ct * 128, 128)
        wait_dyn(("uv", 0), ct, lambda i: [(wuv_hbm.at[pl.ds(s, 128)], luv.at[pl.ds(s, 128)])])
        t = jnp.swapaxes(luv[pl.ds(s, 128)], 0, 1)
        s2 = pl.multiple_of(ct * 64, 64)
        for h in range(H):
            wuv[h, pl.ds(s2, 64), :] = pltpu.bitcast(t[h], u32)
        ctx = list(ctx)
        cc = cc_s[ct]
        for h in range(H):
            g, r = divmod(h, 8)
            out = _dot(cc[g * 8:(g + 1) * 8], pltpu.bitcast(wuv[h, pl.ds(s2, 64), :], bf16))
            ctx[g] = jnp.where(masks[r], ctx[g] + out, ctx[g])
        return tuple(ctx)

    ctx = lax.fori_loop(0, NC, e_body, (zero8,) * 4)
    for g in range(4):
        ctx_s[g] = ctx[g] * linv[g * 8:(g + 1) * 8]

    def f_body(g, acc):
        s = pl.multiple_of(g * 8, 8)
        wait_dyn(("o", 0), g, lambda i: [(wo_hbm.at[pl.ds(s, 8)], lo.at[pl.ds(s, 8)])])
        acc = list(acc)
        cg = ctx_s[g]
        for r in range(8):
            lhs = jnp.where(masks[r], cg, 0.0)
            for n in range(NM):
                acc[n] = acc[n] + _dot(lhs, lo[g * 8 + r, :, pl.ds(n * 128, 128)])
        return tuple(acc)

    acc = lax.fori_loop(0, 4, f_body, (zero8,) * NM)
    x1 = [_rbf(x0[n] + _rbf(_rowsum(acc[n]))) for n in range(NM)]

    mean1, rstd1 = _stats(x1)
    ln1 = [(x - mean1) * rstd1 for x in x1]
    sig1 = _router(ln1, wr)
    lhs1 = [jnp.concatenate([x1[kt], ones8], axis=0) for kt in range(NM)]

    hh1 = []
    for ft in range(NF):
        og = ou = None
        for kt in range(NM):
            a = _dot(lhs1[kt], _tile(gt, ft, kt))
            b = _dot(lhs1[kt], _tile(ut, ft, kt))
            og = a if og is None else og + a
            ou = b if ou is None else ou + b
        csg[ft] = og[8:16]
        csu[ft] = ou[8:16]
        g = rstd1 * (og[0:8] - mean1 * og[8:16])
        u = rstd1 * (ou[0:8] - mean1 * ou[8:16])
        hh1.append(_silu(g) * u)

    def down(ft, n, hh):
        if ft < 13:
            return _dot(hh, ld[pl.ds(ft * 128, 128), pl.ds(n * 128, 128)])
        return _dot(hh[:, :64], ld[pl.ds(13 * 128, 64), pl.ds(n * 128, 128)])

    y = [None] * NM
    for i, (s, nrows) in enumerate(DS):
        wait(("d", i))
        for ft in range(s // 128, (s + nrows + 127) // 128):
            hh = hh1[ft]
            for n in range(NM):
                o = down(ft, n, hh)
                y[n] = o if y[n] is None else y[n] + o
    x2 = [_rbf(x1[n] + _rbf(ln1[n] + _rbf(y[n] * sig1))) for n in range(NM)]

    mean2, rstd2 = _stats(x2)
    q = []
    for g in range(4):
        rawg = zero8
        for r in range(8):
            h = g * 8 + r
            o = None
            for kt in range(NM):
                t = _dot(x2[kt], _tile(wq, h, pl.ds(kt * 64, 64)))
                o = t if o is None else o + t
            rawg = jnp.where(masks[r], o, rawg)
        q.append(rstd2 * (rawg - mean2 * csq[g]))
    qa = []
    for ct in range(NC):
        qg = [zero8] * 4
        for h in range(H):
            g, r = divmod(h, 8)
            qg[g] = jnp.where(masks[r], _dot(q[g], _tile(wukt, h, ct)), qg[g])
        qa.append(jnp.concatenate(qg, axis=0))

    def scores(b):
        ss = []
        for j in range(KB):
            kt = b * KB + j
            sc = None
            for ct in range(NC):
                o = _dot(qa[ct], _tile(ckvt, kt, ct))
                sc = o if sc is None else sc + o
            ss.append(sc * SCALE)
        return ss

    def soft(ss, m, l):
        mb = ss[0]
        for j in range(1, KB):
            mb = jnp.maximum(mb, ss[j])
        mb = jnp.max(mb, axis=1, keepdims=True)
        m_new = mb if m is None else jnp.maximum(m, mb)
        ps = [jnp.exp(sj - m_new) for sj in ss]
        lb = ps[0]
        for j in range(1, KB):
            lb = lb + ps[j]
        if m is None:
            return ps, m_new, lb, None
        alpha = jnp.exp(m - m_new)
        return ps, m_new, l * alpha + lb, alpha

    def ctxc(b, ps, alpha, acc):
        if acc is not None:
            acc = [a * alpha for a in acc]
        else:
            acc = [None] * NC
        acc = list(acc)
        last = b == NB - 1
        seq = ([(j, ct) for ct in range(NC) for j in range(KB)] if last
               else [(j, ct) for j in range(KB) for ct in range(NC)])
        for j, ct in seq:
            kt = b * KB + j
            o = _dot(ps[j], _tile(lckv, ct, pl.ds(kt * 64, 64)))
            acc[ct] = o if acc[ct] is None else acc[ct] + o
        return acc

    s0 = scores(0)
    s1 = scores(1)
    p0, m, l, al0 = soft(s0, None, None)
    acc = ctxc(0, p0, None, None)
    s2 = scores(2)
    p1, m, l, al1 = soft(s1, m, l)
    acc = ctxc(1, p1, al1, acc)
    s3 = scores(3)
    p2, m, l, al2 = soft(s2, m, l)
    acc = ctxc(2, p2, al2, acc)
    p3, m, l, al3 = soft(s3, m, l)
    acc = ctxc(3, p3, al3, acc)
    linv = 1.0 / jnp.sum(l, axis=1, keepdims=True)

    ctx = [zero8] * 4
    for ct in range(NC):
        for h in range(H):
            g, r = divmod(h, 8)
            o = _dot(acc[ct][g * 8:(g + 1) * 8], _tile(wuv, h, pl.ds(ct * 64, 64)))
            ctx[g] = jnp.where(masks[r], ctx[g] + o, ctx[g])
    ctx = [ctx[g] * linv[g * 8:(g + 1) * 8] for g in range(4)]
    x3 = []
    for n in range(NM):
        a = None
        for h in range(H):
            g, r = divmod(h, 8)
            o = _dot(jnp.where(masks[r], ctx[g], 0.0), lo[h, :, pl.ds(n * 128, 128)])
            a = o if a is None else a + o
        x3.append(_rbf(x2[n] + _rbf(_rowsum(a))))
    mean3, rstd3 = _stats(x3)
    ln3 = [(x - mean3) * rstd3 for x in x3]
    sig3 = _router(ln3, wr)
    hh = []
    for ft in range(NF):
        og = ou = None
        for kt in range(NM):
            a = _dot(x3[kt], _tile(gt, ft, kt))
            b = _dot(x3[kt], _tile(ut, ft, kt))
            og = a if og is None else og + a
            ou = b if ou is None else ou + b
        g = rstd3 * (og - mean3 * csg[ft])
        u = rstd3 * (ou - mean3 * csu[ft])
        hh.append(_silu(g) * u)
    y = [None] * NM
    for ft in range(NF):
        for n in range(NM):
            o = down(ft, n, hh[ft])
            y[n] = o if y[n] is None else y[n] + o
    x4 = [x3[n] + _rbf(ln3[n] + _rbf(y[n] * sig3)) for n in range(NM)]
    out = jnp.concatenate([x[0:1, :] for x in x4], axis=1)
    o_ref[0] = out.astype(bf16)


@jax.jit
def pallas_interleave_layers__compressed_kv_cla__moe_arch_mod__decode_kernel(
    A_x: jax.Array,
    A_c_kv: jax.Array,
    A_w_q: jax.Array,
    A_w_uk: jax.Array,
    A_w_uv: jax.Array,
    A_w_o: jax.Array,
    B_x: jax.Array,
    B_w_r: jax.Array,
    B_w_gate: jax.Array,
    B_w_up: jax.Array,
    B_w_down: jax.Array,
):
    del B_x
    any_spec = pl.BlockSpec(memory_space=pl.ANY)
    V = pltpu.VMEM
    scratch = [
        V((1, 1, M), bf16),
        V((NM, 128), bf16),
        V((M, H, D), bf16),
        V((DC, H, D), bf16),
        V((DC, H, D), bf16),
        V((NC, SK // 2, 128), u32),
        V((H, D, M), bf16),
        V((F, M), bf16),
        V((F, M), bf16),
        V((F, M), bf16),
        V((H, M // 2, D), u32),
        V((H, NC, D // 2, 128), u32),
        V((H, DC // 2, D), u32),
        V((NK, NC, 64, 128), u32),
        V((NF, NM, 64, 128), u32),
        V((NF, NM, 64, 128), u32),
        V((4, 8, 128), f32),
        V((NF, 8, 128), f32),
        V((NF, 8, 128), f32),
        V((NC, H, 128), f32),
        V((NC, H, 128), f32),
        V((4, 8, 128), f32),
        V((NF, 8, 128), f32),
        V((NM, 8, 128), f32),
        pltpu.SemaphoreType.DMA((32,)),
    ]
    return pl.pallas_call(
        _kernel,
        out_shape=jax.ShapeDtypeStruct((1, 1, M), bf16),
        in_specs=[any_spec] * 10,
        out_specs=pl.BlockSpec(memory_space=pltpu.VMEM),
        scratch_shapes=scratch,
        compiler_params=pltpu.CompilerParams(
            vmem_limit_bytes=100 * 1024 * 1024,
            disable_semaphore_checks=True,
        ),
    )(A_x, A_c_kv, A_w_q, A_w_uk, A_w_uv, A_w_o, B_w_r.reshape(NM, 128),
      B_w_gate.T, B_w_up.T, B_w_down)
```

```python
import functools

import jax
import jax.numpy as jnp
from jax import lax
import jax.experimental.pallas as pl
import jax.experimental.pallas.tpu as pltpu

f32 = jnp.float32
bf16 = jnp.bfloat16
u32 = jnp.uint32
i32 = jnp.int32

M = 640
H = 32
D = 128
DC = 512
SK = 4096
F = 1728
NM = M // 128
NC = DC // 128
NK = SK // 128
NF = 14
EPS = 1e-5
SCALE = float(D) ** -0.5
KB = 8
NB = NK // KB
GV = 2
DV = 6
OV = 12
BV = 12


def _dot(a, b):
    return jnp.dot(a, b, preferred_element_type=f32)


def _rbf(x):
    return x.astype(bf16).astype(f32)


def _tile(ref, *idx):
    return pltpu.bitcast(ref[idx], bf16)


def _stats(xs):
    s = xs[0] + xs[1] + xs[2] + xs[3] + xs[4]
    mean = jnp.sum(s, axis=1, keepdims=True) * (1.0 / M)
    ds = [x - mean for x in xs]
    q = ds[0] * ds[0] + ds[1] * ds[1] + ds[2] * ds[2] + ds[3] * ds[3] + ds[4] * ds[4]
    var = jnp.sum(q, axis=1, keepdims=True) * (1.0 / M)
    rstd = 1.0 / jnp.sqrt(var + EPS)
    return mean, rstd


def _router(lns, wr):
    s = lns[0] * wr[0] + lns[1] * wr[1] + lns[2] * wr[2] + lns[3] * wr[3] + lns[4] * wr[4]
    r = jnp.sum(s, axis=1, keepdims=True)
    return jax.nn.sigmoid(r)


def _rowsum(x):
    return jnp.broadcast_to(jnp.sum(x, axis=0, keepdims=True), x.shape)


def _xb(row):
    t = jnp.broadcast_to(row, (128, 128)).T
    return [t[s * 8:(s + 1) * 8] for s in range(16)]


def _vmac(acc, xb, load):
    for s, xs in enumerate(xb):
        p = xs * load(s)
        acc = p if acc is None else acc + p
    return acc


def _vmacs(accs, xb, load):
    accs = list(accs)
    for s, xs in enumerate(xb):
        for i in range(len(accs)):
            p = xs * load(s, i)
            accs[i] = p if accs[i] is None else accs[i] + p
    return accs


def _vmac3(accs, xbs, load):
    accs = list(accs)
    for s in range(16):
        for j, xb in enumerate(xbs):
            for i in range(len(accs)):
                p = xb[s] * load(j, s, i)
                accs[i] = p if accs[i] is None else accs[i] + p
    return accs


def _silu(g):
    return g * jax.nn.sigmoid(g)


def _kernel(x_hbm, ckv_hbm, wq_hbm, wuk_hbm, wuv_hbm, wo_hbm, wr_hbm, wg_hbm, wu_hbm, wd_hbm,
            o_ref,
            x_v, wr_v, lq, luk, luv, lckv, lo, lg, lu, ld,
            wq, wukt, wuv, ckvt, gt, ut, g32, u32s, d32, o32, b32, wo2, wd2,
            csq, csg, csu, qa_s, cc_s, ctx_s, hh_s, x_s,
            sems):
    row8 = lax.broadcasted_iota(i32, (8, 128), 0)
    masks = [row8 == r for r in range(8)]

    copies = {}
    order = []

    def add(name, pairs):
        sem = sems.at[len(copies)]
        cs = [pltpu.make_async_copy(s, d, sem) for s, d in pairs]
        copies[name] = cs
        order.append(name)

    add("x", [(x_hbm, x_v)])
    add("wr", [(wr_hbm, wr_v)])
    for i in range(NM):
        add(("q", i), [(wq_hbm.at[pl.ds(i * 128, 128)], lq.at[pl.ds(i * 128, 128)])])
    for i in range(NC):
        add(("uk", i), [(wuk_hbm.at[pl.ds(i * 128, 128)], luk.at[pl.ds(i * 128, 128)])])
    ckv32 = ckv_hbm.at[0].bitcast(u32)
    for b in range(NB):
        add(("ckv", b), [(ckv32.at[pl.ds(b * 512, 512), pl.ds(ct * 128, 128)],
                          lckv.at[ct, pl.ds(b * 512, 512)]) for ct in range(NC)])
    FS = [(0, 896), (896, F - 896)]
    for i, (s, n) in enumerate(FS):
        add(("g", i), [(wg_hbm.at[pl.ds(s, n)], lg.at[pl.ds(s, n)])])
    for i, (s, n) in enumerate(FS):
        add(("u", i), [(wu_hbm.at[pl.ds(s, n)], lu.at[pl.ds(s, n)])])
    for i in range(NC):
        add(("uv", i), [(wuv_hbm.at[pl.ds(i * 128, 128)], luv.at[pl.ds(i * 128, 128)])])
    for g in range(4):
        add(("o", g), [(wo_hbm.at[pl.ds(g * 8, 8)], lo.at[pl.ds(g * 8, 8)])])
    DS = [(0, 512), (512, 512), (1024, 512), (1536, F - 1536)]
    for i, (s, n) in enumerate(DS):
        add(("d", i), [(wd_hbm.at[pl.ds(s, n)], ld.at[pl.ds(s, n)])])

    for name in order:
        for c in copies[name]:
            c.start()

    def wait(name):
        for c in copies[name]:
            c.wait()

    names = list(copies)

    def wait_dyn(first_name, i, pairs_fn):
        base = names.index(first_name)
        for s, d in pairs_fn(i):
            pltpu.make_async_copy(s, d, sems.at[base + i]).wait()

    wait("x")
    wait("wr")
    xr = x_v[0].astype(f32)
    x0 = [jnp.broadcast_to(xr[:, n * 128:(n + 1) * 128], (8, 128)) for n in range(NM)]
    wrf = wr_v[...].astype(f32)
    wr = [jnp.broadcast_to(wrf[n:n + 1, :], (8, 128)) for n in range(NM)]
    for n in range(NM):
        x_s[n] = x0[n]
    mean0, rstd0 = _stats(x0)
    ones8 = jnp.ones((8, 128), f32)
    zero8 = jnp.zeros((8, 128), f32)

    def a_body(kt, carry):
        raw, cs = carry
        s = pl.multiple_of(kt * 128, 128)
        wait_dyn(("q", 0), kt, lambda i: [(wq_hbm.at[pl.ds(s, 128)], lq.at[pl.ds(s, 128)])])
        t = jnp.swapaxes(lq[pl.ds(s, 128)], 0, 1)
        s2 = pl.multiple_of(kt * 64, 64)
        for h in range(H):
            wq[h, pl.ds(s2, 64), :] = pltpu.bitcast(t[h], u32)
        lhs = jnp.concatenate([x_s[kt], ones8], axis=0)
        raw, cs = list(raw), list(cs)
        for h in range(H):
            g, r = divmod(h, 8)
            out = _dot(lhs, pltpu.bitcast(wq[h, pl.ds(s2, 64), :], bf16))
            raw[g] = jnp.where(masks[r], raw[g] + out[0:8], raw[g])
            cs[g] = jnp.where(masks[r], cs[g] + out[8:16], cs[g])
        return tuple(raw), tuple(cs)

    raw, cs = lax.fori_loop(0, NM, a_body, ((zero8,) * 4, (zero8,) * 4))
    for g in range(4):
        csq[g] = cs[g]
    q = [rstd0 * (raw[g] - mean0 * cs[g]) for g in range(4)]

    def b_body(ct, _):
        s = pl.multiple_of(ct * 128, 128)
        wait_dyn(("uk", 0), ct, lambda i: [(wuk_hbm.at[pl.ds(s, 128)], luk.at[pl.ds(s, 128)])])
        t = jnp.swapaxes(luk[pl.ds(s, 128)], 0, 1)
        for h in range(H):
            th = t[h].T
            wukt[h, ct] = pltpu.bitcast(th, u32)
            if h < BV:
                b32[h, ct] = th.astype(f32)
        qa = [zero8] * 4
        for h in range(H):
            g, r = divmod(h, 8)
            out = _dot(q[g], pltpu.bitcast(wukt[h, ct], bf16))
            qa[g] = jnp.where(masks[r], out, qa[g])
        qa_s[ct] = jnp.concatenate(qa, axis=0)
        return _

    lax.fori_loop(0, NC, b_body, 0)

    def cd_body(b, carry):
        m, l, acc = carry
        s = pl.multiple_of(b * 512, 512)
        wait_dyn(("ckv", 0), b, lambda i: [(ckv32.at[pl.ds(s, 512), pl.ds(ct * 128, 128)],
                                            lckv.at[ct, pl.ds(s, 512)]) for ct in range(NC)])
        ss = []
        for j in range(KB):
            kt = b * KB + j
            sk = pl.multiple_of(s + j * 64, 64)
            sc = None
            for ct in range(NC):
                t = pltpu.bitcast(lckv[ct, pl.ds(sk, 64), :], bf16).T
                ckvt[kt, ct] = pltpu.bitcast(t, u32)
                o = _dot(qa_s[ct], t)
                sc = o if sc is None else sc + o
            ss.append(sc * SCALE)
        mb = ss[0]
        for j in range(1, KB):
            mb = jnp.maximum(mb, ss[j])
        m_new = jnp.maximum(m, jnp.max(mb, axis=1, keepdims=True))
        alpha = jnp.exp(m - m_new)
        ps = [jnp.exp(sj - m_new) for sj in ss]
        lb = ps[0]
        for j in range(1, KB):
            lb = lb + ps[j]
        l = l * alpha + lb
        acc = [a * alpha for a in acc]
        for j in range(KB):
            sk = pl.multiple_of(s + j * 64, 64)
            for ct in range(NC):
                acc[ct] = acc[ct] + _dot(ps[j], pltpu.bitcast(lckv[ct, pl.ds(sk, 64), :], bf16))
        return m_new, l, acc

    m_init = jnp.full((H, 128), -jnp.inf, f32)
    _, l, acc = lax.fori_loop(0, NB, cd_body,
                              (m_init, jnp.zeros((H, 128), f32),
                               [jnp.zeros((H, 128), f32)] * NC))
    linv = 1.0 / jnp.sum(l, axis=1, keepdims=True)
    for ct in range(NC):
        cc_s[ct] = acc[ct]

    def transpose_ffn(land, dst, dst32, fam):
        def body(ft, _):
            s = pl.multiple_of(ft * 128, 128)
            for kt in range(NM):
                t = land[pl.ds(s, 128), pl.ds(kt * 128, 128)].T
                dst[ft, kt] = pltpu.bitcast(t, u32)
                if kt < GV:
                    dst32[ft, pl.ds(kt * 128, 128), :] = t.astype(f32)
            return _
        wait((fam, 0))
        lax.fori_loop(0, 7, body, 0)
        wait((fam, 1))
        lax.fori_loop(7, 13, body, 0)
        for kt in range(NM):
            t = land[pl.ds(13 * 128, 64), pl.ds(kt * 128, 128)]
            t = jnp.concatenate([t, jnp.zeros((64, 128), bf16)], axis=0)
            t = t.T
            dst[13, kt] = pltpu.bitcast(t, u32)
            if kt < GV:
                dst32[13, pl.ds(kt * 128, 128), :] = t.astype(f32)

    transpose_ffn(lg, gt, g32, "g")
    transpose_ffn(lu, ut, u32s, "u")

    def e_body(ct, ctx):
        s = pl.multiple_of(ct * 128, 128)
        wait_dyn(("uv", 0), ct, lambda i: [(wuv_hbm.at[pl.ds(s, 128)], luv.at[pl.ds(s, 128)])])
        t = jnp.swapaxes(luv[pl.ds(s, 128)], 0, 1)
        s2 = pl.multiple_of(ct * 64, 64)
        for h in range(H):
            wuv[h, pl.ds(s2, 64), :] = pltpu.bitcast(t[h], u32)
        ctx = list(ctx)
        cc = cc_s[ct]
        for h in range(H):
            g, r = divmod(h, 8)
            out = _dot(cc[g * 8:(g + 1) * 8], pltpu.bitcast(wuv[h, pl.ds(s2, 64), :], bf16))
            ctx[g] = jnp.where(masks[r], ctx[g] + out, ctx[g])
        return tuple(ctx)

    ctx = lax.fori_loop(0, NC, e_body, (zero8,) * 4)
    for g in range(4):
        ctx_s[g] = ctx[g] * linv[g * 8:(g + 1) * 8]

    def f_body(g, acc):
        s = pl.multiple_of(g * 8, 8)
        wait_dyn(("o", 0), g, lambda i: [(wo_hbm.at[pl.ds(s, 8)], lo.at[pl.ds(s, 8)])])
        acc = list(acc)
        cg = ctx_s[g]
        for r in range(8):
            lhs = jnp.where(masks[r], cg, 0.0)
            for n in range(NM):
                t = lo[s + r, :, pl.ds(n * 128, 128)]
                wo2[s + r, n] = pltpu.bitcast(t, u32)
                acc[n] = acc[n] + _dot(lhs, t)
        for r in range(8):
            @pl.when(s + r < OV)
            def _():
                o32[jnp.minimum(s + r, OV - 1)] = lo[s + r].astype(f32)
        return tuple(acc)

    acc = lax.fori_loop(0, 4, f_body, (zero8,) * NM)
    x1 = [_rbf(x0[n] + _rbf(_rowsum(acc[n]))) for n in range(NM)]

    mean1, rstd1 = _stats(x1)
    ln1 = [(x - mean1) * rstd1 for x in x1]
    sig1 = _router(ln1, wr)
    lhs1 = [jnp.concatenate([x1[kt], ones8], axis=0) for kt in range(NM)]

    hh1 = []
    for ft in range(NF):
        og = ou = None
        for kt in range(NM):
            a = _dot(lhs1[kt], _tile(gt, ft, kt))
            b = _dot(lhs1[kt], _tile(ut, ft, kt))
            og = a if og is None else og + a
            ou = b if ou is None else ou + b
        csg[ft] = og[8:16]
        csu[ft] = ou[8:16]
        g = rstd1 * (og[0:8] - mean1 * og[8:16])
        u = rstd1 * (ou[0:8] - mean1 * ou[8:16])
        hh1.append(_silu(g) * u)
        if ft < 12:
            hh_s[ft] = hh1[ft]

    def down2(ft, n, hh):
        if ft < 12:
            return _dot(hh, _tile(wd2, ft, n))
        if ft == 12:
            return _dot(hh, ld[pl.ds(12 * 128, 128), pl.ds(n * 128, 128)])
        return _dot(hh[:, :64], ld[pl.ds(13 * 128, 64), pl.ds(n * 128, 128)])

    def h_body(i, y):
        s = pl.multiple_of(i * 512, 512)
        wait_dyn(("d", 0), i, lambda _: [(wd_hbm.at[pl.ds(s, 512)], ld.at[pl.ds(s, 512)])])
        y = list(y)
        for j in range(4):
            ft = i * 4 + j
            sf = pl.multiple_of(s + j * 128, 128)
            hh = hh_s[ft]
            for n in range(NM):
                t = ld[pl.ds(sf, 128), pl.ds(n * 128, 128)]
                wd2[ft, n] = pltpu.bitcast(t, u32)
                y[n] = y[n] + _dot(hh, t)
        for j in range(4):
            ft = i * 4 + j
            sf = pl.multiple_of(s + j * 128, 128)

            @pl.when(ft < DV)
            def _():
                sd = pl.multiple_of(jnp.minimum(ft, DV - 1) * 128, 128)
                d32[pl.ds(sd, 128), :] = ld[pl.ds(sf, 128), :].astype(f32)
        return tuple(y)

    y = list(lax.fori_loop(0, 3, h_body, (zero8,) * NM))
    wait(("d", 3))
    for ft in (12, 13):
        for n in range(NM):
            y[n] = y[n] + down2(ft, n, hh1[ft])
    x2 = [_rbf(x1[n] + _rbf(ln1[n] + _rbf(y[n] * sig1))) for n in range(NM)]

    mean2, rstd2 = _stats(x2)
    q = []
    for g in range(4):
        rawg = zero8
        for r in range(8):
            h = g * 8 + r
            o = None
            for kt in range(NM):
                t = _dot(x2[kt], _tile(wq, h, pl.ds(kt * 64, 64)))
                o = t if o is None else o + t
            rawg = jnp.where(masks[r], o, rawg)
        q.append(rstd2 * (rawg - mean2 * csq[g]))
    qv = {}
    for i in range(0, BV, 3):
        hs = list(range(i, min(i + 3, BV)))
        xbs = [_xb(q[h // 8][h % 8:h % 8 + 1]) for h in hs]
        accs = [[None] * NC for _ in hs]
        for s in range(16):
            for j, h in enumerate(hs):
                for ct in range(NC):
                    p = xbs[j][s] * b32[h, ct, pl.ds(s * 8, 8), :]
                    accs[j][ct] = p if accs[j][ct] is None else accs[j][ct] + p
        for j, h in enumerate(hs):
            for ct in range(NC):
                qv[h, ct] = _rowsum(accs[j][ct])
    qa = []
    for ct in range(NC):
        qg = [zero8] * 4
        for h in range(H):
            g, r = divmod(h, 8)
            o = qv[h, ct] if h < BV else _dot(q[g], _tile(wukt, h, ct))
            qg[g] = jnp.where(masks[r], o, qg[g])
        qa.append(jnp.concatenate(qg, axis=0))

    def scores(b):
        ss = []
        for j in range(KB):
            kt = b * KB + j
            sc = None
            for ct in range(NC):
                o = _dot(qa[ct], _tile(ckvt, kt, ct))
                sc = o if sc is None else sc + o
            ss.append(sc * SCALE)
        return ss

    def soft(ss, m, l):
        mb = ss[0]
        for j in range(1, KB):
            mb = jnp.maximum(mb, ss[j])
        mb = jnp.max(mb, axis=1, keepdims=True)
        m_new = mb if m is None else jnp.maximum(m, mb)
        ps = [jnp.exp(sj - m_new) for sj in ss]
        lb = ps[0]
        for j in range(1, KB):
            lb = lb + ps[j]
        if m is None:
            return ps, m_new, lb, None
        alpha = jnp.exp(m - m_new)
        return ps, m_new, l * alpha + lb, alpha

    def ctxc(b, ps, alpha, acc):
        if acc is not None:
            acc = [a * alpha for a in acc]
        else:
            acc = [None] * NC
        acc = list(acc)
        last = b == NB - 1
        seq = ([(j, ct) for ct in range(NC) for j in range(KB)] if last
               else [(j, ct) for j in range(KB) for ct in range(NC)])
        for j, ct in seq:
            kt = b * KB + j
            o = _dot(ps[j], _tile(lckv, ct, pl.ds(kt * 64, 64)))
            acc[ct] = o if acc[ct] is None else acc[ct] + o
        return acc

    s0 = scores(0)
    s1 = scores(1)
    p0, m, l, al0 = soft(s0, None, None)
    acc = ctxc(0, p0, None, None)
    s2 = scores(2)
    p1, m, l, al1 = soft(s1, m, l)
    acc = ctxc(1, p1, al1, acc)
    s3 = scores(3)
    p2, m, l, al2 = soft(s2, m, l)
    acc = ctxc(2, p2, al2, acc)
    p3, m, l, al3 = soft(s3, m, l)
    acc = ctxc(3, p3, al3, acc)
    linv = 1.0 / jnp.sum(l, axis=1, keepdims=True)

    ctx = [zero8] * 4
    for ct in range(NC):
        for h in range(H):
            g, r = divmod(h, 8)
            o = _dot(acc[ct][g * 8:(g + 1) * 8], _tile(wuv, h, pl.ds(ct * 64, 64)))
            ctx[g] = jnp.where(masks[r], ctx[g] + o, ctx[g])
    ctx = [ctx[g] * linv[g * 8:(g + 1) * 8] for g in range(4)]
    accv = [None] * NM
    accm = [None] * NM
    mseq = [(n, h) for n in range(NM) for h in range(OV, H)]
    trip = [list(range(i, min(i + 3, OV))) for i in range(0, OV, 3)]
    per = -(-len(mseq) // len(trip))
    for t, hs in enumerate(trip):
        xbs = [_xb(ctx[h // 8][h % 8:h % 8 + 1]) for h in hs]
        accv = _vmac3(accv, xbs,
                      lambda j, s, n: o32[hs[j], pl.ds(s * 8, 8), pl.ds(n * 128, 128)])
        for n, h in mseq[t * per:(t + 1) * per]:
            g, r = divmod(h, 8)
            o = _dot(jnp.where(masks[r], ctx[g], 0.0), _tile(wo2, h, n))
            accm[n] = o if accm[n] is None else accm[n] + o
    x3 = [_rbf(x2[n] + _rbf(_rowsum(accm[n] + accv[n]))) for n in range(NM)]
    mean3, rstd3 = _stats(x3)
    ln3 = [(x - mean3) * rstd3 for x in x3]
    sig3 = _router(ln3, wr)
    xb3 = []
    for kt in range(GV):
        xb3 += _xb(x3[kt][0:1])
    hh = []
    for ft in range(NF):
        og = ou = None
        for kt in range(GV, NM):
            a = _dot(x3[kt], _tile(gt, ft, kt))
            b = _dot(x3[kt], _tile(ut, ft, kt))
            og = a if og is None else og + a
            ou = b if ou is None else ou + b
        if GV:
            ag = au = None
            for s in range(16):
                for kt in range(GV):
                    xs = xb3[kt * 16 + s]
                    pg = xs * g32[ft, pl.ds(kt * 128 + s * 8, 8), :]
                    pu = xs * u32s[ft, pl.ds(kt * 128 + s * 8, 8), :]
                    ag = pg if ag is None else ag + pg
                    au = pu if au is None else au + pu
            og = og + _rowsum(ag)
            ou = ou + _rowsum(au)
        g = rstd3 * (og - mean3 * csg[ft])
        u = rstd3 * (ou - mean3 * csu[ft])
        hh.append(_silu(g) * u)
    yv = [None] * NM
    y = [None] * NM
    mseq = [(ft, n) for ft in range(DV, NF) for n in range(NM)]
    trip = [list(range(i, min(i + 3, DV))) for i in range(0, DV, 3)]
    per = -(-len(mseq) // len(trip))
    for t, fs in enumerate(trip):
        yv = _vmac3(yv, [_xb(hh[ft][0:1]) for ft in fs],
                    lambda j, s, n: d32[pl.ds(fs[j] * 128 + s * 8, 8), pl.ds(n * 128, 128)])
        for f2, n in mseq[t * per:(t + 1) * per]:
            o = down2(f2, n, hh[f2])
            y[n] = o if y[n] is None else y[n] + o
    y = [y[n] + _rowsum(yv[n]) for n in range(NM)]
    x4 = [x3[n] + _rbf(ln3[n] + _rbf(y[n] * sig3)) for n in range(NM)]
    out = jnp.concatenate([x[0:1, :] for x in x4], axis=1)
    o_ref[0] = out.astype(bf16)


@jax.jit
def pallas_interleave_layers__compressed_kv_cla__moe_arch_mod__decode_kernel(
    A_x: jax.Array,
    A_c_kv: jax.Array,
    A_w_q: jax.Array,
    A_w_uk: jax.Array,
    A_w_uv: jax.Array,
    A_w_o: jax.Array,
    B_x: jax.Array,
    B_w_r: jax.Array,
    B_w_gate: jax.Array,
    B_w_up: jax.Array,
    B_w_down: jax.Array,
):
    del B_x
    any_spec = pl.BlockSpec(memory_space=pl.ANY)
    V = pltpu.VMEM
    scratch = [
        V((1, 1, M), bf16),
        V((NM, 128), bf16),
        V((M, H, D), bf16),
        V((DC, H, D), bf16),
        V((DC, H, D), bf16),
        V((NC, SK // 2, 128), u32),
        V((H, D, M), bf16),
        V((F, M), bf16),
        V((F, M), bf16),
        V((F, M), bf16),
        V((H, M // 2, D), u32),
        V((H, NC, D // 2, 128), u32),
        V((H, DC // 2, D), u32),
        V((NK, NC, 64, 128), u32),
        V((NF, NM, 64, 128), u32),
        V((NF, NM, 64, 128), u32),
        V((NF, max(GV, 1) * 128, 128), f32),
        V((NF, max(GV, 1) * 128, 128), f32),
        V((max(DV, 1) * 128, M), f32),
        V((max(OV, 1), D, M), f32),
        V((max(BV, 1), NC, D, 128), f32),
        V((H, NM, 64, 128), u32),
        V((NF, NM, 64, 128), u32),
        V((4, 8, 128), f32),
        V((NF, 8, 128), f32),
        V((NF, 8, 128), f32),
        V((NC, H, 128), f32),
        V((NC, H, 128), f32),
        V((4, 8, 128), f32),
        V((NF, 8, 128), f32),
        V((NM, 8, 128), f32),
        pltpu.SemaphoreType.DMA((32,)),
    ]
    return pl.pallas_call(
        _kernel,
        out_shape=jax.ShapeDtypeStruct((1, 1, M), bf16),
        in_specs=[any_spec] * 10,
        out_specs=pl.BlockSpec(memory_space=pltpu.VMEM),
        scratch_shapes=scratch,
        compiler_params=pltpu.CompilerParams(
            vmem_limit_bytes=100 * 1024 * 1024,
            disable_semaphore_checks=True,
        ),
    )(A_x, A_c_kv, A_w_q, A_w_uk, A_w_uv, A_w_o, B_w_r.reshape(NM, 128),
      B_w_gate.T, B_w_up.T, B_w_down)
```

```python
import functools

import jax
import jax.numpy as jnp
from jax import lax
import jax.experimental.pallas as pl
import jax.experimental.pallas.tpu as pltpu

f32 = jnp.float32
bf16 = jnp.bfloat16
u32 = jnp.uint32
i32 = jnp.int32

M = 640
H = 32
D = 128
DC = 512
SK = 4096
F = 1728
NM = M // 128
NC = DC // 128
NK = SK // 128
NF = 14
EPS = 1e-5
SCALE = float(D) ** -0.5
KB = 8
NB = NK // KB
GV = 1
DV = 9
OV = 21
AV = 0
GB = 2
G0 = 3
BV = 26


def _dot(a, b):
    return jnp.dot(a, b, preferred_element_type=f32)


def _rbf(x):
    return x.astype(bf16).astype(f32)


def _tile(ref, *idx):
    return pltpu.bitcast(ref[idx], bf16)


def _stats(xs):
    s = xs[0] + xs[1] + xs[2] + xs[3] + xs[4]
    mean = jnp.sum(s, axis=1, keepdims=True) * (1.0 / M)
    ds = [x - mean for x in xs]
    q = ds[0] * ds[0] + ds[1] * ds[1] + ds[2] * ds[2] + ds[3] * ds[3] + ds[4] * ds[4]
    var = jnp.sum(q, axis=1, keepdims=True) * (1.0 / M)
    rstd = 1.0 / jnp.sqrt(var + EPS)
    return mean, rstd


def _router(lns, wr):
    s = lns[0] * wr[0] + lns[1] * wr[1] + lns[2] * wr[2] + lns[3] * wr[3] + lns[4] * wr[4]
    r = jnp.sum(s, axis=1, keepdims=True)
    return jax.nn.sigmoid(r)


def _rowsum(x):
    return jnp.broadcast_to(jnp.sum(x, axis=0, keepdims=True), x.shape)


def _xb(row):
    t = jnp.broadcast_to(row, (128, 128)).T
    return [t[s * 8:(s + 1) * 8] for s in range(16)]


def _vmac(acc, xb, load):
    for s, xs in enumerate(xb):
        p = xs * load(s)
        acc = p if acc is None else acc + p
    return acc


def _vmacs(accs, xb, load):
    accs = list(accs)
    for s, xs in enumerate(xb):
        for i in range(len(accs)):
            p = xs * load(s, i)
            accs[i] = p if accs[i] is None else accs[i] + p
    return accs


def _vmac3(accs, xbs, load):
    accs = [list(a) for a in accs]
    for s in range(16):
        for j, xb in enumerate(xbs):
            for i in range(len(accs[j])):
                p = xb[s] * load(j, s, i)
                accs[j][i] = p if accs[j][i] is None else accs[j][i] + p
    return accs


def _fold3(accs, i):
    t = [a[i] for a in accs if a[i] is not None]
    return functools.reduce(lambda a, b: a + b, t)


def _silu(g):
    return g * jax.nn.sigmoid(g)


def _kernel(x_hbm, ckv_hbm, wq_hbm, wuk_hbm, wuv_hbm, wo_hbm, wr_hbm, wg_hbm, wu_hbm, wd_hbm,
            o_ref,
            x_v, wr_v, lq, luk, luv, lckv, lo, lg, lu, ld,
            wq, wukt, wuv, ckvt, gt, ut, g32, u32s, d32, o32, b32, q32, wo2, wd2,
            csq, csg, csu, qa_s, cc_s, ctx_s, hh_s, x_s,
            sems):
    row8 = lax.broadcasted_iota(i32, (8, 128), 0)
    masks = [row8 == r for r in range(8)]

    copies = {}
    order = []

    def add(name, pairs):
        sem = sems.at[len(copies)]
        cs = [pltpu.make_async_copy(s, d, sem) for s, d in pairs]
        copies[name] = cs
        order.append(name)

    add("x", [(x_hbm, x_v)])
    add("wr", [(wr_hbm, wr_v)])
    for i in range(NM):
        add(("q", i), [(wq_hbm.at[pl.ds(i * 128, 128)], lq.at[pl.ds(i * 128, 128)])])
    for i in range(NC):
        add(("uk", i), [(wuk_hbm.at[pl.ds(i * 128, 128)], luk.at[pl.ds(i * 128, 128)])])
    ckv32 = ckv_hbm.at[0].bitcast(u32)
    for b in range(NB):
        add(("ckv", b), [(ckv32.at[pl.ds(b * 512, 512), pl.ds(ct * 128, 128)],
                          lckv.at[ct, pl.ds(b * 512, 512)]) for ct in range(NC)])
    FS = [(0, 896), (896, F - 896)]
    for i, (s, n) in enumerate(FS):
        add(("g", i), [(wg_hbm.at[pl.ds(s, n)], lg.at[pl.ds(s, n)])])
    for i, (s, n) in enumerate(FS):
        add(("u", i), [(wu_hbm.at[pl.ds(s, n)], lu.at[pl.ds(s, n)])])
    for i in range(NC):
        add(("uv", i), [(wuv_hbm.at[pl.ds(i * 128, 128)], luv.at[pl.ds(i * 128, 128)])])
    for g in range(4):
        add(("o", g), [(wo_hbm.at[pl.ds(g * 8, 8)], lo.at[pl.ds(g * 8, 8)])])
    DS = [(0, 512), (512, 512), (1024, 512), (1536, F - 1536)]
    for i, (s, n) in enumerate(DS):
        add(("d", i), [(wd_hbm.at[pl.ds(s, n)], ld.at[pl.ds(s, n)])])

    for name in order:
        for c in copies[name]:
            c.start()

    def wait(name):
        for c in copies[name]:
            c.wait()

    names = list(copies)

    def wait_dyn(first_name, i, pairs_fn):
        base = names.index(first_name)
        for s, d in pairs_fn(i):
            pltpu.make_async_copy(s, d, sems.at[base + i]).wait()

    wait("x")
    wait("wr")
    xr = x_v[0].astype(f32)
    x0 = [jnp.broadcast_to(xr[:, n * 128:(n + 1) * 128], (8, 128)) for n in range(NM)]
    wrf = wr_v[...].astype(f32)
    wr = [jnp.broadcast_to(wrf[n:n + 1, :], (8, 128)) for n in range(NM)]
    for n in range(NM):
        x_s[n] = x0[n]
    mean0, rstd0 = _stats(x0)
    ones8 = jnp.ones((8, 128), f32)
    zero8 = jnp.zeros((8, 128), f32)

    def a_body(kt, carry):
        raw, cs = carry
        s = pl.multiple_of(kt * 128, 128)
        wait_dyn(("q", 0), kt, lambda i: [(wq_hbm.at[pl.ds(s, 128)], lq.at[pl.ds(s, 128)])])
        t = jnp.swapaxes(lq[pl.ds(s, 128)], 0, 1)
        s2 = pl.multiple_of(kt * 64, 64)
        for h in range(H):
            wq[h, pl.ds(s2, 64), :] = pltpu.bitcast(t[h], u32)
        if AV:
            @pl.when(kt < AV)
            def _():
                sv = pl.multiple_of(jnp.minimum(kt, AV - 1) * 128, 128)
                for h in range(H):
                    w = wq[h, pl.ds(s2, 64), :]
                    q32[h, pl.ds(sv, 128), :] = pltpu.bitcast(w, bf16).astype(f32)
        lhs = jnp.concatenate([x_s[kt], ones8], axis=0)
        raw, cs = list(raw), list(cs)
        for h in range(H):
            g, r = divmod(h, 8)
            out = _dot(lhs, pltpu.bitcast(wq[h, pl.ds(s2, 64), :], bf16))
            raw[g] = jnp.where(masks[r], raw[g] + out[0:8], raw[g])
            cs[g] = jnp.where(masks[r], cs[g] + out[8:16], cs[g])
        return tuple(raw), tuple(cs)

    raw, cs = lax.fori_loop(0, NM, a_body, ((zero8,) * 4, (zero8,) * 4))
    for g in range(4):
        csq[g] = cs[g]
    q = [rstd0 * (raw[g] - mean0 * cs[g]) for g in range(4)]

    def b_body(ct, _):
        s = pl.multiple_of(ct * 128, 128)
        wait_dyn(("uk", 0), ct, lambda i: [(wuk_hbm.at[pl.ds(s, 128)], luk.at[pl.ds(s, 128)])])
        t = jnp.swapaxes(luk[pl.ds(s, 128)], 0, 1)
        for h in range(H):
            th = t[h].T
            wukt[h, ct] = pltpu.bitcast(th, u32)
            if h < BV:
                b32[h, ct] = th.astype(f32)
        qa = [zero8] * 4
        for h in range(H):
            g, r = divmod(h, 8)
            out = _dot(q[g], pltpu.bitcast(wukt[h, ct], bf16))
            qa[g] = jnp.where(masks[r], out, qa[g])
        qa_s[ct] = jnp.concatenate(qa, axis=0)
        return _

    lax.fori_loop(0, NC, b_body, 0)

    def cd_body(b, carry):
        m, l, acc = carry
        s = pl.multiple_of(b * 512, 512)
        wait_dyn(("ckv", 0), b, lambda i: [(ckv32.at[pl.ds(s, 512), pl.ds(ct * 128, 128)],
                                            lckv.at[ct, pl.ds(s, 512)]) for ct in range(NC)])
        ss = []
        for j in range(KB):
            kt = b * KB + j
            sk = pl.multiple_of(s + j * 64, 64)
            sc = None
            for ct in range(NC):
                t = pltpu.bitcast(lckv[ct, pl.ds(sk, 64), :], bf16).T
                ckvt[kt, ct] = pltpu.bitcast(t, u32)
                o = _dot(qa_s[ct], t)
                sc = o if sc is None else sc + o
            ss.append(sc * SCALE)
        mb = ss[0]
        for j in range(1, KB):
            mb = jnp.maximum(mb, ss[j])
        m_new = jnp.maximum(m, jnp.max(mb, axis=1, keepdims=True))
        alpha = jnp.exp(m - m_new)
        ps = [jnp.exp(sj - m_new) for sj in ss]
        lb = ps[0]
        for j in range(1, KB):
            lb = lb + ps[j]
        l = l * alpha + lb
        acc = [a * alpha for a in acc]
        for j in range(KB):
            sk = pl.multiple_of(s + j * 64, 64)
            for ct in range(NC):
                acc[ct] = acc[ct] + _dot(ps[j], pltpu.bitcast(lckv[ct, pl.ds(sk, 64), :], bf16))
        return m_new, l, acc

    m_init = jnp.full((H, 128), -jnp.inf, f32)
    _, l, acc = lax.fori_loop(0, NB, cd_body,
                              (m_init, jnp.zeros((H, 128), f32),
                               [jnp.zeros((H, 128), f32)] * NC))
    linv = 1.0 / jnp.sum(l, axis=1, keepdims=True)
    for ct in range(NC):
        cc_s[ct] = acc[ct]

    def transpose_ffn(land, dst, dst32, fam):
        def body(ft, _):
            s = pl.multiple_of(ft * 128, 128)
            for kt in range(NM):
                t = land[pl.ds(s, 128), pl.ds(kt * 128, 128)].T
                dst[ft, kt] = pltpu.bitcast(t, u32)
                if kt < GV:
                    dst32[ft, pl.ds(kt * 128, 128), :] = t.astype(f32)
            return _
        wait((fam, 0))
        lax.fori_loop(0, 7, body, 0)
        wait((fam, 1))
        lax.fori_loop(7, 13, body, 0)
        for kt in range(NM):
            t = land[pl.ds(13 * 128, 64), pl.ds(kt * 128, 128)]
            t = jnp.concatenate([t, jnp.zeros((64, 128), bf16)], axis=0)
            t = t.T
            dst[13, kt] = pltpu.bitcast(t, u32)
            if kt < GV:
                dst32[13, pl.ds(kt * 128, 128), :] = t.astype(f32)

    transpose_ffn(lg, gt, g32, "g")
    transpose_ffn(lu, ut, u32s, "u")

    def e_body(ct, ctx):
        s = pl.multiple_of(ct * 128, 128)
        wait_dyn(("uv", 0), ct, lambda i: [(wuv_hbm.at[pl.ds(s, 128)], luv.at[pl.ds(s, 128)])])
        t = jnp.swapaxes(luv[pl.ds(s, 128)], 0, 1)
        s2 = pl.multiple_of(ct * 64, 64)
        for h in range(H):
            wuv[h, pl.ds(s2, 64), :] = pltpu.bitcast(t[h], u32)
        ctx = list(ctx)
        cc = cc_s[ct]
        for h in range(H):
            g, r = divmod(h, 8)
            out = _dot(cc[g * 8:(g + 1) * 8], pltpu.bitcast(wuv[h, pl.ds(s2, 64), :], bf16))
            ctx[g] = jnp.where(masks[r], ctx[g] + out, ctx[g])
        return tuple(ctx)

    ctx = lax.fori_loop(0, NC, e_body, (zero8,) * 4)
    for g in range(4):
        ctx_s[g] = ctx[g] * linv[g * 8:(g + 1) * 8]

    def f_body(g, acc):
        s = pl.multiple_of(g * 8, 8)
        wait_dyn(("o", 0), g, lambda i: [(wo_hbm.at[pl.ds(s, 8)], lo.at[pl.ds(s, 8)])])
        acc = list(acc)
        cg = ctx_s[g]
        for r in range(8):
            lhs = jnp.where(masks[r], cg, 0.0)
            for n in range(NM):
                t = lo[s + r, :, pl.ds(n * 128, 128)]
                wo2[s + r, n] = pltpu.bitcast(t, u32)
                acc[n] = acc[n] + _dot(lhs, t)
        for r in range(8):
            @pl.when(s + r < OV)
            def _():
                o32[jnp.minimum(s + r, OV - 1)] = lo[s + r].astype(f32)
        return tuple(acc)

    acc = lax.fori_loop(0, 4, f_body, (zero8,) * NM)
    x1 = [_rbf(x0[n] + _rbf(_rowsum(acc[n]))) for n in range(NM)]

    mean1, rstd1 = _stats(x1)
    ln1 = [(x - mean1) * rstd1 for x in x1]
    sig1 = _router(ln1, wr)
    lhs1 = [jnp.concatenate([x1[kt], ones8], axis=0) for kt in range(NM)]

    hh1 = []
    for ft in range(NF):
        og = ou = None
        for kt in range(NM):
            a = _dot(lhs1[kt], _tile(gt, ft, kt))
            b = _dot(lhs1[kt], _tile(ut, ft, kt))
            og = a if og is None else og + a
            ou = b if ou is None else ou + b
        csg[ft] = og[8:16]
        csu[ft] = ou[8:16]
        g = rstd1 * (og[0:8] - mean1 * og[8:16])
        u = rstd1 * (ou[0:8] - mean1 * ou[8:16])
        hh1.append(_silu(g) * u)
        if ft < 12:
            hh_s[ft] = hh1[ft]

    def down2(ft, n, hh):
        if ft < 12:
            return _dot(hh, _tile(wd2, ft, n))
        if ft == 12:
            return _dot(hh, ld[pl.ds(12 * 128, 128), pl.ds(n * 128, 128)])
        return _dot(hh[:, :64], ld[pl.ds(13 * 128, 64), pl.ds(n * 128, 128)])

    def h_body(i, y):
        s = pl.multiple_of(i * 512, 512)
        wait_dyn(("d", 0), i, lambda _: [(wd_hbm.at[pl.ds(s, 512)], ld.at[pl.ds(s, 512)])])
        y = list(y)
        for j in range(4):
            ft = i * 4 + j
            sf = pl.multiple_of(s + j * 128, 128)
            hh = hh_s[ft]
            for n in range(NM):
                t = ld[pl.ds(sf, 128), pl.ds(n * 128, 128)]
                wd2[ft, n] = pltpu.bitcast(t, u32)
                y[n] = y[n] + _dot(hh, t)
        for j in range(4):
            ft = i * 4 + j
            sf = pl.multiple_of(s + j * 128, 128)

            if DV:
                @pl.when(ft < DV)
                def _():
                    sd = pl.multiple_of(jnp.minimum(ft, DV - 1) * 128, 128)
                    d32[pl.ds(sd, 128), :] = ld[pl.ds(sf, 128), :].astype(f32)
        return tuple(y)

    y = list(lax.fori_loop(0, 3, h_body, (zero8,) * NM))
    wait(("d", 3))
    for ft in (12, 13):
        for n in range(NM):
            y[n] = y[n] + down2(ft, n, hh1[ft])
    x2 = [_rbf(x1[n] + _rbf(ln1[n] + _rbf(y[n] * sig1))) for n in range(NM)]

    mean2, rstd2 = _stats(x2)
    raw = {}
    for h in range(H):
        o = None
        for kt in range(NM):
            t = _dot(x2[kt], _tile(wq, h, pl.ds(kt * 64, 64)))
            o = t if o is None else o + t
        raw[h] = o
    qv = {}
    for i in range(0, BV, 3):
        hs = list(range(i, min(i + 3, BV)))
        xbs = []
        for h in hs:
            g, r = divmod(h, 8)
            qh = raw[h][0:1] - mean2[0:1] * csq[g, pl.ds(r, 1), :]
            xbs.append(_xb(qh))
        accs = _vmac3([[None] * NC for _ in hs], xbs,
                      lambda j, s, ct: b32[hs[j], ct, pl.ds(s * 8, 8), :])
        for j, h in enumerate(hs):
            for ct in range(NC):
                qv[h, ct] = _rowsum(accs[j][ct]) * rstd2
    q = {}
    for g in range(BV // 8, 4):
        rawg = zero8
        for r in range(8):
            if g * 8 + r >= BV:
                rawg = jnp.where(masks[r], raw[g * 8 + r], rawg)
        q[g] = rstd2 * (rawg - mean2 * csq[g])
    qa = []
    for ct in range(NC):
        qg = [zero8] * 4
        for h in range(H):
            g, r = divmod(h, 8)
            o = qv[h, ct] if h < BV else _dot(q[g], _tile(wukt, h, ct))
            qg[g] = jnp.where(masks[r], o, qg[g])
        qa.append(jnp.concatenate(qg, axis=0))

    def scores(b):
        ss = []
        for j in range(KB):
            kt = b * KB + j
            sc = None
            for ct in range(NC):
                o = _dot(qa[ct], _tile(ckvt, kt, ct))
                sc = o if sc is None else sc + o
            ss.append(sc * SCALE)
        return ss

    def soft(ss, m, l):
        mb = ss[0]
        for j in range(1, KB):
            mb = jnp.maximum(mb, ss[j])
        mb = jnp.max(mb, axis=1, keepdims=True)
        m_new = mb if m is None else jnp.maximum(m, mb)
        ps = [jnp.exp(sj - m_new) for sj in ss]
        lb = ps[0]
        for j in range(1, KB):
            lb = lb + ps[j]
        if m is None:
            return ps, m_new, lb, None
        alpha = jnp.exp(m - m_new)
        return ps, m_new, l * alpha + lb, alpha

    def ctxc(b, ps, alpha, acc):
        if acc is not None:
            acc = [a * alpha for a in acc]
        else:
            acc = [None] * NC
        acc = list(acc)
        last = b == NB - 1
        seq = ([(j, ct) for ct in range(NC) for j in range(KB)] if last
               else [(j, ct) for j in range(KB) for ct in range(NC)])
        for j, ct in seq:
            kt = b * KB + j
            o = _dot(ps[j], _tile(lckv, ct, pl.ds(kt * 64, 64)))
            acc[ct] = o if acc[ct] is None else acc[ct] + o
        return acc

    s0 = scores(0)
    s1 = scores(1)
    p0, m, l, al0 = soft(s0, None, None)
    acc = ctxc(0, p0, None, None)
    s2 = scores(2)
    p1, m, l, al1 = soft(s1, m, l)
    acc = ctxc(1, p1, al1, acc)
    s3 = scores(3)
    p2, m, l, al2 = soft(s2, m, l)
    acc = ctxc(2, p2, al2, acc)
    p3, m, l, al3 = soft(s3, m, l)
    acc = ctxc(3, p3, al3, acc)
    linv = 1.0 / jnp.sum(l, axis=1, keepdims=True)

    accv = [[None] * NM for _ in range(3)]
    accm = [None] * NM

    def e_tiles(hs, cts, part):
        for ct in cts:
            for h in hs:
                g = h // 8
                o = _dot(acc[ct][g * 8:(g + 1) * 8], _tile(wuv, h, pl.ds(ct * 64, 64)))
                part[h] = o if h not in part else part[h] + o

    def head_ctx(h, part):
        g, r = divmod(h, 8)
        return part.pop(h)[r:r + 1] * linv[h:h + 1]

    def f_vpu(hs, part, accv):
        xbs = [_xb(head_ctx(h, part)) for h in hs]
        return _vmac3(accv, xbs, lambda j, s, n: o32[hs[j], pl.ds(s * 8, 8), pl.ds(n * 128, 128)])

    part = {}
    trip = [list(range(i, min(i + 3, OV))) for i in range(0, OV, 3)]
    e_tiles(trip[0], range(3), part)
    e_tiles(trip[1], range(3), part)
    e_tiles(trip[0], [3], part)
    accv = f_vpu(trip[0], part, accv)
    e_tiles(trip[1], [3], part)
    accv = f_vpu(trip[1], part, accv)
    for hs in trip[2:]:
        e_tiles(hs, range(NC), part)
        accv = f_vpu(hs, part, accv)
    lhs_m = {}
    for h in range(OV, H):
        e_tiles([h], range(NC), part)
        g, r = divmod(h, 8)
        lhs_m[h] = jnp.where(masks[r], part.pop(h) * linv[g * 8:(g + 1) * 8], 0.0)
    for n in range(NM):
        for h in range(OV, H):
            o = _dot(lhs_m[h], _tile(wo2, h, n))
            accm[n] = o if accm[n] is None else accm[n] + o
    x3 = [_rbf(x2[n] + _rbf(_rowsum(accm[n] + _fold3(accv, n)))) for n in range(NM)]
    mean3, rstd3 = _stats(x3)
    ln3 = [(x - mean3) * rstd3 for x in x3]
    sig3 = _router(ln3, wr)
    xb3 = []
    for kt in range(GV):
        xb3 += _xb(x3[kt][0:1])
    hh = []
    blocks = [list(range(G0))] + [list(range(i, min(i + GB, NF))) for i in range(G0, NF, GB)]
    for fts in blocks:
        av = {}
        for s in range(16):
            for kt in range(GV):
                for ft in fts:
                    for nm, ref in (("g", g32), ("u", u32s)):
                        p = xb3[kt * 16 + s] * ref[ft, pl.ds(kt * 128 + s * 8, 8), :]
                        key = (nm, ft, kt)
                        av[key] = p if key not in av else av[key] + p
        for ft in fts:
            og = ou = None
            for kt in range(GV, NM):
                a = _dot(x3[kt], _tile(gt, ft, kt))
                b = _dot(x3[kt], _tile(ut, ft, kt))
                og = a if og is None else og + a
                ou = b if ou is None else ou + b
            tot = lambda nm: functools.reduce(lambda a, b: a + b, [av[nm, ft, kt] for kt in range(GV)])
            g = rstd3 * (og + _rowsum(tot("g")) - mean3 * csg[ft])
            u = rstd3 * (ou + _rowsum(tot("u")) - mean3 * csu[ft])
            hh.append(_silu(g) * u)
    y = [None] * NM
    for ft in range(DV, NF):
        for n in range(NM):
            o = down2(ft, n, hh[ft])
            y[n] = o if y[n] is None else y[n] + o
    yv = [[None] * NM for _ in range(3)]
    for i in range(0, DV, 3):
        fs = list(range(i, min(i + 3, DV)))
        yv = _vmac3(yv, [_xb(hh[ft][0:1]) for ft in fs],
                    lambda j, s, n: d32[pl.ds(fs[j] * 128 + s * 8, 8), pl.ds(n * 128, 128)])
    if DV:
        y = [y[n] + _rowsum(_fold3(yv, n)) for n in range(NM)]
    x4 = [x3[n] + _rbf(ln3[n] + _rbf(y[n] * sig3)) for n in range(NM)]
    out = jnp.concatenate([x[0:1, :] for x in x4], axis=1)
    o_ref[0] = out.astype(bf16)


@jax.jit
def pallas_interleave_layers__compressed_kv_cla__moe_arch_mod__decode_kernel(
    A_x: jax.Array,
    A_c_kv: jax.Array,
    A_w_q: jax.Array,
    A_w_uk: jax.Array,
    A_w_uv: jax.Array,
    A_w_o: jax.Array,
    B_x: jax.Array,
    B_w_r: jax.Array,
    B_w_gate: jax.Array,
    B_w_up: jax.Array,
    B_w_down: jax.Array,
):
    del B_x
    any_spec = pl.BlockSpec(memory_space=pl.ANY)
    V = pltpu.VMEM
    scratch = [
        V((1, 1, M), bf16),
        V((NM, 128), bf16),
        V((M, H, D), bf16),
        V((DC, H, D), bf16),
        V((DC, H, D), bf16),
        V((NC, SK // 2, 128), u32),
        V((H, D, M), bf16),
        V((F, M), bf16),
        V((F, M), bf16),
        V((F, M), bf16),
        V((H, M // 2, D), u32),
        V((H, NC, D // 2, 128), u32),
        V((H, DC // 2, D), u32),
        V((NK, NC, 64, 128), u32),
        V((NF, NM, 64, 128), u32),
        V((NF, NM, 64, 128), u32),
        V((NF, max(GV, 1) * 128, 128), f32),
        V((NF, max(GV, 1) * 128, 128), f32),
        V((max(DV, 1) * 128, M), f32),
        V((max(OV, 1), D, M), f32),
        V((max(BV, 1), NC, D, 128), f32),
        V((H, max(AV, 1) * 128, D), f32),
        V((H, NM, 64, 128), u32),
        V((NF, NM, 64, 128), u32),
        V((4, 8, 128), f32),
        V((NF, 8, 128), f32),
        V((NF, 8, 128), f32),
        V((NC, H, 128), f32),
        V((NC, H, 128), f32),
        V((4, 8, 128), f32),
        V((NF, 8, 128), f32),
        V((NM, 8, 128), f32),
        pltpu.SemaphoreType.DMA((32,)),
    ]
    return pl.pallas_call(
        _kernel,
        out_shape=jax.ShapeDtypeStruct((1, 1, M), bf16),
        in_specs=[any_spec] * 10,
        out_specs=pl.BlockSpec(memory_space=pltpu.VMEM),
        scratch_shapes=scratch,
        compiler_params=pltpu.CompilerParams(
            vmem_limit_bytes=100 * 1024 * 1024,
            disable_semaphore_checks=True,
        ),
    )(A_x, A_c_kv, A_w_q, A_w_uk, A_w_uv, A_w_o, B_w_r.reshape(NM, 128),
      B_w_gate.T, B_w_up.T, B_w_down)
```

```python
import functools

import jax
import jax.numpy as jnp
from jax import lax
import jax.experimental.pallas as pl
import jax.experimental.pallas.tpu as pltpu

f32 = jnp.float32
bf16 = jnp.bfloat16
u32 = jnp.uint32
i32 = jnp.int32

M = 640
H = 32
D = 128
DC = 512
SK = 4096
F = 1728
NM = M // 128
NC = DC // 128
NK = SK // 128
NF = 14
EPS = 1e-5
SCALE = float(D) ** -0.5
KB = 8
NB = NK // KB
GV = 1
DV = 9
OV = 21
AV = 0
GB = 2
DRC = 384
DR0 = 768
DGROUPS = ((0,1),(2,3),(4,))
G0 = 3
BV = 12


def _dot(a, b):
    return jnp.dot(a, b, preferred_element_type=f32)


def _rbf(x):
    return x.astype(bf16).astype(f32)


def _tile(ref, *idx):
    return pltpu.bitcast(ref[idx], bf16)


def _stats(xs):
    s = xs[0] + xs[1] + xs[2] + xs[3] + xs[4]
    mean = jnp.sum(s, axis=1, keepdims=True) * (1.0 / M)
    ds = [x - mean for x in xs]
    q = ds[0] * ds[0] + ds[1] * ds[1] + ds[2] * ds[2] + ds[3] * ds[3] + ds[4] * ds[4]
    var = jnp.sum(q, axis=1, keepdims=True) * (1.0 / M)
    rstd = 1.0 / jnp.sqrt(var + EPS)
    return mean, rstd


def _router(lns, wr):
    s = lns[0] * wr[0] + lns[1] * wr[1] + lns[2] * wr[2] + lns[3] * wr[3] + lns[4] * wr[4]
    r = jnp.sum(s, axis=1, keepdims=True)
    return jax.nn.sigmoid(r)


def _rowsum(x):
    return jnp.broadcast_to(jnp.sum(x, axis=0, keepdims=True), x.shape)


def _xb(row):
    t = jnp.broadcast_to(row, (128, 128)).T
    return [t[s * 8:(s + 1) * 8] for s in range(16)]


def _vmac(acc, xb, load):
    for s, xs in enumerate(xb):
        p = xs * load(s)
        acc = p if acc is None else acc + p
    return acc


def _vmacs(accs, xb, load):
    accs = list(accs)
    for s, xs in enumerate(xb):
        for i in range(len(accs)):
            p = xs * load(s, i)
            accs[i] = p if accs[i] is None else accs[i] + p
    return accs


def _vmac3(accs, xbs, load):
    accs = [list(a) for a in accs]
    for s in range(16):
        for j, xb in enumerate(xbs):
            for i in range(len(accs[j])):
                p = xb[s] * load(j, s, i)
                accs[j][i] = p if accs[j][i] is None else accs[j][i] + p
    return accs


def _fold3(accs, i):
    t = [a[i] for a in accs if a[i] is not None]
    return functools.reduce(lambda a, b: a + b, t)


def _silu(g):
    return g * jax.nn.sigmoid(g)


def _kernel(x_hbm, ckv_hbm, wq_hbm, wuk_hbm, wuv_hbm, wo_hbm, wr_hbm, wg_hbm, wu_hbm, wd_hbm,
            o_ref,
            x_v, wr_v, lq, luk, luv, lckv, lo, lg, lu, ld,
            wq, wukt, wuv, ckvt, gt, ut, g32, u32s, d32, o32, b32, q32, wo2, wd2,
            csq, csg, csu, qa_s, cc_s, ctx_s, hh_s, x_s,
            sems):
    row8 = lax.broadcasted_iota(i32, (8, 128), 0)
    masks = [row8 == r for r in range(8)]

    copies = {}
    order = []

    def add(name, pairs):
        sem = sems.at[len(copies)]
        cs = [pltpu.make_async_copy(s, d, sem) for s, d in pairs]
        copies[name] = cs
        order.append(name)

    add("x", [(x_hbm, x_v)])
    add("wr", [(wr_hbm, wr_v)])
    for i in range(NM):
        add(("q", i), [(wq_hbm.at[pl.ds(i * 128, 128)], lq.at[pl.ds(i * 128, 128)])])
    for i in range(NC):
        add(("uk", i), [(wuk_hbm.at[pl.ds(i * 128, 128)], luk.at[pl.ds(i * 128, 128)])])
    ckv32 = ckv_hbm.at[0].bitcast(u32)
    for b in range(NB):
        add(("ckv", b), [(ckv32.at[pl.ds(b * 512, 512), pl.ds(ct * 128, 128)],
                          lckv.at[ct, pl.ds(b * 512, 512)]) for ct in range(NC)])
    FS = [(0, 896), (896, F - 896)]
    for i, (s, n) in enumerate(FS):
        add(("g", i), [(wg_hbm.at[pl.ds(s, n)], lg.at[pl.ds(s, n)])])
    for i, (s, n) in enumerate(FS):
        add(("u", i), [(wu_hbm.at[pl.ds(s, n)], lu.at[pl.ds(s, n)])])
    for i in range(NC):
        add(("uv", i), [(wuv_hbm.at[pl.ds(i * 128, 128)], luv.at[pl.ds(i * 128, 128)])])
    for g in range(4):
        add(("o", g), [(wo_hbm.at[pl.ds(g * 8, 8)], lo.at[pl.ds(g * 8, 8)])])
    for i in range(DR0 // DRC):
        add(("d", i), [(wd_hbm.at[pl.ds(i * DRC, DRC)], ld.at[pl.ds(i * DRC, DRC)])])
    for i, cols in enumerate(DGROUPS):
        c0, nc = cols[0] * 128, len(cols) * 128
        add(("dc", i), [(wd_hbm.at[pl.ds(DR0, F - DR0), pl.ds(c0, nc)],
                         ld.at[pl.ds(DR0, F - DR0), pl.ds(c0, nc)])])

    for name in order:
        for c in copies[name]:
            c.start()

    def wait(name):
        for c in copies[name]:
            c.wait()

    names = list(copies)

    def wait_dyn(first_name, i, pairs_fn):
        base = names.index(first_name)
        for s, d in pairs_fn(i):
            pltpu.make_async_copy(s, d, sems.at[base + i]).wait()

    wait("x")
    wait("wr")
    xr = x_v[0].astype(f32)
    x0 = [jnp.broadcast_to(xr[:, n * 128:(n + 1) * 128], (8, 128)) for n in range(NM)]
    wrf = wr_v[...].astype(f32)
    wr = [jnp.broadcast_to(wrf[n:n + 1, :], (8, 128)) for n in range(NM)]
    for n in range(NM):
        x_s[n] = x0[n]
    mean0, rstd0 = _stats(x0)
    ones8 = jnp.ones((8, 128), f32)
    zero8 = jnp.zeros((8, 128), f32)

    def a_body(kt, carry):
        raw, cs = carry
        s = pl.multiple_of(kt * 128, 128)
        wait_dyn(("q", 0), kt, lambda i: [(wq_hbm.at[pl.ds(s, 128)], lq.at[pl.ds(s, 128)])])
        t = jnp.swapaxes(lq[pl.ds(s, 128)], 0, 1)
        s2 = pl.multiple_of(kt * 64, 64)
        for h in range(H):
            wq[h, pl.ds(s2, 64), :] = pltpu.bitcast(t[h], u32)
        if AV:
            @pl.when(kt < AV)
            def _():
                sv = pl.multiple_of(jnp.minimum(kt, AV - 1) * 128, 128)
                for h in range(H):
                    w = wq[h, pl.ds(s2, 64), :]
                    q32[h, pl.ds(sv, 128), :] = pltpu.bitcast(w, bf16).astype(f32)
        lhs = jnp.concatenate([x_s[kt], ones8], axis=0)
        raw, cs = list(raw), list(cs)
        for h in range(H):
            g, r = divmod(h, 8)
            out = _dot(lhs, pltpu.bitcast(wq[h, pl.ds(s2, 64), :], bf16))
            raw[g] = jnp.where(masks[r], raw[g] + out[0:8], raw[g])
            cs[g] = jnp.where(masks[r], cs[g] + out[8:16], cs[g])
        return tuple(raw), tuple(cs)

    raw, cs = lax.fori_loop(0, NM, a_body, ((zero8,) * 4, (zero8,) * 4))
    for g in range(4):
        csq[g] = cs[g]
    q = [rstd0 * (raw[g] - mean0 * cs[g]) for g in range(4)]

    def b_body(ct, _):
        s = pl.multiple_of(ct * 128, 128)
        wait_dyn(("uk", 0), ct, lambda i: [(wuk_hbm.at[pl.ds(s, 128)], luk.at[pl.ds(s, 128)])])
        t = jnp.swapaxes(luk[pl.ds(s, 128)], 0, 1)
        for h in range(H):
            th = t[h].T
            wukt[h, ct] = pltpu.bitcast(th, u32)
            if h < BV:
                b32[h, ct] = th.astype(f32)
        qa = [zero8] * 4
        for h in range(H):
            g, r = divmod(h, 8)
            out = _dot(q[g], pltpu.bitcast(wukt[h, ct], bf16))
            qa[g] = jnp.where(masks[r], out, qa[g])
        qa_s[ct] = jnp.concatenate(qa, axis=0)
        return _

    lax.fori_loop(0, NC, b_body, 0)

    def cd_body(b, carry):
        m, l, acc = carry
        s = pl.multiple_of(b * 512, 512)
        wait_dyn(("ckv", 0), b, lambda i: [(ckv32.at[pl.ds(s, 512), pl.ds(ct * 128, 128)],
                                            lckv.at[ct, pl.ds(s, 512)]) for ct in range(NC)])
        ss = []
        for j in range(KB):
            kt = b * KB + j
            sk = pl.multiple_of(s + j * 64, 64)
            sc = None
            for ct in range(NC):
                t = pltpu.bitcast(lckv[ct, pl.ds(sk, 64), :], bf16).T
                ckvt[kt, ct] = pltpu.bitcast(t, u32)
                o = _dot(qa_s[ct], t)
                sc = o if sc is None else sc + o
            ss.append(sc * SCALE)
        mb = ss[0]
        for j in range(1, KB):
            mb = jnp.maximum(mb, ss[j])
        m_new = jnp.maximum(m, jnp.max(mb, axis=1, keepdims=True))
        alpha = jnp.exp(m - m_new)
        ps = [jnp.exp(sj - m_new) for sj in ss]
        lb = ps[0]
        for j in range(1, KB):
            lb = lb + ps[j]
        l = l * alpha + lb
        acc = [a * alpha for a in acc]
        for j in range(KB):
            sk = pl.multiple_of(s + j * 64, 64)
            for ct in range(NC):
                acc[ct] = acc[ct] + _dot(ps[j], pltpu.bitcast(lckv[ct, pl.ds(sk, 64), :], bf16))
        return m_new, l, acc

    m_init = jnp.full((H, 128), -jnp.inf, f32)
    _, l, acc = lax.fori_loop(0, NB, cd_body,
                              (m_init, jnp.zeros((H, 128), f32),
                               [jnp.zeros((H, 128), f32)] * NC))
    linv = 1.0 / jnp.sum(l, axis=1, keepdims=True)
    for ct in range(NC):
        cc_s[ct] = acc[ct]

    def transpose_ffn(land, dst, dst32, fam):
        def body(ft, _):
            s = pl.multiple_of(ft * 128, 128)
            for kt in range(NM):
                t = land[pl.ds(s, 128), pl.ds(kt * 128, 128)].T
                dst[ft, kt] = pltpu.bitcast(t, u32)
                if kt < GV:
                    dst32[ft, pl.ds(kt * 128, 128), :] = t.astype(f32)
            return _
        wait((fam, 0))
        lax.fori_loop(0, 7, body, 0)
        wait((fam, 1))
        lax.fori_loop(7, 13, body, 0)
        for kt in range(NM):
            t = land[pl.ds(13 * 128, 64), pl.ds(kt * 128, 128)]
            t = jnp.concatenate([t, jnp.zeros((64, 128), bf16)], axis=0)
            t = t.T
            dst[13, kt] = pltpu.bitcast(t, u32)
            if kt < GV:
                dst32[13, pl.ds(kt * 128, 128), :] = t.astype(f32)

    transpose_ffn(lg, gt, g32, "g")
    transpose_ffn(lu, ut, u32s, "u")

    def e_body(ct, ctx):
        s = pl.multiple_of(ct * 128, 128)
        wait_dyn(("uv", 0), ct, lambda i: [(wuv_hbm.at[pl.ds(s, 128)], luv.at[pl.ds(s, 128)])])
        t = jnp.swapaxes(luv[pl.ds(s, 128)], 0, 1)
        s2 = pl.multiple_of(ct * 64, 64)
        for h in range(H):
            wuv[h, pl.ds(s2, 64), :] = pltpu.bitcast(t[h], u32)
        ctx = list(ctx)
        cc = cc_s[ct]
        for h in range(H):
            g, r = divmod(h, 8)
            out = _dot(cc[g * 8:(g + 1) * 8], pltpu.bitcast(wuv[h, pl.ds(s2, 64), :], bf16))
            ctx[g] = jnp.where(masks[r], ctx[g] + out, ctx[g])
        return tuple(ctx)

    ctx = lax.fori_loop(0, NC, e_body, (zero8,) * 4)
    for g in range(4):
        ctx_s[g] = ctx[g] * linv[g * 8:(g + 1) * 8]

    def f_body(g, acc):
        s = pl.multiple_of(g * 8, 8)
        wait_dyn(("o", 0), g, lambda i: [(wo_hbm.at[pl.ds(s, 8)], lo.at[pl.ds(s, 8)])])
        acc = list(acc)
        cg = ctx_s[g]
        for r in range(8):
            lhs = jnp.where(masks[r], cg, 0.0)
            for n in range(NM):
                t = lo[s + r, :, pl.ds(n * 128, 128)]
                wo2[s + r, n] = pltpu.bitcast(t, u32)
                acc[n] = acc[n] + _dot(lhs, t)
        for r in range(8):
            @pl.when(s + r < OV)
            def _():
                o32[jnp.minimum(s + r, OV - 1)] = lo[s + r].astype(f32)
        return tuple(acc)

    acc = lax.fori_loop(0, 4, f_body, (zero8,) * NM)
    x1 = [_rbf(x0[n] + _rbf(_rowsum(acc[n]))) for n in range(NM)]

    mean1, rstd1 = _stats(x1)
    ln1 = [(x - mean1) * rstd1 for x in x1]
    sig1 = _router(ln1, wr)
    lhs1 = [jnp.concatenate([x1[kt], ones8], axis=0) for kt in range(NM)]

    hh1 = []
    NE_ = DR0 // 128
    for ft in range(NF):
        og = ou = None
        for kt in range(NM):
            a = _dot(lhs1[kt], _tile(gt, ft, kt))
            b = _dot(lhs1[kt], _tile(ut, ft, kt))
            og = a if og is None else og + a
            ou = b if ou is None else ou + b
        csg[ft] = og[8:16]
        csu[ft] = ou[8:16]
        g = rstd1 * (og[0:8] - mean1 * og[8:16])
        u = rstd1 * (ou[0:8] - mean1 * ou[8:16])
        hh1.append(_silu(g) * u)
        if ft < NE_:
            hh_s[ft] = hh1[ft]

    NE = DR0 // 128

    def wd_tile(ft, n):
        if ft < NE:
            return _tile(wd2, ft, n)
        return ld[pl.ds(ft * 128, min(128, F - ft * 128)), pl.ds(n * 128, 128)]

    def down2(ft, n, hh):
        return _dot(hh if ft < 13 else hh[:, :64], wd_tile(ft, n))

    def wd_f32(ft, s, n):
        if ft < NE:
            return d32[pl.ds(ft * 128 + s * 8, 8), pl.ds(n * 128, 128)]
        return wd_tile(ft, n).astype(f32)[s * 8:(s + 1) * 8]

    FPC = DRC // 128

    def h_body(i, y):
        s = pl.multiple_of(i * DRC, 128)
        wait_dyn(("d", 0), i, lambda _: [(wd_hbm.at[pl.ds(s, DRC)], ld.at[pl.ds(s, DRC)])])
        y = list(y)
        for j in range(FPC):
            ft = i * FPC + j
            sf = pl.multiple_of(s + j * 128, 128)
            hh = hh_s[ft]
            for n in range(NM):
                t = ld[pl.ds(sf, 128), pl.ds(n * 128, 128)]
                wd2[ft, n] = pltpu.bitcast(t, u32)
                y[n] = y[n] + _dot(hh, t)
        for j in range(FPC):
            ft = i * FPC + j
            sf = pl.multiple_of(s + j * 128, 128)
            if DV:
                @pl.when(ft < DV)
                def _():
                    sd = pl.multiple_of(jnp.minimum(ft, min(DV, NE) - 1) * 128, 128)
                    d32[pl.ds(sd, 128), :] = ld[pl.ds(sf, 128), :].astype(f32)
        return tuple(y)

    y = list(lax.fori_loop(0, DR0 // DRC, h_body, (zero8,) * NM))

    x2 = [None] * NM
    racc = [None] * 4

    def h_late(n):
        for ft in range(NE, NF):
            y[n] = y[n] + down2(ft, n, hh1[ft])
        x2[n] = _rbf(x1[n] + _rbf(ln1[n] + _rbf(y[n] * sig1)))

    def a_pass(kt):
        for h in range(H):
            g, r = divmod(h, 8)
            o = _dot(jnp.where(masks[r], x2[kt], 0.0), _tile(wq, h, pl.ds(kt * 64, 64)))
            racc[g] = o if racc[g] is None else racc[g] + o

    wait(("dc", 0))
    h_late(0)
    h_late(1)
    a_pass(0)
    a_pass(1)
    wait(("dc", 1))
    h_late(2)
    h_late(3)
    a_pass(2)
    wait(("dc", 2))
    h_late(4)
    a_pass(3)
    mean2, rstd2 = _stats(x2)
    raw = {}
    KL = DGROUPS[-1][-1]
    horder = list(range(0, 3)) + list(range(BV, H)) + list(range(3, BV))
    for h in horder:
        raw[h] = racc[h // 8] + _dot(x2[KL], _tile(wq, h, pl.ds(KL * 64, 64)))
    qv = {}
    for i in range(0, BV, 3):
        hs = list(range(i, min(i + 3, BV)))
        xbs = []
        for h in hs:
            g, r = divmod(h, 8)
            qh = raw[h][r:r + 1] - mean2[0:1] * csq[g, pl.ds(r, 1), :]
            xbs.append(_xb(qh))
        accs = _vmac3([[None] * NC for _ in hs], xbs,
                      lambda j, s, ct: b32[hs[j], ct, pl.ds(s * 8, 8), :])
        for j, h in enumerate(hs):
            for ct in range(NC):
                qv[h, ct] = _rowsum(accs[j][ct]) * rstd2
    q = {}
    for g in range(BV // 8, 4):
        rawg = zero8
        for r in range(8):
            if g * 8 + r >= BV:
                rawg = jnp.where(masks[r], raw[g * 8 + r], rawg)
        q[g] = rstd2 * (rawg - mean2 * csq[g])
    qa = []
    for ct in range(NC):
        qg = [zero8] * 4
        for h in range(H):
            g, r = divmod(h, 8)
            o = qv[h, ct] if h < BV else _dot(q[g], _tile(wukt, h, ct))
            qg[g] = jnp.where(masks[r], o, qg[g])
        qa.append(jnp.concatenate(qg, axis=0))

    def scores(b):
        ss = []
        for j in range(KB):
            kt = b * KB + j
            sc = None
            for ct in range(NC):
                o = _dot(qa[ct], _tile(ckvt, kt, ct))
                sc = o if sc is None else sc + o
            ss.append(sc * SCALE)
        return ss

    def soft(ss, m, l):
        mb = ss[0]
        for j in range(1, KB):
            mb = jnp.maximum(mb, ss[j])
        mb = jnp.max(mb, axis=1, keepdims=True)
        m_new = mb if m is None else jnp.maximum(m, mb)
        ps = [jnp.exp(sj - m_new) for sj in ss]
        lb = ps[0]
        for j in range(1, KB):
            lb = lb + ps[j]
        if m is None:
            return ps, m_new, lb, None
        alpha = jnp.exp(m - m_new)
        return ps, m_new, l * alpha + lb, alpha

    def ctxc(b, ps, alpha, acc):
        if acc is not None:
            acc = [a * alpha for a in acc]
        else:
            acc = [None] * NC
        acc = list(acc)
        last = b == NB - 1
        seq = ([(j, ct) for ct in range(NC) for j in range(KB)] if last
               else [(j, ct) for j in range(KB) for ct in range(NC)])
        for j, ct in seq:
            kt = b * KB + j
            o = _dot(ps[j], _tile(lckv, ct, pl.ds(kt * 64, 64)))
            acc[ct] = o if acc[ct] is None else acc[ct] + o
        return acc

    s0 = scores(0)
    s1 = scores(1)
    p0, m, l, al0 = soft(s0, None, None)
    acc = ctxc(0, p0, None, None)
    s2 = scores(2)
    p1, m, l, al1 = soft(s1, m, l)
    acc = ctxc(1, p1, al1, acc)
    s3 = scores(3)
    p2, m, l, al2 = soft(s2, m, l)
    acc = ctxc(2, p2, al2, acc)
    p3, m, l, al3 = soft(s3, m, l)
    acc = ctxc(3, p3, al3, acc)
    linv = 1.0 / jnp.sum(l, axis=1, keepdims=True)

    accv = [[None] * NM for _ in range(3)]
    accm = [None] * NM

    def e_tiles(hs, cts, part):
        for ct in cts:
            for h in hs:
                g = h // 8
                o = _dot(acc[ct][g * 8:(g + 1) * 8], _tile(wuv, h, pl.ds(ct * 64, 64)))
                part[h] = o if h not in part else part[h] + o

    def head_ctx(h, part):
        g, r = divmod(h, 8)
        return part.pop(h)[r:r + 1] * linv[h:h + 1]

    def f_vpu(hs, part, accv):
        xbs = [_xb(head_ctx(h, part)) for h in hs]
        return _vmac3(accv, xbs, lambda j, s, n: o32[hs[j], pl.ds(s * 8, 8), pl.ds(n * 128, 128)])

    part = {}
    trip = [list(range(i, min(i + 3, OV))) for i in range(0, OV, 3)]
    e_tiles(trip[0], range(3), part)
    e_tiles(trip[1], range(3), part)
    e_tiles(trip[0], [3], part)
    accv = f_vpu(trip[0], part, accv)
    e_tiles(trip[1], [3], part)
    accv = f_vpu(trip[1], part, accv)
    for hs in trip[2:]:
        e_tiles(hs, range(NC), part)
        accv = f_vpu(hs, part, accv)
    lhs_m = {}
    for h in range(OV, H):
        e_tiles([h], range(NC), part)
        g, r = divmod(h, 8)
        lhs_m[h] = jnp.where(masks[r], part.pop(h) * linv[g * 8:(g + 1) * 8], 0.0)
    for n in range(NM):
        for h in range(OV, H):
            o = _dot(lhs_m[h], _tile(wo2, h, n))
            accm[n] = o if accm[n] is None else accm[n] + o
    x3 = [_rbf(x2[n] + _rbf(_rowsum(accm[n] + _fold3(accv, n)))) for n in range(NM)]
    mean3, rstd3 = _stats(x3)
    ln3 = [(x - mean3) * rstd3 for x in x3]
    sig3 = _router(ln3, wr)
    xb3 = []
    for kt in range(GV):
        xb3 += _xb(x3[kt][0:1])
    hh = []
    blocks = [list(range(G0))] + [list(range(i, min(i + GB, NF))) for i in range(G0, NF, GB)]
    for fts in blocks:
        av = {}
        for s in range(16):
            for kt in range(GV):
                for ft in fts:
                    for nm, ref in (("g", g32), ("u", u32s)):
                        p = xb3[kt * 16 + s] * ref[ft, pl.ds(kt * 128 + s * 8, 8), :]
                        key = (nm, ft, kt)
                        av[key] = p if key not in av else av[key] + p
        for ft in fts:
            og = ou = None
            for kt in range(GV, NM):
                a = _dot(x3[kt], _tile(gt, ft, kt))
                b = _dot(x3[kt], _tile(ut, ft, kt))
                og = a if og is None else og + a
                ou = b if ou is None else ou + b
            tot = lambda nm: functools.reduce(lambda a, b: a + b, [av[nm, ft, kt] for kt in range(GV)])
            g = rstd3 * (og + _rowsum(tot("g")) - mean3 * csg[ft])
            u = rstd3 * (ou + _rowsum(tot("u")) - mean3 * csu[ft])
            hh.append(_silu(g) * u)
    y = [None] * NM
    for ft in range(DV, NF):
        for n in range(NM):
            o = down2(ft, n, hh[ft])
            y[n] = o if y[n] is None else y[n] + o
    yv = [[None] * NM for _ in range(3)]
    for i in range(0, DV, 3):
        fs = list(range(i, min(i + 3, DV)))
        yv = _vmac3(yv, [_xb(hh[ft][0:1]) for ft in fs],
                    lambda j, s, n: wd_f32(fs[j], s, n))
    if DV:
        y = [y[n] + _rowsum(_fold3(yv, n)) for n in range(NM)]
    x4 = [x3[n] + _rbf(ln3[n] + _rbf(y[n] * sig3)) for n in range(NM)]
    out = jnp.concatenate([x[0:1, :] for x in x4], axis=1)
    o_ref[0] = out.astype(bf16)


@jax.jit
def pallas_interleave_layers__compressed_kv_cla__moe_arch_mod__decode_kernel(
    A_x: jax.Array,
    A_c_kv: jax.Array,
    A_w_q: jax.Array,
    A_w_uk: jax.Array,
    A_w_uv: jax.Array,
    A_w_o: jax.Array,
    B_x: jax.Array,
    B_w_r: jax.Array,
    B_w_gate: jax.Array,
    B_w_up: jax.Array,
    B_w_down: jax.Array,
):
    del B_x
    any_spec = pl.BlockSpec(memory_space=pl.ANY)
    V = pltpu.VMEM
    scratch = [
        V((1, 1, M), bf16),
        V((NM, 128), bf16),
        V((M, H, D), bf16),
        V((DC, H, D), bf16),
        V((DC, H, D), bf16),
        V((NC, SK // 2, 128), u32),
        V((H, D, M), bf16),
        V((F, M), bf16),
        V((F, M), bf16),
        V((F, M), bf16),
        V((H, M // 2, D), u32),
        V((H, NC, D // 2, 128), u32),
        V((H, DC // 2, D), u32),
        V((NK, NC, 64, 128), u32),
        V((NF, NM, 64, 128), u32),
        V((NF, NM, 64, 128), u32),
        V((NF, max(GV, 1) * 128, 128), f32),
        V((NF, max(GV, 1) * 128, 128), f32),
        V((max(min(DV, DR0 // 128), 1) * 128, M), f32),
        V((max(OV, 1), D, M), f32),
        V((max(BV, 1), NC, D, 128), f32),
        V((H, max(AV, 1) * 128, D), f32),
        V((H, NM, 64, 128), u32),
        V((NF, NM, 64, 128), u32),
        V((4, 8, 128), f32),
        V((NF, 8, 128), f32),
        V((NF, 8, 128), f32),
        V((NC, H, 128), f32),
        V((NC, H, 128), f32),
        V((4, 8, 128), f32),
        V((NF, 8, 128), f32),
        V((NM, 8, 128), f32),
        pltpu.SemaphoreType.DMA((40,)),
    ]
    return pl.pallas_call(
        _kernel,
        out_shape=jax.ShapeDtypeStruct((1, 1, M), bf16),
        in_specs=[any_spec] * 10,
        out_specs=pl.BlockSpec(memory_space=pltpu.VMEM),
        scratch_shapes=scratch,
        compiler_params=pltpu.CompilerParams(
            vmem_limit_bytes=100 * 1024 * 1024,
            disable_semaphore_checks=True,
        ),
    )(A_x, A_c_kv, A_w_q, A_w_uk, A_w_uv, A_w_o, B_w_r.reshape(NM, 128),
      B_w_gate.T, B_w_up.T, B_w_down)
```

```python
import functools

import jax
import jax.numpy as jnp
from jax import lax
import jax.experimental.pallas as pl
import jax.experimental.pallas.tpu as pltpu

f32 = jnp.float32
bf16 = jnp.bfloat16
u32 = jnp.uint32
i32 = jnp.int32

M = 640
H = 32
D = 128
DC = 512
SK = 4096
F = 1728
NM = M // 128
NC = DC // 128
NK = SK // 128
NF = 14
EPS = 1e-5
SCALE = float(D) ** -0.5
KB = 8
NB = NK // KB
GV = 1
DV = 9
OV = 21
AV = 0
GB = 2
PRECONV = (0,1,2,3)
DRC = 384
DR0 = 768
DGROUPS = ((0,1),(2,3),(4,))
G0 = 3
BV = 12


def _dot(a, b):
    return jnp.dot(a, b, preferred_element_type=f32)


def _rbf(x):
    return x.astype(bf16).astype(f32)


def _tile(ref, *idx):
    return pltpu.bitcast(ref[idx], bf16)


def _stats(xs):
    s = xs[0] + xs[1] + xs[2] + xs[3] + xs[4]
    mean = jnp.sum(s, axis=1, keepdims=True) * (1.0 / M)
    ds = [x - mean for x in xs]
    q = ds[0] * ds[0] + ds[1] * ds[1] + ds[2] * ds[2] + ds[3] * ds[3] + ds[4] * ds[4]
    var = jnp.sum(q, axis=1, keepdims=True) * (1.0 / M)
    rstd = 1.0 / jnp.sqrt(var + EPS)
    return mean, rstd


def _router(lns, wr):
    s = lns[0] * wr[0] + lns[1] * wr[1] + lns[2] * wr[2] + lns[3] * wr[3] + lns[4] * wr[4]
    r = jnp.sum(s, axis=1, keepdims=True)
    return jax.nn.sigmoid(r)


def _rowsum(x):
    return jnp.broadcast_to(jnp.sum(x, axis=0, keepdims=True), x.shape)


def _xb(row):
    t = jnp.broadcast_to(row, (128, 128)).T
    return [t[s * 8:(s + 1) * 8] for s in range(16)]


def _vmac(acc, xb, load):
    for s, xs in enumerate(xb):
        p = xs * load(s)
        acc = p if acc is None else acc + p
    return acc


def _vmacs(accs, xb, load):
    accs = list(accs)
    for s, xs in enumerate(xb):
        for i in range(len(accs)):
            p = xs * load(s, i)
            accs[i] = p if accs[i] is None else accs[i] + p
    return accs


def _vmac3(accs, xbs, load):
    accs = [list(a) for a in accs]
    for s in range(16):
        for j, xb in enumerate(xbs):
            for i in range(len(accs[j])):
                p = xb[s] * load(j, s, i)
                accs[j][i] = p if accs[j][i] is None else accs[j][i] + p
    return accs


def _fold3(accs, i):
    t = [a[i] for a in accs if a[i] is not None]
    return functools.reduce(lambda a, b: a + b, t)


def _silu(g):
    return g * jax.nn.sigmoid(g)


def _kernel(x_hbm, ckv_hbm, wq_hbm, wuk_hbm, wuv_hbm, wo_hbm, wr_hbm, wg_hbm, wu_hbm, wd_hbm,
            o_ref,
            x_v, wr_v, lq, luk, luv, lckv, lo, lg, lu, ld,
            wq, wukt, wuv, ckvt, gt, ut, g32, u32s, d32, o32, b32, q32, wo2, wd2,
            csq, csg, csu, qa_s, cc_s, ctx_s, hh_s, x_s,
            sems):
    row8 = lax.broadcasted_iota(i32, (8, 128), 0)
    masks = [row8 == r for r in range(8)]

    copies = {}
    order = []

    def add(name, pairs):
        sem = sems.at[len(copies)]
        cs = [pltpu.make_async_copy(s, d, sem) for s, d in pairs]
        copies[name] = cs
        order.append(name)

    add("x", [(x_hbm, x_v)])
    add("wr", [(wr_hbm, wr_v)])
    for i in range(NM):
        add(("q", i), [(wq_hbm.at[pl.ds(i * 128, 128)], lq.at[pl.ds(i * 128, 128)])])
    for i in range(NC):
        add(("uk", i), [(wuk_hbm.at[pl.ds(i * 128, 128)], luk.at[pl.ds(i * 128, 128)])])
    ckv32 = ckv_hbm.at[0].bitcast(u32)
    for b in range(NB):
        add(("ckv", b), [(ckv32.at[pl.ds(b * 512, 512), pl.ds(ct * 128, 128)],
                          lckv.at[ct, pl.ds(b * 512, 512)]) for ct in range(NC)])
    FS = [(0, 896), (896, F - 896)]
    for i, (s, n) in enumerate(FS):
        add(("g", i), [(wg_hbm.at[pl.ds(s, n)], lg.at[pl.ds(s, n)])])
    for i, (s, n) in enumerate(FS):
        add(("u", i), [(wu_hbm.at[pl.ds(s, n)], lu.at[pl.ds(s, n)])])
    for i in range(NC):
        add(("uv", i), [(wuv_hbm.at[pl.ds(i * 128, 128)], luv.at[pl.ds(i * 128, 128)])])
    for g in range(4):
        add(("o", g), [(wo_hbm.at[pl.ds(g * 8, 8)], lo.at[pl.ds(g * 8, 8)])])
    for i in range(DR0 // DRC):
        add(("d", i), [(wd_hbm.at[pl.ds(i * DRC, DRC)], ld.at[pl.ds(i * DRC, DRC)])])
    for i, cols in enumerate(DGROUPS):
        c0, nc = cols[0] * 128, len(cols) * 128
        add(("dc", i), [(wd_hbm.at[pl.ds(DR0, F - DR0), pl.ds(c0, nc)],
                         ld.at[pl.ds(DR0, F - DR0), pl.ds(c0, nc)])])

    for name in order:
        for c in copies[name]:
            c.start()

    def wait(name):
        for c in copies[name]:
            c.wait()

    names = list(copies)

    def wait_dyn(first_name, i, pairs_fn):
        base = names.index(first_name)
        for s, d in pairs_fn(i):
            pltpu.make_async_copy(s, d, sems.at[base + i]).wait()

    wait("x")
    wait("wr")
    xr = x_v[0].astype(f32)
    x0 = [jnp.broadcast_to(xr[:, n * 128:(n + 1) * 128], (8, 128)) for n in range(NM)]
    wrf = wr_v[...].astype(f32)
    wr = [jnp.broadcast_to(wrf[n:n + 1, :], (8, 128)) for n in range(NM)]
    for n in range(NM):
        x_s[n] = x0[n]
    mean0, rstd0 = _stats(x0)
    ones8 = jnp.ones((8, 128), f32)
    zero8 = jnp.zeros((8, 128), f32)

    def a_body(kt, carry):
        raw, cs = carry
        s = pl.multiple_of(kt * 128, 128)
        wait_dyn(("q", 0), kt, lambda i: [(wq_hbm.at[pl.ds(s, 128)], lq.at[pl.ds(s, 128)])])
        t = jnp.swapaxes(lq[pl.ds(s, 128)], 0, 1)
        s2 = pl.multiple_of(kt * 64, 64)
        for h in range(H):
            wq[h, pl.ds(s2, 64), :] = pltpu.bitcast(t[h], u32)
        if AV:
            @pl.when(kt < AV)
            def _():
                sv = pl.multiple_of(jnp.minimum(kt, AV - 1) * 128, 128)
                for h in range(H):
                    w = wq[h, pl.ds(s2, 64), :]
                    q32[h, pl.ds(sv, 128), :] = pltpu.bitcast(w, bf16).astype(f32)
        lhs = jnp.concatenate([x_s[kt], ones8], axis=0)
        raw, cs = list(raw), list(cs)
        for h in range(H):
            g, r = divmod(h, 8)
            out = _dot(lhs, pltpu.bitcast(wq[h, pl.ds(s2, 64), :], bf16))
            raw[g] = jnp.where(masks[r], raw[g] + out[0:8], raw[g])
            cs[g] = jnp.where(masks[r], cs[g] + out[8:16], cs[g])
        return tuple(raw), tuple(cs)

    raw, cs = lax.fori_loop(0, NM, a_body, ((zero8,) * 4, (zero8,) * 4))
    for g in range(4):
        csq[g] = cs[g]
    q = [rstd0 * (raw[g] - mean0 * cs[g]) for g in range(4)]

    def b_body(ct, _):
        s = pl.multiple_of(ct * 128, 128)
        wait_dyn(("uk", 0), ct, lambda i: [(wuk_hbm.at[pl.ds(s, 128)], luk.at[pl.ds(s, 128)])])
        t = jnp.swapaxes(luk[pl.ds(s, 128)], 0, 1)
        for h in range(H):
            th = t[h].T
            wukt[h, ct] = pltpu.bitcast(th, u32)
            if h < BV:
                b32[h, ct] = th.astype(f32)
        qa = [zero8] * 4
        for h in range(H):
            g, r = divmod(h, 8)
            out = _dot(q[g], pltpu.bitcast(wukt[h, ct], bf16))
            qa[g] = jnp.where(masks[r], out, qa[g])
        qa_s[ct] = jnp.concatenate(qa, axis=0)
        return _

    lax.fori_loop(0, NC, b_body, 0)

    def cd_body(b, carry):
        m, l, acc = carry
        s = pl.multiple_of(b * 512, 512)
        wait_dyn(("ckv", 0), b, lambda i: [(ckv32.at[pl.ds(s, 512), pl.ds(ct * 128, 128)],
                                            lckv.at[ct, pl.ds(s, 512)]) for ct in range(NC)])
        ss = []
        for j in range(KB):
            kt = b * KB + j
            sk = pl.multiple_of(s + j * 64, 64)
            sc = None
            for ct in range(NC):
                t = pltpu.bitcast(lckv[ct, pl.ds(sk, 64), :], bf16).T
                ckvt[kt, ct] = pltpu.bitcast(t, u32)
                o = _dot(qa_s[ct], t)
                sc = o if sc is None else sc + o
            ss.append(sc * SCALE)
        mb = ss[0]
        for j in range(1, KB):
            mb = jnp.maximum(mb, ss[j])
        m_new = jnp.maximum(m, jnp.max(mb, axis=1, keepdims=True))
        alpha = jnp.exp(m - m_new)
        ps = [jnp.exp(sj - m_new) for sj in ss]
        lb = ps[0]
        for j in range(1, KB):
            lb = lb + ps[j]
        l = l * alpha + lb
        acc = [a * alpha for a in acc]
        for j in range(KB):
            sk = pl.multiple_of(s + j * 64, 64)
            for ct in range(NC):
                acc[ct] = acc[ct] + _dot(ps[j], pltpu.bitcast(lckv[ct, pl.ds(sk, 64), :], bf16))
        return m_new, l, acc

    m_init = jnp.full((H, 128), -jnp.inf, f32)
    _, l, acc = lax.fori_loop(0, NB, cd_body,
                              (m_init, jnp.zeros((H, 128), f32),
                               [jnp.zeros((H, 128), f32)] * NC))
    linv = 1.0 / jnp.sum(l, axis=1, keepdims=True)
    for ct in range(NC):
        cc_s[ct] = acc[ct]

    def transpose_ffn(land, dst, dst32, fam):
        def body(ft, _):
            s = pl.multiple_of(ft * 128, 128)
            for kt in range(NM):
                t = land[pl.ds(s, 128), pl.ds(kt * 128, 128)].T
                dst[ft, kt] = pltpu.bitcast(t, u32)
                if kt < GV:
                    dst32[ft, pl.ds(kt * 128, 128), :] = t.astype(f32)
            return _
        wait((fam, 0))
        lax.fori_loop(0, 7, body, 0)
        wait((fam, 1))
        lax.fori_loop(7, 13, body, 0)
        for kt in range(NM):
            t = land[pl.ds(13 * 128, 64), pl.ds(kt * 128, 128)]
            t = jnp.concatenate([t, jnp.zeros((64, 128), bf16)], axis=0)
            t = t.T
            dst[13, kt] = pltpu.bitcast(t, u32)
            if kt < GV:
                dst32[13, pl.ds(kt * 128, 128), :] = t.astype(f32)

    transpose_ffn(lg, gt, g32, "g")
    transpose_ffn(lu, ut, u32s, "u")

    def e_body(ct, ctx):
        s = pl.multiple_of(ct * 128, 128)
        wait_dyn(("uv", 0), ct, lambda i: [(wuv_hbm.at[pl.ds(s, 128)], luv.at[pl.ds(s, 128)])])
        t = jnp.swapaxes(luv[pl.ds(s, 128)], 0, 1)
        s2 = pl.multiple_of(ct * 64, 64)
        for h in range(H):
            wuv[h, pl.ds(s2, 64), :] = pltpu.bitcast(t[h], u32)
        ctx = list(ctx)
        cc = cc_s[ct]
        for h in range(H):
            g, r = divmod(h, 8)
            out = _dot(cc[g * 8:(g + 1) * 8], pltpu.bitcast(wuv[h, pl.ds(s2, 64), :], bf16))
            ctx[g] = jnp.where(masks[r], ctx[g] + out, ctx[g])
        return tuple(ctx)

    ctx = lax.fori_loop(0, NC, e_body, (zero8,) * 4)
    for g in range(4):
        ctx_s[g] = ctx[g] * linv[g * 8:(g + 1) * 8]

    def f_body(g, acc):
        s = pl.multiple_of(g * 8, 8)
        wait_dyn(("o", 0), g, lambda i: [(wo_hbm.at[pl.ds(s, 8)], lo.at[pl.ds(s, 8)])])
        acc = list(acc)
        cg = ctx_s[g]
        for r in range(8):
            lhs = jnp.where(masks[r], cg, 0.0)
            for n in range(NM):
                t = lo[s + r, :, pl.ds(n * 128, 128)]
                wo2[s + r, n] = pltpu.bitcast(t, u32)
                acc[n] = acc[n] + _dot(lhs, t)
        for r in range(8):
            @pl.when(s + r < OV)
            def _():
                o32[jnp.minimum(s + r, OV - 1)] = lo[s + r].astype(f32)
        return tuple(acc)

    acc = lax.fori_loop(0, 4, f_body, (zero8,) * NM)
    x1 = [_rbf(x0[n] + _rbf(_rowsum(acc[n]))) for n in range(NM)]

    mean1, rstd1 = _stats(x1)
    ln1 = [(x - mean1) * rstd1 for x in x1]
    sig1 = _router(ln1, wr)
    lhs1 = [jnp.concatenate([x1[kt], ones8], axis=0) for kt in range(NM)]

    hh1 = []
    NE_ = DR0 // 128
    for ft in range(NF):
        og = ou = None
        for kt in range(NM):
            a = _dot(lhs1[kt], _tile(gt, ft, kt))
            b = _dot(lhs1[kt], _tile(ut, ft, kt))
            og = a if og is None else og + a
            ou = b if ou is None else ou + b
        csg[ft] = og[8:16]
        csu[ft] = ou[8:16]
        g = rstd1 * (og[0:8] - mean1 * og[8:16])
        u = rstd1 * (ou[0:8] - mean1 * ou[8:16])
        hh1.append(_silu(g) * u)
        if ft < NE_:
            hh_s[ft] = hh1[ft]

    NE = DR0 // 128

    def wd_tile(ft, n):
        if ft < NE:
            return _tile(wd2, ft, n)
        return ld[pl.ds(ft * 128, min(128, F - ft * 128)), pl.ds(n * 128, 128)]

    def down2(ft, n, hh):
        return _dot(hh if ft < 13 else hh[:, :64], wd_tile(ft, n))

    def wd_f32(ft, s, n):
        if ft < NE or n in PRECONV:
            return d32[pl.ds(ft * 128 + s * 8, 8), pl.ds(n * 128, 128)]
        return wd_tile(ft, n).astype(f32)[s * 8:(s + 1) * 8]

    FPC = DRC // 128

    def h_body(i, y):
        s = pl.multiple_of(i * DRC, 128)
        wait_dyn(("d", 0), i, lambda _: [(wd_hbm.at[pl.ds(s, DRC)], ld.at[pl.ds(s, DRC)])])
        y = list(y)
        for j in range(FPC):
            ft = i * FPC + j
            sf = pl.multiple_of(s + j * 128, 128)
            hh = hh_s[ft]
            for n in range(NM):
                t = ld[pl.ds(sf, 128), pl.ds(n * 128, 128)]
                wd2[ft, n] = pltpu.bitcast(t, u32)
                y[n] = y[n] + _dot(hh, t)
        for j in range(FPC):
            ft = i * FPC + j
            sf = pl.multiple_of(s + j * 128, 128)
            if DV:
                @pl.when(ft < DV)
                def _():
                    sd = pl.multiple_of(jnp.minimum(ft, DV - 1) * 128, 128)
                    d32[pl.ds(sd, 128), :] = ld[pl.ds(sf, 128), :].astype(f32)
        return tuple(y)

    y = list(lax.fori_loop(0, DR0 // DRC, h_body, (zero8,) * NM))

    x2 = [None] * NM
    racc = [None] * 4

    def h_late(n):
        for ft in range(NE, NF):
            y[n] = y[n] + down2(ft, n, hh1[ft])
        x2[n] = _rbf(x1[n] + _rbf(ln1[n] + _rbf(y[n] * sig1)))
        if n in PRECONV:
            for ft in range(NE, DV):
                d32[pl.ds(ft * 128, 128), pl.ds(n * 128, 128)] = wd_tile(ft, n).astype(f32)

    def a_pass(kt):
        for h in range(H):
            g, r = divmod(h, 8)
            o = _dot(jnp.where(masks[r], x2[kt], 0.0), _tile(wq, h, pl.ds(kt * 64, 64)))
            racc[g] = o if racc[g] is None else racc[g] + o

    wait(("dc", 0))
    h_late(0)
    h_late(1)
    a_pass(0)
    a_pass(1)
    wait(("dc", 1))
    h_late(2)
    h_late(3)
    a_pass(2)
    wait(("dc", 2))
    h_late(4)
    a_pass(3)
    mean2, rstd2 = _stats(x2)
    raw = {}
    KL = DGROUPS[-1][-1]
    horder = list(range(0, 3)) + list(range(BV, H)) + list(range(3, BV))
    for h in horder:
        raw[h] = racc[h // 8] + _dot(x2[KL], _tile(wq, h, pl.ds(KL * 64, 64)))
    qv = {}
    for i in range(0, BV, 3):
        hs = list(range(i, min(i + 3, BV)))
        xbs = []
        for h in hs:
            g, r = divmod(h, 8)
            qh = raw[h][r:r + 1] - mean2[0:1] * csq[g, pl.ds(r, 1), :]
            xbs.append(_xb(qh))
        accs = _vmac3([[None] * NC for _ in hs], xbs,
                      lambda j, s, ct: b32[hs[j], ct, pl.ds(s * 8, 8), :])
        for j, h in enumerate(hs):
            for ct in range(NC):
                qv[h, ct] = _rowsum(accs[j][ct]) * rstd2
    q = {}
    for g in range(BV // 8, 4):
        rawg = zero8
        for r in range(8):
            if g * 8 + r >= BV:
                rawg = jnp.where(masks[r], raw[g * 8 + r], rawg)
        q[g] = rstd2 * (rawg - mean2 * csq[g])
    qa = []
    for ct in range(NC):
        qg = [zero8] * 4
        for h in range(H):
            g, r = divmod(h, 8)
            o = qv[h, ct] if h < BV else _dot(q[g], _tile(wukt, h, ct))
            qg[g] = jnp.where(masks[r], o, qg[g])
        qa.append(jnp.concatenate(qg, axis=0))

    def scores(b):
        ss = []
        for j in range(KB):
            kt = b * KB + j
            sc = None
            for ct in range(NC):
                o = _dot(qa[ct], _tile(ckvt, kt, ct))
                sc = o if sc is None else sc + o
            ss.append(sc * SCALE)
        return ss

    def soft(ss, m, l):
        mb = ss[0]
        for j in range(1, KB):
            mb = jnp.maximum(mb, ss[j])
        mb = jnp.max(mb, axis=1, keepdims=True)
        m_new = mb if m is None else jnp.maximum(m, mb)
        ps = [jnp.exp(sj - m_new) for sj in ss]
        lb = ps[0]
        for j in range(1, KB):
            lb = lb + ps[j]
        if m is None:
            return ps, m_new, lb, None
        alpha = jnp.exp(m - m_new)
        return ps, m_new, l * alpha + lb, alpha

    def ctxc(b, ps, alpha, acc):
        if acc is not None:
            acc = [a * alpha for a in acc]
        else:
            acc = [None] * NC
        acc = list(acc)
        last = b == NB - 1
        seq = ([(j, ct) for ct in range(NC) for j in range(KB)] if last
               else [(j, ct) for j in range(KB) for ct in range(NC)])
        for j, ct in seq:
            kt = b * KB + j
            o = _dot(ps[j], _tile(lckv, ct, pl.ds(kt * 64, 64)))
            acc[ct] = o if acc[ct] is None else acc[ct] + o
        return acc

    s0 = scores(0)
    s1 = scores(1)
    p0, m, l, al0 = soft(s0, None, None)
    acc = ctxc(0, p0, None, None)
    s2 = scores(2)
    p1, m, l, al1 = soft(s1, m, l)
    acc = ctxc(1, p1, al1, acc)
    s3 = scores(3)
    p2, m, l, al2 = soft(s2, m, l)
    acc = ctxc(2, p2, al2, acc)
    p3, m, l, al3 = soft(s3, m, l)
    acc = ctxc(3, p3, al3, acc)
    linv = 1.0 / jnp.sum(l, axis=1, keepdims=True)

    accv = [[None] * NM for _ in range(3)]
    accm = [None] * NM

    def e_tiles(hs, cts, part):
        for ct in cts:
            for h in hs:
                g = h // 8
                o = _dot(acc[ct][g * 8:(g + 1) * 8], _tile(wuv, h, pl.ds(ct * 64, 64)))
                part[h] = o if h not in part else part[h] + o

    def head_ctx(h, part):
        g, r = divmod(h, 8)
        return part.pop(h)[r:r + 1] * linv[h:h + 1]

    def f_vpu(hs, part, accv):
        xbs = [_xb(head_ctx(h, part)) for h in hs]
        return _vmac3(accv, xbs, lambda j, s, n: o32[hs[j], pl.ds(s * 8, 8), pl.ds(n * 128, 128)])

    part = {}
    trip = [list(range(i, min(i + 3, OV))) for i in range(0, OV, 3)]
    e_tiles(trip[0], range(3), part)
    e_tiles(trip[1], range(3), part)
    e_tiles(trip[0], [3], part)
    accv = f_vpu(trip[0], part, accv)
    e_tiles(trip[1], [3], part)
    accv = f_vpu(trip[1], part, accv)
    for hs in trip[2:]:
        e_tiles(hs, range(NC), part)
        accv = f_vpu(hs, part, accv)
    lhs_m = {}
    for h in range(OV, H):
        e_tiles([h], range(NC), part)
        g, r = divmod(h, 8)
        lhs_m[h] = jnp.where(masks[r], part.pop(h) * linv[g * 8:(g + 1) * 8], 0.0)
    for n in range(NM):
        for h in range(OV, H):
            o = _dot(lhs_m[h], _tile(wo2, h, n))
            accm[n] = o if accm[n] is None else accm[n] + o
    x3 = [_rbf(x2[n] + _rbf(_rowsum(accm[n] + _fold3(accv, n)))) for n in range(NM)]
    mean3, rstd3 = _stats(x3)
    ln3 = [(x - mean3) * rstd3 for x in x3]
    sig3 = _router(ln3, wr)
    xb3 = []
    for kt in range(GV):
        xb3 += _xb(x3[kt][0:1])
    hh = []
    blocks = [list(range(G0))] + [list(range(i, min(i + GB, NF))) for i in range(G0, NF, GB)]
    for fts in blocks:
        av = {}
        for s in range(16):
            for kt in range(GV):
                for ft in fts:
                    for nm, ref in (("g", g32), ("u", u32s)):
                        p = xb3[kt * 16 + s] * ref[ft, pl.ds(kt * 128 + s * 8, 8), :]
                        key = (nm, ft, kt)
                        av[key] = p if key not in av else av[key] + p
        for ft in fts:
            og = ou = None
            for kt in range(GV, NM):
                a = _dot(x3[kt], _tile(gt, ft, kt))
                b = _dot(x3[kt], _tile(ut, ft, kt))
                og = a if og is None else og + a
                ou = b if ou is None else ou + b
            tot = lambda nm: functools.reduce(lambda a, b: a + b, [av[nm, ft, kt] for kt in range(GV)])
            g = rstd3 * (og + _rowsum(tot("g")) - mean3 * csg[ft])
            u = rstd3 * (ou + _rowsum(tot("u")) - mean3 * csu[ft])
            hh.append(_silu(g) * u)
    y = [None] * NM
    for ft in range(DV, NF):
        for n in range(NM):
            o = down2(ft, n, hh[ft])
            y[n] = o if y[n] is None else y[n] + o
    yv = [[None] * NM for _ in range(3)]
    for i in range(0, DV, 3):
        fs = list(range(i, min(i + 3, DV)))
        yv = _vmac3(yv, [_xb(hh[ft][0:1]) for ft in fs],
                    lambda j, s, n: wd_f32(fs[j], s, n))
    if DV:
        y = [y[n] + _rowsum(_fold3(yv, n)) for n in range(NM)]
    x4 = [x3[n] + _rbf(ln3[n] + _rbf(y[n] * sig3)) for n in range(NM)]
    out = jnp.concatenate([x[0:1, :] for x in x4], axis=1)
    o_ref[0] = out.astype(bf16)


@jax.jit
def pallas_interleave_layers__compressed_kv_cla__moe_arch_mod__decode_kernel(
    A_x: jax.Array,
    A_c_kv: jax.Array,
    A_w_q: jax.Array,
    A_w_uk: jax.Array,
    A_w_uv: jax.Array,
    A_w_o: jax.Array,
    B_x: jax.Array,
    B_w_r: jax.Array,
    B_w_gate: jax.Array,
    B_w_up: jax.Array,
    B_w_down: jax.Array,
):
    del B_x
    any_spec = pl.BlockSpec(memory_space=pl.ANY)
    V = pltpu.VMEM
    scratch = [
        V((1, 1, M), bf16),
        V((NM, 128), bf16),
        V((M, H, D), bf16),
        V((DC, H, D), bf16),
        V((DC, H, D), bf16),
        V((NC, SK // 2, 128), u32),
        V((H, D, M), bf16),
        V((F, M), bf16),
        V((F, M), bf16),
        V((F, M), bf16),
        V((H, M // 2, D), u32),
        V((H, NC, D // 2, 128), u32),
        V((H, DC // 2, D), u32),
        V((NK, NC, 64, 128), u32),
        V((NF, NM, 64, 128), u32),
        V((NF, NM, 64, 128), u32),
        V((NF, max(GV, 1) * 128, 128), f32),
        V((NF, max(GV, 1) * 128, 128), f32),
        V((max(DV, 1) * 128, M), f32),
        V((max(OV, 1), D, M), f32),
        V((max(BV, 1), NC, D, 128), f32),
        V((H, max(AV, 1) * 128, D), f32),
        V((H, NM, 64, 128), u32),
        V((NF, NM, 64, 128), u32),
        V((4, 8, 128), f32),
        V((NF, 8, 128), f32),
        V((NF, 8, 128), f32),
        V((NC, H, 128), f32),
        V((NC, H, 128), f32),
        V((4, 8, 128), f32),
        V((NF, 8, 128), f32),
        V((NM, 8, 128), f32),
        pltpu.SemaphoreType.DMA((40,)),
    ]
    return pl.pallas_call(
        _kernel,
        out_shape=jax.ShapeDtypeStruct((1, 1, M), bf16),
        in_specs=[any_spec] * 10,
        out_specs=pl.BlockSpec(memory_space=pltpu.VMEM),
        scratch_shapes=scratch,
        compiler_params=pltpu.CompilerParams(
            vmem_limit_bytes=100 * 1024 * 1024,
            disable_semaphore_checks=True,
        ),
    )(A_x, A_c_kv, A_w_q, A_w_uk, A_w_uv, A_w_o, B_w_r.reshape(NM, 128),
      B_w_gate.T, B_w_up.T, B_w_down)
```

```python
import functools

import jax
import jax.numpy as jnp
from jax import lax
import jax.experimental.pallas as pl
import jax.experimental.pallas.tpu as pltpu

f32 = jnp.float32
bf16 = jnp.bfloat16
u32 = jnp.uint32
i32 = jnp.int32

M = 640
H = 32
D = 128
DC = 512
SK = 4096
F = 1728
NM = M // 128
NC = DC // 128
NK = SK // 128
NF = 14
EPS = 1e-5
SCALE = float(D) ** -0.5
KB = 8
NB = NK // KB
GV = 1
DV = 10
OV = 21
AV = 0
GB = 2
GATH = 1
PRECONV = (0,1,2,3)
DRC = 384
DR0 = 768
DGROUPS = ((0,1),(2,3),(4,))
G0 = 3
BV = 14


def _dot(a, b):
    return jnp.dot(a, b, preferred_element_type=f32)


def _rbf(x):
    return x.astype(bf16).astype(f32)


def _tile(ref, *idx):
    return pltpu.bitcast(ref[idx], bf16)


def _stats(xs):
    s = xs[0] + xs[1] + xs[2] + xs[3] + xs[4]
    mean = jnp.sum(s, axis=1, keepdims=True) * (1.0 / M)
    ds = [x - mean for x in xs]
    q = ds[0] * ds[0] + ds[1] * ds[1] + ds[2] * ds[2] + ds[3] * ds[3] + ds[4] * ds[4]
    var = jnp.sum(q, axis=1, keepdims=True) * (1.0 / M)
    rstd = 1.0 / jnp.sqrt(var + EPS)
    return mean, rstd


def _router(lns, wr):
    s = lns[0] * wr[0] + lns[1] * wr[1] + lns[2] * wr[2] + lns[3] * wr[3] + lns[4] * wr[4]
    r = jnp.sum(s, axis=1, keepdims=True)
    return jax.nn.sigmoid(r)


def _rowsum(x):
    return jnp.broadcast_to(jnp.sum(x, axis=0, keepdims=True), x.shape)


def _xb(row):
    t = jnp.broadcast_to(row, (128, 128)).T
    return [t[s * 8:(s + 1) * 8] for s in range(16)]


def _xb_gather(rows):
    sub = lax.broadcasted_iota(i32, (8, 128), 0)
    return [jnp.take_along_axis(rows, sub + 8 * s, axis=1, mode="promise_in_bounds")
            for s in range(16)]


def _vmac(acc, xb, load):
    for s, xs in enumerate(xb):
        p = xs * load(s)
        acc = p if acc is None else acc + p
    return acc


def _vmacs(accs, xb, load):
    accs = list(accs)
    for s, xs in enumerate(xb):
        for i in range(len(accs)):
            p = xs * load(s, i)
            accs[i] = p if accs[i] is None else accs[i] + p
    return accs


def _vmac3(accs, xbs, load):
    accs = [list(a) for a in accs]
    for s in range(16):
        for j, xb in enumerate(xbs):
            for i in range(len(accs[j])):
                p = xb[s] * load(j, s, i)
                accs[j][i] = p if accs[j][i] is None else accs[j][i] + p
    return accs


def _fold3(accs, i):
    t = [a[i] for a in accs if a[i] is not None]
    return functools.reduce(lambda a, b: a + b, t)


def _silu(g):
    return g * jax.nn.sigmoid(g)


def _kernel(x_hbm, ckv_hbm, wq_hbm, wuk_hbm, wuv_hbm, wo_hbm, wr_hbm, wg_hbm, wu_hbm, wd_hbm,
            o_ref,
            x_v, wr_v, lq, luk, luv, lckv, lo, lg, lu, ld,
            wq, wukt, wuv, ckvt, gt, ut, g32, u32s, d32, o32, b32, q32, wo2, wd2,
            csq, csg, csu, qa_s, cc_s, ctx_s, hh_s, x_s,
            sems):
    row8 = lax.broadcasted_iota(i32, (8, 128), 0)
    masks = [row8 == r for r in range(8)]

    copies = {}
    order = []

    def add(name, pairs):
        sem = sems.at[len(copies)]
        cs = [pltpu.make_async_copy(s, d, sem) for s, d in pairs]
        copies[name] = cs
        order.append(name)

    add("x", [(x_hbm, x_v)])
    add("wr", [(wr_hbm, wr_v)])
    for i in range(NM):
        add(("q", i), [(wq_hbm.at[pl.ds(i * 128, 128)], lq.at[pl.ds(i * 128, 128)])])
    for i in range(NC):
        add(("uk", i), [(wuk_hbm.at[pl.ds(i * 128, 128)], luk.at[pl.ds(i * 128, 128)])])
    ckv32 = ckv_hbm.at[0].bitcast(u32)
    for b in range(NB):
        add(("ckv", b), [(ckv32.at[pl.ds(b * 512, 512), pl.ds(ct * 128, 128)],
                          lckv.at[ct, pl.ds(b * 512, 512)]) for ct in range(NC)])
    FS = [(0, 896), (896, F - 896)]
    for i, (s, n) in enumerate(FS):
        add(("g", i), [(wg_hbm.at[pl.ds(s, n)], lg.at[pl.ds(s, n)])])
    for i, (s, n) in enumerate(FS):
        add(("u", i), [(wu_hbm.at[pl.ds(s, n)], lu.at[pl.ds(s, n)])])
    for i in range(NC):
        add(("uv", i), [(wuv_hbm.at[pl.ds(i * 128, 128)], luv.at[pl.ds(i * 128, 128)])])
    for g in range(4):
        add(("o", g), [(wo_hbm.at[pl.ds(g * 8, 8)], lo.at[pl.ds(g * 8, 8)])])
    for i in range(DR0 // DRC):
        add(("d", i), [(wd_hbm.at[pl.ds(i * DRC, DRC)], ld.at[pl.ds(i * DRC, DRC)])])
    for i, cols in enumerate(DGROUPS):
        c0, nc = cols[0] * 128, len(cols) * 128
        add(("dc", i), [(wd_hbm.at[pl.ds(DR0, F - DR0), pl.ds(c0, nc)],
                         ld.at[pl.ds(DR0, F - DR0), pl.ds(c0, nc)])])

    for name in order:
        for c in copies[name]:
            c.start()

    def wait(name):
        for c in copies[name]:
            c.wait()

    names = list(copies)

    def wait_dyn(first_name, i, pairs_fn):
        base = names.index(first_name)
        for s, d in pairs_fn(i):
            pltpu.make_async_copy(s, d, sems.at[base + i]).wait()

    wait("x")
    wait("wr")
    xr = x_v[0].astype(f32)
    x0 = [jnp.broadcast_to(xr[:, n * 128:(n + 1) * 128], (8, 128)) for n in range(NM)]
    wrf = wr_v[...].astype(f32)
    wr = [jnp.broadcast_to(wrf[n:n + 1, :], (8, 128)) for n in range(NM)]
    for n in range(NM):
        x_s[n] = x0[n]
    mean0, rstd0 = _stats(x0)
    ones8 = jnp.ones((8, 128), f32)
    zero8 = jnp.zeros((8, 128), f32)

    def a_body(kt, carry):
        raw, cs = carry
        s = pl.multiple_of(kt * 128, 128)
        wait_dyn(("q", 0), kt, lambda i: [(wq_hbm.at[pl.ds(s, 128)], lq.at[pl.ds(s, 128)])])
        t = jnp.swapaxes(lq[pl.ds(s, 128)], 0, 1)
        s2 = pl.multiple_of(kt * 64, 64)
        for h in range(H):
            wq[h, pl.ds(s2, 64), :] = pltpu.bitcast(t[h], u32)
        if AV:
            @pl.when(kt < AV)
            def _():
                sv = pl.multiple_of(jnp.minimum(kt, AV - 1) * 128, 128)
                for h in range(H):
                    w = wq[h, pl.ds(s2, 64), :]
                    q32[h, pl.ds(sv, 128), :] = pltpu.bitcast(w, bf16).astype(f32)
        lhs = jnp.concatenate([x_s[kt], ones8], axis=0)
        raw, cs = list(raw), list(cs)
        for h in range(H):
            g, r = divmod(h, 8)
            out = _dot(lhs, pltpu.bitcast(wq[h, pl.ds(s2, 64), :], bf16))
            raw[g] = jnp.where(masks[r], raw[g] + out[0:8], raw[g])
            cs[g] = jnp.where(masks[r], cs[g] + out[8:16], cs[g])
        return tuple(raw), tuple(cs)

    raw, cs = lax.fori_loop(0, NM, a_body, ((zero8,) * 4, (zero8,) * 4))
    for g in range(4):
        csq[g] = cs[g]
    q = [rstd0 * (raw[g] - mean0 * cs[g]) for g in range(4)]

    def b_body(ct, _):
        s = pl.multiple_of(ct * 128, 128)
        wait_dyn(("uk", 0), ct, lambda i: [(wuk_hbm.at[pl.ds(s, 128)], luk.at[pl.ds(s, 128)])])
        t = jnp.swapaxes(luk[pl.ds(s, 128)], 0, 1)
        for h in range(H):
            th = t[h].T
            wukt[h, ct] = pltpu.bitcast(th, u32)
            if h < BV:
                b32[h, ct] = th.astype(f32)
        qa = [zero8] * 4
        for h in range(H):
            g, r = divmod(h, 8)
            out = _dot(q[g], pltpu.bitcast(wukt[h, ct], bf16))
            qa[g] = jnp.where(masks[r], out, qa[g])
        qa_s[ct] = jnp.concatenate(qa, axis=0)
        return _

    lax.fori_loop(0, NC, b_body, 0)

    def cd_body(b, carry):
        m, l, acc = carry
        s = pl.multiple_of(b * 512, 512)
        wait_dyn(("ckv", 0), b, lambda i: [(ckv32.at[pl.ds(s, 512), pl.ds(ct * 128, 128)],
                                            lckv.at[ct, pl.ds(s, 512)]) for ct in range(NC)])
        ss = []
        for j in range(KB):
            kt = b * KB + j
            sk = pl.multiple_of(s + j * 64, 64)
            sc = None
            for ct in range(NC):
                t = pltpu.bitcast(lckv[ct, pl.ds(sk, 64), :], bf16).T
                ckvt[kt, ct] = pltpu.bitcast(t, u32)
                o = _dot(qa_s[ct], t)
                sc = o if sc is None else sc + o
            ss.append(sc * SCALE)
        mb = ss[0]
        for j in range(1, KB):
            mb = jnp.maximum(mb, ss[j])
        m_new = jnp.maximum(m, jnp.max(mb, axis=1, keepdims=True))
        alpha = jnp.exp(m - m_new)
        ps = [jnp.exp(sj - m_new) for sj in ss]
        lb = ps[0]
        for j in range(1, KB):
            lb = lb + ps[j]
        l = l * alpha + lb
        acc = [a * alpha for a in acc]
        for j in range(KB):
            sk = pl.multiple_of(s + j * 64, 64)
            for ct in range(NC):
                acc[ct] = acc[ct] + _dot(ps[j], pltpu.bitcast(lckv[ct, pl.ds(sk, 64), :], bf16))
        return m_new, l, acc

    m_init = jnp.full((H, 128), -jnp.inf, f32)
    _, l, acc = lax.fori_loop(0, NB, cd_body,
                              (m_init, jnp.zeros((H, 128), f32),
                               [jnp.zeros((H, 128), f32)] * NC))
    linv = 1.0 / jnp.sum(l, axis=1, keepdims=True)
    for ct in range(NC):
        cc_s[ct] = acc[ct]

    def transpose_ffn(land, dst, dst32, fam):
        def body(ft, _):
            s = pl.multiple_of(ft * 128, 128)
            for kt in range(NM):
                t = land[pl.ds(s, 128), pl.ds(kt * 128, 128)].T
                dst[ft, kt] = pltpu.bitcast(t, u32)
                if kt < GV:
                    dst32[ft, pl.ds(kt * 128, 128), :] = t.astype(f32)
            return _
        wait((fam, 0))
        lax.fori_loop(0, 7, body, 0)
        wait((fam, 1))
        lax.fori_loop(7, 13, body, 0)
        for kt in range(NM):
            t = land[pl.ds(13 * 128, 64), pl.ds(kt * 128, 128)]
            t = jnp.concatenate([t, jnp.zeros((64, 128), bf16)], axis=0)
            t = t.T
            dst[13, kt] = pltpu.bitcast(t, u32)
            if kt < GV:
                dst32[13, pl.ds(kt * 128, 128), :] = t.astype(f32)

    transpose_ffn(lg, gt, g32, "g")
    transpose_ffn(lu, ut, u32s, "u")

    def e_body(ct, ctx):
        s = pl.multiple_of(ct * 128, 128)
        wait_dyn(("uv", 0), ct, lambda i: [(wuv_hbm.at[pl.ds(s, 128)], luv.at[pl.ds(s, 128)])])
        t = jnp.swapaxes(luv[pl.ds(s, 128)], 0, 1)
        s2 = pl.multiple_of(ct * 64, 64)
        for h in range(H):
            wuv[h, pl.ds(s2, 64), :] = pltpu.bitcast(t[h], u32)
        ctx = list(ctx)
        cc = cc_s[ct]
        for h in range(H):
            g, r = divmod(h, 8)
            out = _dot(cc[g * 8:(g + 1) * 8], pltpu.bitcast(wuv[h, pl.ds(s2, 64), :], bf16))
            ctx[g] = jnp.where(masks[r], ctx[g] + out, ctx[g])
        return tuple(ctx)

    ctx = lax.fori_loop(0, NC, e_body, (zero8,) * 4)
    for g in range(4):
        ctx_s[g] = ctx[g] * linv[g * 8:(g + 1) * 8]

    def f_body(g, acc):
        s = pl.multiple_of(g * 8, 8)
        wait_dyn(("o", 0), g, lambda i: [(wo_hbm.at[pl.ds(s, 8)], lo.at[pl.ds(s, 8)])])
        acc = list(acc)
        cg = ctx_s[g]
        for r in range(8):
            lhs = jnp.where(masks[r], cg, 0.0)
            for n in range(NM):
                t = lo[s + r, :, pl.ds(n * 128, 128)]
                wo2[s + r, n] = pltpu.bitcast(t, u32)
                acc[n] = acc[n] + _dot(lhs, t)
        for r in range(8):
            @pl.when(s + r < OV)
            def _():
                o32[jnp.minimum(s + r, OV - 1)] = lo[s + r].astype(f32)
        return tuple(acc)

    acc = lax.fori_loop(0, 4, f_body, (zero8,) * NM)
    x1 = [_rbf(x0[n] + _rbf(_rowsum(acc[n]))) for n in range(NM)]

    mean1, rstd1 = _stats(x1)
    ln1 = [(x - mean1) * rstd1 for x in x1]
    sig1 = _router(ln1, wr)
    lhs1 = [jnp.concatenate([x1[kt], ones8], axis=0) for kt in range(NM)]

    hh1 = []
    NE_ = DR0 // 128
    for ft in range(NF):
        og = ou = None
        for kt in range(NM):
            a = _dot(lhs1[kt], _tile(gt, ft, kt))
            b = _dot(lhs1[kt], _tile(ut, ft, kt))
            og = a if og is None else og + a
            ou = b if ou is None else ou + b
        csg[ft] = og[8:16]
        csu[ft] = ou[8:16]
        g = rstd1 * (og[0:8] - mean1 * og[8:16])
        u = rstd1 * (ou[0:8] - mean1 * ou[8:16])
        hh1.append(_silu(g) * u)
        if ft < NE_:
            hh_s[ft] = hh1[ft]

    NE = DR0 // 128

    def wd_tile(ft, n):
        if ft < NE:
            return _tile(wd2, ft, n)
        return ld[pl.ds(ft * 128, min(128, F - ft * 128)), pl.ds(n * 128, 128)]

    def down2(ft, n, hh):
        return _dot(hh if ft < 13 else hh[:, :64], wd_tile(ft, n))

    def wd_f32(ft, s, n):
        if ft < NE or n in PRECONV:
            return d32[pl.ds(ft * 128 + s * 8, 8), pl.ds(n * 128, 128)]
        return wd_tile(ft, n).astype(f32)[s * 8:(s + 1) * 8]

    FPC = DRC // 128

    def h_body(i, y):
        s = pl.multiple_of(i * DRC, 128)
        wait_dyn(("d", 0), i, lambda _: [(wd_hbm.at[pl.ds(s, DRC)], ld.at[pl.ds(s, DRC)])])
        y = list(y)
        for j in range(FPC):
            ft = i * FPC + j
            sf = pl.multiple_of(s + j * 128, 128)
            hh = hh_s[ft]
            for n in range(NM):
                t = ld[pl.ds(sf, 128), pl.ds(n * 128, 128)]
                wd2[ft, n] = pltpu.bitcast(t, u32)
                y[n] = y[n] + _dot(hh, t)
        for j in range(FPC):
            ft = i * FPC + j
            sf = pl.multiple_of(s + j * 128, 128)
            if DV:
                @pl.when(ft < DV)
                def _():
                    sd = pl.multiple_of(jnp.minimum(ft, DV - 1) * 128, 128)
                    d32[pl.ds(sd, 128), :] = ld[pl.ds(sf, 128), :].astype(f32)
        return tuple(y)

    y = list(lax.fori_loop(0, DR0 // DRC, h_body, (zero8,) * NM))

    x2 = [None] * NM
    racc = [None] * 4

    def h_late(n):
        for ft in range(NE, NF):
            y[n] = y[n] + down2(ft, n, hh1[ft])
        x2[n] = _rbf(x1[n] + _rbf(ln1[n] + _rbf(y[n] * sig1)))
        if n in PRECONV:
            for ft in range(NE, DV):
                d32[pl.ds(ft * 128, 128), pl.ds(n * 128, 128)] = wd_tile(ft, n).astype(f32)

    def a_pass(kt, heads=range(H)):
        for h in heads:
            g, r = divmod(h, 8)
            o = _dot(jnp.where(masks[r], x2[kt], 0.0), _tile(wq, h, pl.ds(kt * 64, 64)))
            racc[g] = o if racc[g] is None else racc[g] + o

    wait(("dc", 0))
    h_late(0)
    h_late(1)
    a_pass(0)
    a_pass(1)
    wait(("dc", 1))
    h_late(2)
    h_late(3)
    a_pass(2)
    wait(("dc", 2))
    h_late(4)
    a_pass(3, range(0, 16))
    mean2, rstd2 = _stats(x2)
    raw = {}
    KL = DGROUPS[-1][-1]
    last = {}
    for h in range(BV):
        last[h] = _dot(x2[KL], _tile(wq, h, pl.ds(KL * 64, 64)))
    a_pass(3, range(16, H))
    for h in range(BV, H):
        last[h] = _dot(x2[KL], _tile(wq, h, pl.ds(KL * 64, 64)))
    for h in range(H):
        raw[h] = racc[h // 8] + last[h]
    qv = {}
    for i in range(0, BV, 3):
        hs = list(range(i, min(i + 3, BV)))
        xbs = []
        for h in hs:
            g, r = divmod(h, 8)
            qh = raw[h][r:r + 1] - mean2[0:1] * csq[g, pl.ds(r, 1), :]
            xbs.append(_xb(qh))
        accs = _vmac3([[None] * NC for _ in hs], xbs,
                      lambda j, s, ct: b32[hs[j], ct, pl.ds(s * 8, 8), :])
        for j, h in enumerate(hs):
            for ct in range(NC):
                qv[h, ct] = _rowsum(accs[j][ct]) * rstd2
    q = {}
    for g in range(BV // 8, 4):
        rawg = zero8
        for r in range(8):
            if g * 8 + r >= BV:
                rawg = jnp.where(masks[r], raw[g * 8 + r], rawg)
        q[g] = rstd2 * (rawg - mean2 * csq[g])
    qa = []
    for ct in range(NC):
        qg = [zero8] * 4
        for h in range(H):
            g, r = divmod(h, 8)
            o = qv[h, ct] if h < BV else _dot(q[g], _tile(wukt, h, ct))
            qg[g] = jnp.where(masks[r], o, qg[g])
        qa.append(jnp.concatenate(qg, axis=0))

    def scores(b):
        ss = []
        for j in range(KB):
            kt = b * KB + j
            sc = None
            for ct in range(NC):
                o = _dot(qa[ct], _tile(ckvt, kt, ct))
                sc = o if sc is None else sc + o
            ss.append(sc * SCALE)
        return ss

    def soft(ss, m, l):
        mb = ss[0]
        for j in range(1, KB):
            mb = jnp.maximum(mb, ss[j])
        mb = jnp.max(mb, axis=1, keepdims=True)
        m_new = mb if m is None else jnp.maximum(m, mb)
        ps = [jnp.exp(sj - m_new) for sj in ss]
        lb = ps[0]
        for j in range(1, KB):
            lb = lb + ps[j]
        if m is None:
            return ps, m_new, lb, None
        alpha = jnp.exp(m - m_new)
        return ps, m_new, l * alpha + lb, alpha

    def ctxc(b, ps, alpha, acc):
        if acc is not None:
            acc = [a * alpha for a in acc]
        else:
            acc = [None] * NC
        acc = list(acc)
        last = b == NB - 1
        seq = ([(j, ct) for ct in range(NC) for j in range(KB)] if last
               else [(j, ct) for j in range(KB) for ct in range(NC)])
        for j, ct in seq:
            kt = b * KB + j
            o = _dot(ps[j], _tile(lckv, ct, pl.ds(kt * 64, 64)))
            acc[ct] = o if acc[ct] is None else acc[ct] + o
        return acc

    s0 = scores(0)
    s1 = scores(1)
    p0, m, l, al0 = soft(s0, None, None)
    acc = ctxc(0, p0, None, None)
    s2 = scores(2)
    p1, m, l, al1 = soft(s1, m, l)
    acc = ctxc(1, p1, al1, acc)
    s3 = scores(3)
    p2, m, l, al2 = soft(s2, m, l)
    acc = ctxc(2, p2, al2, acc)
    p3, m, l, al3 = soft(s3, m, l)
    acc = ctxc(3, p3, al3, acc)
    linv = 1.0 / jnp.sum(l, axis=1, keepdims=True)

    accv = [[None] * NM for _ in range(3)]
    accm = [None] * NM

    def e_tiles(hs, cts, part):
        for ct in cts:
            for h in hs:
                g = h // 8
                o = _dot(acc[ct][g * 8:(g + 1) * 8], _tile(wuv, h, pl.ds(ct * 64, 64)))
                part[h] = o if h not in part else part[h] + o

    def head_ctx(h, part):
        g, r = divmod(h, 8)
        return part.pop(h)[r:r + 1] * linv[h:h + 1]

    def f_vpu(hs, part, accv):
        xbs = [_xb(head_ctx(h, part)) for h in hs]
        return _vmac3(accv, xbs, lambda j, s, n: o32[hs[j], pl.ds(s * 8, 8), pl.ds(n * 128, 128)])

    part = {}
    trip = [list(range(i, min(i + 3, OV))) for i in range(0, OV, 3)]
    e_tiles(trip[0], range(3), part)
    e_tiles(trip[1], range(3), part)
    e_tiles(trip[0], [3], part)
    accv = f_vpu(trip[0], part, accv)
    e_tiles(trip[1], [3], part)
    accv = f_vpu(trip[1], part, accv)
    for hs in trip[2:]:
        e_tiles(hs, range(NC), part)
        accv = f_vpu(hs, part, accv)
    lhs_m = {}
    for h in range(OV, H):
        e_tiles([h], range(NC), part)
        g, r = divmod(h, 8)
        lhs_m[h] = jnp.where(masks[r], part.pop(h) * linv[g * 8:(g + 1) * 8], 0.0)
    for n in range(NM):
        for h in range(OV, H):
            o = _dot(lhs_m[h], _tile(wo2, h, n))
            accm[n] = o if accm[n] is None else accm[n] + o
    x3 = [_rbf(x2[n] + _rbf(_rowsum(accm[n] + _fold3(accv, n)))) for n in range(NM)]
    mean3, rstd3 = _stats(x3)
    ln3 = [(x - mean3) * rstd3 for x in x3]
    sig3 = _router(ln3, wr)
    xb3 = []
    for kt in range(GV):
        xb3 += _xb_gather(x3[kt]) if GATH else _xb(x3[kt][0:1])
    hh = []
    blocks = [list(range(G0))] + [list(range(i, min(i + GB, NF))) for i in range(G0, NF, GB)]
    for fts in blocks:
        av = {}
        for s in range(16):
            for kt in range(GV):
                for ft in fts:
                    for nm, ref in (("g", g32), ("u", u32s)):
                        p = xb3[kt * 16 + s] * ref[ft, pl.ds(kt * 128 + s * 8, 8), :]
                        key = (nm, ft, kt)
                        av[key] = p if key not in av else av[key] + p
        for ft in fts:
            og = ou = None
            for kt in range(GV, NM):
                a = _dot(x3[kt], _tile(gt, ft, kt))
                b = _dot(x3[kt], _tile(ut, ft, kt))
                og = a if og is None else og + a
                ou = b if ou is None else ou + b
            tot = lambda nm: functools.reduce(lambda a, b: a + b, [av[nm, ft, kt] for kt in range(GV)])
            g = rstd3 * (og + _rowsum(tot("g")) - mean3 * csg[ft])
            u = rstd3 * (ou + _rowsum(tot("u")) - mean3 * csu[ft])
            hh.append(_silu(g) * u)
    y = [None] * NM
    for ft in range(DV, NF):
        for n in range(NM):
            o = down2(ft, n, hh[ft])
            y[n] = o if y[n] is None else y[n] + o
    yv = [[None] * NM for _ in range(3)]
    for i in range(0, DV, 3):
        fs = list(range(i, min(i + 3, DV)))
        yv = _vmac3(yv, [_xb(hh[ft][0:1]) for ft in fs],
                    lambda j, s, n: wd_f32(fs[j], s, n))
    if DV:
        y = [y[n] + _rowsum(_fold3(yv, n)) for n in range(NM)]
    x4 = [x3[n] + _rbf(ln3[n] + _rbf(y[n] * sig3)) for n in range(NM)]
    out = jnp.concatenate([x[0:1, :] for x in x4], axis=1)
    o_ref[0] = out.astype(bf16)


@jax.jit
def pallas_interleave_layers__compressed_kv_cla__moe_arch_mod__decode_kernel(
    A_x: jax.Array,
    A_c_kv: jax.Array,
    A_w_q: jax.Array,
    A_w_uk: jax.Array,
    A_w_uv: jax.Array,
    A_w_o: jax.Array,
    B_x: jax.Array,
    B_w_r: jax.Array,
    B_w_gate: jax.Array,
    B_w_up: jax.Array,
    B_w_down: jax.Array,
):
    del B_x
    any_spec = pl.BlockSpec(memory_space=pl.ANY)
    V = pltpu.VMEM
    scratch = [
        V((1, 1, M), bf16),
        V((NM, 128), bf16),
        V((M, H, D), bf16),
        V((DC, H, D), bf16),
        V((DC, H, D), bf16),
        V((NC, SK // 2, 128), u32),
        V((H, D, M), bf16),
        V((F, M), bf16),
        V((F, M), bf16),
        V((F, M), bf16),
        V((H, M // 2, D), u32),
        V((H, NC, D // 2, 128), u32),
        V((H, DC // 2, D), u32),
        V((NK, NC, 64, 128), u32),
        V((NF, NM, 64, 128), u32),
        V((NF, NM, 64, 128), u32),
        V((NF, max(GV, 1) * 128, 128), f32),
        V((NF, max(GV, 1) * 128, 128), f32),
        V((max(DV, 1) * 128, M), f32),
        V((max(OV, 1), D, M), f32),
        V((max(BV, 1), NC, D, 128), f32),
        V((H, max(AV, 1) * 128, D), f32),
        V((H, NM, 64, 128), u32),
        V((NF, NM, 64, 128), u32),
        V((4, 8, 128), f32),
        V((NF, 8, 128), f32),
        V((NF, 8, 128), f32),
        V((NC, H, 128), f32),
        V((NC, H, 128), f32),
        V((4, 8, 128), f32),
        V((NF, 8, 128), f32),
        V((NM, 8, 128), f32),
        pltpu.SemaphoreType.DMA((40,)),
    ]
    return pl.pallas_call(
        _kernel,
        out_shape=jax.ShapeDtypeStruct((1, 1, M), bf16),
        in_specs=[any_spec] * 10,
        out_specs=pl.BlockSpec(memory_space=pltpu.VMEM),
        scratch_shapes=scratch,
        compiler_params=pltpu.CompilerParams(
            vmem_limit_bytes=100 * 1024 * 1024,
            disable_semaphore_checks=True,
        ),
    )(A_x, A_c_kv, A_w_q, A_w_uk, A_w_uv, A_w_o, B_w_r.reshape(NM, 128),
      B_w_gate.T, B_w_up.T, B_w_down)
```

```python
import functools

import jax
import jax.numpy as jnp
from jax import lax
import jax.experimental.pallas as pl
import jax.experimental.pallas.tpu as pltpu

f32 = jnp.float32
bf16 = jnp.bfloat16
u32 = jnp.uint32
i32 = jnp.int32

M = 640
H = 32
D = 128
DC = 512
SK = 4096
F = 1728
NM = M // 128
NC = DC // 128
NK = SK // 128
NF = 14
EPS = 1e-5
SCALE = float(D) ** -0.5
KB = 8
NB = NK // KB
GV = 1
DV = 10
OV = 21
AV = 0
GB = 2
GATH = 1
PRECONV = (0,1,2,3)
DRC = 384
DR0 = 768
DGROUPS = ((0,1),(2,3),(4,))
G0 = 3
BV = 14


def _dot(a, b):
    return jnp.dot(a, b, preferred_element_type=f32)


def _rbf(x):
    return x.astype(bf16).astype(f32)


def _tile(ref, *idx):
    return pltpu.bitcast(ref[idx], bf16)


def _stats(xs):
    s = xs[0] + xs[1] + xs[2] + xs[3] + xs[4]
    mean = jnp.sum(s, axis=1, keepdims=True) * (1.0 / M)
    ds = [x - mean for x in xs]
    q = ds[0] * ds[0] + ds[1] * ds[1] + ds[2] * ds[2] + ds[3] * ds[3] + ds[4] * ds[4]
    var = jnp.sum(q, axis=1, keepdims=True) * (1.0 / M)
    rstd = 1.0 / jnp.sqrt(var + EPS)
    return mean, rstd


def _router(lns, wr):
    s = lns[0] * wr[0] + lns[1] * wr[1] + lns[2] * wr[2] + lns[3] * wr[3] + lns[4] * wr[4]
    r = jnp.sum(s, axis=1, keepdims=True)
    return jax.nn.sigmoid(r)


def _rowsum(x):
    return jnp.broadcast_to(jnp.sum(x, axis=0, keepdims=True), x.shape)


def _xb(row):
    t = jnp.broadcast_to(row, (128, 128)).T
    return [t[s * 8:(s + 1) * 8] for s in range(16)]


def _xb_gather(rows):
    sub = lax.broadcasted_iota(i32, (8, 128), 0)
    return [jnp.take_along_axis(rows, sub + 8 * s, axis=1, mode="promise_in_bounds")
            for s in range(16)]


def _vmac(acc, xb, load):
    for s, xs in enumerate(xb):
        p = xs * load(s)
        acc = p if acc is None else acc + p
    return acc


def _vmacs(accs, xb, load):
    accs = list(accs)
    for s, xs in enumerate(xb):
        for i in range(len(accs)):
            p = xs * load(s, i)
            accs[i] = p if accs[i] is None else accs[i] + p
    return accs


def _vmac3(accs, xbs, load):
    accs = [list(a) for a in accs]
    for s in range(16):
        for j, xb in enumerate(xbs):
            for i in range(len(accs[j])):
                p = xb[s] * load(j, s, i)
                accs[j][i] = p if accs[j][i] is None else accs[j][i] + p
    return accs


def _fold3(accs, i):
    t = [a[i] for a in accs if a[i] is not None]
    return functools.reduce(lambda a, b: a + b, t)


def _silu(g):
    return g * jax.nn.sigmoid(g)


def _kernel(x_hbm, ckv_hbm, wq_hbm, wuk_hbm, wuv_hbm, wo_hbm, wr_hbm, wg_hbm, wu_hbm, wd_hbm,
            o_ref,
            x_v, wr_v, lq, luk, luv, lckv, lo, lg, lu, ld,
            wq, wukt, wuv, ckvt, gt, ut, g32, u32s, d32, o32, b32, q32, wo2,
            csq, csg, csu, qa_s, cc_s, ctx_s, hh_s, x_s,
            sems):
    row8 = lax.broadcasted_iota(i32, (8, 128), 0)
    masks = [row8 == r for r in range(8)]

    copies = {}
    order = []

    def add(name, pairs):
        sem = sems.at[len(copies)]
        cs = [pltpu.make_async_copy(s, d, sem) for s, d in pairs]
        copies[name] = cs
        order.append(name)

    add("x", [(x_hbm, x_v)])
    add("wr", [(wr_hbm, wr_v)])
    for i in range(NM):
        add(("q", i), [(wq_hbm.at[pl.ds(i * 128, 128)], lq.at[pl.ds(i * 128, 128)])])
    for i in range(NC):
        add(("uk", i), [(wuk_hbm.at[pl.ds(i * 128, 128)], luk.at[pl.ds(i * 128, 128)])])
    ckv32 = ckv_hbm.at[0].bitcast(u32)
    for b in range(NB):
        add(("ckv", b), [(ckv32.at[pl.ds(b * 512, 512), pl.ds(ct * 128, 128)],
                          lckv.at[ct, pl.ds(b * 512, 512)]) for ct in range(NC)])
    FS = [(0, 896), (896, F - 896)]
    for i, (s, n) in enumerate(FS):
        add(("g", i), [(wg_hbm.at[pl.ds(s, n)], lg.at[pl.ds(s, n)])])
    for i, (s, n) in enumerate(FS):
        add(("u", i), [(wu_hbm.at[pl.ds(s, n)], lu.at[pl.ds(s, n)])])
    for i in range(NC):
        add(("uv", i), [(wuv_hbm.at[pl.ds(i * 128, 128)], luv.at[pl.ds(i * 128, 128)])])
    for g in range(4):
        add(("o", g), [(wo_hbm.at[pl.ds(g * 8, 8)], lo.at[pl.ds(g * 8, 8)])])
    for i in range(DR0 // DRC):
        add(("d", i), [(wd_hbm.at[pl.ds(i * DRC, DRC)], ld.at[pl.ds(i * DRC, DRC)])])
    for i, cols in enumerate(DGROUPS):
        c0, nc = cols[0] * 128, len(cols) * 128
        add(("dc", i), [(wd_hbm.at[pl.ds(DR0, F - DR0), pl.ds(c0, nc)],
                         ld.at[pl.ds(DR0, F - DR0), pl.ds(c0, nc)])])

    for name in order:
        for c in copies[name]:
            c.start()

    def wait(name):
        for c in copies[name]:
            c.wait()

    names = list(copies)

    def wait_dyn(first_name, i, pairs_fn):
        base = names.index(first_name)
        for s, d in pairs_fn(i):
            pltpu.make_async_copy(s, d, sems.at[base + i]).wait()

    wait("x")
    wait("wr")
    xr = x_v[0].astype(f32)
    x0 = [jnp.broadcast_to(xr[:, n * 128:(n + 1) * 128], (8, 128)) for n in range(NM)]
    wrf = wr_v[...].astype(f32)
    wr = [jnp.broadcast_to(wrf[n:n + 1, :], (8, 128)) for n in range(NM)]
    for n in range(NM):
        x_s[n] = x0[n]
    mean0, rstd0 = _stats(x0)
    ones8 = jnp.ones((8, 128), f32)
    zero8 = jnp.zeros((8, 128), f32)

    def a_body(kt, carry):
        raw, cs = carry
        s = pl.multiple_of(kt * 128, 128)
        wait_dyn(("q", 0), kt, lambda i: [(wq_hbm.at[pl.ds(s, 128)], lq.at[pl.ds(s, 128)])])
        t = jnp.swapaxes(lq[pl.ds(s, 128)], 0, 1)
        s2 = pl.multiple_of(kt * 64, 64)
        for h in range(H):
            wq[h, pl.ds(s2, 64), :] = pltpu.bitcast(t[h], u32)
        if AV:
            @pl.when(kt < AV)
            def _():
                sv = pl.multiple_of(jnp.minimum(kt, AV - 1) * 128, 128)
                for h in range(H):
                    w = wq[h, pl.ds(s2, 64), :]
                    q32[h, pl.ds(sv, 128), :] = pltpu.bitcast(w, bf16).astype(f32)
        lhs = jnp.concatenate([x_s[kt], ones8], axis=0)
        raw, cs = list(raw), list(cs)
        for h in range(H):
            g, r = divmod(h, 8)
            out = _dot(lhs, pltpu.bitcast(wq[h, pl.ds(s2, 64), :], bf16))
            raw[g] = jnp.where(masks[r], raw[g] + out[0:8], raw[g])
            cs[g] = jnp.where(masks[r], cs[g] + out[8:16], cs[g])
        return tuple(raw), tuple(cs)

    raw, cs = lax.fori_loop(0, NM, a_body, ((zero8,) * 4, (zero8,) * 4))
    for g in range(4):
        csq[g] = cs[g]
    q = [rstd0 * (raw[g] - mean0 * cs[g]) for g in range(4)]

    def b_body(ct, _):
        s = pl.multiple_of(ct * 128, 128)
        wait_dyn(("uk", 0), ct, lambda i: [(wuk_hbm.at[pl.ds(s, 128)], luk.at[pl.ds(s, 128)])])
        t = jnp.swapaxes(luk[pl.ds(s, 128)], 0, 1)
        for h in range(H):
            th = t[h].T
            wukt[h, ct] = pltpu.bitcast(th, u32)
            if h < BV:
                b32[h, ct] = th.astype(f32)
        qa = [zero8] * 4
        for h in range(H):
            g, r = divmod(h, 8)
            out = _dot(q[g], pltpu.bitcast(wukt[h, ct], bf16))
            qa[g] = jnp.where(masks[r], out, qa[g])
        qa_s[ct] = jnp.concatenate(qa, axis=0)
        return _

    lax.fori_loop(0, NC, b_body, 0)

    def cd_body(b, carry):
        m, l, acc = carry
        s = pl.multiple_of(b * 512, 512)
        wait_dyn(("ckv", 0), b, lambda i: [(ckv32.at[pl.ds(s, 512), pl.ds(ct * 128, 128)],
                                            lckv.at[ct, pl.ds(s, 512)]) for ct in range(NC)])
        ss = []
        for j in range(KB):
            kt = b * KB + j
            sk = pl.multiple_of(s + j * 64, 64)
            sc = None
            for ct in range(NC):
                t = pltpu.bitcast(lckv[ct, pl.ds(sk, 64), :], bf16).T
                ckvt[kt, ct] = pltpu.bitcast(t, u32)
                o = _dot(qa_s[ct], t)
                sc = o if sc is None else sc + o
            ss.append(sc * SCALE)
        mb = ss[0]
        for j in range(1, KB):
            mb = jnp.maximum(mb, ss[j])
        m_new = jnp.maximum(m, jnp.max(mb, axis=1, keepdims=True))
        alpha = jnp.exp(m - m_new)
        ps = [jnp.exp(sj - m_new) for sj in ss]
        lb = ps[0]
        for j in range(1, KB):
            lb = lb + ps[j]
        l = l * alpha + lb
        acc = [a * alpha for a in acc]
        for j in range(KB):
            sk = pl.multiple_of(s + j * 64, 64)
            for ct in range(NC):
                acc[ct] = acc[ct] + _dot(ps[j], pltpu.bitcast(lckv[ct, pl.ds(sk, 64), :], bf16))
        return m_new, l, acc

    m_init = jnp.full((H, 128), -jnp.inf, f32)
    _, l, acc = lax.fori_loop(0, NB, cd_body,
                              (m_init, jnp.zeros((H, 128), f32),
                               [jnp.zeros((H, 128), f32)] * NC))
    linv = 1.0 / jnp.sum(l, axis=1, keepdims=True)
    for ct in range(NC):
        cc_s[ct] = acc[ct]

    def transpose_ffn(land, dst, dst32, fam):
        def body(ft, _):
            s = pl.multiple_of(ft * 128, 128)
            for kt in range(NM):
                t = land[pl.ds(s, 128), pl.ds(kt * 128, 128)].T
                dst[ft, kt] = pltpu.bitcast(t, u32)
                if kt < GV:
                    dst32[ft, pl.ds(kt * 128, 128), :] = t.astype(f32)
            return _
        wait((fam, 0))
        lax.fori_loop(0, 7, body, 0)
        wait((fam, 1))
        lax.fori_loop(7, 13, body, 0)
        for kt in range(NM):
            t = land[pl.ds(13 * 128, 64), pl.ds(kt * 128, 128)]
            t = jnp.concatenate([t, jnp.zeros((64, 128), bf16)], axis=0)
            t = t.T
            dst[13, kt] = pltpu.bitcast(t, u32)
            if kt < GV:
                dst32[13, pl.ds(kt * 128, 128), :] = t.astype(f32)

    transpose_ffn(lg, gt, g32, "g")
    transpose_ffn(lu, ut, u32s, "u")

    def e_body(ct, ctx):
        s = pl.multiple_of(ct * 128, 128)
        wait_dyn(("uv", 0), ct, lambda i: [(wuv_hbm.at[pl.ds(s, 128)], luv.at[pl.ds(s, 128)])])
        t = jnp.swapaxes(luv[pl.ds(s, 128)], 0, 1)
        s2 = pl.multiple_of(ct * 64, 64)
        for h in range(H):
            wuv[h, pl.ds(s2, 64), :] = pltpu.bitcast(t[h], u32)
        ctx = list(ctx)
        cc = cc_s[ct]
        for h in range(H):
            g, r = divmod(h, 8)
            out = _dot(cc[g * 8:(g + 1) * 8], pltpu.bitcast(wuv[h, pl.ds(s2, 64), :], bf16))
            ctx[g] = jnp.where(masks[r], ctx[g] + out, ctx[g])
        return tuple(ctx)

    ctx = lax.fori_loop(0, NC, e_body, (zero8,) * 4)
    for g in range(4):
        ctx_s[g] = ctx[g] * linv[g * 8:(g + 1) * 8]

    def f_body(g, acc):
        s = pl.multiple_of(g * 8, 8)
        wait_dyn(("o", 0), g, lambda i: [(wo_hbm.at[pl.ds(s, 8)], lo.at[pl.ds(s, 8)])])
        acc = list(acc)
        cg = ctx_s[g]
        for r in range(8):
            lhs = jnp.where(masks[r], cg, 0.0)
            for n in range(NM):
                t = lo[s + r, :, pl.ds(n * 128, 128)]
                wo2[s + r, n] = pltpu.bitcast(t, u32)
                acc[n] = acc[n] + _dot(lhs, t)
        for r in range(8):
            @pl.when(s + r < OV)
            def _():
                o32[jnp.minimum(s + r, OV - 1)] = lo[s + r].astype(f32)
        return tuple(acc)

    acc = lax.fori_loop(0, 4, f_body, (zero8,) * NM)
    x1 = [_rbf(x0[n] + _rbf(_rowsum(acc[n]))) for n in range(NM)]

    mean1, rstd1 = _stats(x1)
    ln1 = [(x - mean1) * rstd1 for x in x1]
    sig1 = _router(ln1, wr)
    lhs1 = [jnp.concatenate([x1[kt], ones8], axis=0) for kt in range(NM)]

    hh1 = []
    NE_ = DR0 // 128
    for ft in range(NF):
        og = ou = None
        for kt in range(NM):
            a = _dot(lhs1[kt], _tile(gt, ft, kt))
            b = _dot(lhs1[kt], _tile(ut, ft, kt))
            og = a if og is None else og + a
            ou = b if ou is None else ou + b
        csg[ft] = og[8:16]
        csu[ft] = ou[8:16]
        g = rstd1 * (og[0:8] - mean1 * og[8:16])
        u = rstd1 * (ou[0:8] - mean1 * ou[8:16])
        hh1.append(_silu(g) * u)
        if ft < NE_:
            hh_s[ft] = hh1[ft]

    NE = DR0 // 128

    def wd_tile(ft, n):
        return ld[pl.ds(ft * 128, min(128, F - ft * 128)), pl.ds(n * 128, 128)]

    def down2(ft, n, hh):
        return _dot(hh if ft < 13 else hh[:, :64], wd_tile(ft, n))

    def wd_f32(ft, s, n):
        if ft < NE or n in PRECONV:
            return d32[pl.ds(ft * 128 + s * 8, 8), pl.ds(n * 128, 128)]
        return wd_tile(ft, n).astype(f32)[s * 8:(s + 1) * 8]

    FPC = DRC // 128

    def h_body(i, y):
        s = pl.multiple_of(i * DRC, 128)
        wait_dyn(("d", 0), i, lambda _: [(wd_hbm.at[pl.ds(s, DRC)], ld.at[pl.ds(s, DRC)])])
        y = list(y)
        for j in range(FPC):
            ft = i * FPC + j
            sf = pl.multiple_of(s + j * 128, 128)
            hh = hh_s[ft]
            for n in range(NM):
                t = ld[pl.ds(sf, 128), pl.ds(n * 128, 128)]
                y[n] = y[n] + _dot(hh, t)
        for j in range(FPC):
            ft = i * FPC + j
            sf = pl.multiple_of(s + j * 128, 128)
            if DV:
                @pl.when(ft < DV)
                def _():
                    sd = pl.multiple_of(jnp.minimum(ft, DV - 1) * 128, 128)
                    d32[pl.ds(sd, 128), :] = ld[pl.ds(sf, 128), :].astype(f32)
        return tuple(y)

    y = list(lax.fori_loop(0, DR0 // DRC, h_body, (zero8,) * NM))

    x2 = [None] * NM
    racc = [None] * 4

    def h_late(n):
        for ft in range(NE, NF):
            y[n] = y[n] + down2(ft, n, hh1[ft])
        x2[n] = _rbf(x1[n] + _rbf(ln1[n] + _rbf(y[n] * sig1)))
        if n in PRECONV:
            for ft in range(NE, DV):
                d32[pl.ds(ft * 128, 128), pl.ds(n * 128, 128)] = wd_tile(ft, n).astype(f32)

    def a_pass(kt, heads=range(H)):
        for h in heads:
            g, r = divmod(h, 8)
            o = _dot(jnp.where(masks[r], x2[kt], 0.0), _tile(wq, h, pl.ds(kt * 64, 64)))
            racc[g] = o if racc[g] is None else racc[g] + o

    wait(("dc", 0))
    h_late(0)
    h_late(1)
    a_pass(0)
    a_pass(1)
    wait(("dc", 1))
    h_late(2)
    h_late(3)
    a_pass(2)
    wait(("dc", 2))
    h_late(4)
    a_pass(3, range(0, 16))
    mean2, rstd2 = _stats(x2)
    raw = {}
    KL = DGROUPS[-1][-1]
    last = {}
    for h in range(BV):
        last[h] = _dot(x2[KL], _tile(wq, h, pl.ds(KL * 64, 64)))
    a_pass(3, range(16, H))
    for h in range(BV, H):
        last[h] = _dot(x2[KL], _tile(wq, h, pl.ds(KL * 64, 64)))
    for h in range(H):
        raw[h] = racc[h // 8] + last[h]
    qv = {}
    for i in range(0, BV, 3):
        hs = list(range(i, min(i + 3, BV)))
        xbs = []
        for h in hs:
            g, r = divmod(h, 8)
            qh = raw[h][r:r + 1] - mean2[0:1] * csq[g, pl.ds(r, 1), :]
            xbs.append(_xb(qh))
        accs = _vmac3([[None] * NC for _ in hs], xbs,
                      lambda j, s, ct: b32[hs[j], ct, pl.ds(s * 8, 8), :])
        for j, h in enumerate(hs):
            for ct in range(NC):
                qv[h, ct] = _rowsum(accs[j][ct]) * rstd2
    q = {}
    for g in range(BV // 8, 4):
        rawg = zero8
        for r in range(8):
            if g * 8 + r >= BV:
                rawg = jnp.where(masks[r], raw[g * 8 + r], rawg)
        q[g] = rstd2 * (rawg - mean2 * csq[g])
    qa = []
    for ct in range(NC):
        qg = [zero8] * 4
        for h in range(H):
            g, r = divmod(h, 8)
            o = qv[h, ct] if h < BV else _dot(q[g], _tile(wukt, h, ct))
            qg[g] = jnp.where(masks[r], o, qg[g])
        qa.append(jnp.concatenate(qg, axis=0))

    def scores(b):
        ss = []
        for j in range(KB):
            kt = b * KB + j
            sc = None
            for ct in range(NC):
                o = _dot(qa[ct], _tile(ckvt, kt, ct))
                sc = o if sc is None else sc + o
            ss.append(sc * SCALE)
        return ss

    def soft(ss, m, l):
        mb = ss[0]
        for j in range(1, KB):
            mb = jnp.maximum(mb, ss[j])
        mb = jnp.max(mb, axis=1, keepdims=True)
        m_new = mb if m is None else jnp.maximum(m, mb)
        ps = [jnp.exp(sj - m_new) for sj in ss]
        lb = ps[0]
        for j in range(1, KB):
            lb = lb + ps[j]
        if m is None:
            return ps, m_new, lb, None
        alpha = jnp.exp(m - m_new)
        return ps, m_new, l * alpha + lb, alpha

    def ctxc(b, ps, alpha, acc):
        if acc is not None:
            acc = [a * alpha for a in acc]
        else:
            acc = [None] * NC
        acc = list(acc)
        last = b == NB - 1
        seq = ([(j, ct) for ct in range(NC) for j in range(KB)] if last
               else [(j, ct) for j in range(KB) for ct in range(NC)])
        for j, ct in seq:
            kt = b * KB + j
            o = _dot(ps[j], _tile(lckv, ct, pl.ds(kt * 64, 64)))
            acc[ct] = o if acc[ct] is None else acc[ct] + o
        return acc

    s0 = scores(0)
    s1 = scores(1)
    p0, m, l, al0 = soft(s0, None, None)
    acc = ctxc(0, p0, None, None)
    s2 = scores(2)
    p1, m, l, al1 = soft(s1, m, l)
    acc = ctxc(1, p1, al1, acc)
    s3 = scores(3)
    p2, m, l, al2 = soft(s2, m, l)
    acc = ctxc(2, p2, al2, acc)
    p3, m, l, al3 = soft(s3, m, l)
    acc = ctxc(3, p3, al3, acc)
    linv = 1.0 / jnp.sum(l, axis=1, keepdims=True)

    accv = [[None] * NM for _ in range(3)]
    accm = [None] * NM

    def e_tiles(hs, cts, part):
        for ct in cts:
            for h in hs:
                g = h // 8
                o = _dot(acc[ct][g * 8:(g + 1) * 8], _tile(wuv, h, pl.ds(ct * 64, 64)))
                part[h] = o if h not in part else part[h] + o

    def head_ctx(h, part):
        g, r = divmod(h, 8)
        return part.pop(h)[r:r + 1] * linv[h:h + 1]

    def f_vpu(hs, part, accv):
        xbs = [_xb(head_ctx(h, part)) for h in hs]
        return _vmac3(accv, xbs, lambda j, s, n: o32[hs[j], pl.ds(s * 8, 8), pl.ds(n * 128, 128)])

    part = {}
    trip = [list(range(i, min(i + 3, OV))) for i in range(0, OV, 3)]
    e_tiles(trip[0], range(3), part)
    e_tiles(trip[1], range(3), part)
    e_tiles(trip[0], [3], part)
    accv = f_vpu(trip[0], part, accv)
    e_tiles(trip[1], [3], part)
    accv = f_vpu(trip[1], part, accv)
    for hs in trip[2:]:
        e_tiles(hs, range(NC), part)
        accv = f_vpu(hs, part, accv)
    lhs_m = {}
    for h in range(OV, H):
        e_tiles([h], range(NC), part)
        g, r = divmod(h, 8)
        lhs_m[h] = jnp.where(masks[r], part.pop(h) * linv[g * 8:(g + 1) * 8], 0.0)
    for n in range(NM):
        for h in range(OV, H):
            o = _dot(lhs_m[h], _tile(wo2, h, n))
            accm[n] = o if accm[n] is None else accm[n] + o
    x3 = [_rbf(x2[n] + _rbf(_rowsum(accm[n] + _fold3(accv, n)))) for n in range(NM)]
    mean3, rstd3 = _stats(x3)
    ln3 = [(x - mean3) * rstd3 for x in x3]
    sig3 = _router(ln3, wr)
    xb3 = []
    for kt in range(GV):
        xb3 += _xb_gather(x3[kt]) if GATH else _xb(x3[kt][0:1])
    hh = []
    blocks = [list(range(G0))] + [list(range(i, min(i + GB, NF))) for i in range(G0, NF, GB)]
    for fts in blocks:
        av = {}
        for s in range(16):
            for kt in range(GV):
                for ft in fts:
                    for nm, ref in (("g", g32), ("u", u32s)):
                        p = xb3[kt * 16 + s] * ref[ft, pl.ds(kt * 128 + s * 8, 8), :]
                        key = (nm, ft, kt)
                        av[key] = p if key not in av else av[key] + p
        for ft in fts:
            og = ou = None
            for kt in range(GV, NM):
                a = _dot(x3[kt], _tile(gt, ft, kt))
                b = _dot(x3[kt], _tile(ut, ft, kt))
                og = a if og is None else og + a
                ou = b if ou is None else ou + b
            tot = lambda nm: functools.reduce(lambda a, b: a + b, [av[nm, ft, kt] for kt in range(GV)])
            g = rstd3 * (og + _rowsum(tot("g")) - mean3 * csg[ft])
            u = rstd3 * (ou + _rowsum(tot("u")) - mean3 * csu[ft])
            hh.append(_silu(g) * u)
    y = [None] * NM
    for ft in range(DV, NF):
        for n in range(NM):
            o = down2(ft, n, hh[ft])
            y[n] = o if y[n] is None else y[n] + o
    yv = [[None] * NM for _ in range(3)]
    for i in range(0, DV, 3):
        fs = list(range(i, min(i + 3, DV)))
        yv = _vmac3(yv, [_xb(hh[ft][0:1]) for ft in fs],
                    lambda j, s, n: wd_f32(fs[j], s, n))
    if DV:
        y = [y[n] + _rowsum(_fold3(yv, n)) for n in range(NM)]
    x4 = [x3[n] + _rbf(ln3[n] + _rbf(y[n] * sig3)) for n in range(NM)]
    out = jnp.concatenate([x[0:1, :] for x in x4], axis=1)
    o_ref[0] = out.astype(bf16)


@jax.jit
def pallas_interleave_layers__compressed_kv_cla__moe_arch_mod__decode_kernel(
    A_x: jax.Array,
    A_c_kv: jax.Array,
    A_w_q: jax.Array,
    A_w_uk: jax.Array,
    A_w_uv: jax.Array,
    A_w_o: jax.Array,
    B_x: jax.Array,
    B_w_r: jax.Array,
    B_w_gate: jax.Array,
    B_w_up: jax.Array,
    B_w_down: jax.Array,
):
    del B_x
    any_spec = pl.BlockSpec(memory_space=pl.ANY)
    V = pltpu.VMEM
    scratch = [
        V((1, 1, M), bf16),
        V((NM, 128), bf16),
        V((M, H, D), bf16),
        V((DC, H, D), bf16),
        V((DC, H, D), bf16),
        V((NC, SK // 2, 128), u32),
        V((H, D, M), bf16),
        V((F, M), bf16),
        V((F, M), bf16),
        V((F, M), bf16),
        V((H, M // 2, D), u32),
        V((H, NC, D // 2, 128), u32),
        V((H, DC // 2, D), u32),
        V((NK, NC, 64, 128), u32),
        V((NF, NM, 64, 128), u32),
        V((NF, NM, 64, 128), u32),
        V((NF, max(GV, 1) * 128, 128), f32),
        V((NF, max(GV, 1) * 128, 128), f32),
        V((max(DV, 1) * 128, M), f32),
        V((max(OV, 1), D, M), f32),
        V((max(BV, 1), NC, D, 128), f32),
        V((H, max(AV, 1) * 128, D), f32),
        V((H, NM, 64, 128), u32),
        V((4, 8, 128), f32),
        V((NF, 8, 128), f32),
        V((NF, 8, 128), f32),
        V((NC, H, 128), f32),
        V((NC, H, 128), f32),
        V((4, 8, 128), f32),
        V((NF, 8, 128), f32),
        V((NM, 8, 128), f32),
        pltpu.SemaphoreType.DMA((40,)),
    ]
    return pl.pallas_call(
        _kernel,
        out_shape=jax.ShapeDtypeStruct((1, 1, M), bf16),
        in_specs=[any_spec] * 10,
        out_specs=pl.BlockSpec(memory_space=pltpu.VMEM),
        scratch_shapes=scratch,
        compiler_params=pltpu.CompilerParams(
            vmem_limit_bytes=100 * 1024 * 1024,
            disable_semaphore_checks=True,
            flags={"XLA_TPU_RESCHEDULE_DMA_DONES": True},
        ),
    )(A_x, A_c_kv, A_w_q, A_w_uk, A_w_uv, A_w_o, B_w_r.reshape(NM, 128),
      B_w_gate.T, B_w_up.T, B_w_down)
```

```python
import functools

import jax
import jax.numpy as jnp
from jax import lax
import jax.experimental.pallas as pl
import jax.experimental.pallas.tpu as pltpu

f32 = jnp.float32
bf16 = jnp.bfloat16
u32 = jnp.uint32
i32 = jnp.int32

M = 640
H = 32
D = 128
DC = 512
SK = 4096
F = 1728
NM = M // 128
NC = DC // 128
NK = SK // 128
NF = 14
EPS = 1e-5
SCALE = float(D) ** -0.5
KB = 8
NB = NK // KB
GV = 1
DV = 10
OV = 21
AV = 0
GB = 2
GORD = list(range(10)) + [13, 10, 11, 12]
GATH = 1
PRECONV = (0,1,2,3)
DRC = 384
DR0 = 768
DGROUPS = ((0,1),(2,3),(4,))
G0 = 3
BV = 14


def _dot(a, b):
    return jnp.dot(a, b, preferred_element_type=f32)


def _rbf(x):
    return x.astype(bf16).astype(f32)


def _tile(ref, *idx):
    return pltpu.bitcast(ref[idx], bf16)


def _stats(xs):
    s = xs[0] + xs[1] + xs[2] + xs[3] + xs[4]
    mean = jnp.sum(s, axis=1, keepdims=True) * (1.0 / M)
    ds = [x - mean for x in xs]
    q = ds[0] * ds[0] + ds[1] * ds[1] + ds[2] * ds[2] + ds[3] * ds[3] + ds[4] * ds[4]
    var = jnp.sum(q, axis=1, keepdims=True) * (1.0 / M)
    rstd = 1.0 / jnp.sqrt(var + EPS)
    return mean, rstd


def _router(lns, wr):
    s = lns[0] * wr[0] + lns[1] * wr[1] + lns[2] * wr[2] + lns[3] * wr[3] + lns[4] * wr[4]
    r = jnp.sum(s, axis=1, keepdims=True)
    return jax.nn.sigmoid(r)


def _rowsum(x):
    return jnp.broadcast_to(jnp.sum(x, axis=0, keepdims=True), x.shape)


def _xb(row):
    t = jnp.broadcast_to(row, (128, 128)).T
    return [t[s * 8:(s + 1) * 8] for s in range(16)]


def _xb_gather(rows):
    sub = lax.broadcasted_iota(i32, (8, 128), 0)
    return [jnp.take_along_axis(rows, sub + 8 * s, axis=1, mode="promise_in_bounds")
            for s in range(16)]


def _vmac(acc, xb, load):
    for s, xs in enumerate(xb):
        p = xs * load(s)
        acc = p if acc is None else acc + p
    return acc


def _vmacs(accs, xb, load):
    accs = list(accs)
    for s, xs in enumerate(xb):
        for i in range(len(accs)):
            p = xs * load(s, i)
            accs[i] = p if accs[i] is None else accs[i] + p
    return accs


def _vmac3(accs, xbs, load):
    accs = [list(a) for a in accs]
    for s in range(16):
        for j, xb in enumerate(xbs):
            for i in range(len(accs[j])):
                p = xb[s] * load(j, s, i)
                accs[j][i] = p if accs[j][i] is None else accs[j][i] + p
    return accs


def _fold3(accs, i):
    t = [a[i] for a in accs if a[i] is not None]
    return functools.reduce(lambda a, b: a + b, t)


def _silu(g):
    return g * jax.nn.sigmoid(g)


def _kernel(x_hbm, ckv_hbm, wq_hbm, wuk_hbm, wuv_hbm, wo_hbm, wr_hbm, wg_hbm, wu_hbm, wd_hbm,
            o_ref,
            x_v, wr_v, lq, luk, luv, lckv, lo, lg, lu, ld,
            wq, wukt, wuv, ckvt, gt, ut, g32, u32s, d32, o32, b32, q32, wo2,
            csq, csg, csu, qa_s, cc_s, ctx_s, hh_s, x_s,
            sems):
    row8 = lax.broadcasted_iota(i32, (8, 128), 0)
    masks = [row8 == r for r in range(8)]

    copies = {}
    order = []

    def add(name, pairs):
        sem = sems.at[len(copies)]
        cs = [pltpu.make_async_copy(s, d, sem) for s, d in pairs]
        copies[name] = cs
        order.append(name)

    add("x", [(x_hbm, x_v)])
    add("wr", [(wr_hbm, wr_v)])
    for i in range(NM):
        add(("q", i), [(wq_hbm.at[pl.ds(i * 128, 128)], lq.at[pl.ds(i * 128, 128)])])
    for i in range(NC):
        add(("uk", i), [(wuk_hbm.at[pl.ds(i * 128, 128)], luk.at[pl.ds(i * 128, 128)])])
    ckv32 = ckv_hbm.at[0].bitcast(u32)
    for b in range(NB):
        add(("ckv", b), [(ckv32.at[pl.ds(b * 512, 512), pl.ds(ct * 128, 128)],
                          lckv.at[ct, pl.ds(b * 512, 512)]) for ct in range(NC)])
    FS = [(0, 896), (896, F - 896)]
    for i, (s, n) in enumerate(FS):
        add(("g", i), [(wg_hbm.at[pl.ds(s, n)], lg.at[pl.ds(s, n)])])
    for i, (s, n) in enumerate(FS):
        add(("u", i), [(wu_hbm.at[pl.ds(s, n)], lu.at[pl.ds(s, n)])])
    for i in range(NC):
        add(("uv", i), [(wuv_hbm.at[pl.ds(i * 128, 128)], luv.at[pl.ds(i * 128, 128)])])
    for g in range(4):
        add(("o", g), [(wo_hbm.at[pl.ds(g * 8, 8)], lo.at[pl.ds(g * 8, 8)])])
    for i in range(DR0 // DRC):
        add(("d", i), [(wd_hbm.at[pl.ds(i * DRC, DRC)], ld.at[pl.ds(i * DRC, DRC)])])
    for i, cols in enumerate(DGROUPS):
        c0, nc = cols[0] * 128, len(cols) * 128
        add(("dc", i), [(wd_hbm.at[pl.ds(DR0, F - DR0), pl.ds(c0, nc)],
                         ld.at[pl.ds(DR0, F - DR0), pl.ds(c0, nc)])])

    for name in order:
        for c in copies[name]:
            c.start()

    def wait(name):
        for c in copies[name]:
            c.wait()

    names = list(copies)

    def wait_dyn(first_name, i, pairs_fn):
        base = names.index(first_name)
        for s, d in pairs_fn(i):
            pltpu.make_async_copy(s, d, sems.at[base + i]).wait()

    wait("x")
    wait("wr")
    xr = x_v[0].astype(f32)
    x0 = [jnp.broadcast_to(xr[:, n * 128:(n + 1) * 128], (8, 128)) for n in range(NM)]
    wrf = wr_v[...].astype(f32)
    wr = [jnp.broadcast_to(wrf[n:n + 1, :], (8, 128)) for n in range(NM)]
    for n in range(NM):
        x_s[n] = x0[n]
    mean0, rstd0 = _stats(x0)
    ones8 = jnp.ones((8, 128), f32)
    zero8 = jnp.zeros((8, 128), f32)

    def a_body(kt, carry):
        raw, cs = carry
        s = pl.multiple_of(kt * 128, 128)
        wait_dyn(("q", 0), kt, lambda i: [(wq_hbm.at[pl.ds(s, 128)], lq.at[pl.ds(s, 128)])])
        t = jnp.swapaxes(lq[pl.ds(s, 128)], 0, 1)
        s2 = pl.multiple_of(kt * 64, 64)
        for h in range(H):
            wq[h, pl.ds(s2, 64), :] = pltpu.bitcast(t[h], u32)
        if AV:
            @pl.when(kt < AV)
            def _():
                sv = pl.multiple_of(jnp.minimum(kt, AV - 1) * 128, 128)
                for h in range(H):
                    w = wq[h, pl.ds(s2, 64), :]
                    q32[h, pl.ds(sv, 128), :] = pltpu.bitcast(w, bf16).astype(f32)
        lhs = jnp.concatenate([x_s[kt], ones8], axis=0)
        raw, cs = list(raw), list(cs)
        for h in range(H):
            g, r = divmod(h, 8)
            out = _dot(lhs, pltpu.bitcast(wq[h, pl.ds(s2, 64), :], bf16))
            raw[g] = jnp.where(masks[r], raw[g] + out[0:8], raw[g])
            cs[g] = jnp.where(masks[r], cs[g] + out[8:16], cs[g])
        return tuple(raw), tuple(cs)

    raw, cs = lax.fori_loop(0, NM, a_body, ((zero8,) * 4, (zero8,) * 4))
    for g in range(4):
        csq[g] = cs[g]
    q = [rstd0 * (raw[g] - mean0 * cs[g]) for g in range(4)]

    def b_body(ct, _):
        s = pl.multiple_of(ct * 128, 128)
        wait_dyn(("uk", 0), ct, lambda i: [(wuk_hbm.at[pl.ds(s, 128)], luk.at[pl.ds(s, 128)])])
        t = jnp.swapaxes(luk[pl.ds(s, 128)], 0, 1)
        for h in range(H):
            th = t[h].T
            wukt[h, ct] = pltpu.bitcast(th, u32)
            if h < BV:
                b32[h, ct] = th.astype(f32)
        qa = [zero8] * 4
        for h in range(H):
            g, r = divmod(h, 8)
            out = _dot(q[g], pltpu.bitcast(wukt[h, ct], bf16))
            qa[g] = jnp.where(masks[r], out, qa[g])
        qa_s[ct] = jnp.concatenate(qa, axis=0)
        return _

    lax.fori_loop(0, NC, b_body, 0)

    def cd_body(b, carry):
        m, l, acc = carry
        s = pl.multiple_of(b * 512, 512)
        wait_dyn(("ckv", 0), b, lambda i: [(ckv32.at[pl.ds(s, 512), pl.ds(ct * 128, 128)],
                                            lckv.at[ct, pl.ds(s, 512)]) for ct in range(NC)])
        ss = []
        for j in range(KB):
            kt = b * KB + j
            sk = pl.multiple_of(s + j * 64, 64)
            sc = None
            for ct in range(NC):
                t = pltpu.bitcast(lckv[ct, pl.ds(sk, 64), :], bf16).T
                ckvt[kt, ct] = pltpu.bitcast(t, u32)
                o = _dot(qa_s[ct], t)
                sc = o if sc is None else sc + o
            ss.append(sc * SCALE)
        mb = ss[0]
        for j in range(1, KB):
            mb = jnp.maximum(mb, ss[j])
        m_new = jnp.maximum(m, jnp.max(mb, axis=1, keepdims=True))
        alpha = jnp.exp(m - m_new)
        ps = [jnp.exp(sj - m_new) for sj in ss]
        lb = ps[0]
        for j in range(1, KB):
            lb = lb + ps[j]
        l = l * alpha + lb
        acc = [a * alpha for a in acc]
        for j in range(KB):
            sk = pl.multiple_of(s + j * 64, 64)
            for ct in range(NC):
                acc[ct] = acc[ct] + _dot(ps[j], pltpu.bitcast(lckv[ct, pl.ds(sk, 64), :], bf16))
        return m_new, l, acc

    m_init = jnp.full((H, 128), -jnp.inf, f32)
    _, l, acc = lax.fori_loop(0, NB, cd_body,
                              (m_init, jnp.zeros((H, 128), f32),
                               [jnp.zeros((H, 128), f32)] * NC))
    linv = 1.0 / jnp.sum(l, axis=1, keepdims=True)
    for ct in range(NC):
        cc_s[ct] = acc[ct]

    def transpose_ffn(land, dst, dst32, fam):
        def body(ft, _):
            s = pl.multiple_of(ft * 128, 128)
            for kt in range(NM):
                t = land[pl.ds(s, 128), pl.ds(kt * 128, 128)].T
                dst[ft, kt] = pltpu.bitcast(t, u32)
                if kt < GV:
                    dst32[ft, pl.ds(kt * 128, 128), :] = t.astype(f32)
            return _
        wait((fam, 0))
        lax.fori_loop(0, 7, body, 0)
        wait((fam, 1))
        lax.fori_loop(7, 13, body, 0)

    transpose_ffn(lg, gt, g32, "g")
    transpose_ffn(lu, ut, u32s, "u")
    for kt in range(NM):
        t = jnp.concatenate([lg[pl.ds(13 * 128, 64), pl.ds(kt * 128, 128)],
                             lu[pl.ds(13 * 128, 64), pl.ds(kt * 128, 128)]], axis=0).T
        gt[13, kt] = pltpu.bitcast(t, u32)
        if kt < GV:
            g32[13, pl.ds(kt * 128, 128), :] = t.astype(f32)

    def e_body(ct, ctx):
        s = pl.multiple_of(ct * 128, 128)
        wait_dyn(("uv", 0), ct, lambda i: [(wuv_hbm.at[pl.ds(s, 128)], luv.at[pl.ds(s, 128)])])
        t = jnp.swapaxes(luv[pl.ds(s, 128)], 0, 1)
        s2 = pl.multiple_of(ct * 64, 64)
        for h in range(H):
            wuv[h, pl.ds(s2, 64), :] = pltpu.bitcast(t[h], u32)
        ctx = list(ctx)
        cc = cc_s[ct]
        for h in range(H):
            g, r = divmod(h, 8)
            out = _dot(cc[g * 8:(g + 1) * 8], pltpu.bitcast(wuv[h, pl.ds(s2, 64), :], bf16))
            ctx[g] = jnp.where(masks[r], ctx[g] + out, ctx[g])
        return tuple(ctx)

    ctx = lax.fori_loop(0, NC, e_body, (zero8,) * 4)
    for g in range(4):
        ctx_s[g] = ctx[g] * linv[g * 8:(g + 1) * 8]

    def f_body(g, acc):
        s = pl.multiple_of(g * 8, 8)
        wait_dyn(("o", 0), g, lambda i: [(wo_hbm.at[pl.ds(s, 8)], lo.at[pl.ds(s, 8)])])
        acc = list(acc)
        cg = ctx_s[g]
        for r in range(8):
            lhs = jnp.where(masks[r], cg, 0.0)
            for n in range(NM):
                t = lo[s + r, :, pl.ds(n * 128, 128)]
                wo2[s + r, n] = pltpu.bitcast(t, u32)
                acc[n] = acc[n] + _dot(lhs, t)
        for r in range(8):
            @pl.when(s + r < OV)
            def _():
                o32[jnp.minimum(s + r, OV - 1)] = lo[s + r].astype(f32)
        return tuple(acc)

    acc = lax.fori_loop(0, 4, f_body, (zero8,) * NM)
    x1 = [_rbf(x0[n] + _rbf(_rowsum(acc[n]))) for n in range(NM)]

    mean1, rstd1 = _stats(x1)
    ln1 = [(x - mean1) * rstd1 for x in x1]
    sig1 = _router(ln1, wr)
    lhs1 = [jnp.concatenate([x1[kt], ones8], axis=0) for kt in range(NM)]

    hh1 = []
    NE_ = DR0 // 128
    for ft in range(NF):
        og = ou = None
        for kt in range(NM):
            a = _dot(lhs1[kt], _tile(gt, ft, kt))
            og = a if og is None else og + a
            if ft < 13:
                b = _dot(lhs1[kt], _tile(ut, ft, kt))
                ou = b if ou is None else ou + b
        csg[ft] = og[8:16]
        g = rstd1 * (og[0:8] - mean1 * og[8:16])
        if ft < 13:
            csu[ft] = ou[8:16]
            u = rstd1 * (ou[0:8] - mean1 * ou[8:16])
        else:
            u = pltpu.roll(g, 64, 1)
        hh1.append(_silu(g) * u)
        if ft < NE_:
            hh_s[ft] = hh1[ft]

    NE = DR0 // 128

    def wd_tile(ft, n):
        return ld[pl.ds(ft * 128, min(128, F - ft * 128)), pl.ds(n * 128, 128)]

    def down2(ft, n, hh):
        return _dot(hh if ft < 13 else hh[:, :64], wd_tile(ft, n))

    def wd_f32(ft, s, n):
        if ft < NE or n in PRECONV:
            return d32[pl.ds(ft * 128 + s * 8, 8), pl.ds(n * 128, 128)]
        return wd_tile(ft, n).astype(f32)[s * 8:(s + 1) * 8]

    FPC = DRC // 128

    def h_body(i, y):
        s = pl.multiple_of(i * DRC, 128)
        wait_dyn(("d", 0), i, lambda _: [(wd_hbm.at[pl.ds(s, DRC)], ld.at[pl.ds(s, DRC)])])
        y = list(y)
        for j in range(FPC):
            ft = i * FPC + j
            sf = pl.multiple_of(s + j * 128, 128)
            hh = hh_s[ft]
            for n in range(NM):
                t = ld[pl.ds(sf, 128), pl.ds(n * 128, 128)]
                y[n] = y[n] + _dot(hh, t)
        for j in range(FPC):
            ft = i * FPC + j
            sf = pl.multiple_of(s + j * 128, 128)
            if DV:
                @pl.when(ft < DV)
                def _():
                    sd = pl.multiple_of(jnp.minimum(ft, DV - 1) * 128, 128)
                    d32[pl.ds(sd, 128), :] = ld[pl.ds(sf, 128), :].astype(f32)
        return tuple(y)

    y = list(lax.fori_loop(0, DR0 // DRC, h_body, (zero8,) * NM))

    x2 = [None] * NM
    racc = [None] * 4

    def h_late(n):
        for ft in range(NE, NF):
            y[n] = y[n] + down2(ft, n, hh1[ft])
        x2[n] = _rbf(x1[n] + _rbf(ln1[n] + _rbf(y[n] * sig1)))
        if n in PRECONV:
            for ft in range(NE, DV):
                d32[pl.ds(ft * 128, 128), pl.ds(n * 128, 128)] = wd_tile(ft, n).astype(f32)

    def a_pass(kt, heads=range(H)):
        for h in heads:
            g, r = divmod(h, 8)
            o = _dot(jnp.where(masks[r], x2[kt], 0.0), _tile(wq, h, pl.ds(kt * 64, 64)))
            racc[g] = o if racc[g] is None else racc[g] + o

    wait(("dc", 0))
    h_late(0)
    h_late(1)
    a_pass(0)
    a_pass(1)
    wait(("dc", 1))
    h_late(2)
    h_late(3)
    a_pass(2)
    wait(("dc", 2))
    h_late(4)
    a_pass(3, range(0, 16))
    mean2, rstd2 = _stats(x2)
    raw = {}
    KL = DGROUPS[-1][-1]
    last = {}
    for h in range(BV):
        last[h] = _dot(x2[KL], _tile(wq, h, pl.ds(KL * 64, 64)))
    a_pass(3, range(16, H))
    for h in range(BV, H):
        last[h] = _dot(x2[KL], _tile(wq, h, pl.ds(KL * 64, 64)))
    for h in range(H):
        raw[h] = racc[h // 8] + last[h]
    qv = {}
    for i in range(0, BV, 3):
        hs = list(range(i, min(i + 3, BV)))
        xbs = []
        for h in hs:
            g, r = divmod(h, 8)
            qh = raw[h][r:r + 1] - mean2[0:1] * csq[g, pl.ds(r, 1), :]
            xbs.append(_xb(qh))
        accs = _vmac3([[None] * NC for _ in hs], xbs,
                      lambda j, s, ct: b32[hs[j], ct, pl.ds(s * 8, 8), :])
        for j, h in enumerate(hs):
            for ct in range(NC):
                qv[h, ct] = _rowsum(accs[j][ct]) * rstd2
    q = {}
    for g in range(BV // 8, 4):
        rawg = zero8
        for r in range(8):
            if g * 8 + r >= BV:
                rawg = jnp.where(masks[r], raw[g * 8 + r], rawg)
        q[g] = rstd2 * (rawg - mean2 * csq[g])
    qa = []
    for ct in range(NC):
        qg = [zero8] * 4
        for h in range(H):
            g, r = divmod(h, 8)
            o = qv[h, ct] if h < BV else _dot(q[g], _tile(wukt, h, ct))
            qg[g] = jnp.where(masks[r], o, qg[g])
        qa.append(jnp.concatenate(qg, axis=0))

    def scores(b):
        ss = []
        for j in range(KB):
            kt = b * KB + j
            sc = None
            for ct in range(NC):
                o = _dot(qa[ct], _tile(ckvt, kt, ct))
                sc = o if sc is None else sc + o
            ss.append(sc * SCALE)
        return ss

    def soft(ss, m, l):
        mb = ss[0]
        for j in range(1, KB):
            mb = jnp.maximum(mb, ss[j])
        mb = jnp.max(mb, axis=1, keepdims=True)
        m_new = mb if m is None else jnp.maximum(m, mb)
        ps = [jnp.exp(sj - m_new) for sj in ss]
        lb = ps[0]
        for j in range(1, KB):
            lb = lb + ps[j]
        if m is None:
            return ps, m_new, lb, None
        alpha = jnp.exp(m - m_new)
        return ps, m_new, l * alpha + lb, alpha

    def ctxc(b, ps, alpha, acc):
        if acc is not None:
            acc = [a * alpha for a in acc]
        else:
            acc = [None] * NC
        acc = list(acc)
        last = b == NB - 1
        seq = ([(j, ct) for ct in range(NC) for j in range(KB)] if last
               else [(j, ct) for j in range(KB) for ct in range(NC)])
        for j, ct in seq:
            kt = b * KB + j
            o = _dot(ps[j], _tile(lckv, ct, pl.ds(kt * 64, 64)))
            acc[ct] = o if acc[ct] is None else acc[ct] + o
        return acc

    s0 = scores(0)
    s1 = scores(1)
    p0, m, l, al0 = soft(s0, None, None)
    acc = ctxc(0, p0, None, None)
    s2 = scores(2)
    p1, m, l, al1 = soft(s1, m, l)
    acc = ctxc(1, p1, al1, acc)
    s3 = scores(3)
    p2, m, l, al2 = soft(s2, m, l)
    acc = ctxc(2, p2, al2, acc)
    p3, m, l, al3 = soft(s3, m, l)
    acc = ctxc(3, p3, al3, acc)
    linv = 1.0 / jnp.sum(l, axis=1, keepdims=True)

    accv = [[None] * NM for _ in range(3)]
    accm = [None] * NM

    def e_tiles(hs, cts, part):
        for ct in cts:
            for h in hs:
                g = h // 8
                o = _dot(acc[ct][g * 8:(g + 1) * 8], _tile(wuv, h, pl.ds(ct * 64, 64)))
                part[h] = o if h not in part else part[h] + o

    def head_ctx(h, part):
        g, r = divmod(h, 8)
        return part.pop(h)[r:r + 1] * linv[h:h + 1]

    def f_vpu(hs, part, accv):
        xbs = [_xb(head_ctx(h, part)) for h in hs]
        return _vmac3(accv, xbs, lambda j, s, n: o32[hs[j], pl.ds(s * 8, 8), pl.ds(n * 128, 128)])

    part = {}
    trip = [list(range(i, min(i + 3, OV))) for i in range(0, OV, 3)]
    e_tiles(trip[0], range(3), part)
    e_tiles(trip[1], range(3), part)
    e_tiles(trip[0], [3], part)
    accv = f_vpu(trip[0], part, accv)
    e_tiles(trip[1], [3], part)
    accv = f_vpu(trip[1], part, accv)
    for hs in trip[2:]:
        e_tiles(hs, range(NC), part)
        accv = f_vpu(hs, part, accv)
    lhs_m = {}
    for h in range(OV, H):
        e_tiles([h], range(NC), part)
        g, r = divmod(h, 8)
        lhs_m[h] = jnp.where(masks[r], part.pop(h) * linv[g * 8:(g + 1) * 8], 0.0)
    for n in range(NM):
        for h in range(OV, H):
            o = _dot(lhs_m[h], _tile(wo2, h, n))
            accm[n] = o if accm[n] is None else accm[n] + o
    x3 = [_rbf(x2[n] + _rbf(_rowsum(accm[n] + _fold3(accv, n)))) for n in range(NM)]
    mean3, rstd3 = _stats(x3)
    ln3 = [(x - mean3) * rstd3 for x in x3]
    sig3 = _router(ln3, wr)
    xb3 = []
    for kt in range(GV):
        xb3 += _xb_gather(x3[kt]) if GATH else _xb(x3[kt][0:1])
    hh = {}
    for ft in GORD:
        srcs = (("g", g32, gt), ("u", u32s, ut)) if ft < 13 else (("g", g32, gt),)
        val = {}
        for nm, ref, mref in srcs:
            av = None
            for s in range(16):
                for kt in range(GV):
                    p = xb3[kt * 16 + s] * ref[ft, pl.ds(kt * 128 + s * 8, 8), :]
                    av = p if av is None else av + p
            om = None
            for kt in range(GV, NM):
                a = _dot(x3[kt], _tile(mref, ft, kt))
                om = a if om is None else om + a
            cs_ = csg[ft] if nm == "g" else csu[ft]
            val[nm] = rstd3 * (om + _rowsum(av) - mean3 * cs_)
        u = val["u"] if ft < 13 else pltpu.roll(val["g"], 64, 1)
        hh[ft] = _silu(val["g"]) * u
    y = [None] * NM
    for ft in range(DV, NF):
        for n in range(NM):
            o = down2(ft, n, hh[ft])
            y[n] = o if y[n] is None else y[n] + o
    yv = [[None] * NM for _ in range(3)]
    for i in range(0, DV, 3):
        fs = list(range(i, min(i + 3, DV)))
        yv = _vmac3(yv, [_xb(hh[ft][0:1]) for ft in fs],
                    lambda j, s, n: wd_f32(fs[j], s, n))
    if DV:
        y = [y[n] + _rowsum(_fold3(yv, n)) for n in range(NM)]
    x4 = [x3[n] + _rbf(ln3[n] + _rbf(y[n] * sig3)) for n in range(NM)]
    out = jnp.concatenate([x[0:1, :] for x in x4], axis=1)
    o_ref[0] = out.astype(bf16)


@jax.jit
def pallas_interleave_layers__compressed_kv_cla__moe_arch_mod__decode_kernel(
    A_x: jax.Array,
    A_c_kv: jax.Array,
    A_w_q: jax.Array,
    A_w_uk: jax.Array,
    A_w_uv: jax.Array,
    A_w_o: jax.Array,
    B_x: jax.Array,
    B_w_r: jax.Array,
    B_w_gate: jax.Array,
    B_w_up: jax.Array,
    B_w_down: jax.Array,
):
    del B_x
    any_spec = pl.BlockSpec(memory_space=pl.ANY)
    V = pltpu.VMEM
    scratch = [
        V((1, 1, M), bf16),
        V((NM, 128), bf16),
        V((M, H, D), bf16),
        V((DC, H, D), bf16),
        V((DC, H, D), bf16),
        V((NC, SK // 2, 128), u32),
        V((H, D, M), bf16),
        V((F, M), bf16),
        V((F, M), bf16),
        V((F, M), bf16),
        V((H, M // 2, D), u32),
        V((H, NC, D // 2, 128), u32),
        V((H, DC // 2, D), u32),
        V((NK, NC, 64, 128), u32),
        V((NF, NM, 64, 128), u32),
        V((NF, NM, 64, 128), u32),
        V((NF, max(GV, 1) * 128, 128), f32),
        V((NF, max(GV, 1) * 128, 128), f32),
        V((max(DV, 1) * 128, M), f32),
        V((max(OV, 1), D, M), f32),
        V((max(BV, 1), NC, D, 128), f32),
        V((H, max(AV, 1) * 128, D), f32),
        V((H, NM, 64, 128), u32),
        V((4, 8, 128), f32),
        V((NF, 8, 128), f32),
        V((NF, 8, 128), f32),
        V((NC, H, 128), f32),
        V((NC, H, 128), f32),
        V((4, 8, 128), f32),
        V((NF, 8, 128), f32),
        V((NM, 8, 128), f32),
        pltpu.SemaphoreType.DMA((40,)),
    ]
    return pl.pallas_call(
        _kernel,
        out_shape=jax.ShapeDtypeStruct((1, 1, M), bf16),
        in_specs=[any_spec] * 10,
        out_specs=pl.BlockSpec(memory_space=pltpu.VMEM),
        scratch_shapes=scratch,
        compiler_params=pltpu.CompilerParams(
            vmem_limit_bytes=100 * 1024 * 1024,
            disable_semaphore_checks=True,
            flags={"XLA_TPU_RESCHEDULE_DMA_DONES": True},
        ),
    )(A_x, A_c_kv, A_w_q, A_w_uk, A_w_uv, A_w_o, B_w_r.reshape(NM, 128),
      B_w_gate.T, B_w_up.T, B_w_down)
```

```python
import functools

import jax
import jax.numpy as jnp
from jax import lax
import jax.experimental.pallas as pl
import jax.experimental.pallas.tpu as pltpu

f32 = jnp.float32
bf16 = jnp.bfloat16
u32 = jnp.uint32
i32 = jnp.int32

M = 640
H = 32
D = 128
DC = 512
SK = 4096
F = 1728
NM = M // 128
NC = DC // 128
NK = SK // 128
NF = 14
EPS = 1e-5
SCALE = float(D) ** -0.5
KB = 8
NB = NK // KB
GV = 1
DV = 10
OV = 21
AV = 1
AVT = 4
A3M = 12
GB = 2
GORD = list(range(10)) + [13, 10, 11, 12]
GATH = 1
PRECONV = (0,1,2,3)
DRC = 384
DR0 = 768
DGROUPS = ((0,1),(2,3),(4,))
G0 = 3
BV = 12


def _dot(a, b):
    return jnp.dot(a, b, preferred_element_type=f32)


def _rbf(x):
    return x.astype(bf16).astype(f32)


def _tile(ref, *idx):
    return pltpu.bitcast(ref[idx], bf16)


def _stats(xs):
    s = xs[0] + xs[1] + xs[2] + xs[3] + xs[4]
    mean = jnp.sum(s, axis=1, keepdims=True) * (1.0 / M)
    ds = [x - mean for x in xs]
    q = ds[0] * ds[0] + ds[1] * ds[1] + ds[2] * ds[2] + ds[3] * ds[3] + ds[4] * ds[4]
    var = jnp.sum(q, axis=1, keepdims=True) * (1.0 / M)
    rstd = 1.0 / jnp.sqrt(var + EPS)
    return mean, rstd


def _router(lns, wr):
    s = lns[0] * wr[0] + lns[1] * wr[1] + lns[2] * wr[2] + lns[3] * wr[3] + lns[4] * wr[4]
    r = jnp.sum(s, axis=1, keepdims=True)
    return jax.nn.sigmoid(r)


def _rowsum(x):
    return jnp.broadcast_to(jnp.sum(x, axis=0, keepdims=True), x.shape)


def _xb(row):
    t = jnp.broadcast_to(row, (128, 128)).T
    return [t[s * 8:(s + 1) * 8] for s in range(16)]


def _xb_gather(rows):
    sub = lax.broadcasted_iota(i32, (8, 128), 0)
    return [jnp.take_along_axis(rows, sub + 8 * s, axis=1, mode="promise_in_bounds")
            for s in range(16)]


def _vmac(acc, xb, load):
    for s, xs in enumerate(xb):
        p = xs * load(s)
        acc = p if acc is None else acc + p
    return acc


def _vmacs(accs, xb, load):
    accs = list(accs)
    for s, xs in enumerate(xb):
        for i in range(len(accs)):
            p = xs * load(s, i)
            accs[i] = p if accs[i] is None else accs[i] + p
    return accs


def _vmac3(accs, xbs, load):
    accs = [list(a) for a in accs]
    for s in range(16):
        for j, xb in enumerate(xbs):
            for i in range(len(accs[j])):
                p = xb[s] * load(j, s, i)
                accs[j][i] = p if accs[j][i] is None else accs[j][i] + p
    return accs


def _fold3(accs, i):
    t = [a[i] for a in accs if a[i] is not None]
    return functools.reduce(lambda a, b: a + b, t)


def _silu(g):
    return g * jax.nn.sigmoid(g)


def _kernel(x_hbm, ckv_hbm, wq_hbm, wuk_hbm, wuv_hbm, wo_hbm, wr_hbm, wg_hbm, wu_hbm, wd_hbm,
            o_ref,
            x_v, wr_v, lq, luk, luv, lckv, lo, lg, lu, ld,
            wq, wukt, wuv, ckvt, gt, ut, g32, u32s, d32, o32, b32, q32, wo2,
            csq, csg, csu, qa_s, cc_s, ctx_s, hh_s, x_s,
            sems):
    row8 = lax.broadcasted_iota(i32, (8, 128), 0)
    masks = [row8 == r for r in range(8)]

    copies = {}
    order = []

    def add(name, pairs):
        sem = sems.at[len(copies)]
        cs = [pltpu.make_async_copy(s, d, sem) for s, d in pairs]
        copies[name] = cs
        order.append(name)

    add("x", [(x_hbm, x_v)])
    add("wr", [(wr_hbm, wr_v)])
    for i in range(NM):
        add(("q", i), [(wq_hbm.at[pl.ds(i * 128, 128)], lq.at[pl.ds(i * 128, 128)])])
    for i in range(NC):
        add(("uk", i), [(wuk_hbm.at[pl.ds(i * 128, 128)], luk.at[pl.ds(i * 128, 128)])])
    ckv32 = ckv_hbm.at[0].bitcast(u32)
    for b in range(NB):
        add(("ckv", b), [(ckv32.at[pl.ds(b * 512, 512), pl.ds(ct * 128, 128)],
                          lckv.at[ct, pl.ds(b * 512, 512)]) for ct in range(NC)])
    FS = [(0, 896), (896, F - 896)]
    for i, (s, n) in enumerate(FS):
        add(("g", i), [(wg_hbm.at[pl.ds(s, n)], lg.at[pl.ds(s, n)])])
    for i, (s, n) in enumerate(FS):
        add(("u", i), [(wu_hbm.at[pl.ds(s, n)], lu.at[pl.ds(s, n)])])
    for i in range(NC):
        add(("uv", i), [(wuv_hbm.at[pl.ds(i * 128, 128)], luv.at[pl.ds(i * 128, 128)])])
    for g in range(4):
        add(("o", g), [(wo_hbm.at[pl.ds(g * 8, 8)], lo.at[pl.ds(g * 8, 8)])])
    for i in range(DR0 // DRC):
        add(("d", i), [(wd_hbm.at[pl.ds(i * DRC, DRC)], ld.at[pl.ds(i * DRC, DRC)])])
    for i, cols in enumerate(DGROUPS):
        c0, nc = cols[0] * 128, len(cols) * 128
        add(("dc", i), [(wd_hbm.at[pl.ds(DR0, F - DR0), pl.ds(c0, nc)],
                         ld.at[pl.ds(DR0, F - DR0), pl.ds(c0, nc)])])

    for name in order:
        for c in copies[name]:
            c.start()

    def wait(name):
        for c in copies[name]:
            c.wait()

    names = list(copies)

    def wait_dyn(first_name, i, pairs_fn):
        base = names.index(first_name)
        for s, d in pairs_fn(i):
            pltpu.make_async_copy(s, d, sems.at[base + i]).wait()

    wait("x")
    wait("wr")
    xr = x_v[0].astype(f32)
    x0 = [jnp.broadcast_to(xr[:, n * 128:(n + 1) * 128], (8, 128)) for n in range(NM)]
    wrf = wr_v[...].astype(f32)
    wr = [jnp.broadcast_to(wrf[n:n + 1, :], (8, 128)) for n in range(NM)]
    for n in range(NM):
        x_s[n] = x0[n]
    mean0, rstd0 = _stats(x0)
    ones8 = jnp.ones((8, 128), f32)
    zero8 = jnp.zeros((8, 128), f32)

    def a_body(kt, carry):
        raw, cs = carry
        s = pl.multiple_of(kt * 128, 128)
        wait_dyn(("q", 0), kt, lambda i: [(wq_hbm.at[pl.ds(s, 128)], lq.at[pl.ds(s, 128)])])
        t = jnp.swapaxes(lq[pl.ds(s, 128)], 0, 1)
        s2 = pl.multiple_of(kt * 64, 64)
        for h in range(H):
            wq[h, pl.ds(s2, 64), :] = pltpu.bitcast(t[h], u32)
        if AV:
            @pl.when((kt >= AVT - AV) & (kt < AVT))
            def _():
                sv = pl.multiple_of(jnp.clip(kt - (AVT - AV), 0, AV - 1) * 128, 128)
                for h in range(H):
                    w = wq[h, pl.ds(s2, 64), :]
                    q32[h, pl.ds(sv, 128), :] = pltpu.bitcast(w, bf16).astype(f32)
        lhs = jnp.concatenate([x_s[kt], ones8], axis=0)
        raw, cs = list(raw), list(cs)
        for h in range(H):
            g, r = divmod(h, 8)
            out = _dot(lhs, pltpu.bitcast(wq[h, pl.ds(s2, 64), :], bf16))
            raw[g] = jnp.where(masks[r], raw[g] + out[0:8], raw[g])
            cs[g] = jnp.where(masks[r], cs[g] + out[8:16], cs[g])
        return tuple(raw), tuple(cs)

    raw, cs = lax.fori_loop(0, NM, a_body, ((zero8,) * 4, (zero8,) * 4))
    for g in range(4):
        csq[g] = cs[g]
    q = [rstd0 * (raw[g] - mean0 * cs[g]) for g in range(4)]

    def b_body(ct, _):
        s = pl.multiple_of(ct * 128, 128)
        wait_dyn(("uk", 0), ct, lambda i: [(wuk_hbm.at[pl.ds(s, 128)], luk.at[pl.ds(s, 128)])])
        t = jnp.swapaxes(luk[pl.ds(s, 128)], 0, 1)
        for h in range(H):
            th = t[h].T
            wukt[h, ct] = pltpu.bitcast(th, u32)
            if h < BV:
                b32[h, ct] = th.astype(f32)
        qa = [zero8] * 4
        for h in range(H):
            g, r = divmod(h, 8)
            out = _dot(q[g], pltpu.bitcast(wukt[h, ct], bf16))
            qa[g] = jnp.where(masks[r], out, qa[g])
        qa_s[ct] = jnp.concatenate(qa, axis=0)
        return _

    lax.fori_loop(0, NC, b_body, 0)

    def cd_body(b, carry):
        m, l, acc = carry
        s = pl.multiple_of(b * 512, 512)
        wait_dyn(("ckv", 0), b, lambda i: [(ckv32.at[pl.ds(s, 512), pl.ds(ct * 128, 128)],
                                            lckv.at[ct, pl.ds(s, 512)]) for ct in range(NC)])
        ss = []
        for j in range(KB):
            kt = b * KB + j
            sk = pl.multiple_of(s + j * 64, 64)
            sc = None
            for ct in range(NC):
                t = pltpu.bitcast(lckv[ct, pl.ds(sk, 64), :], bf16).T
                ckvt[kt, ct] = pltpu.bitcast(t, u32)
                o = _dot(qa_s[ct], t)
                sc = o if sc is None else sc + o
            ss.append(sc * SCALE)
        mb = ss[0]
        for j in range(1, KB):
            mb = jnp.maximum(mb, ss[j])
        m_new = jnp.maximum(m, jnp.max(mb, axis=1, keepdims=True))
        alpha = jnp.exp(m - m_new)
        ps = [jnp.exp(sj - m_new) for sj in ss]
        lb = ps[0]
        for j in range(1, KB):
            lb = lb + ps[j]
        l = l * alpha + lb
        acc = [a * alpha for a in acc]
        for j in range(KB):
            sk = pl.multiple_of(s + j * 64, 64)
            for ct in range(NC):
                acc[ct] = acc[ct] + _dot(ps[j], pltpu.bitcast(lckv[ct, pl.ds(sk, 64), :], bf16))
        return m_new, l, acc

    m_init = jnp.full((H, 128), -jnp.inf, f32)
    _, l, acc = lax.fori_loop(0, NB, cd_body,
                              (m_init, jnp.zeros((H, 128), f32),
                               [jnp.zeros((H, 128), f32)] * NC))
    linv = 1.0 / jnp.sum(l, axis=1, keepdims=True)
    for ct in range(NC):
        cc_s[ct] = acc[ct]

    def transpose_ffn(land, dst, dst32, fam):
        def body(ft, _):
            s = pl.multiple_of(ft * 128, 128)
            for kt in range(NM):
                t = land[pl.ds(s, 128), pl.ds(kt * 128, 128)].T
                dst[ft, kt] = pltpu.bitcast(t, u32)
                if kt < GV:
                    dst32[ft, pl.ds(kt * 128, 128), :] = t.astype(f32)
            return _
        wait((fam, 0))
        lax.fori_loop(0, 7, body, 0)
        wait((fam, 1))
        lax.fori_loop(7, 13, body, 0)

    transpose_ffn(lg, gt, g32, "g")
    transpose_ffn(lu, ut, u32s, "u")
    for kt in range(NM):
        t = jnp.concatenate([lg[pl.ds(13 * 128, 64), pl.ds(kt * 128, 128)],
                             lu[pl.ds(13 * 128, 64), pl.ds(kt * 128, 128)]], axis=0).T
        gt[13, kt] = pltpu.bitcast(t, u32)
        if kt < GV:
            g32[13, pl.ds(kt * 128, 128), :] = t.astype(f32)

    def e_body(ct, ctx):
        s = pl.multiple_of(ct * 128, 128)
        wait_dyn(("uv", 0), ct, lambda i: [(wuv_hbm.at[pl.ds(s, 128)], luv.at[pl.ds(s, 128)])])
        t = jnp.swapaxes(luv[pl.ds(s, 128)], 0, 1)
        s2 = pl.multiple_of(ct * 64, 64)
        for h in range(H):
            wuv[h, pl.ds(s2, 64), :] = pltpu.bitcast(t[h], u32)
        ctx = list(ctx)
        cc = cc_s[ct]
        for h in range(H):
            g, r = divmod(h, 8)
            out = _dot(cc[g * 8:(g + 1) * 8], pltpu.bitcast(wuv[h, pl.ds(s2, 64), :], bf16))
            ctx[g] = jnp.where(masks[r], ctx[g] + out, ctx[g])
        return tuple(ctx)

    ctx = lax.fori_loop(0, NC, e_body, (zero8,) * 4)
    for g in range(4):
        ctx_s[g] = ctx[g] * linv[g * 8:(g + 1) * 8]

    def f_body(g, acc):
        s = pl.multiple_of(g * 8, 8)
        wait_dyn(("o", 0), g, lambda i: [(wo_hbm.at[pl.ds(s, 8)], lo.at[pl.ds(s, 8)])])
        acc = list(acc)
        cg = ctx_s[g]
        for r in range(8):
            lhs = jnp.where(masks[r], cg, 0.0)
            for n in range(NM):
                t = lo[s + r, :, pl.ds(n * 128, 128)]
                wo2[s + r, n] = pltpu.bitcast(t, u32)
                acc[n] = acc[n] + _dot(lhs, t)
        for r in range(8):
            @pl.when(s + r < OV)
            def _():
                o32[jnp.minimum(s + r, OV - 1)] = lo[s + r].astype(f32)
        return tuple(acc)

    acc = lax.fori_loop(0, 4, f_body, (zero8,) * NM)
    x1 = [_rbf(x0[n] + _rbf(_rowsum(acc[n]))) for n in range(NM)]

    mean1, rstd1 = _stats(x1)
    ln1 = [(x - mean1) * rstd1 for x in x1]
    sig1 = _router(ln1, wr)
    lhs1 = [jnp.concatenate([x1[kt], ones8], axis=0) for kt in range(NM)]

    hh1 = []
    NE_ = DR0 // 128
    for ft in range(NF):
        og = ou = None
        for kt in range(NM):
            a = _dot(lhs1[kt], _tile(gt, ft, kt))
            og = a if og is None else og + a
            if ft < 13:
                b = _dot(lhs1[kt], _tile(ut, ft, kt))
                ou = b if ou is None else ou + b
        csg[ft] = og[8:16]
        g = rstd1 * (og[0:8] - mean1 * og[8:16])
        if ft < 13:
            csu[ft] = ou[8:16]
            u = rstd1 * (ou[0:8] - mean1 * ou[8:16])
        else:
            u = pltpu.roll(g, 64, 1)
        hh1.append(_silu(g) * u)
        if ft < NE_:
            hh_s[ft] = hh1[ft]

    NE = DR0 // 128

    def wd_tile(ft, n):
        return ld[pl.ds(ft * 128, min(128, F - ft * 128)), pl.ds(n * 128, 128)]

    def down2(ft, n, hh):
        return _dot(hh if ft < 13 else hh[:, :64], wd_tile(ft, n))

    def wd_f32(ft, s, n):
        if ft < NE or n in PRECONV:
            return d32[pl.ds(ft * 128 + s * 8, 8), pl.ds(n * 128, 128)]
        return wd_tile(ft, n).astype(f32)[s * 8:(s + 1) * 8]

    FPC = DRC // 128

    def h_body(i, y):
        s = pl.multiple_of(i * DRC, 128)
        wait_dyn(("d", 0), i, lambda _: [(wd_hbm.at[pl.ds(s, DRC)], ld.at[pl.ds(s, DRC)])])
        y = list(y)
        for j in range(FPC):
            ft = i * FPC + j
            sf = pl.multiple_of(s + j * 128, 128)
            hh = hh_s[ft]
            for n in range(NM):
                t = ld[pl.ds(sf, 128), pl.ds(n * 128, 128)]
                y[n] = y[n] + _dot(hh, t)
        for j in range(FPC):
            ft = i * FPC + j
            sf = pl.multiple_of(s + j * 128, 128)
            if DV:
                @pl.when(ft < DV)
                def _():
                    sd = pl.multiple_of(jnp.minimum(ft, DV - 1) * 128, 128)
                    d32[pl.ds(sd, 128), :] = ld[pl.ds(sf, 128), :].astype(f32)
        return tuple(y)

    y = list(lax.fori_loop(0, DR0 // DRC, h_body, (zero8,) * NM))

    x2 = [None] * NM
    racc = [None] * 4

    def h_late(n):
        for ft in range(NE, NF):
            y[n] = y[n] + down2(ft, n, hh1[ft])
        x2[n] = _rbf(x1[n] + _rbf(ln1[n] + _rbf(y[n] * sig1)))
        if n in PRECONV:
            for ft in range(NE, DV):
                d32[pl.ds(ft * 128, 128), pl.ds(n * 128, 128)] = wd_tile(ft, n).astype(f32)

    def a_pass(kt, heads=range(H)):
        for h in heads:
            g, r = divmod(h, 8)
            o = _dot(jnp.where(masks[r], x2[kt], 0.0), _tile(wq, h, pl.ds(kt * 64, 64)))
            racc[g] = o if racc[g] is None else racc[g] + o

    VK = list(range(AVT - AV, AVT))

    def a_mxu(kt, heads=range(H)):
        a_pass(kt, [h for h in heads if kt not in VK or h < A3M])

    wait(("dc", 0))
    h_late(0)
    h_late(1)
    a_mxu(0)
    a_mxu(1)
    wait(("dc", 1))
    h_late(2)
    h_late(3)
    a_mxu(2)
    av = {}
    if AV:
        xb2 = [_xb_gather(x2[kt]) for kt in VK]
        for h in range(A3M, H):
            a = None
            for s in range(16):
                for j in range(AV):
                    p = xb2[j][s] * q32[h, pl.ds(j * 128 + s * 8, 8), :]
                    a = p if a is None else a + p
            av[h] = _rowsum(a)
    wait(("dc", 2))
    h_late(4)
    a_mxu(3, range(0, 16))
    mean2, rstd2 = _stats(x2)
    raw = {}
    KL = DGROUPS[-1][-1]
    last = {}
    for h in range(BV):
        last[h] = _dot(x2[KL], _tile(wq, h, pl.ds(KL * 64, 64)))
    a_mxu(3, range(16, H))
    for h in range(BV, H):
        last[h] = _dot(x2[KL], _tile(wq, h, pl.ds(KL * 64, 64)))
    for h in range(H):
        raw[h] = racc[h // 8] + last[h]
        if h in av:
            raw[h] = raw[h] + av[h]
    qv = {}
    for i in range(0, BV, 3):
        hs = list(range(i, min(i + 3, BV)))
        xbs = []
        for h in hs:
            g, r = divmod(h, 8)
            qh = raw[h][r:r + 1] - mean2[0:1] * csq[g, pl.ds(r, 1), :]
            xbs.append(_xb(qh))
        accs = _vmac3([[None] * NC for _ in hs], xbs,
                      lambda j, s, ct: b32[hs[j], ct, pl.ds(s * 8, 8), :])
        for j, h in enumerate(hs):
            for ct in range(NC):
                qv[h, ct] = _rowsum(accs[j][ct]) * rstd2
    q = {}
    for g in range(BV // 8, 4):
        rawg = zero8
        for r in range(8):
            if g * 8 + r >= BV:
                rawg = jnp.where(masks[r], raw[g * 8 + r], rawg)
        q[g] = rstd2 * (rawg - mean2 * csq[g])
    qa = []
    for ct in range(NC):
        qg = [zero8] * 4
        for h in range(H):
            g, r = divmod(h, 8)
            o = qv[h, ct] if h < BV else _dot(q[g], _tile(wukt, h, ct))
            qg[g] = jnp.where(masks[r], o, qg[g])
        qa.append(jnp.concatenate(qg, axis=0))

    def scores(b):
        ss = []
        for j in range(KB):
            kt = b * KB + j
            sc = None
            for ct in range(NC):
                o = _dot(qa[ct], _tile(ckvt, kt, ct))
                sc = o if sc is None else sc + o
            ss.append(sc * SCALE)
        return ss

    def soft(ss, m, l):
        mb = ss[0]
        for j in range(1, KB):
            mb = jnp.maximum(mb, ss[j])
        mb = jnp.max(mb, axis=1, keepdims=True)
        m_new = mb if m is None else jnp.maximum(m, mb)
        ps = [jnp.exp(sj - m_new) for sj in ss]
        lb = ps[0]
        for j in range(1, KB):
            lb = lb + ps[j]
        if m is None:
            return ps, m_new, lb, None
        alpha = jnp.exp(m - m_new)
        return ps, m_new, l * alpha + lb, alpha

    def ctxc(b, ps, alpha, acc):
        if acc is not None:
            acc = [a * alpha for a in acc]
        else:
            acc = [None] * NC
        acc = list(acc)
        last = b == NB - 1
        seq = ([(j, ct) for ct in range(NC) for j in range(KB)] if last
               else [(j, ct) for j in range(KB) for ct in range(NC)])
        for j, ct in seq:
            kt = b * KB + j
            o = _dot(ps[j], _tile(lckv, ct, pl.ds(kt * 64, 64)))
            acc[ct] = o if acc[ct] is None else acc[ct] + o
        return acc

    s0 = scores(0)
    s1 = scores(1)
    p0, m, l, al0 = soft(s0, None, None)
    acc = ctxc(0, p0, None, None)
    s2 = scores(2)
    p1, m, l, al1 = soft(s1, m, l)
    acc = ctxc(1, p1, al1, acc)
    s3 = scores(3)
    p2, m, l, al2 = soft(s2, m, l)
    acc = ctxc(2, p2, al2, acc)
    p3, m, l, al3 = soft(s3, m, l)
    acc = ctxc(3, p3, al3, acc)
    linv = 1.0 / jnp.sum(l, axis=1, keepdims=True)

    accv = [[None] * NM for _ in range(3)]
    accm = [None] * NM

    def e_tiles(hs, cts, part):
        for ct in cts:
            for h in hs:
                g = h // 8
                o = _dot(acc[ct][g * 8:(g + 1) * 8], _tile(wuv, h, pl.ds(ct * 64, 64)))
                part[h] = o if h not in part else part[h] + o

    def head_ctx(h, part):
        g, r = divmod(h, 8)
        return part.pop(h)[r:r + 1] * linv[h:h + 1]

    def f_vpu(hs, part, accv):
        xbs = [_xb(head_ctx(h, part)) for h in hs]
        return _vmac3(accv, xbs, lambda j, s, n: o32[hs[j], pl.ds(s * 8, 8), pl.ds(n * 128, 128)])

    part = {}
    trip = [list(range(i, min(i + 3, OV))) for i in range(0, OV, 3)]
    e_tiles(trip[0], range(3), part)
    e_tiles(trip[1], range(3), part)
    e_tiles(trip[0], [3], part)
    accv = f_vpu(trip[0], part, accv)
    e_tiles(trip[1], [3], part)
    accv = f_vpu(trip[1], part, accv)
    for hs in trip[2:]:
        e_tiles(hs, range(NC), part)
        accv = f_vpu(hs, part, accv)
    lhs_m = {}
    for h in range(OV, H):
        e_tiles([h], range(NC), part)
        g, r = divmod(h, 8)
        lhs_m[h] = jnp.where(masks[r], part.pop(h) * linv[g * 8:(g + 1) * 8], 0.0)
    for n in range(NM):
        for h in range(OV, H):
            o = _dot(lhs_m[h], _tile(wo2, h, n))
            accm[n] = o if accm[n] is None else accm[n] + o
    x3 = [_rbf(x2[n] + _rbf(_rowsum(accm[n] + _fold3(accv, n)))) for n in range(NM)]
    mean3, rstd3 = _stats(x3)
    ln3 = [(x - mean3) * rstd3 for x in x3]
    sig3 = _router(ln3, wr)
    xb3 = []
    for kt in range(GV):
        xb3 += _xb_gather(x3[kt]) if GATH else _xb(x3[kt][0:1])
    hh = {}
    for ft in GORD:
        srcs = (("g", g32, gt), ("u", u32s, ut)) if ft < 13 else (("g", g32, gt),)
        val = {}
        for nm, ref, mref in srcs:
            av = None
            for s in range(16):
                for kt in range(GV):
                    p = xb3[kt * 16 + s] * ref[ft, pl.ds(kt * 128 + s * 8, 8), :]
                    av = p if av is None else av + p
            om = None
            for kt in range(GV, NM):
                a = _dot(x3[kt], _tile(mref, ft, kt))
                om = a if om is None else om + a
            cs_ = csg[ft] if nm == "g" else csu[ft]
            val[nm] = rstd3 * (om + _rowsum(av) - mean3 * cs_)
        u = val["u"] if ft < 13 else pltpu.roll(val["g"], 64, 1)
        hh[ft] = _silu(val["g"]) * u
    y = [None] * NM
    for ft in range(DV, NF):
        for n in range(NM):
            o = down2(ft, n, hh[ft])
            y[n] = o if y[n] is None else y[n] + o
    yv = [[None] * NM for _ in range(3)]
    for i in range(0, DV, 3):
        fs = list(range(i, min(i + 3, DV)))
        yv = _vmac3(yv, [_xb(hh[ft][0:1]) for ft in fs],
                    lambda j, s, n: wd_f32(fs[j], s, n))
    if DV:
        y = [y[n] + _rowsum(_fold3(yv, n)) for n in range(NM)]
    x4 = [x3[n] + _rbf(ln3[n] + _rbf(y[n] * sig3)) for n in range(NM)]
    out = jnp.concatenate([x[0:1, :] for x in x4], axis=1)
    o_ref[0] = out.astype(bf16)


@jax.jit
def pallas_interleave_layers__compressed_kv_cla__moe_arch_mod__decode_kernel(
    A_x: jax.Array,
    A_c_kv: jax.Array,
    A_w_q: jax.Array,
    A_w_uk: jax.Array,
    A_w_uv: jax.Array,
    A_w_o: jax.Array,
    B_x: jax.Array,
    B_w_r: jax.Array,
    B_w_gate: jax.Array,
    B_w_up: jax.Array,
    B_w_down: jax.Array,
):
    del B_x
    any_spec = pl.BlockSpec(memory_space=pl.ANY)
    V = pltpu.VMEM
    scratch = [
        V((1, 1, M), bf16),
        V((NM, 128), bf16),
        V((M, H, D), bf16),
        V((DC, H, D), bf16),
        V((DC, H, D), bf16),
        V((NC, SK // 2, 128), u32),
        V((H, D, M), bf16),
        V((F, M), bf16),
        V((F, M), bf16),
        V((F, M), bf16),
        V((H, M // 2, D), u32),
        V((H, NC, D // 2, 128), u32),
        V((H, DC // 2, D), u32),
        V((NK, NC, 64, 128), u32),
        V((NF, NM, 64, 128), u32),
        V((NF, NM, 64, 128), u32),
        V((NF, max(GV, 1) * 128, 128), f32),
        V((NF, max(GV, 1) * 128, 128), f32),
        V((max(DV, 1) * 128, M), f32),
        V((max(OV, 1), D, M), f32),
        V((max(BV, 1), NC, D, 128), f32),
        V((H, max(AV, 1) * 128, D), f32),
        V((H, NM, 64, 128), u32),
        V((4, 8, 128), f32),
        V((NF, 8, 128), f32),
        V((NF, 8, 128), f32),
        V((NC, H, 128), f32),
        V((NC, H, 128), f32),
        V((4, 8, 128), f32),
        V((NF, 8, 128), f32),
        V((NM, 8, 128), f32),
        pltpu.SemaphoreType.DMA((40,)),
    ]
    return pl.pallas_call(
        _kernel,
        out_shape=jax.ShapeDtypeStruct((1, 1, M), bf16),
        in_specs=[any_spec] * 10,
        out_specs=pl.BlockSpec(memory_space=pltpu.VMEM),
        scratch_shapes=scratch,
        compiler_params=pltpu.CompilerParams(
            vmem_limit_bytes=100 * 1024 * 1024,
            disable_semaphore_checks=True,
        ),
    )(A_x, A_c_kv, A_w_q, A_w_uk, A_w_uv, A_w_o, B_w_r.reshape(NM, 128),
      B_w_gate.T, B_w_up.T, B_w_down)
```

```python
import functools

import jax
import jax.numpy as jnp
from jax import lax
import jax.experimental.pallas as pl
import jax.experimental.pallas.tpu as pltpu

f32 = jnp.float32
bf16 = jnp.bfloat16
u32 = jnp.uint32
i32 = jnp.int32

M = 640
H = 32
D = 128
DC = 512
SK = 4096
F = 1728
NM = M // 128
NC = DC // 128
NK = SK // 128
NF = 14
EPS = 1e-5
SCALE = float(D) ** -0.5
KB = 8
NB = NK // KB
GV = 1
DV = 10
OV = 21
AV = 2
AVT = 4
A3M = 16
A2M = 24
GB = 2
GORD = list(range(10)) + [13, 10, 11, 12]
GATH = 1
PRECONV = (0,1,2,3)
DRC = 384
DR0 = 768
DGROUPS = ((0,1),(2,3),(4,))
G0 = 3
BV = 12


def _dot(a, b):
    return jnp.dot(a, b, preferred_element_type=f32)


def _rbf(x):
    return x.astype(bf16).astype(f32)


def _tile(ref, *idx):
    return pltpu.bitcast(ref[idx], bf16)


def _stats(xs):
    s = xs[0] + xs[1] + xs[2] + xs[3] + xs[4]
    mean = jnp.sum(s, axis=1, keepdims=True) * (1.0 / M)
    ds = [x - mean for x in xs]
    q = ds[0] * ds[0] + ds[1] * ds[1] + ds[2] * ds[2] + ds[3] * ds[3] + ds[4] * ds[4]
    var = jnp.sum(q, axis=1, keepdims=True) * (1.0 / M)
    rstd = 1.0 / jnp.sqrt(var + EPS)
    return mean, rstd


def _router(lns, wr):
    s = lns[0] * wr[0] + lns[1] * wr[1] + lns[2] * wr[2] + lns[3] * wr[3] + lns[4] * wr[4]
    r = jnp.sum(s, axis=1, keepdims=True)
    return jax.nn.sigmoid(r)


def _rowsum(x):
    return jnp.broadcast_to(jnp.sum(x, axis=0, keepdims=True), x.shape)


def _xb(row):
    t = jnp.broadcast_to(row, (128, 128)).T
    return [t[s * 8:(s + 1) * 8] for s in range(16)]


def _xb_gather(rows):
    sub = lax.broadcasted_iota(i32, (8, 128), 0)
    return [jnp.take_along_axis(rows, sub + 8 * s, axis=1, mode="promise_in_bounds")
            for s in range(16)]


def _vmac(acc, xb, load):
    for s, xs in enumerate(xb):
        p = xs * load(s)
        acc = p if acc is None else acc + p
    return acc


def _vmacs(accs, xb, load):
    accs = list(accs)
    for s, xs in enumerate(xb):
        for i in range(len(accs)):
            p = xs * load(s, i)
            accs[i] = p if accs[i] is None else accs[i] + p
    return accs


def _vmac3(accs, xbs, load):
    accs = [list(a) for a in accs]
    for s in range(16):
        for j, xb in enumerate(xbs):
            for i in range(len(accs[j])):
                p = xb[s] * load(j, s, i)
                accs[j][i] = p if accs[j][i] is None else accs[j][i] + p
    return accs


def _fold3(accs, i):
    t = [a[i] for a in accs if a[i] is not None]
    return functools.reduce(lambda a, b: a + b, t)


def _silu(g):
    return g * jax.nn.sigmoid(g)


def _kernel(x_hbm, ckv_hbm, wq_hbm, wuk_hbm, wuv_hbm, wo_hbm, wr_hbm, wg_hbm, wu_hbm, wd_hbm,
            o_ref,
            x_v, wr_v, lq, luk, luv, lckv, lo, lg, lu, ld,
            wq, wukt, wuv, ckvt, gt, ut, g32, u32s, d32, o32, b32, q32, wo2,
            csq, csg, csu, qa_s, cc_s, ctx_s, hh_s, x_s,
            sems):
    row8 = lax.broadcasted_iota(i32, (8, 128), 0)
    masks = [row8 == r for r in range(8)]

    copies = {}
    order = []

    def add(name, pairs):
        sem = sems.at[len(copies)]
        cs = [pltpu.make_async_copy(s, d, sem) for s, d in pairs]
        copies[name] = cs
        order.append(name)

    add("x", [(x_hbm, x_v)])
    add("wr", [(wr_hbm, wr_v)])
    for i in range(NM):
        add(("q", i), [(wq_hbm.at[pl.ds(i * 128, 128)], lq.at[pl.ds(i * 128, 128)])])
    for i in range(NC):
        add(("uk", i), [(wuk_hbm.at[pl.ds(i * 128, 128)], luk.at[pl.ds(i * 128, 128)])])
    ckv32 = ckv_hbm.at[0].bitcast(u32)
    for b in range(NB):
        add(("ckv", b), [(ckv32.at[pl.ds(b * 512, 512), pl.ds(ct * 128, 128)],
                          lckv.at[ct, pl.ds(b * 512, 512)]) for ct in range(NC)])
    FS = [(0, 896), (896, F - 896)]
    for i, (s, n) in enumerate(FS):
        add(("g", i), [(wg_hbm.at[pl.ds(s, n)], lg.at[pl.ds(s, n)])])
    for i, (s, n) in enumerate(FS):
        add(("u", i), [(wu_hbm.at[pl.ds(s, n)], lu.at[pl.ds(s, n)])])
    for i in range(NC):
        add(("uv", i), [(wuv_hbm.at[pl.ds(i * 128, 128)], luv.at[pl.ds(i * 128, 128)])])
    for g in range(4):
        add(("o", g), [(wo_hbm.at[pl.ds(g * 8, 8)], lo.at[pl.ds(g * 8, 8)])])
    for i in range(DR0 // DRC):
        add(("d", i), [(wd_hbm.at[pl.ds(i * DRC, DRC)], ld.at[pl.ds(i * DRC, DRC)])])
    for i, cols in enumerate(DGROUPS):
        c0, nc = cols[0] * 128, len(cols) * 128
        add(("dc", i), [(wd_hbm.at[pl.ds(DR0, F - DR0), pl.ds(c0, nc)],
                         ld.at[pl.ds(DR0, F - DR0), pl.ds(c0, nc)])])

    for name in order:
        for c in copies[name]:
            c.start()

    def wait(name):
        for c in copies[name]:
            c.wait()

    names = list(copies)

    def wait_dyn(first_name, i, pairs_fn):
        base = names.index(first_name)
        for s, d in pairs_fn(i):
            pltpu.make_async_copy(s, d, sems.at[base + i]).wait()

    wait("x")
    wait("wr")
    xr = x_v[0].astype(f32)
    x0 = [jnp.broadcast_to(xr[:, n * 128:(n + 1) * 128], (8, 128)) for n in range(NM)]
    wrf = wr_v[...].astype(f32)
    wr = [jnp.broadcast_to(wrf[n:n + 1, :], (8, 128)) for n in range(NM)]
    for n in range(NM):
        x_s[n] = x0[n]
    mean0, rstd0 = _stats(x0)
    ones8 = jnp.ones((8, 128), f32)
    zero8 = jnp.zeros((8, 128), f32)

    def a_body(kt, carry):
        raw, cs = carry
        s = pl.multiple_of(kt * 128, 128)
        wait_dyn(("q", 0), kt, lambda i: [(wq_hbm.at[pl.ds(s, 128)], lq.at[pl.ds(s, 128)])])
        t = jnp.swapaxes(lq[pl.ds(s, 128)], 0, 1)
        s2 = pl.multiple_of(kt * 64, 64)
        for h in range(H):
            wq[h, pl.ds(s2, 64), :] = pltpu.bitcast(t[h], u32)
        if AV:
            @pl.when((kt >= AVT - AV) & (kt < AVT))
            def _():
                sv = pl.multiple_of(jnp.clip(kt - (AVT - AV), 0, AV - 1) * 128, 128)
                for h in range(H):
                    w = wq[h, pl.ds(s2, 64), :]
                    q32[h, pl.ds(sv, 128), :] = pltpu.bitcast(w, bf16).astype(f32)
        lhs = jnp.concatenate([x_s[kt], ones8], axis=0)
        raw, cs = list(raw), list(cs)
        for h in range(H):
            g, r = divmod(h, 8)
            out = _dot(lhs, pltpu.bitcast(wq[h, pl.ds(s2, 64), :], bf16))
            raw[g] = jnp.where(masks[r], raw[g] + out[0:8], raw[g])
            cs[g] = jnp.where(masks[r], cs[g] + out[8:16], cs[g])
        return tuple(raw), tuple(cs)

    raw, cs = lax.fori_loop(0, NM, a_body, ((zero8,) * 4, (zero8,) * 4))
    for g in range(4):
        csq[g] = cs[g]
    q = [rstd0 * (raw[g] - mean0 * cs[g]) for g in range(4)]

    def b_body(ct, _):
        s = pl.multiple_of(ct * 128, 128)
        wait_dyn(("uk", 0), ct, lambda i: [(wuk_hbm.at[pl.ds(s, 128)], luk.at[pl.ds(s, 128)])])
        t = jnp.swapaxes(luk[pl.ds(s, 128)], 0, 1)
        for h in range(H):
            th = t[h].T
            wukt[h, ct] = pltpu.bitcast(th, u32)
            if h < BV:
                b32[h, ct] = th.astype(f32)
        qa = [zero8] * 4
        for h in range(H):
            g, r = divmod(h, 8)
            out = _dot(q[g], pltpu.bitcast(wukt[h, ct], bf16))
            qa[g] = jnp.where(masks[r], out, qa[g])
        qa_s[ct] = jnp.concatenate(qa, axis=0)
        return _

    lax.fori_loop(0, NC, b_body, 0)

    def cd_body(b, carry):
        m, l, acc = carry
        s = pl.multiple_of(b * 512, 512)
        wait_dyn(("ckv", 0), b, lambda i: [(ckv32.at[pl.ds(s, 512), pl.ds(ct * 128, 128)],
                                            lckv.at[ct, pl.ds(s, 512)]) for ct in range(NC)])
        ss = []
        for j in range(KB):
            kt = b * KB + j
            sk = pl.multiple_of(s + j * 64, 64)
            sc = None
            for ct in range(NC):
                t = pltpu.bitcast(lckv[ct, pl.ds(sk, 64), :], bf16).T
                ckvt[kt, ct] = pltpu.bitcast(t, u32)
                o = _dot(qa_s[ct], t)
                sc = o if sc is None else sc + o
            ss.append(sc * SCALE)
        mb = ss[0]
        for j in range(1, KB):
            mb = jnp.maximum(mb, ss[j])
        m_new = jnp.maximum(m, jnp.max(mb, axis=1, keepdims=True))
        alpha = jnp.exp(m - m_new)
        ps = [jnp.exp(sj - m_new) for sj in ss]
        lb = ps[0]
        for j in range(1, KB):
            lb = lb + ps[j]
        l = l * alpha + lb
        acc = [a * alpha for a in acc]
        for j in range(KB):
            sk = pl.multiple_of(s + j * 64, 64)
            for ct in range(NC):
                acc[ct] = acc[ct] + _dot(ps[j], pltpu.bitcast(lckv[ct, pl.ds(sk, 64), :], bf16))
        return m_new, l, acc

    m_init = jnp.full((H, 128), -jnp.inf, f32)
    _, l, acc = lax.fori_loop(0, NB, cd_body,
                              (m_init, jnp.zeros((H, 128), f32),
                               [jnp.zeros((H, 128), f32)] * NC))
    linv = 1.0 / jnp.sum(l, axis=1, keepdims=True)
    for ct in range(NC):
        cc_s[ct] = acc[ct]

    def transpose_ffn(land, dst, dst32, fam):
        def body(ft, _):
            s = pl.multiple_of(ft * 128, 128)
            for kt in range(NM):
                t = land[pl.ds(s, 128), pl.ds(kt * 128, 128)].T
                dst[ft, kt] = pltpu.bitcast(t, u32)
                if kt < GV:
                    dst32[ft, pl.ds(kt * 128, 128), :] = t.astype(f32)
            return _
        wait((fam, 0))
        lax.fori_loop(0, 7, body, 0)
        wait((fam, 1))
        lax.fori_loop(7, 13, body, 0)

    transpose_ffn(lg, gt, g32, "g")
    transpose_ffn(lu, ut, u32s, "u")
    for kt in range(NM):
        t = jnp.concatenate([lg[pl.ds(13 * 128, 64), pl.ds(kt * 128, 128)],
                             lu[pl.ds(13 * 128, 64), pl.ds(kt * 128, 128)]], axis=0).T
        gt[13, kt] = pltpu.bitcast(t, u32)
        if kt < GV:
            g32[13, pl.ds(kt * 128, 128), :] = t.astype(f32)

    def e_body(ct, ctx):
        s = pl.multiple_of(ct * 128, 128)
        wait_dyn(("uv", 0), ct, lambda i: [(wuv_hbm.at[pl.ds(s, 128)], luv.at[pl.ds(s, 128)])])
        t = jnp.swapaxes(luv[pl.ds(s, 128)], 0, 1)
        s2 = pl.multiple_of(ct * 64, 64)
        for h in range(H):
            wuv[h, pl.ds(s2, 64), :] = pltpu.bitcast(t[h], u32)
        ctx = list(ctx)
        cc = cc_s[ct]
        for h in range(H):
            g, r = divmod(h, 8)
            out = _dot(cc[g * 8:(g + 1) * 8], pltpu.bitcast(wuv[h, pl.ds(s2, 64), :], bf16))
            ctx[g] = jnp.where(masks[r], ctx[g] + out, ctx[g])
        return tuple(ctx)

    ctx = lax.fori_loop(0, NC, e_body, (zero8,) * 4)
    for g in range(4):
        ctx_s[g] = ctx[g] * linv[g * 8:(g + 1) * 8]

    def f_body(g, acc):
        s = pl.multiple_of(g * 8, 8)
        wait_dyn(("o", 0), g, lambda i: [(wo_hbm.at[pl.ds(s, 8)], lo.at[pl.ds(s, 8)])])
        acc = list(acc)
        cg = ctx_s[g]
        for r in range(8):
            lhs = jnp.where(masks[r], cg, 0.0)
            for n in range(NM):
                t = lo[s + r, :, pl.ds(n * 128, 128)]
                wo2[s + r, n] = pltpu.bitcast(t, u32)
                acc[n] = acc[n] + _dot(lhs, t)
        for r in range(8):
            @pl.when(s + r < OV)
            def _():
                o32[jnp.minimum(s + r, OV - 1)] = lo[s + r].astype(f32)
        return tuple(acc)

    acc = lax.fori_loop(0, 4, f_body, (zero8,) * NM)
    x1 = [_rbf(x0[n] + _rbf(_rowsum(acc[n]))) for n in range(NM)]

    mean1, rstd1 = _stats(x1)
    ln1 = [(x - mean1) * rstd1 for x in x1]
    sig1 = _router(ln1, wr)
    lhs1 = [jnp.concatenate([x1[kt], ones8], axis=0) for kt in range(NM)]

    hh1 = []
    NE_ = DR0 // 128
    for ft in range(NF):
        og = ou = None
        for kt in range(NM):
            a = _dot(lhs1[kt], _tile(gt, ft, kt))
            og = a if og is None else og + a
            if ft < 13:
                b = _dot(lhs1[kt], _tile(ut, ft, kt))
                ou = b if ou is None else ou + b
        csg[ft] = og[8:16]
        g = rstd1 * (og[0:8] - mean1 * og[8:16])
        if ft < 13:
            csu[ft] = ou[8:16]
            u = rstd1 * (ou[0:8] - mean1 * ou[8:16])
        else:
            u = pltpu.roll(g, 64, 1)
        hh1.append(_silu(g) * u)
        if ft < NE_:
            hh_s[ft] = hh1[ft]

    NE = DR0 // 128

    def wd_tile(ft, n):
        return ld[pl.ds(ft * 128, min(128, F - ft * 128)), pl.ds(n * 128, 128)]

    def down2(ft, n, hh):
        return _dot(hh if ft < 13 else hh[:, :64], wd_tile(ft, n))

    def wd_f32(ft, s, n):
        if ft < NE or n in PRECONV:
            return d32[pl.ds(ft * 128 + s * 8, 8), pl.ds(n * 128, 128)]
        return wd_tile(ft, n).astype(f32)[s * 8:(s + 1) * 8]

    FPC = DRC // 128

    def h_body(i, y):
        s = pl.multiple_of(i * DRC, 128)
        wait_dyn(("d", 0), i, lambda _: [(wd_hbm.at[pl.ds(s, DRC)], ld.at[pl.ds(s, DRC)])])
        y = list(y)
        for j in range(FPC):
            ft = i * FPC + j
            sf = pl.multiple_of(s + j * 128, 128)
            hh = hh_s[ft]
            for n in range(NM):
                t = ld[pl.ds(sf, 128), pl.ds(n * 128, 128)]
                y[n] = y[n] + _dot(hh, t)
        for j in range(FPC):
            ft = i * FPC + j
            sf = pl.multiple_of(s + j * 128, 128)
            if DV:
                @pl.when(ft < DV)
                def _():
                    sd = pl.multiple_of(jnp.minimum(ft, DV - 1) * 128, 128)
                    d32[pl.ds(sd, 128), :] = ld[pl.ds(sf, 128), :].astype(f32)
        return tuple(y)

    y = list(lax.fori_loop(0, DR0 // DRC, h_body, (zero8,) * NM))

    x2 = [None] * NM
    racc = [None] * 4

    def h_late(n):
        for ft in range(NE, NF):
            y[n] = y[n] + down2(ft, n, hh1[ft])
        x2[n] = _rbf(x1[n] + _rbf(ln1[n] + _rbf(y[n] * sig1)))
        if n in PRECONV:
            for ft in range(NE, DV):
                d32[pl.ds(ft * 128, 128), pl.ds(n * 128, 128)] = wd_tile(ft, n).astype(f32)

    def a_pass(kt, heads=range(H)):
        for h in heads:
            g, r = divmod(h, 8)
            o = _dot(jnp.where(masks[r], x2[kt], 0.0), _tile(wq, h, pl.ds(kt * 64, 64)))
            racc[g] = o if racc[g] is None else racc[g] + o

    VK = list(range(AVT - AV, AVT))

    def a_mxu(kt, heads=range(H)):
        a_pass(kt, [h for h in heads if kt not in VK or h < (A3M if kt == 3 else A2M)])

    wait(("dc", 0))
    h_late(0)
    h_late(1)
    a_mxu(0)
    a_mxu(1)
    wait(("dc", 1))
    h_late(2)
    h_late(3)
    a_mxu(2)
    wait(("dc", 2))
    av = {}
    for j, kt in enumerate(VK):
        hs = range(A3M if kt == 3 else A2M, H)
        if len(hs):
            xb = _xb_gather(x2[kt])
            for h in hs:
                a = None
                for s in range(16):
                    p = xb[s] * q32[h, pl.ds(j * 128 + s * 8, 8), :]
                    a = p if a is None else a + p
                av[h] = a if h not in av else av[h] + a
    h_late(4)
    a_mxu(3, range(0, 16))
    mean2, rstd2 = _stats(x2)
    raw = {}
    KL = DGROUPS[-1][-1]
    last = {}
    for h in range(BV):
        last[h] = _dot(x2[KL], _tile(wq, h, pl.ds(KL * 64, 64)))
    a_mxu(3, range(16, H))
    for h in range(BV, H):
        last[h] = _dot(x2[KL], _tile(wq, h, pl.ds(KL * 64, 64)))
    for h in range(H):
        raw[h] = racc[h // 8] + last[h]
        if h in av:
            raw[h] = raw[h] + _rowsum(av[h])
    qv = {}
    for i in range(0, BV, 3):
        hs = list(range(i, min(i + 3, BV)))
        xbs = []
        for h in hs:
            g, r = divmod(h, 8)
            qh = raw[h][r:r + 1] - mean2[0:1] * csq[g, pl.ds(r, 1), :]
            xbs.append(_xb(qh))
        accs = _vmac3([[None] * NC for _ in hs], xbs,
                      lambda j, s, ct: b32[hs[j], ct, pl.ds(s * 8, 8), :])
        for j, h in enumerate(hs):
            for ct in range(NC):
                qv[h, ct] = _rowsum(accs[j][ct]) * rstd2
    q = {}
    for g in range(BV // 8, 4):
        rawg = zero8
        for r in range(8):
            if g * 8 + r >= BV:
                rawg = jnp.where(masks[r], raw[g * 8 + r], rawg)
        q[g] = rstd2 * (rawg - mean2 * csq[g])
    qa = []
    for ct in range(NC):
        qg = [zero8] * 4
        for h in range(H):
            g, r = divmod(h, 8)
            o = qv[h, ct] if h < BV else _dot(q[g], _tile(wukt, h, ct))
            qg[g] = jnp.where(masks[r], o, qg[g])
        qa.append(jnp.concatenate(qg, axis=0))

    def scores(b):
        ss = []
        for j in range(KB):
            kt = b * KB + j
            sc = None
            for ct in range(NC):
                o = _dot(qa[ct], _tile(ckvt, kt, ct))
                sc = o if sc is None else sc + o
            ss.append(sc * SCALE)
        return ss

    def soft(ss, m, l):
        mb = ss[0]
        for j in range(1, KB):
            mb = jnp.maximum(mb, ss[j])
        mb = jnp.max(mb, axis=1, keepdims=True)
        m_new = mb if m is None else jnp.maximum(m, mb)
        ps = [jnp.exp(sj - m_new) for sj in ss]
        lb = ps[0]
        for j in range(1, KB):
            lb = lb + ps[j]
        if m is None:
            return ps, m_new, lb, None
        alpha = jnp.exp(m - m_new)
        return ps, m_new, l * alpha + lb, alpha

    def ctxc(b, ps, alpha, acc):
        if acc is not None:
            acc = [a * alpha for a in acc]
        else:
            acc = [None] * NC
        acc = list(acc)
        last = b == NB - 1
        seq = ([(j, ct) for ct in range(NC) for j in range(KB)] if last
               else [(j, ct) for j in range(KB) for ct in range(NC)])
        for j, ct in seq:
            kt = b * KB + j
            o = _dot(ps[j], _tile(lckv, ct, pl.ds(kt * 64, 64)))
            acc[ct] = o if acc[ct] is None else acc[ct] + o
        return acc

    s0 = scores(0)
    s1 = scores(1)
    p0, m, l, al0 = soft(s0, None, None)
    acc = ctxc(0, p0, None, None)
    s2 = scores(2)
    p1, m, l, al1 = soft(s1, m, l)
    acc = ctxc(1, p1, al1, acc)
    s3 = scores(3)
    p2, m, l, al2 = soft(s2, m, l)
    acc = ctxc(2, p2, al2, acc)
    p3, m, l, al3 = soft(s3, m, l)
    acc = ctxc(3, p3, al3, acc)
    linv = 1.0 / jnp.sum(l, axis=1, keepdims=True)

    accv = [[None] * NM for _ in range(3)]
    accm = [None] * NM

    def e_tiles(hs, cts, part):
        for ct in cts:
            for h in hs:
                g = h // 8
                o = _dot(acc[ct][g * 8:(g + 1) * 8], _tile(wuv, h, pl.ds(ct * 64, 64)))
                part[h] = o if h not in part else part[h] + o

    def head_ctx(h, part):
        g, r = divmod(h, 8)
        return part.pop(h)[r:r + 1] * linv[h:h + 1]

    def f_vpu(hs, part, accv):
        xbs = [_xb(head_ctx(h, part)) for h in hs]
        return _vmac3(accv, xbs, lambda j, s, n: o32[hs[j], pl.ds(s * 8, 8), pl.ds(n * 128, 128)])

    part = {}
    trip = [list(range(i, min(i + 3, OV))) for i in range(0, OV, 3)]
    e_tiles(trip[0], range(3), part)
    e_tiles(trip[1], range(3), part)
    e_tiles(trip[0], [3], part)
    accv = f_vpu(trip[0], part, accv)
    e_tiles(trip[1], [3], part)
    accv = f_vpu(trip[1], part, accv)
    for hs in trip[2:]:
        e_tiles(hs, range(NC), part)
        accv = f_vpu(hs, part, accv)
    lhs_m = {}
    for h in range(OV, H):
        e_tiles([h], range(NC), part)
        g, r = divmod(h, 8)
        lhs_m[h] = jnp.where(masks[r], part.pop(h) * linv[g * 8:(g + 1) * 8], 0.0)
    for n in range(NM):
        for h in range(OV, H):
            o = _dot(lhs_m[h], _tile(wo2, h, n))
            accm[n] = o if accm[n] is None else accm[n] + o
    x3 = [_rbf(x2[n] + _rbf(_rowsum(accm[n] + _fold3(accv, n)))) for n in range(NM)]
    mean3, rstd3 = _stats(x3)
    ln3 = [(x - mean3) * rstd3 for x in x3]
    sig3 = _router(ln3, wr)
    xb3 = []
    for kt in range(GV):
        xb3 += _xb_gather(x3[kt]) if GATH else _xb(x3[kt][0:1])
    hh = {}
    for ft in GORD:
        srcs = (("g", g32, gt), ("u", u32s, ut)) if ft < 13 else (("g", g32, gt),)
        val = {}
        for nm, ref, mref in srcs:
            av = None
            for s in range(16):
                for kt in range(GV):
                    p = xb3[kt * 16 + s] * ref[ft, pl.ds(kt * 128 + s * 8, 8), :]
                    av = p if av is None else av + p
            om = None
            for kt in range(GV, NM):
                a = _dot(x3[kt], _tile(mref, ft, kt))
                om = a if om is None else om + a
            cs_ = csg[ft] if nm == "g" else csu[ft]
            val[nm] = rstd3 * (om + _rowsum(av) - mean3 * cs_)
        u = val["u"] if ft < 13 else pltpu.roll(val["g"], 64, 1)
        hh[ft] = _silu(val["g"]) * u
    y = [None] * NM
    for ft in range(DV, NF):
        for n in range(NM):
            o = down2(ft, n, hh[ft])
            y[n] = o if y[n] is None else y[n] + o
    yv = [[None] * NM for _ in range(3)]
    for i in range(0, DV, 3):
        fs = list(range(i, min(i + 3, DV)))
        yv = _vmac3(yv, [_xb(hh[ft][0:1]) for ft in fs],
                    lambda j, s, n: wd_f32(fs[j], s, n))
    if DV:
        y = [y[n] + _rowsum(_fold3(yv, n)) for n in range(NM)]
    x4 = [x3[n] + _rbf(ln3[n] + _rbf(y[n] * sig3)) for n in range(NM)]
    out = jnp.concatenate([x[0:1, :] for x in x4], axis=1)
    o_ref[0] = out.astype(bf16)


@jax.jit
def pallas_interleave_layers__compressed_kv_cla__moe_arch_mod__decode_kernel(
    A_x: jax.Array,
    A_c_kv: jax.Array,
    A_w_q: jax.Array,
    A_w_uk: jax.Array,
    A_w_uv: jax.Array,
    A_w_o: jax.Array,
    B_x: jax.Array,
    B_w_r: jax.Array,
    B_w_gate: jax.Array,
    B_w_up: jax.Array,
    B_w_down: jax.Array,
):
    del B_x
    any_spec = pl.BlockSpec(memory_space=pl.ANY)
    V = pltpu.VMEM
    scratch = [
        V((1, 1, M), bf16),
        V((NM, 128), bf16),
        V((M, H, D), bf16),
        V((DC, H, D), bf16),
        V((DC, H, D), bf16),
        V((NC, SK // 2, 128), u32),
        V((H, D, M), bf16),
        V((F, M), bf16),
        V((F, M), bf16),
        V((F, M), bf16),
        V((H, M // 2, D), u32),
        V((H, NC, D // 2, 128), u32),
        V((H, DC // 2, D), u32),
        V((NK, NC, 64, 128), u32),
        V((NF, NM, 64, 128), u32),
        V((NF, NM, 64, 128), u32),
        V((NF, max(GV, 1) * 128, 128), f32),
        V((NF, max(GV, 1) * 128, 128), f32),
        V((max(DV, 1) * 128, M), f32),
        V((max(OV, 1), D, M), f32),
        V((max(BV, 1), NC, D, 128), f32),
        V((H, max(AV, 1) * 128, D), f32),
        V((H, NM, 64, 128), u32),
        V((4, 8, 128), f32),
        V((NF, 8, 128), f32),
        V((NF, 8, 128), f32),
        V((NC, H, 128), f32),
        V((NC, H, 128), f32),
        V((4, 8, 128), f32),
        V((NF, 8, 128), f32),
        V((NM, 8, 128), f32),
        pltpu.SemaphoreType.DMA((40,)),
    ]
    return pl.pallas_call(
        _kernel,
        out_shape=jax.ShapeDtypeStruct((1, 1, M), bf16),
        in_specs=[any_spec] * 10,
        out_specs=pl.BlockSpec(memory_space=pltpu.VMEM),
        scratch_shapes=scratch,
        compiler_params=pltpu.CompilerParams(
            vmem_limit_bytes=100 * 1024 * 1024,
            disable_semaphore_checks=True,
        ),
    )(A_x, A_c_kv, A_w_q, A_w_uk, A_w_uv, A_w_o, B_w_r.reshape(NM, 128),
      B_w_gate.T, B_w_up.T, B_w_down)
```

```python
import functools

import jax
import jax.numpy as jnp
from jax import lax
import jax.experimental.pallas as pl
import jax.experimental.pallas.tpu as pltpu

f32 = jnp.float32
bf16 = jnp.bfloat16
u32 = jnp.uint32
i32 = jnp.int32

M = 640
H = 32
D = 128
DC = 512
SK = 4096
F = 1728
NM = M // 128
NC = DC // 128
NK = SK // 128
NF = 14
EPS = 1e-5
SCALE = float(D) ** -0.5
KB = 8
NB = NK // KB

QV = {2: 24, 3: 16}
BV = 12
OV = 21
DV = 10
DRC = 384
DR0 = 768
DGROUPS = ((0, 1), (2, 3), (4,))
NE = DR0 // 128
GORD = list(range(10)) + [13, 10, 11, 12]


def _dot(a, b):
    return jnp.dot(a, b, preferred_element_type=f32)


def _rbf(x):
    return x.astype(bf16).astype(f32)


def _tile(ref, *idx):
    return pltpu.bitcast(ref[idx], bf16)


def _stats(xs):
    s = xs[0] + xs[1] + xs[2] + xs[3] + xs[4]
    mean = jnp.sum(s, axis=1, keepdims=True) * (1.0 / M)
    ds = [x - mean for x in xs]
    q = ds[0] * ds[0] + ds[1] * ds[1] + ds[2] * ds[2] + ds[3] * ds[3] + ds[4] * ds[4]
    var = jnp.sum(q, axis=1, keepdims=True) * (1.0 / M)
    rstd = 1.0 / jnp.sqrt(var + EPS)
    return mean, rstd


def _router(lns, wr):
    s = lns[0] * wr[0] + lns[1] * wr[1] + lns[2] * wr[2] + lns[3] * wr[3] + lns[4] * wr[4]
    r = jnp.sum(s, axis=1, keepdims=True)
    return jax.nn.sigmoid(r)


def _rowsum(x):
    return jnp.broadcast_to(jnp.sum(x, axis=0, keepdims=True), x.shape)


def _xb(row):
    t = jnp.broadcast_to(row, (128, 128)).T
    return [t[s * 8:(s + 1) * 8] for s in range(16)]


def _xb_gather(rows):
    sub = lax.broadcasted_iota(i32, (8, 128), 0)
    return [jnp.take_along_axis(rows, sub + 8 * s, axis=1, mode="promise_in_bounds")
            for s in range(16)]


def _vmac3(accs, xbs, load):
    accs = [list(a) for a in accs]
    for s in range(16):
        for j, xb in enumerate(xbs):
            for i in range(len(accs[j])):
                p = xb[s] * load(j, s, i)
                accs[j][i] = p if accs[j][i] is None else accs[j][i] + p
    return accs


def _fold3(accs, i):
    t = [a[i] for a in accs if a[i] is not None]
    return functools.reduce(lambda a, b: a + b, t)


def _silu(g):
    return g * jax.nn.sigmoid(g)


def _kernel(x_hbm, ckv_hbm, wq_hbm, wuk_hbm, wuv_hbm, wo_hbm, wr_hbm, wg_hbm, wu_hbm, wd_hbm,
            o_ref,
            x_v, wr_v, lq, luk, luv, lckv, lo, lg, lu, ld,
            wq, wukt, wuv, ckvt, gt, ut, g32, u32s, d32, o32, b32, q32, wo2,
            csq, csg, csu, qa_s, cc_s, ctx_s, hh_s, x_s,
            sems):
    row8 = lax.broadcasted_iota(i32, (8, 128), 0)
    masks = [row8 == r for r in range(8)]

    copies = {}
    order = []

    def add(name, pairs):
        sem = sems.at[len(copies)]
        cs = [pltpu.make_async_copy(s, d, sem) for s, d in pairs]
        copies[name] = cs
        order.append(name)

    add("x", [(x_hbm, x_v)])
    add("wr", [(wr_hbm, wr_v)])
    for i in range(NM):
        add(("q", i), [(wq_hbm.at[pl.ds(i * 128, 128)], lq.at[pl.ds(i * 128, 128)])])
    for i in range(NC):
        add(("uk", i), [(wuk_hbm.at[pl.ds(i * 128, 128)], luk.at[pl.ds(i * 128, 128)])])
    ckv32 = ckv_hbm.at[0].bitcast(u32)
    for b in range(NB):
        add(("ckv", b), [(ckv32.at[pl.ds(b * 512, 512), pl.ds(ct * 128, 128)],
                          lckv.at[ct, pl.ds(b * 512, 512)]) for ct in range(NC)])
    FS = [(0, 896), (896, F - 896)]
    for i, (s, n) in enumerate(FS):
        add(("g", i), [(wg_hbm.at[pl.ds(s, n)], lg.at[pl.ds(s, n)])])
    for i, (s, n) in enumerate(FS):
        add(("u", i), [(wu_hbm.at[pl.ds(s, n)], lu.at[pl.ds(s, n)])])
    for i in range(NC):
        add(("uv", i), [(wuv_hbm.at[pl.ds(i * 128, 128)], luv.at[pl.ds(i * 128, 128)])])
    for g in range(4):
        add(("o", g), [(wo_hbm.at[pl.ds(g * 8, 8)], lo.at[pl.ds(g * 8, 8)])])
    for i in range(DR0 // DRC):
        add(("d", i), [(wd_hbm.at[pl.ds(i * DRC, DRC)], ld.at[pl.ds(i * DRC, DRC)])])
    for i, cols in enumerate(DGROUPS):
        c0, nc = cols[0] * 128, len(cols) * 128
        add(("dc", i), [(wd_hbm.at[pl.ds(DR0, F - DR0), pl.ds(c0, nc)],
                         ld.at[pl.ds(DR0, F - DR0), pl.ds(c0, nc)])])

    for name in order:
        for c in copies[name]:
            c.start()

    def wait(name):
        for c in copies[name]:
            c.wait()

    names = list(copies)

    def wait_dyn(first_name, i, pairs_fn):
        base = names.index(first_name)
        for s, d in pairs_fn(i):
            pltpu.make_async_copy(s, d, sems.at[base + i]).wait()

    wait("x")
    wait("wr")
    xr = x_v[0].astype(f32)
    x0 = [jnp.broadcast_to(xr[:, n * 128:(n + 1) * 128], (8, 128)) for n in range(NM)]
    wrf = wr_v[...].astype(f32)
    wr = [jnp.broadcast_to(wrf[n:n + 1, :], (8, 128)) for n in range(NM)]
    for n in range(NM):
        x_s[n] = x0[n]
    mean0, rstd0 = _stats(x0)
    ones8 = jnp.ones((8, 128), f32)
    zero8 = jnp.zeros((8, 128), f32)

    def a_body(kt, carry):
        raw, cs = carry
        s = pl.multiple_of(kt * 128, 128)
        wait_dyn(("q", 0), kt, lambda i: [(wq_hbm.at[pl.ds(s, 128)], lq.at[pl.ds(s, 128)])])
        t = jnp.swapaxes(lq[pl.ds(s, 128)], 0, 1)
        s2 = pl.multiple_of(kt * 64, 64)
        for h in range(H):
            wq[h, pl.ds(s2, 64), :] = pltpu.bitcast(t[h], u32)
        for j, (ktv, h0) in enumerate(sorted(QV.items())):
            @pl.when(kt == ktv)
            def _():
                for h in range(h0, H):
                    w = wq[h, pl.ds(s2, 64), :]
                    q32[h, pl.ds(j * 128, 128), :] = pltpu.bitcast(w, bf16).astype(f32)
        lhs = jnp.concatenate([x_s[kt], ones8], axis=0)
        raw, cs = list(raw), list(cs)
        for h in range(H):
            g, r = divmod(h, 8)
            out = _dot(lhs, pltpu.bitcast(wq[h, pl.ds(s2, 64), :], bf16))
            raw[g] = jnp.where(masks[r], raw[g] + out[0:8], raw[g])
            cs[g] = jnp.where(masks[r], cs[g] + out[8:16], cs[g])
        return tuple(raw), tuple(cs)

    raw, cs = lax.fori_loop(0, NM, a_body, ((zero8,) * 4, (zero8,) * 4))
    for g in range(4):
        csq[g] = cs[g]
    q = [rstd0 * (raw[g] - mean0 * cs[g]) for g in range(4)]

    def b_body(ct, _):
        s = pl.multiple_of(ct * 128, 128)
        wait_dyn(("uk", 0), ct, lambda i: [(wuk_hbm.at[pl.ds(s, 128)], luk.at[pl.ds(s, 128)])])
        t = jnp.swapaxes(luk[pl.ds(s, 128)], 0, 1)
        for h in range(H):
            th = t[h].T
            wukt[h, ct] = pltpu.bitcast(th, u32)
            if h < BV:
                b32[h, ct] = th.astype(f32)
        qa = [zero8] * 4
        for h in range(H):
            g, r = divmod(h, 8)
            out = _dot(q[g], pltpu.bitcast(wukt[h, ct], bf16))
            qa[g] = jnp.where(masks[r], out, qa[g])
        qa_s[ct] = jnp.concatenate(qa, axis=0)
        return _

    lax.fori_loop(0, NC, b_body, 0)

    def cd_body(b, carry):
        m, l, acc = carry
        s = pl.multiple_of(b * 512, 512)
        wait_dyn(("ckv", 0), b, lambda i: [(ckv32.at[pl.ds(s, 512), pl.ds(ct * 128, 128)],
                                            lckv.at[ct, pl.ds(s, 512)]) for ct in range(NC)])
        ss = []
        for j in range(KB):
            kt = b * KB + j
            sk = pl.multiple_of(s + j * 64, 64)
            sc = None
            for ct in range(NC):
                t = pltpu.bitcast(lckv[ct, pl.ds(sk, 64), :], bf16).T
                ckvt[kt, ct] = pltpu.bitcast(t, u32)
                o = _dot(qa_s[ct], t)
                sc = o if sc is None else sc + o
            ss.append(sc * SCALE)
        mb = ss[0]
        for j in range(1, KB):
            mb = jnp.maximum(mb, ss[j])
        m_new = jnp.maximum(m, jnp.max(mb, axis=1, keepdims=True))
        alpha = jnp.exp(m - m_new)
        ps = [jnp.exp(sj - m_new) for sj in ss]
        lb = ps[0]
        for j in range(1, KB):
            lb = lb + ps[j]
        l = l * alpha + lb
        acc = [a * alpha for a in acc]
        for j in range(KB):
            sk = pl.multiple_of(s + j * 64, 64)
            for ct in range(NC):
                acc[ct] = acc[ct] + _dot(ps[j], pltpu.bitcast(lckv[ct, pl.ds(sk, 64), :], bf16))
        return m_new, l, acc

    m_init = jnp.full((H, 128), -jnp.inf, f32)
    _, l, acc = lax.fori_loop(0, NB, cd_body,
                              (m_init, jnp.zeros((H, 128), f32),
                               [jnp.zeros((H, 128), f32)] * NC))
    linv = 1.0 / jnp.sum(l, axis=1, keepdims=True)
    for ct in range(NC):
        cc_s[ct] = acc[ct]

    def transpose_ffn(land, dst, dst32, fam):
        def body(ft, _):
            s = pl.multiple_of(ft * 128, 128)
            for kt in range(NM):
                t = land[pl.ds(s, 128), pl.ds(kt * 128, 128)].T
                dst[ft, kt] = pltpu.bitcast(t, u32)
                if kt == 0:
                    dst32[ft] = t.astype(f32)
            return _
        wait((fam, 0))
        lax.fori_loop(0, 7, body, 0)
        wait((fam, 1))
        lax.fori_loop(7, 13, body, 0)

    transpose_ffn(lg, gt, g32, "g")
    transpose_ffn(lu, ut, u32s, "u")
    for kt in range(NM):
        t = jnp.concatenate([lg[pl.ds(13 * 128, 64), pl.ds(kt * 128, 128)],
                             lu[pl.ds(13 * 128, 64), pl.ds(kt * 128, 128)]], axis=0).T
        gt[13, kt] = pltpu.bitcast(t, u32)
        if kt == 0:
            g32[13] = t.astype(f32)

    def e_body(ct, ctx):
        s = pl.multiple_of(ct * 128, 128)
        wait_dyn(("uv", 0), ct, lambda i: [(wuv_hbm.at[pl.ds(s, 128)], luv.at[pl.ds(s, 128)])])
        t = jnp.swapaxes(luv[pl.ds(s, 128)], 0, 1)
        s2 = pl.multiple_of(ct * 64, 64)
        for h in range(H):
            wuv[h, pl.ds(s2, 64), :] = pltpu.bitcast(t[h], u32)
        ctx = list(ctx)
        cc = cc_s[ct]
        for h in range(H):
            g, r = divmod(h, 8)
            out = _dot(cc[g * 8:(g + 1) * 8], pltpu.bitcast(wuv[h, pl.ds(s2, 64), :], bf16))
            ctx[g] = jnp.where(masks[r], ctx[g] + out, ctx[g])
        return tuple(ctx)

    ctx = lax.fori_loop(0, NC, e_body, (zero8,) * 4)
    for g in range(4):
        ctx_s[g] = ctx[g] * linv[g * 8:(g + 1) * 8]

    def f_body(g, acc):
        s = pl.multiple_of(g * 8, 8)
        wait_dyn(("o", 0), g, lambda i: [(wo_hbm.at[pl.ds(s, 8)], lo.at[pl.ds(s, 8)])])
        acc = list(acc)
        cg = ctx_s[g]
        for r in range(8):
            lhs = jnp.where(masks[r], cg, 0.0)
            for n in range(NM):
                t = lo[s + r, :, pl.ds(n * 128, 128)]
                wo2[s + r, n] = pltpu.bitcast(t, u32)
                acc[n] = acc[n] + _dot(lhs, t)
        for r in range(8):
            @pl.when(s + r < OV)
            def _():
                o32[jnp.minimum(s + r, OV - 1)] = lo[s + r].astype(f32)
        return tuple(acc)

    acc = lax.fori_loop(0, 4, f_body, (zero8,) * NM)
    x1 = [_rbf(x0[n] + _rbf(_rowsum(acc[n]))) for n in range(NM)]

    mean1, rstd1 = _stats(x1)
    ln1 = [(x - mean1) * rstd1 for x in x1]
    sig1 = _router(ln1, wr)
    lhs1 = [jnp.concatenate([x1[kt], ones8], axis=0) for kt in range(NM)]

    hh1 = []
    for ft in range(NF):
        og = ou = None
        for kt in range(NM):
            a = _dot(lhs1[kt], _tile(gt, ft, kt))
            og = a if og is None else og + a
            if ft < 13:
                b = _dot(lhs1[kt], _tile(ut, ft, kt))
                ou = b if ou is None else ou + b
        csg[ft] = og[8:16]
        g = rstd1 * (og[0:8] - mean1 * og[8:16])
        if ft < 13:
            csu[ft] = ou[8:16]
            u = rstd1 * (ou[0:8] - mean1 * ou[8:16])
        else:
            u = pltpu.roll(g, 64, 1)
        hh1.append(_silu(g) * u)
        if ft < NE:
            hh_s[ft] = hh1[ft]


    def wd_tile(ft, n):
        return ld[pl.ds(ft * 128, min(128, F - ft * 128)), pl.ds(n * 128, 128)]

    def down2(ft, n, hh):
        return _dot(hh if ft < 13 else hh[:, :64], wd_tile(ft, n))

    def wd_f32(ft, s, n):
        if ft < NE or n < 4:
            return d32[pl.ds(ft * 128 + s * 8, 8), pl.ds(n * 128, 128)]
        return wd_tile(ft, n).astype(f32)[s * 8:(s + 1) * 8]

    FPC = DRC // 128

    def h_body(i, y):
        s = pl.multiple_of(i * DRC, 128)
        wait_dyn(("d", 0), i, lambda _: [(wd_hbm.at[pl.ds(s, DRC)], ld.at[pl.ds(s, DRC)])])
        y = list(y)
        for j in range(FPC):
            ft = i * FPC + j
            sf = pl.multiple_of(s + j * 128, 128)
            hh = hh_s[ft]
            for n in range(NM):
                t = ld[pl.ds(sf, 128), pl.ds(n * 128, 128)]
                y[n] = y[n] + _dot(hh, t)
        for j in range(FPC):
            ft = i * FPC + j
            sf = pl.multiple_of(s + j * 128, 128)
            sd = pl.multiple_of(ft * 128, 128)
            d32[pl.ds(sd, 128), :] = ld[pl.ds(sf, 128), :].astype(f32)
        return tuple(y)

    y = list(lax.fori_loop(0, DR0 // DRC, h_body, (zero8,) * NM))

    x2 = [None] * NM
    racc = [None] * 4

    def h_late(n):
        for ft in range(NE, NF):
            y[n] = y[n] + down2(ft, n, hh1[ft])
        x2[n] = _rbf(x1[n] + _rbf(ln1[n] + _rbf(y[n] * sig1)))
        if n < 4:
            for ft in range(NE, DV):
                d32[pl.ds(ft * 128, 128), pl.ds(n * 128, 128)] = wd_tile(ft, n).astype(f32)

    def a_pass(kt, heads=range(H)):
        for h in heads:
            g, r = divmod(h, 8)
            o = _dot(jnp.where(masks[r], x2[kt], 0.0), _tile(wq, h, pl.ds(kt * 64, 64)))
            racc[g] = o if racc[g] is None else racc[g] + o

    def a_mxu(kt, heads=range(H)):
        a_pass(kt, [h for h in heads if h < QV.get(kt, H)])

    wait(("dc", 0))
    h_late(0)
    h_late(1)
    a_mxu(0)
    a_mxu(1)
    wait(("dc", 1))
    h_late(2)
    h_late(3)
    a_mxu(2)
    wait(("dc", 2))
    av = {}
    for j, (kt, h0) in enumerate(sorted(QV.items())):
        xb = _xb_gather(x2[kt])
        for h in range(h0, H):
            a = None
            for s in range(16):
                p = xb[s] * q32[h, pl.ds(j * 128 + s * 8, 8), :]
                a = p if a is None else a + p
            av[h] = a if h not in av else av[h] + a
    h_late(4)
    a_mxu(3, range(0, 16))
    mean2, rstd2 = _stats(x2)
    raw = {}
    KL = DGROUPS[-1][-1]
    last = {}
    for h in range(BV):
        last[h] = _dot(x2[KL], _tile(wq, h, pl.ds(KL * 64, 64)))
    a_mxu(3, range(16, H))
    for h in range(BV, H):
        last[h] = _dot(x2[KL], _tile(wq, h, pl.ds(KL * 64, 64)))
    for h in range(H):
        raw[h] = racc[h // 8] + last[h]
        if h in av:
            raw[h] = raw[h] + _rowsum(av[h])
    qv = {}
    for i in range(0, BV, 3):
        hs = list(range(i, min(i + 3, BV)))
        xbs = []
        for h in hs:
            g, r = divmod(h, 8)
            qh = raw[h][r:r + 1] - mean2[0:1] * csq[g, pl.ds(r, 1), :]
            xbs.append(_xb(qh))
        accs = _vmac3([[None] * NC for _ in hs], xbs,
                      lambda j, s, ct: b32[hs[j], ct, pl.ds(s * 8, 8), :])
        for j, h in enumerate(hs):
            for ct in range(NC):
                qv[h, ct] = _rowsum(accs[j][ct]) * rstd2
    q = {}
    for g in range(BV // 8, 4):
        rawg = zero8
        for r in range(8):
            if g * 8 + r >= BV:
                rawg = jnp.where(masks[r], raw[g * 8 + r], rawg)
        q[g] = rstd2 * (rawg - mean2 * csq[g])
    qa = []
    for ct in range(NC):
        qg = [zero8] * 4
        for h in range(H):
            g, r = divmod(h, 8)
            o = qv[h, ct] if h < BV else _dot(q[g], _tile(wukt, h, ct))
            qg[g] = jnp.where(masks[r], o, qg[g])
        qa.append(jnp.concatenate(qg, axis=0))

    def scores(b):
        ss = []
        for j in range(KB):
            kt = b * KB + j
            sc = None
            for ct in range(NC):
                o = _dot(qa[ct], _tile(ckvt, kt, ct))
                sc = o if sc is None else sc + o
            ss.append(sc * SCALE)
        return ss

    def soft(ss, m, l):
        mb = ss[0]
        for j in range(1, KB):
            mb = jnp.maximum(mb, ss[j])
        mb = jnp.max(mb, axis=1, keepdims=True)
        m_new = mb if m is None else jnp.maximum(m, mb)
        ps = [jnp.exp(sj - m_new) for sj in ss]
        lb = ps[0]
        for j in range(1, KB):
            lb = lb + ps[j]
        if m is None:
            return ps, m_new, lb, None
        alpha = jnp.exp(m - m_new)
        return ps, m_new, l * alpha + lb, alpha

    def ctxc(b, ps, alpha, acc):
        if acc is not None:
            acc = [a * alpha for a in acc]
        else:
            acc = [None] * NC
        acc = list(acc)
        last = b == NB - 1
        seq = ([(j, ct) for ct in range(NC) for j in range(KB)] if last
               else [(j, ct) for j in range(KB) for ct in range(NC)])
        for j, ct in seq:
            kt = b * KB + j
            o = _dot(ps[j], _tile(lckv, ct, pl.ds(kt * 64, 64)))
            acc[ct] = o if acc[ct] is None else acc[ct] + o
        return acc

    s0 = scores(0)
    s1 = scores(1)
    p0, m, l, al0 = soft(s0, None, None)
    acc = ctxc(0, p0, None, None)
    s2 = scores(2)
    p1, m, l, al1 = soft(s1, m, l)
    acc = ctxc(1, p1, al1, acc)
    s3 = scores(3)
    p2, m, l, al2 = soft(s2, m, l)
    acc = ctxc(2, p2, al2, acc)
    p3, m, l, al3 = soft(s3, m, l)
    acc = ctxc(3, p3, al3, acc)
    linv = 1.0 / jnp.sum(l, axis=1, keepdims=True)

    accv = [[None] * NM for _ in range(3)]
    accm = [None] * NM

    def e_tiles(hs, cts, part):
        for ct in cts:
            for h in hs:
                g = h // 8
                o = _dot(acc[ct][g * 8:(g + 1) * 8], _tile(wuv, h, pl.ds(ct * 64, 64)))
                part[h] = o if h not in part else part[h] + o

    def head_ctx(h, part):
        g, r = divmod(h, 8)
        return part.pop(h)[r:r + 1] * linv[h:h + 1]

    def f_vpu(hs, part, accv):
        xbs = [_xb(head_ctx(h, part)) for h in hs]
        return _vmac3(accv, xbs, lambda j, s, n: o32[hs[j], pl.ds(s * 8, 8), pl.ds(n * 128, 128)])

    part = {}
    trip = [list(range(i, min(i + 3, OV))) for i in range(0, OV, 3)]
    e_tiles(trip[0], range(3), part)
    e_tiles(trip[1], range(3), part)
    e_tiles(trip[0], [3], part)
    accv = f_vpu(trip[0], part, accv)
    e_tiles(trip[1], [3], part)
    accv = f_vpu(trip[1], part, accv)
    for hs in trip[2:]:
        e_tiles(hs, range(NC), part)
        accv = f_vpu(hs, part, accv)
    lhs_m = {}
    for h in range(OV, H):
        e_tiles([h], range(NC), part)
        g, r = divmod(h, 8)
        lhs_m[h] = jnp.where(masks[r], part.pop(h) * linv[g * 8:(g + 1) * 8], 0.0)
    for n in range(NM):
        for h in range(OV, H):
            o = _dot(lhs_m[h], _tile(wo2, h, n))
            accm[n] = o if accm[n] is None else accm[n] + o
    x3 = [_rbf(x2[n] + _rbf(_rowsum(accm[n] + _fold3(accv, n)))) for n in range(NM)]
    mean3, rstd3 = _stats(x3)
    ln3 = [(x - mean3) * rstd3 for x in x3]
    sig3 = _router(ln3, wr)
    xb3 = _xb_gather(x3[0])
    hh = {}
    for ft in GORD:
        srcs = (("g", g32, gt), ("u", u32s, ut)) if ft < 13 else (("g", g32, gt),)
        val = {}
        for nm, ref, mref in srcs:
            av_ = None
            for s in range(16):
                p = xb3[s] * ref[ft, pl.ds(s * 8, 8), :]
                av_ = p if av_ is None else av_ + p
            om = None
            for kt in range(1, NM):
                a = _dot(x3[kt], _tile(mref, ft, kt))
                om = a if om is None else om + a
            cs_ = csg[ft] if nm == "g" else csu[ft]
            val[nm] = rstd3 * (om + _rowsum(av_) - mean3 * cs_)
        u = val["u"] if ft < 13 else pltpu.roll(val["g"], 64, 1)
        hh[ft] = _silu(val["g"]) * u
    y = [None] * NM
    for ft in range(DV, NF):
        for n in range(NM):
            o = down2(ft, n, hh[ft])
            y[n] = o if y[n] is None else y[n] + o
    yv = [[None] * NM for _ in range(3)]
    for i in range(0, DV, 3):
        fs = list(range(i, min(i + 3, DV)))
        yv = _vmac3(yv, [_xb(hh[ft][0:1]) for ft in fs],
                    lambda j, s, n: wd_f32(fs[j], s, n))
    y = [y[n] + _rowsum(_fold3(yv, n)) for n in range(NM)]
    x4 = [x3[n] + _rbf(ln3[n] + _rbf(y[n] * sig3)) for n in range(NM)]
    out = jnp.concatenate([x[0:1, :] for x in x4], axis=1)
    o_ref[0] = out.astype(bf16)


@jax.jit
def pallas_interleave_layers__compressed_kv_cla__moe_arch_mod__decode_kernel(
    A_x: jax.Array,
    A_c_kv: jax.Array,
    A_w_q: jax.Array,
    A_w_uk: jax.Array,
    A_w_uv: jax.Array,
    A_w_o: jax.Array,
    B_x: jax.Array,
    B_w_r: jax.Array,
    B_w_gate: jax.Array,
    B_w_up: jax.Array,
    B_w_down: jax.Array,
):
    del B_x
    any_spec = pl.BlockSpec(memory_space=pl.ANY)
    V = pltpu.VMEM
    scratch = [
        V((1, 1, M), bf16),
        V((NM, 128), bf16),
        V((M, H, D), bf16),
        V((DC, H, D), bf16),
        V((DC, H, D), bf16),
        V((NC, SK // 2, 128), u32),
        V((H, D, M), bf16),
        V((F, M), bf16),
        V((F, M), bf16),
        V((F, M), bf16),
        V((H, M // 2, D), u32),
        V((H, NC, D // 2, 128), u32),
        V((H, DC // 2, D), u32),
        V((NK, NC, 64, 128), u32),
        V((NF, NM, 64, 128), u32),
        V((NF, NM, 64, 128), u32),
        V((NF, 128, 128), f32),
        V((NF, 128, 128), f32),
        V((DV * 128, M), f32),
        V((OV, D, M), f32),
        V((BV, NC, D, 128), f32),
        V((H, len(QV) * 128, D), f32),
        V((H, NM, 64, 128), u32),
        V((4, 8, 128), f32),
        V((NF, 8, 128), f32),
        V((NF, 8, 128), f32),
        V((NC, H, 128), f32),
        V((NC, H, 128), f32),
        V((4, 8, 128), f32),
        V((NF, 8, 128), f32),
        V((NM, 8, 128), f32),
        pltpu.SemaphoreType.DMA((40,)),
    ]
    return pl.pallas_call(
        _kernel,
        out_shape=jax.ShapeDtypeStruct((1, 1, M), bf16),
        in_specs=[any_spec] * 10,
        out_specs=pl.BlockSpec(memory_space=pltpu.VMEM),
        scratch_shapes=scratch,
        compiler_params=pltpu.CompilerParams(
            vmem_limit_bytes=100 * 1024 * 1024,
            disable_semaphore_checks=True,
        ),
    )(A_x, A_c_kv, A_w_q, A_w_uk, A_w_uv, A_w_o, B_w_r.reshape(NM, 128),
      B_w_gate.T, B_w_up.T, B_w_down)
```

```python
import functools

import jax
import jax.numpy as jnp
from jax import lax
import jax.experimental.pallas as pl
import jax.experimental.pallas.tpu as pltpu

f32 = jnp.float32
bf16 = jnp.bfloat16
u32 = jnp.uint32
i32 = jnp.int32

M = 640
H = 32
D = 128
DC = 512
SK = 4096
F = 1728
NM = M // 128
NC = DC // 128
NK = SK // 128
NF = 14
EPS = 1e-5
SCALE = float(D) ** -0.5
KB = 8
NB = NK // KB

QV = {2: 24, 3: 16}
BV = 12
OV = 21
DV = 8
GX = 32
DRC = 384
DR0 = 768
DGROUPS = ((0, 1), (2, 3), (4,))
NE = DR0 // 128
GORD = list(range(10)) + [13, 10, 11, 12]


def _dot(a, b):
    return jnp.dot(a, b, preferred_element_type=f32)


def _rbf(x):
    return x.astype(bf16).astype(f32)


def _tile(ref, *idx):
    return pltpu.bitcast(ref[idx], bf16)


def _stats(xs):
    s = xs[0] + xs[1] + xs[2] + xs[3] + xs[4]
    mean = jnp.sum(s, axis=1, keepdims=True) * (1.0 / M)
    ds = [x - mean for x in xs]
    q = ds[0] * ds[0] + ds[1] * ds[1] + ds[2] * ds[2] + ds[3] * ds[3] + ds[4] * ds[4]
    var = jnp.sum(q, axis=1, keepdims=True) * (1.0 / M)
    rstd = 1.0 / jnp.sqrt(var + EPS)
    return mean, rstd


def _router(lns, wr):
    s = lns[0] * wr[0] + lns[1] * wr[1] + lns[2] * wr[2] + lns[3] * wr[3] + lns[4] * wr[4]
    r = jnp.sum(s, axis=1, keepdims=True)
    return jax.nn.sigmoid(r)


def _rowsum(x):
    return jnp.broadcast_to(jnp.sum(x, axis=0, keepdims=True), x.shape)


def _xb(row):
    t = jnp.broadcast_to(row, (128, 128)).T
    return [t[s * 8:(s + 1) * 8] for s in range(16)]


def _xb_gather(rows):
    sub = lax.broadcasted_iota(i32, (8, 128), 0)
    return [jnp.take_along_axis(rows, sub + 8 * s, axis=1, mode="promise_in_bounds")
            for s in range(16)]


def _vmac3(accs, xbs, load):
    accs = [list(a) for a in accs]
    for s in range(16):
        for j, xb in enumerate(xbs):
            for i in range(len(accs[j])):
                p = xb[s] * load(j, s, i)
                accs[j][i] = p if accs[j][i] is None else accs[j][i] + p
    return accs


def _fold3(accs, i):
    t = [a[i] for a in accs if a[i] is not None]
    return functools.reduce(lambda a, b: a + b, t)


def _silu(g):
    return g * jax.nn.sigmoid(g)


def _kernel(x_hbm, ckv_hbm, wq_hbm, wuk_hbm, wuv_hbm, wo_hbm, wr_hbm, wg_hbm, wu_hbm, wd_hbm,
            o_ref,
            x_v, wr_v, lq, luk, luv, lckv, lo, lg, lu, ld,
            wq, wukt, wuv, ckvt, gt, ut, g32, u32s, d32, o32, b32, q32, wo2,
            csq, csg, csu, qa_s, cc_s, ctx_s, hh_s, x_s,
            sems):
    row8 = lax.broadcasted_iota(i32, (8, 128), 0)
    masks = [row8 == r for r in range(8)]

    copies = {}
    order = []

    def add(name, pairs):
        sem = sems.at[len(copies)]
        cs = [pltpu.make_async_copy(s, d, sem) for s, d in pairs]
        copies[name] = cs
        order.append(name)

    add("x", [(x_hbm, x_v)])
    add("wr", [(wr_hbm, wr_v)])
    for i in range(NM):
        add(("q", i), [(wq_hbm.at[pl.ds(i * 128, 128)], lq.at[pl.ds(i * 128, 128)])])
    for i in range(NC):
        add(("uk", i), [(wuk_hbm.at[pl.ds(i * 128, 128)], luk.at[pl.ds(i * 128, 128)])])
    ckv32 = ckv_hbm.at[0].bitcast(u32)
    for b in range(NB):
        add(("ckv", b), [(ckv32.at[pl.ds(b * 512, 512), pl.ds(ct * 128, 128)],
                          lckv.at[ct, pl.ds(b * 512, 512)]) for ct in range(NC)])
    FS = [(0, 896), (896, F - 896)]
    for i, (s, n) in enumerate(FS):
        add(("g", i), [(wg_hbm.at[pl.ds(s, n)], lg.at[pl.ds(s, n)])])
    for i, (s, n) in enumerate(FS):
        add(("u", i), [(wu_hbm.at[pl.ds(s, n)], lu.at[pl.ds(s, n)])])
    for i in range(NC):
        add(("uv", i), [(wuv_hbm.at[pl.ds(i * 128, 128)], luv.at[pl.ds(i * 128, 128)])])
    for g in range(4):
        add(("o", g), [(wo_hbm.at[pl.ds(g * 8, 8)], lo.at[pl.ds(g * 8, 8)])])
    for i in range(DR0 // DRC):
        add(("d", i), [(wd_hbm.at[pl.ds(i * DRC, DRC)], ld.at[pl.ds(i * DRC, DRC)])])
    for i, cols in enumerate(DGROUPS):
        c0, nc = cols[0] * 128, len(cols) * 128
        add(("dc", i), [(wd_hbm.at[pl.ds(DR0, F - DR0), pl.ds(c0, nc)],
                         ld.at[pl.ds(DR0, F - DR0), pl.ds(c0, nc)])])

    for name in order:
        for c in copies[name]:
            c.start()

    def wait(name):
        for c in copies[name]:
            c.wait()

    names = list(copies)

    def wait_dyn(first_name, i, pairs_fn):
        base = names.index(first_name)
        for s, d in pairs_fn(i):
            pltpu.make_async_copy(s, d, sems.at[base + i]).wait()

    wait("x")
    wait("wr")
    xr = x_v[0].astype(f32)
    x0 = [jnp.broadcast_to(xr[:, n * 128:(n + 1) * 128], (8, 128)) for n in range(NM)]
    wrf = wr_v[...].astype(f32)
    wr = [jnp.broadcast_to(wrf[n:n + 1, :], (8, 128)) for n in range(NM)]
    for n in range(NM):
        x_s[n] = x0[n]
    mean0, rstd0 = _stats(x0)
    ones8 = jnp.ones((8, 128), f32)
    zero8 = jnp.zeros((8, 128), f32)

    def a_body(kt, carry):
        raw, cs = carry
        s = pl.multiple_of(kt * 128, 128)
        wait_dyn(("q", 0), kt, lambda i: [(wq_hbm.at[pl.ds(s, 128)], lq.at[pl.ds(s, 128)])])
        t = jnp.swapaxes(lq[pl.ds(s, 128)], 0, 1)
        s2 = pl.multiple_of(kt * 64, 64)
        for h in range(H):
            wq[h, pl.ds(s2, 64), :] = pltpu.bitcast(t[h], u32)
        for j, (ktv, h0) in enumerate(sorted(QV.items())):
            @pl.when(kt == ktv)
            def _():
                for h in range(h0, H):
                    w = wq[h, pl.ds(s2, 64), :]
                    q32[h, pl.ds(j * 128, 128), :] = pltpu.bitcast(w, bf16).astype(f32)
        lhs = jnp.concatenate([x_s[kt], ones8], axis=0)
        raw, cs = list(raw), list(cs)
        for h in range(H):
            g, r = divmod(h, 8)
            out = _dot(lhs, pltpu.bitcast(wq[h, pl.ds(s2, 64), :], bf16))
            raw[g] = jnp.where(masks[r], raw[g] + out[0:8], raw[g])
            cs[g] = jnp.where(masks[r], cs[g] + out[8:16], cs[g])
        return tuple(raw), tuple(cs)

    raw, cs = lax.fori_loop(0, NM, a_body, ((zero8,) * 4, (zero8,) * 4))
    for g in range(4):
        csq[g] = cs[g]
    q = [rstd0 * (raw[g] - mean0 * cs[g]) for g in range(4)]

    def b_body(ct, _):
        s = pl.multiple_of(ct * 128, 128)
        wait_dyn(("uk", 0), ct, lambda i: [(wuk_hbm.at[pl.ds(s, 128)], luk.at[pl.ds(s, 128)])])
        t = jnp.swapaxes(luk[pl.ds(s, 128)], 0, 1)
        for h in range(H):
            th = t[h].T
            wukt[h, ct] = pltpu.bitcast(th, u32)
            if h < BV:
                b32[h, ct] = th.astype(f32)
        qa = [zero8] * 4
        for h in range(H):
            g, r = divmod(h, 8)
            out = _dot(q[g], pltpu.bitcast(wukt[h, ct], bf16))
            qa[g] = jnp.where(masks[r], out, qa[g])
        qa_s[ct] = jnp.concatenate(qa, axis=0)
        return _

    lax.fori_loop(0, NC, b_body, 0)

    def cd_body(b, carry):
        m, l, acc = carry
        s = pl.multiple_of(b * 512, 512)
        wait_dyn(("ckv", 0), b, lambda i: [(ckv32.at[pl.ds(s, 512), pl.ds(ct * 128, 128)],
                                            lckv.at[ct, pl.ds(s, 512)]) for ct in range(NC)])
        ss = []
        for j in range(KB):
            kt = b * KB + j
            sk = pl.multiple_of(s + j * 64, 64)
            sc = None
            for ct in range(NC):
                t = pltpu.bitcast(lckv[ct, pl.ds(sk, 64), :], bf16).T
                ckvt[kt, ct] = pltpu.bitcast(t, u32)
                o = _dot(qa_s[ct], t)
                sc = o if sc is None else sc + o
            ss.append(sc * SCALE)
        mb = ss[0]
        for j in range(1, KB):
            mb = jnp.maximum(mb, ss[j])
        m_new = jnp.maximum(m, jnp.max(mb, axis=1, keepdims=True))
        alpha = jnp.exp(m - m_new)
        ps = [jnp.exp(sj - m_new) for sj in ss]
        lb = ps[0]
        for j in range(1, KB):
            lb = lb + ps[j]
        l = l * alpha + lb
        acc = [a * alpha for a in acc]
        for j in range(KB):
            sk = pl.multiple_of(s + j * 64, 64)
            for ct in range(NC):
                acc[ct] = acc[ct] + _dot(ps[j], pltpu.bitcast(lckv[ct, pl.ds(sk, 64), :], bf16))
        return m_new, l, acc

    m_init = jnp.full((H, 128), -jnp.inf, f32)
    _, l, acc = lax.fori_loop(0, NB, cd_body,
                              (m_init, jnp.zeros((H, 128), f32),
                               [jnp.zeros((H, 128), f32)] * NC))
    linv = 1.0 / jnp.sum(l, axis=1, keepdims=True)
    for ct in range(NC):
        cc_s[ct] = acc[ct]

    def transpose_ffn(land, dst, dst32, fam):
        def body(ft, _):
            s = pl.multiple_of(ft * 128, 128)
            for kt in range(NM):
                t = land[pl.ds(s, 128), pl.ds(kt * 128, 128)].T
                dst[ft, kt] = pltpu.bitcast(t, u32)
                if kt < 2:
                    dst32[ft, pl.ds(kt * 128, 128), :] = t.astype(f32)
            return _
        wait((fam, 0))
        lax.fori_loop(0, 7, body, 0)
        wait((fam, 1))
        lax.fori_loop(7, 13, body, 0)

    transpose_ffn(lg, gt, g32, "g")
    transpose_ffn(lu, ut, u32s, "u")
    for kt in range(NM):
        t = jnp.concatenate([lg[pl.ds(13 * 128, 64), pl.ds(kt * 128, 128)],
                             lu[pl.ds(13 * 128, 64), pl.ds(kt * 128, 128)]], axis=0).T
        gt[13, kt] = pltpu.bitcast(t, u32)
        if kt < 2:
            g32[13, pl.ds(kt * 128, 128), :] = t.astype(f32)

    def e_body(ct, ctx):
        s = pl.multiple_of(ct * 128, 128)
        wait_dyn(("uv", 0), ct, lambda i: [(wuv_hbm.at[pl.ds(s, 128)], luv.at[pl.ds(s, 128)])])
        t = jnp.swapaxes(luv[pl.ds(s, 128)], 0, 1)
        s2 = pl.multiple_of(ct * 64, 64)
        for h in range(H):
            wuv[h, pl.ds(s2, 64), :] = pltpu.bitcast(t[h], u32)
        ctx = list(ctx)
        cc = cc_s[ct]
        for h in range(H):
            g, r = divmod(h, 8)
            out = _dot(cc[g * 8:(g + 1) * 8], pltpu.bitcast(wuv[h, pl.ds(s2, 64), :], bf16))
            ctx[g] = jnp.where(masks[r], ctx[g] + out, ctx[g])
        return tuple(ctx)

    ctx = lax.fori_loop(0, NC, e_body, (zero8,) * 4)
    for g in range(4):
        ctx_s[g] = ctx[g] * linv[g * 8:(g + 1) * 8]

    def f_body(g, acc):
        s = pl.multiple_of(g * 8, 8)
        wait_dyn(("o", 0), g, lambda i: [(wo_hbm.at[pl.ds(s, 8)], lo.at[pl.ds(s, 8)])])
        acc = list(acc)
        cg = ctx_s[g]
        for r in range(8):
            lhs = jnp.where(masks[r], cg, 0.0)
            for n in range(NM):
                t = lo[s + r, :, pl.ds(n * 128, 128)]
                wo2[s + r, n] = pltpu.bitcast(t, u32)
                acc[n] = acc[n] + _dot(lhs, t)
        for r in range(8):
            @pl.when(s + r < OV)
            def _():
                o32[jnp.minimum(s + r, OV - 1)] = lo[s + r].astype(f32)
        return tuple(acc)

    acc = lax.fori_loop(0, 4, f_body, (zero8,) * NM)
    x1 = [_rbf(x0[n] + _rbf(_rowsum(acc[n]))) for n in range(NM)]

    mean1, rstd1 = _stats(x1)
    ln1 = [(x - mean1) * rstd1 for x in x1]
    sig1 = _router(ln1, wr)
    lhs1 = [jnp.concatenate([x1[kt], ones8], axis=0) for kt in range(NM)]

    hh1 = []
    for ft in range(NF):
        og = ou = None
        for kt in range(NM):
            a = _dot(lhs1[kt], _tile(gt, ft, kt))
            og = a if og is None else og + a
            if ft < 13:
                b = _dot(lhs1[kt], _tile(ut, ft, kt))
                ou = b if ou is None else ou + b
        csg[ft] = og[8:16]
        g = rstd1 * (og[0:8] - mean1 * og[8:16])
        if ft < 13:
            csu[ft] = ou[8:16]
            u = rstd1 * (ou[0:8] - mean1 * ou[8:16])
        else:
            u = pltpu.roll(g, 64, 1)
        hh1.append(_silu(g) * u)
        if ft < NE:
            hh_s[ft] = hh1[ft]


    def wd_tile(ft, n):
        return ld[pl.ds(ft * 128, min(128, F - ft * 128)), pl.ds(n * 128, 128)]

    def down2(ft, n, hh):
        return _dot(hh if ft < 13 else hh[:, :64], wd_tile(ft, n))

    def wd_f32(ft, s, n):
        if ft < NE or n < 4:
            return d32[pl.ds(ft * 128 + s * 8, 8), pl.ds(n * 128, 128)]
        return wd_tile(ft, n).astype(f32)[s * 8:(s + 1) * 8]

    FPC = DRC // 128

    def h_body(i, y):
        s = pl.multiple_of(i * DRC, 128)
        wait_dyn(("d", 0), i, lambda _: [(wd_hbm.at[pl.ds(s, DRC)], ld.at[pl.ds(s, DRC)])])
        y = list(y)
        for j in range(FPC):
            ft = i * FPC + j
            sf = pl.multiple_of(s + j * 128, 128)
            hh = hh_s[ft]
            for n in range(NM):
                t = ld[pl.ds(sf, 128), pl.ds(n * 128, 128)]
                y[n] = y[n] + _dot(hh, t)
        for j in range(FPC):
            ft = i * FPC + j
            sf = pl.multiple_of(s + j * 128, 128)
            sd = pl.multiple_of(ft * 128, 128)
            d32[pl.ds(sd, 128), :] = ld[pl.ds(sf, 128), :].astype(f32)
        return tuple(y)

    y = list(lax.fori_loop(0, DR0 // DRC, h_body, (zero8,) * NM))

    x2 = [None] * NM
    racc = [None] * 4

    def h_late(n):
        for ft in range(NE, NF):
            y[n] = y[n] + down2(ft, n, hh1[ft])
        x2[n] = _rbf(x1[n] + _rbf(ln1[n] + _rbf(y[n] * sig1)))
        if n < 4:
            for ft in range(NE, DV):
                d32[pl.ds(ft * 128, 128), pl.ds(n * 128, 128)] = wd_tile(ft, n).astype(f32)

    def a_pass(kt, heads=range(H)):
        for h in heads:
            g, r = divmod(h, 8)
            o = _dot(jnp.where(masks[r], x2[kt], 0.0), _tile(wq, h, pl.ds(kt * 64, 64)))
            racc[g] = o if racc[g] is None else racc[g] + o

    def a_mxu(kt, heads=range(H)):
        a_pass(kt, [h for h in heads if h < QV.get(kt, H)])

    wait(("dc", 0))
    h_late(0)
    h_late(1)
    a_mxu(0)
    a_mxu(1)
    wait(("dc", 1))
    h_late(2)
    h_late(3)
    a_mxu(2)
    wait(("dc", 2))
    av = {}
    for j, (kt, h0) in enumerate(sorted(QV.items())):
        xb = _xb_gather(x2[kt])
        for h in range(h0, H):
            a = None
            for s in range(16):
                p = xb[s] * q32[h, pl.ds(j * 128 + s * 8, 8), :]
                a = p if a is None else a + p
            av[h] = a if h not in av else av[h] + a
    h_late(4)
    a_mxu(3, range(0, 16))
    mean2, rstd2 = _stats(x2)
    raw = {}
    KL = DGROUPS[-1][-1]
    last = {}
    for h in range(BV):
        last[h] = _dot(x2[KL], _tile(wq, h, pl.ds(KL * 64, 64)))
    a_mxu(3, range(16, H))
    for h in range(BV, H):
        last[h] = _dot(x2[KL], _tile(wq, h, pl.ds(KL * 64, 64)))
    for h in range(H):
        raw[h] = racc[h // 8] + last[h]
        if h in av:
            raw[h] = raw[h] + _rowsum(av[h])
    qv = {}
    for i in range(0, BV, 3):
        hs = list(range(i, min(i + 3, BV)))
        xbs = []
        for h in hs:
            g, r = divmod(h, 8)
            qh = raw[h][r:r + 1] - mean2[0:1] * csq[g, pl.ds(r, 1), :]
            xbs.append(_xb(qh))
        accs = _vmac3([[None] * NC for _ in hs], xbs,
                      lambda j, s, ct: b32[hs[j], ct, pl.ds(s * 8, 8), :])
        for j, h in enumerate(hs):
            for ct in range(NC):
                qv[h, ct] = _rowsum(accs[j][ct]) * rstd2
    q = {}
    for g in range(BV // 8, 4):
        rawg = zero8
        for r in range(8):
            if g * 8 + r >= BV:
                rawg = jnp.where(masks[r], raw[g * 8 + r], rawg)
        q[g] = rstd2 * (rawg - mean2 * csq[g])
    qa = []
    for ct in range(NC):
        qg = [zero8] * 4
        for h in range(H):
            g, r = divmod(h, 8)
            o = qv[h, ct] if h < BV else _dot(q[g], _tile(wukt, h, ct))
            qg[g] = jnp.where(masks[r], o, qg[g])
        qa.append(jnp.concatenate(qg, axis=0))

    def scores(b):
        ss = []
        for j in range(KB):
            kt = b * KB + j
            sc = None
            for ct in range(NC):
                o = _dot(qa[ct], _tile(ckvt, kt, ct))
                sc = o if sc is None else sc + o
            ss.append(sc * SCALE)
        return ss

    def soft(ss, m, l):
        mb = ss[0]
        for j in range(1, KB):
            mb = jnp.maximum(mb, ss[j])
        mb = jnp.max(mb, axis=1, keepdims=True)
        m_new = mb if m is None else jnp.maximum(m, mb)
        ps = [jnp.exp(sj - m_new) for sj in ss]
        lb = ps[0]
        for j in range(1, KB):
            lb = lb + ps[j]
        if m is None:
            return ps, m_new, lb, None
        alpha = jnp.exp(m - m_new)
        return ps, m_new, l * alpha + lb, alpha

    def ctxc(b, ps, alpha, acc):
        if acc is not None:
            acc = [a * alpha for a in acc]
        else:
            acc = [None] * NC
        acc = list(acc)
        last = b == NB - 1
        seq = ([(j, ct) for ct in range(NC) for j in range(KB)] if last
               else [(j, ct) for j in range(KB) for ct in range(NC)])
        for j, ct in seq:
            kt = b * KB + j
            o = _dot(ps[j], _tile(lckv, ct, pl.ds(kt * 64, 64)))
            acc[ct] = o if acc[ct] is None else acc[ct] + o
        return acc

    s0 = scores(0)
    s1 = scores(1)
    p0, m, l, al0 = soft(s0, None, None)
    acc = ctxc(0, p0, None, None)
    s2 = scores(2)
    p1, m, l, al1 = soft(s1, m, l)
    acc = ctxc(1, p1, al1, acc)
    s3 = scores(3)
    p2, m, l, al2 = soft(s2, m, l)
    acc = ctxc(2, p2, al2, acc)
    p3, m, l, al3 = soft(s3, m, l)
    acc = ctxc(3, p3, al3, acc)
    linv = 1.0 / jnp.sum(l, axis=1, keepdims=True)

    accv = [[None] * NM for _ in range(3)]
    accm = [None] * NM

    def e_tiles(hs, cts, part):
        for ct in cts:
            for h in hs:
                g = h // 8
                o = _dot(acc[ct][g * 8:(g + 1) * 8], _tile(wuv, h, pl.ds(ct * 64, 64)))
                part[h] = o if h not in part else part[h] + o

    def head_ctx(h, part):
        g, r = divmod(h, 8)
        return part.pop(h)[r:r + 1] * linv[h:h + 1]

    def f_vpu(hs, part, accv):
        xbs = [_xb(head_ctx(h, part)) for h in hs]
        return _vmac3(accv, xbs, lambda j, s, n: o32[hs[j], pl.ds(s * 8, 8), pl.ds(n * 128, 128)])

    part = {}
    trip = [list(range(i, min(i + 3, OV))) for i in range(0, OV, 3)]
    e_tiles(trip[0], range(3), part)
    e_tiles(trip[1], range(3), part)
    e_tiles(trip[0], [3], part)
    accv = f_vpu(trip[0], part, accv)
    e_tiles(trip[1], [3], part)
    accv = f_vpu(trip[1], part, accv)
    for hs in trip[2:]:
        e_tiles(hs, range(NC), part)
        accv = f_vpu(hs, part, accv)
    lhs_m = {}
    for h in range(OV, H):
        e_tiles([h], range(NC), part)
        g, r = divmod(h, 8)
        lhs_m[h] = jnp.where(masks[r], part.pop(h) * linv[g * 8:(g + 1) * 8], 0.0)
    for n in range(NM):
        for h in range(OV, H):
            o = _dot(lhs_m[h], _tile(wo2, h, n))
            accm[n] = o if accm[n] is None else accm[n] + o
    x3 = [_rbf(x2[n] + _rbf(_rowsum(accm[n] + _fold3(accv, n)))) for n in range(NM)]
    mean3, rstd3 = _stats(x3)
    ln3 = [(x - mean3) * rstd3 for x in x3]
    sig3 = _router(ln3, wr)
    xb3 = list(enumerate(_xb_gather(x3[0])))
    KM = 128 - GX
    if GX:
        sub = lax.broadcasted_iota(i32, (8, 128), 0)
        for s in range(KM // 8, 16):
            xb3.append((16 + s, jnp.take_along_axis(x3[1], sub + 8 * s, axis=1,
                                                    mode="promise_in_bounds")))
    hh = {}
    for ft in GORD:
        srcs = (("g", g32, gt), ("u", u32s, ut)) if ft < 13 else (("g", g32, gt),)
        val = {}
        for nm, ref, mref in srcs:
            av_ = None
            for s, xs in xb3:
                p = xs * ref[ft, pl.ds(s * 8, 8), :]
                av_ = p if av_ is None else av_ + p
            om = None
            for kt in range(1, NM):
                if kt == 1 and GX:
                    a = _dot(x3[1][:, :KM], _tile(mref, ft, 1, pl.ds(0, KM // 2)))
                else:
                    a = _dot(x3[kt], _tile(mref, ft, kt))
                om = a if om is None else om + a
            cs_ = csg[ft] if nm == "g" else csu[ft]
            val[nm] = rstd3 * (om + _rowsum(av_) - mean3 * cs_)
        u = val["u"] if ft < 13 else pltpu.roll(val["g"], 64, 1)
        hh[ft] = _silu(val["g"]) * u
    y = [None] * NM
    for ft in range(DV, NF):
        for n in range(NM):
            o = down2(ft, n, hh[ft])
            y[n] = o if y[n] is None else y[n] + o
    yv = [[None] * NM for _ in range(3)]
    for i in range(0, DV, 3):
        fs = list(range(i, min(i + 3, DV)))
        yv = _vmac3(yv, [_xb(hh[ft][0:1]) for ft in fs],
                    lambda j, s, n: wd_f32(fs[j], s, n))
    y = [y[n] + _rowsum(_fold3(yv, n)) for n in range(NM)]
    x4 = [x3[n] + _rbf(ln3[n] + _rbf(y[n] * sig3)) for n in range(NM)]
    out = jnp.concatenate([x[0:1, :] for x in x4], axis=1)
    o_ref[0] = out.astype(bf16)


@jax.jit
def pallas_interleave_layers__compressed_kv_cla__moe_arch_mod__decode_kernel(
    A_x: jax.Array,
    A_c_kv: jax.Array,
    A_w_q: jax.Array,
    A_w_uk: jax.Array,
    A_w_uv: jax.Array,
    A_w_o: jax.Array,
    B_x: jax.Array,
    B_w_r: jax.Array,
    B_w_gate: jax.Array,
    B_w_up: jax.Array,
    B_w_down: jax.Array,
):
    del B_x
    any_spec = pl.BlockSpec(memory_space=pl.ANY)
    V = pltpu.VMEM
    scratch = [
        V((1, 1, M), bf16),
        V((NM, 128), bf16),
        V((M, H, D), bf16),
        V((DC, H, D), bf16),
        V((DC, H, D), bf16),
        V((NC, SK // 2, 128), u32),
        V((H, D, M), bf16),
        V((F, M), bf16),
        V((F, M), bf16),
        V((F, M), bf16),
        V((H, M // 2, D), u32),
        V((H, NC, D // 2, 128), u32),
        V((H, DC // 2, D), u32),
        V((NK, NC, 64, 128), u32),
        V((NF, NM, 64, 128), u32),
        V((NF, NM, 64, 128), u32),
        V((NF, 256, 128), f32),
        V((NF, 256, 128), f32),
        V((DV * 128, M), f32),
        V((OV, D, M), f32),
        V((BV, NC, D, 128), f32),
        V((H, len(QV) * 128, D), f32),
        V((H, NM, 64, 128), u32),
        V((4, 8, 128), f32),
        V((NF, 8, 128), f32),
        V((NF, 8, 128), f32),
        V((NC, H, 128), f32),
        V((NC, H, 128), f32),
        V((4, 8, 128), f32),
        V((NF, 8, 128), f32),
        V((NM, 8, 128), f32),
        pltpu.SemaphoreType.DMA((40,)),
    ]
    return pl.pallas_call(
        _kernel,
        out_shape=jax.ShapeDtypeStruct((1, 1, M), bf16),
        in_specs=[any_spec] * 10,
        out_specs=pl.BlockSpec(memory_space=pltpu.VMEM),
        scratch_shapes=scratch,
        compiler_params=pltpu.CompilerParams(
            vmem_limit_bytes=100 * 1024 * 1024,
            disable_semaphore_checks=True,
        ),
    )(A_x, A_c_kv, A_w_q, A_w_uk, A_w_uv, A_w_o, B_w_r.reshape(NM, 128),
      B_w_gate.T, B_w_up.T, B_w_down)
```

```python
import functools

import jax
import jax.numpy as jnp
from jax import lax
import jax.experimental.pallas as pl
import jax.experimental.pallas.tpu as pltpu

f32 = jnp.float32
bf16 = jnp.bfloat16
u32 = jnp.uint32
i32 = jnp.int32

M = 640
H = 32
D = 128
DC = 512
SK = 4096
F = 1728
NM = M // 128
NC = DC // 128
NK = SK // 128
NF = 14
EPS = 1e-5
SCALE = float(D) ** -0.5
KB = 8
NB = NK // KB

QV = {2: 24, 3: 16}
BV = 12
OV = 21
DV = 8
GX = 32
DRC = 384
DR0 = 768
DGROUPS = ((0, 1), (2, 3), (4,))
NE = DR0 // 128
GORD = list(range(10)) + [13, 10, 11, 12]


def _dot(a, b):
    return jnp.dot(a, b, preferred_element_type=f32)


def _rbf(x):
    return x.astype(bf16).astype(f32)


def _tile(ref, *idx):
    return pltpu.bitcast(ref[idx], bf16)


def _stats(xs):
    s = xs[0] + xs[1] + xs[2] + xs[3] + xs[4]
    mean = jnp.sum(s, axis=1, keepdims=True) * (1.0 / M)
    ds = [x - mean for x in xs]
    q = ds[0] * ds[0] + ds[1] * ds[1] + ds[2] * ds[2] + ds[3] * ds[3] + ds[4] * ds[4]
    var = jnp.sum(q, axis=1, keepdims=True) * (1.0 / M)
    rstd = 1.0 / jnp.sqrt(var + EPS)
    return mean, rstd


def _router(lns, wr):
    s = lns[0] * wr[0] + lns[1] * wr[1] + lns[2] * wr[2] + lns[3] * wr[3] + lns[4] * wr[4]
    r = jnp.sum(s, axis=1, keepdims=True)
    return jax.nn.sigmoid(r)


def _rowsum(x):
    return jnp.broadcast_to(jnp.sum(x, axis=0, keepdims=True), x.shape)


def _xb(row):
    t = jnp.broadcast_to(row, (128, 128)).T
    return [t[s * 8:(s + 1) * 8] for s in range(16)]


def _xb_gather(rows):
    sub = lax.broadcasted_iota(i32, (8, 128), 0)
    return [jnp.take_along_axis(rows, sub + 8 * s, axis=1, mode="promise_in_bounds")
            for s in range(16)]


def _vmac3(accs, xbs, load):
    accs = [list(a) for a in accs]
    for s in range(16):
        for j, xb in enumerate(xbs):
            for i in range(len(accs[j])):
                p = xb[s] * load(j, s, i)
                accs[j][i] = p if accs[j][i] is None else accs[j][i] + p
    return accs


def _fold3(accs, i):
    t = [a[i] for a in accs if a[i] is not None]
    return functools.reduce(lambda a, b: a + b, t)


def _silu(g):
    return g * jax.nn.sigmoid(g)


def _kernel(x_hbm, ckv_hbm, wq_hbm, wuk_hbm, wuv_hbm, wo_hbm, wr_hbm, wg_hbm, wu_hbm, wd_hbm,
            o_ref,
            x_v, wr_v, lq, luk, luv, lckv, lo, lg, lu, ld,
            wq, wukt, wuv, ckvt, ckvn, gt, ut, g32, u32s, d32, o32, b32, q32, wo2,
            csq, csg, csu, qa_s, cc_s, ctx_s, hh_s, x_s,
            sems):
    row8 = lax.broadcasted_iota(i32, (8, 128), 0)
    masks = [row8 == r for r in range(8)]

    copies = {}
    order = []

    def add(name, pairs):
        sem = sems.at[len(copies)]
        cs = [pltpu.make_async_copy(s, d, sem) for s, d in pairs]
        copies[name] = cs
        order.append(name)

    add("x", [(x_hbm, x_v)])
    add("wr", [(wr_hbm, wr_v)])
    for i in range(NM):
        add(("q", i), [(wq_hbm.at[pl.ds(i * 128, 128)], lq.at[pl.ds(i * 128, 128)])])
    for i in range(NC):
        add(("uk", i), [(wuk_hbm.at[pl.ds(i * 128, 128)], luk.at[pl.ds(i * 128, 128)])])
    ckv2 = ckv_hbm.at[0]
    for b in range(NB):
        add(("ckv", b), [(ckv2.at[pl.ds(b * 1024, 1024), pl.ds(ct * 128, 128)],
                          lckv.at[ct, pl.ds(b * 1024, 1024)]) for ct in range(NC)])
    FS = [(0, 896), (896, F - 896)]
    for i, (s, n) in enumerate(FS):
        add(("g", i), [(wg_hbm.at[pl.ds(s, n)], lg.at[pl.ds(s, n)])])
    for i, (s, n) in enumerate(FS):
        add(("u", i), [(wu_hbm.at[pl.ds(s, n)], lu.at[pl.ds(s, n)])])
    for i in range(NC):
        add(("uv", i), [(wuv_hbm.at[pl.ds(i * 128, 128)], luv.at[pl.ds(i * 128, 128)])])
    for g in range(4):
        add(("o", g), [(wo_hbm.at[pl.ds(g * 8, 8)], lo.at[pl.ds(g * 8, 8)])])
    for i in range(DR0 // DRC):
        add(("d", i), [(wd_hbm.at[pl.ds(i * DRC, DRC)], ld.at[pl.ds(i * DRC, DRC)])])
    for i, cols in enumerate(DGROUPS):
        c0, nc = cols[0] * 128, len(cols) * 128
        add(("dc", i), [(wd_hbm.at[pl.ds(DR0, F - DR0), pl.ds(c0, nc)],
                         ld.at[pl.ds(DR0, F - DR0), pl.ds(c0, nc)])])

    order = [("q", 0), "x", "wr"] + [n for n in order if n not in (("q", 0), "x", "wr")]
    for name in order:
        for c in copies[name]:
            c.start()

    def wait(name):
        for c in copies[name]:
            c.wait()

    names = list(copies)

    def wait_dyn(first_name, i, pairs_fn):
        base = names.index(first_name)
        for s, d in pairs_fn(i):
            pltpu.make_async_copy(s, d, sems.at[base + i]).wait()

    wait("x")
    wait("wr")
    xr = x_v[0].astype(f32)
    x0 = [jnp.broadcast_to(xr[:, n * 128:(n + 1) * 128], (8, 128)) for n in range(NM)]
    wrf = wr_v[...].astype(f32)
    wr = [jnp.broadcast_to(wrf[n:n + 1, :], (8, 128)) for n in range(NM)]
    for n in range(NM):
        x_s[n] = x0[n]
    mean0, rstd0 = _stats(x0)
    ones8 = jnp.ones((8, 128), f32)
    zero8 = jnp.zeros((8, 128), f32)

    def a_body(kt, carry):
        raw, cs = carry
        s = pl.multiple_of(kt * 128, 128)
        wait_dyn(("q", 0), kt, lambda i: [(wq_hbm.at[pl.ds(s, 128)], lq.at[pl.ds(s, 128)])])
        t = jnp.swapaxes(lq[pl.ds(s, 128)], 0, 1)
        s2 = pl.multiple_of(kt * 64, 64)
        for h in range(H):
            wq[h, pl.ds(s2, 64), :] = pltpu.bitcast(t[h], u32)
        for j, (ktv, h0) in enumerate(sorted(QV.items())):
            @pl.when(kt == ktv)
            def _():
                for h in range(h0, H):
                    w = wq[h, pl.ds(s2, 64), :]
                    q32[h, pl.ds(j * 128, 128), :] = pltpu.bitcast(w, bf16).astype(f32)
        lhs = jnp.concatenate([x_s[kt], ones8], axis=0)
        raw, cs = list(raw), list(cs)
        for h in range(H):
            g, r = divmod(h, 8)
            out = _dot(lhs, pltpu.bitcast(wq[h, pl.ds(s2, 64), :], bf16))
            raw[g] = jnp.where(masks[r], raw[g] + out[0:8], raw[g])
            cs[g] = jnp.where(masks[r], cs[g] + out[8:16], cs[g])
        return tuple(raw), tuple(cs)

    raw, cs = lax.fori_loop(0, NM, a_body, ((zero8,) * 4, (zero8,) * 4))
    for g in range(4):
        csq[g] = cs[g]
    q = [rstd0 * (raw[g] - mean0 * cs[g]) for g in range(4)]

    def b_body(ct, _):
        s = pl.multiple_of(ct * 128, 128)
        wait_dyn(("uk", 0), ct, lambda i: [(wuk_hbm.at[pl.ds(s, 128)], luk.at[pl.ds(s, 128)])])
        t = jnp.swapaxes(luk[pl.ds(s, 128)], 0, 1)
        for h in range(H):
            th = t[h].T
            wukt[h, ct] = pltpu.bitcast(th, u32)
            if h < BV:
                b32[h, ct] = th.astype(f32)
        qa = [zero8] * 4
        for h in range(H):
            g, r = divmod(h, 8)
            out = _dot(q[g], pltpu.bitcast(wukt[h, ct], bf16))
            qa[g] = jnp.where(masks[r], out, qa[g])
        qa_s[ct] = jnp.concatenate(qa, axis=0)
        return _

    lax.fori_loop(0, NC, b_body, 0)

    def cd_body(b, carry):
        m, l, acc = carry
        s = pl.multiple_of(b * 1024, 1024)
        wait_dyn(("ckv", 0), b, lambda i: [(ckv2.at[pl.ds(s, 1024), pl.ds(ct * 128, 128)],
                                            lckv.at[ct, pl.ds(s, 1024)]) for ct in range(NC)])
        ss = []
        for j in range(KB):
            kt = b * KB + j
            sk = pl.multiple_of(s + j * 128, 128)
            sc = None
            for ct in range(NC):
                t = lckv[ct, pl.ds(sk, 128), :]
                ckvn[kt, ct] = pltpu.bitcast(t, u32)
                t = t.T
                ckvt[kt, ct] = pltpu.bitcast(t, u32)
                o = _dot(qa_s[ct], t)
                sc = o if sc is None else sc + o
            ss.append(sc * SCALE)
        mb = ss[0]
        for j in range(1, KB):
            mb = jnp.maximum(mb, ss[j])
        m_new = jnp.maximum(m, jnp.max(mb, axis=1, keepdims=True))
        alpha = jnp.exp(m - m_new)
        ps = [jnp.exp(sj - m_new) for sj in ss]
        lb = ps[0]
        for j in range(1, KB):
            lb = lb + ps[j]
        l = l * alpha + lb
        acc = [a * alpha for a in acc]
        for j in range(KB):
            sk = pl.multiple_of(s + j * 128, 128)
            for ct in range(NC):
                acc[ct] = acc[ct] + _dot(ps[j], lckv[ct, pl.ds(sk, 128), :])
        return m_new, l, acc

    m_init = jnp.full((H, 128), -jnp.inf, f32)
    _, l, acc = lax.fori_loop(0, NB, cd_body,
                              (m_init, jnp.zeros((H, 128), f32),
                               [jnp.zeros((H, 128), f32)] * NC))
    linv = 1.0 / jnp.sum(l, axis=1, keepdims=True)
    for ct in range(NC):
        cc_s[ct] = acc[ct]

    def transpose_ffn(land, dst, dst32, fam):
        def body(ft, _):
            s = pl.multiple_of(ft * 128, 128)
            for kt in range(NM):
                t = land[pl.ds(s, 128), pl.ds(kt * 128, 128)].T
                dst[ft, kt] = pltpu.bitcast(t, u32)
                if kt < 2:
                    dst32[ft, pl.ds(kt * 128, 128), :] = t.astype(f32)
            return _
        wait((fam, 0))
        lax.fori_loop(0, 7, body, 0)
        wait((fam, 1))
        lax.fori_loop(7, 13, body, 0)

    transpose_ffn(lg, gt, g32, "g")
    transpose_ffn(lu, ut, u32s, "u")
    for kt in range(NM):
        t = jnp.concatenate([lg[pl.ds(13 * 128, 64), pl.ds(kt * 128, 128)],
                             lu[pl.ds(13 * 128, 64), pl.ds(kt * 128, 128)]], axis=0).T
        gt[13, kt] = pltpu.bitcast(t, u32)
        if kt < 2:
            g32[13, pl.ds(kt * 128, 128), :] = t.astype(f32)

    def e_body(ct, ctx):
        s = pl.multiple_of(ct * 128, 128)
        wait_dyn(("uv", 0), ct, lambda i: [(wuv_hbm.at[pl.ds(s, 128)], luv.at[pl.ds(s, 128)])])
        t = jnp.swapaxes(luv[pl.ds(s, 128)], 0, 1)
        s2 = pl.multiple_of(ct * 64, 64)
        for h in range(H):
            wuv[h, pl.ds(s2, 64), :] = pltpu.bitcast(t[h], u32)
        ctx = list(ctx)
        cc = cc_s[ct]
        for h in range(H):
            g, r = divmod(h, 8)
            out = _dot(cc[g * 8:(g + 1) * 8], pltpu.bitcast(wuv[h, pl.ds(s2, 64), :], bf16))
            ctx[g] = jnp.where(masks[r], ctx[g] + out, ctx[g])
        return tuple(ctx)

    ctx = lax.fori_loop(0, NC, e_body, (zero8,) * 4)
    for g in range(4):
        ctx_s[g] = ctx[g] * linv[g * 8:(g + 1) * 8]

    def f_body(g, acc):
        s = pl.multiple_of(g * 8, 8)
        wait_dyn(("o", 0), g, lambda i: [(wo_hbm.at[pl.ds(s, 8)], lo.at[pl.ds(s, 8)])])
        acc = list(acc)
        cg = ctx_s[g]
        for r in range(8):
            lhs = jnp.where(masks[r], cg, 0.0)
            for n in range(NM):
                t = lo[s + r, :, pl.ds(n * 128, 128)]
                wo2[s + r, n] = pltpu.bitcast(t, u32)
                acc[n] = acc[n] + _dot(lhs, t)
        for r in range(8):
            @pl.when(s + r < OV)
            def _():
                o32[jnp.minimum(s + r, OV - 1)] = lo[s + r].astype(f32)
        return tuple(acc)

    acc = lax.fori_loop(0, 4, f_body, (zero8,) * NM)
    x1 = [_rbf(x0[n] + _rbf(_rowsum(acc[n]))) for n in range(NM)]

    mean1, rstd1 = _stats(x1)
    ln1 = [(x - mean1) * rstd1 for x in x1]
    sig1 = _router(ln1, wr)
    lhs1 = [jnp.concatenate([x1[kt], ones8], axis=0) for kt in range(NM)]

    hh1 = []
    for ft in range(NF):
        og = ou = None
        for kt in range(NM):
            a = _dot(lhs1[kt], _tile(gt, ft, kt))
            og = a if og is None else og + a
            if ft < 13:
                b = _dot(lhs1[kt], _tile(ut, ft, kt))
                ou = b if ou is None else ou + b
        csg[ft] = og[8:16]
        g = rstd1 * (og[0:8] - mean1 * og[8:16])
        if ft < 13:
            csu[ft] = ou[8:16]
            u = rstd1 * (ou[0:8] - mean1 * ou[8:16])
        else:
            u = pltpu.roll(g, 64, 1)
        hh1.append(_silu(g) * u)
        if ft < NE:
            hh_s[ft] = hh1[ft]


    def wd_tile(ft, n):
        return ld[pl.ds(ft * 128, min(128, F - ft * 128)), pl.ds(n * 128, 128)]

    def down2(ft, n, hh):
        return _dot(hh if ft < 13 else hh[:, :64], wd_tile(ft, n))

    def wd_f32(ft, s, n):
        if ft < NE or n < 4:
            return d32[pl.ds(ft * 128 + s * 8, 8), pl.ds(n * 128, 128)]
        return wd_tile(ft, n).astype(f32)[s * 8:(s + 1) * 8]

    FPC = DRC // 128

    def h_body(i, y):
        s = pl.multiple_of(i * DRC, 128)
        wait_dyn(("d", 0), i, lambda _: [(wd_hbm.at[pl.ds(s, DRC)], ld.at[pl.ds(s, DRC)])])
        y = list(y)
        for j in range(FPC):
            ft = i * FPC + j
            sf = pl.multiple_of(s + j * 128, 128)
            hh = hh_s[ft]
            for n in range(NM):
                t = ld[pl.ds(sf, 128), pl.ds(n * 128, 128)]
                y[n] = y[n] + _dot(hh, t)
        for j in range(FPC):
            ft = i * FPC + j
            sf = pl.multiple_of(s + j * 128, 128)
            sd = pl.multiple_of(ft * 128, 128)
            d32[pl.ds(sd, 128), :] = ld[pl.ds(sf, 128), :].astype(f32)
        return tuple(y)

    y = list(lax.fori_loop(0, DR0 // DRC, h_body, (zero8,) * NM))

    x2 = [None] * NM
    racc = [None] * 4

    def h_late(n):
        for ft in range(NE, NF):
            y[n] = y[n] + down2(ft, n, hh1[ft])
        x2[n] = _rbf(x1[n] + _rbf(ln1[n] + _rbf(y[n] * sig1)))
        if n < 4:
            for ft in range(NE, DV):
                d32[pl.ds(ft * 128, 128), pl.ds(n * 128, 128)] = wd_tile(ft, n).astype(f32)

    def a_pass(kt, heads=range(H)):
        for h in heads:
            g, r = divmod(h, 8)
            o = _dot(jnp.where(masks[r], x2[kt], 0.0), _tile(wq, h, pl.ds(kt * 64, 64)))
            racc[g] = o if racc[g] is None else racc[g] + o

    def a_mxu(kt, heads=range(H)):
        a_pass(kt, [h for h in heads if h < QV.get(kt, H)])

    wait(("dc", 0))
    h_late(0)
    h_late(1)
    a_mxu(0)
    a_mxu(1)
    wait(("dc", 1))
    h_late(2)
    h_late(3)
    a_mxu(2)
    wait(("dc", 2))
    av = {}
    for j, (kt, h0) in enumerate(sorted(QV.items())):
        xb = _xb_gather(x2[kt])
        for h in range(h0, H):
            a = None
            for s in range(16):
                p = xb[s] * q32[h, pl.ds(j * 128 + s * 8, 8), :]
                a = p if a is None else a + p
            av[h] = a if h not in av else av[h] + a
    h_late(4)
    a_mxu(3, range(0, 16))
    mean2, rstd2 = _stats(x2)
    raw = {}
    KL = DGROUPS[-1][-1]
    last = {}
    for h in range(BV):
        last[h] = _dot(x2[KL], _tile(wq, h, pl.ds(KL * 64, 64)))
    a_mxu(3, range(16, H))
    for h in range(BV, H):
        last[h] = _dot(x2[KL], _tile(wq, h, pl.ds(KL * 64, 64)))
    for h in range(H):
        raw[h] = racc[h // 8] + last[h]
        if h in av:
            raw[h] = raw[h] + _rowsum(av[h])
    qv = {}
    for i in range(0, BV, 3):
        hs = list(range(i, min(i + 3, BV)))
        xbs = []
        for h in hs:
            g, r = divmod(h, 8)
            qh = raw[h][r:r + 1] - mean2[0:1] * csq[g, pl.ds(r, 1), :]
            xbs.append(_xb(qh))
        accs = _vmac3([[None] * NC for _ in hs], xbs,
                      lambda j, s, ct: b32[hs[j], ct, pl.ds(s * 8, 8), :])
        for j, h in enumerate(hs):
            for ct in range(NC):
                qv[h, ct] = _rowsum(accs[j][ct]) * rstd2
    q = {}
    for g in range(BV // 8, 4):
        rawg = zero8
        for r in range(8):
            if g * 8 + r >= BV:
                rawg = jnp.where(masks[r], raw[g * 8 + r], rawg)
        q[g] = rstd2 * (rawg - mean2 * csq[g])
    qa = []
    for ct in range(NC):
        qg = [zero8] * 4
        for h in range(H):
            g, r = divmod(h, 8)
            o = qv[h, ct] if h < BV else _dot(q[g], _tile(wukt, h, ct))
            qg[g] = jnp.where(masks[r], o, qg[g])
        qa.append(jnp.concatenate(qg, axis=0))

    def scores(b):
        ss = []
        for j in range(KB):
            kt = b * KB + j
            sc = None
            for ct in range(NC):
                o = _dot(qa[ct], _tile(ckvt, kt, ct))
                sc = o if sc is None else sc + o
            ss.append(sc * SCALE)
        return ss

    def soft(ss, m, l):
        mb = ss[0]
        for j in range(1, KB):
            mb = jnp.maximum(mb, ss[j])
        mb = jnp.max(mb, axis=1, keepdims=True)
        m_new = mb if m is None else jnp.maximum(m, mb)
        ps = [jnp.exp(sj - m_new) for sj in ss]
        lb = ps[0]
        for j in range(1, KB):
            lb = lb + ps[j]
        if m is None:
            return ps, m_new, lb, None
        alpha = jnp.exp(m - m_new)
        return ps, m_new, l * alpha + lb, alpha

    def ctxc(b, ps, alpha, acc):
        if acc is not None:
            acc = [a * alpha for a in acc]
        else:
            acc = [None] * NC
        acc = list(acc)
        last = b == NB - 1
        seq = ([(j, ct) for ct in range(NC) for j in range(KB)] if last
               else [(j, ct) for j in range(KB) for ct in range(NC)])
        for j, ct in seq:
            kt = b * KB + j
            o = _dot(ps[j], _tile(ckvn, kt, ct))
            acc[ct] = o if acc[ct] is None else acc[ct] + o
        return acc

    s0 = scores(0)
    s1 = scores(1)
    p0, m, l, al0 = soft(s0, None, None)
    acc = ctxc(0, p0, None, None)
    s2 = scores(2)
    p1, m, l, al1 = soft(s1, m, l)
    acc = ctxc(1, p1, al1, acc)
    s3 = scores(3)
    p2, m, l, al2 = soft(s2, m, l)
    acc = ctxc(2, p2, al2, acc)
    p3, m, l, al3 = soft(s3, m, l)
    acc = ctxc(3, p3, al3, acc)
    linv = 1.0 / jnp.sum(l, axis=1, keepdims=True)

    accv = [[None] * NM for _ in range(3)]
    accm = [None] * NM

    def e_tiles(hs, cts, part):
        for ct in cts:
            for h in hs:
                g = h // 8
                o = _dot(acc[ct][g * 8:(g + 1) * 8], _tile(wuv, h, pl.ds(ct * 64, 64)))
                part[h] = o if h not in part else part[h] + o

    def head_ctx(h, part):
        g, r = divmod(h, 8)
        return part.pop(h)[r:r + 1] * linv[h:h + 1]

    def f_vpu(hs, part, accv):
        xbs = [_xb(head_ctx(h, part)) for h in hs]
        return _vmac3(accv, xbs, lambda j, s, n: o32[hs[j], pl.ds(s * 8, 8), pl.ds(n * 128, 128)])

    part = {}
    trip = [list(range(i, min(i + 3, OV))) for i in range(0, OV, 3)]
    e_tiles(trip[0], range(3), part)
    e_tiles(trip[1], range(3), part)
    e_tiles(trip[0], [3], part)
    accv = f_vpu(trip[0], part, accv)
    e_tiles(trip[1], [3], part)
    accv = f_vpu(trip[1], part, accv)
    for hs in trip[2:]:
        e_tiles(hs, range(NC), part)
        accv = f_vpu(hs, part, accv)
    lhs_m = {}
    for h in range(OV, H):
        e_tiles([h], range(NC), part)
        g, r = divmod(h, 8)
        lhs_m[h] = jnp.where(masks[r], part.pop(h) * linv[g * 8:(g + 1) * 8], 0.0)
    for n in range(NM):
        for h in range(OV, H):
            o = _dot(lhs_m[h], _tile(wo2, h, n))
            accm[n] = o if accm[n] is None else accm[n] + o
    x3 = [_rbf(x2[n] + _rbf(_rowsum(accm[n] + _fold3(accv, n)))) for n in range(NM)]
    mean3, rstd3 = _stats(x3)
    ln3 = [(x - mean3) * rstd3 for x in x3]
    sig3 = _router(ln3, wr)
    xb3 = list(enumerate(_xb_gather(x3[0])))
    KM = 128 - GX
    if GX:
        sub = lax.broadcasted_iota(i32, (8, 128), 0)
        for s in range(KM // 8, 16):
            xb3.append((16 + s, jnp.take_along_axis(x3[1], sub + 8 * s, axis=1,
                                                    mode="promise_in_bounds")))
    hh = {}
    for ft in GORD:
        srcs = (("g", g32, gt), ("u", u32s, ut)) if ft < 13 else (("g", g32, gt),)
        val = {}
        for nm, ref, mref in srcs:
            av_ = None
            for s, xs in xb3:
                p = xs * ref[ft, pl.ds(s * 8, 8), :]
                av_ = p if av_ is None else av_ + p
            om = None
            for kt in range(1, NM):
                if kt == 1 and GX:
                    a = _dot(x3[1][:, :KM], _tile(mref, ft, 1, pl.ds(0, KM // 2)))
                else:
                    a = _dot(x3[kt], _tile(mref, ft, kt))
                om = a if om is None else om + a
            cs_ = csg[ft] if nm == "g" else csu[ft]
            val[nm] = rstd3 * (om + _rowsum(av_) - mean3 * cs_)
        u = val["u"] if ft < 13 else pltpu.roll(val["g"], 64, 1)
        hh[ft] = _silu(val["g"]) * u
    y = [None] * NM
    for ft in range(DV, NF):
        for n in range(NM):
            o = down2(ft, n, hh[ft])
            y[n] = o if y[n] is None else y[n] + o
    yv = [[None] * NM for _ in range(3)]
    for i in range(0, DV, 3):
        fs = list(range(i, min(i + 3, DV)))
        yv = _vmac3(yv, [_xb(hh[ft][0:1]) for ft in fs],
                    lambda j, s, n: wd_f32(fs[j], s, n))
    y = [y[n] + _rowsum(_fold3(yv, n)) for n in range(NM)]
    x4 = [x3[n] + _rbf(ln3[n] + _rbf(y[n] * sig3)) for n in range(NM)]
    out = jnp.concatenate([x[0:1, :] for x in x4], axis=1)
    o_ref[0] = out.astype(bf16)


@jax.jit
def pallas_interleave_layers__compressed_kv_cla__moe_arch_mod__decode_kernel(
    A_x: jax.Array,
    A_c_kv: jax.Array,
    A_w_q: jax.Array,
    A_w_uk: jax.Array,
    A_w_uv: jax.Array,
    A_w_o: jax.Array,
    B_x: jax.Array,
    B_w_r: jax.Array,
    B_w_gate: jax.Array,
    B_w_up: jax.Array,
    B_w_down: jax.Array,
):
    del B_x
    any_spec = pl.BlockSpec(memory_space=pl.ANY)
    V = pltpu.VMEM
    scratch = [
        V((1, 1, M), bf16),
        V((NM, 128), bf16),
        V((M, H, D), bf16),
        V((DC, H, D), bf16),
        V((DC, H, D), bf16),
        V((NC, SK, 128), bf16),
        V((H, D, M), bf16),
        V((F, M), bf16),
        V((F, M), bf16),
        V((F, M), bf16),
        V((H, M // 2, D), u32),
        V((H, NC, D // 2, 128), u32),
        V((H, DC // 2, D), u32),
        V((NK, NC, 64, 128), u32),
        V((NK, NC, 64, 128), u32),
        V((NF, NM, 64, 128), u32),
        V((NF, NM, 64, 128), u32),
        V((NF, 256, 128), f32),
        V((NF, 256, 128), f32),
        V((DV * 128, M), f32),
        V((OV, D, M), f32),
        V((BV, NC, D, 128), f32),
        V((H, len(QV) * 128, D), f32),
        V((H, NM, 64, 128), u32),
        V((4, 8, 128), f32),
        V((NF, 8, 128), f32),
        V((NF, 8, 128), f32),
        V((NC, H, 128), f32),
        V((NC, H, 128), f32),
        V((4, 8, 128), f32),
        V((NF, 8, 128), f32),
        V((NM, 8, 128), f32),
        pltpu.SemaphoreType.DMA((40,)),
    ]
    return pl.pallas_call(
        _kernel,
        out_shape=jax.ShapeDtypeStruct((1, 1, M), bf16),
        in_specs=[any_spec] * 10,
        out_specs=pl.BlockSpec(memory_space=pltpu.VMEM),
        scratch_shapes=scratch,
        compiler_params=pltpu.CompilerParams(
            vmem_limit_bytes=100 * 1024 * 1024,
            disable_semaphore_checks=True,
        ),
    )(A_x, A_c_kv, A_w_q, A_w_uk, A_w_uv, A_w_o, B_w_r.reshape(NM, 128),
      B_w_gate.T, B_w_up.T, B_w_down)
```

```python
import functools

import jax
import jax.numpy as jnp
from jax import lax
import jax.experimental.pallas as pl
import jax.experimental.pallas.tpu as pltpu

f32 = jnp.float32
bf16 = jnp.bfloat16
u32 = jnp.uint32
i32 = jnp.int32

M = 640
H = 32
D = 128
DC = 512
SK = 4096
F = 1728
NM = M // 128
NC = DC // 128
NK = SK // 128
NF = 14
EPS = 1e-5
SCALE = float(D) ** -0.5
KB = 8
NB = NK // KB

QV = {2: 24, 3: 16}
BV = 12
OV = 21
DV = 8
GX = 32
BORD = 0
CFIRST = 3
DRC = 384
DR0 = 768
DGROUPS = ((0, 1), (2, 3), (4,))
NE = DR0 // 128
GORD = list(range(10)) + [13, 10, 11, 12]


def _dot(a, b):
    return jnp.dot(a, b, preferred_element_type=f32)


def _rbf(x):
    return x.astype(bf16).astype(f32)


def _tile(ref, *idx):
    return pltpu.bitcast(ref[idx], bf16)


def _stats(xs):
    s = xs[0] + xs[1] + xs[2] + xs[3] + xs[4]
    mean = jnp.sum(s, axis=1, keepdims=True) * (1.0 / M)
    ds = [x - mean for x in xs]
    q = ds[0] * ds[0] + ds[1] * ds[1] + ds[2] * ds[2] + ds[3] * ds[3] + ds[4] * ds[4]
    var = jnp.sum(q, axis=1, keepdims=True) * (1.0 / M)
    rstd = 1.0 / jnp.sqrt(var + EPS)
    return mean, rstd


def _router(lns, wr):
    s = lns[0] * wr[0] + lns[1] * wr[1] + lns[2] * wr[2] + lns[3] * wr[3] + lns[4] * wr[4]
    r = jnp.sum(s, axis=1, keepdims=True)
    return jax.nn.sigmoid(r)


def _rowsum(x):
    return jnp.broadcast_to(jnp.sum(x, axis=0, keepdims=True), x.shape)


def _xb(row):
    t = jnp.broadcast_to(row, (128, 128)).T
    return [t[s * 8:(s + 1) * 8] for s in range(16)]


def _xb_gather(rows):
    sub = lax.broadcasted_iota(i32, (8, 128), 0)
    return [jnp.take_along_axis(rows, sub + 8 * s, axis=1, mode="promise_in_bounds")
            for s in range(16)]


def _vmac3(accs, xbs, load):
    accs = [list(a) for a in accs]
    for s in range(16):
        for j, xb in enumerate(xbs):
            for i in range(len(accs[j])):
                p = xb[s] * load(j, s, i)
                accs[j][i] = p if accs[j][i] is None else accs[j][i] + p
    return accs


def _fold3(accs, i):
    t = [a[i] for a in accs if a[i] is not None]
    return functools.reduce(lambda a, b: a + b, t)


def _silu(g):
    return g * jax.nn.sigmoid(g)


def _kernel(x_hbm, ckv_hbm, wq_hbm, wuk_hbm, wuv_hbm, wo_hbm, wr_hbm, wg_hbm, wu_hbm, wd_hbm,
            o_ref,
            x_v, wr_v, lq, luk, luv, lckv, lo, lg, lu, ld,
            wq, wukt, wuv, ckvt, ckvn, gt, ut, g32, u32s, d32, o32, b32, q32, wo2,
            csq, csg, csu, qa_s, cc_s, ctx_s, hh_s, x_s,
            sems):
    row8 = lax.broadcasted_iota(i32, (8, 128), 0)
    masks = [row8 == r for r in range(8)]

    copies = {}
    order = []

    def add(name, pairs):
        sem = sems.at[len(copies)]
        cs = [pltpu.make_async_copy(s, d, sem) for s, d in pairs]
        copies[name] = cs
        order.append(name)

    add("x", [(x_hbm, x_v)])
    add("wr", [(wr_hbm, wr_v)])
    for i in range(NM):
        add(("q", i), [(wq_hbm.at[pl.ds(i * 128, 128)], lq.at[pl.ds(i * 128, 128)])])
    for i in range(NC):
        add(("uk", i), [(wuk_hbm.at[pl.ds(i * 128, 128)], luk.at[pl.ds(i * 128, 128)])])
    ckv2 = ckv_hbm.at[0]
    for b in range(NB):
        add(("ckv", b), [(ckv2.at[pl.ds(b * 1024, 1024), pl.ds(ct * 128, 128)],
                          lckv.at[ct, pl.ds(b * 1024, 1024)]) for ct in range(NC)])
    FS = [(0, 896), (896, F - 896)]
    for i, (s, n) in enumerate(FS):
        add(("g", i), [(wg_hbm.at[pl.ds(s, n)], lg.at[pl.ds(s, n)])])
    for i, (s, n) in enumerate(FS):
        add(("u", i), [(wu_hbm.at[pl.ds(s, n)], lu.at[pl.ds(s, n)])])
    for i in range(NC):
        add(("uv", i), [(wuv_hbm.at[pl.ds(i * 128, 128)], luv.at[pl.ds(i * 128, 128)])])
    for g in range(4):
        add(("o", g), [(wo_hbm.at[pl.ds(g * 8, 8)], lo.at[pl.ds(g * 8, 8)])])
    for i in range(DR0 // DRC):
        add(("d", i), [(wd_hbm.at[pl.ds(i * DRC, DRC)], ld.at[pl.ds(i * DRC, DRC)])])
    for i, cols in enumerate(DGROUPS):
        c0, nc = cols[0] * 128, len(cols) * 128
        add(("dc", i), [(wd_hbm.at[pl.ds(DR0, F - DR0), pl.ds(c0, nc)],
                         ld.at[pl.ds(DR0, F - DR0), pl.ds(c0, nc)])])

    order = [("q", 0), "x", "wr"] + [n for n in order if n not in (("q", 0), "x", "wr")]
    for name in order:
        for c in copies[name]:
            c.start()

    def wait(name):
        for c in copies[name]:
            c.wait()

    names = list(copies)

    def wait_dyn(first_name, i, pairs_fn):
        base = names.index(first_name)
        for s, d in pairs_fn(i):
            pltpu.make_async_copy(s, d, sems.at[base + i]).wait()

    wait("x")
    wait("wr")
    xr = x_v[0].astype(f32)
    x0 = [jnp.broadcast_to(xr[:, n * 128:(n + 1) * 128], (8, 128)) for n in range(NM)]
    wrf = wr_v[...].astype(f32)
    wr = [jnp.broadcast_to(wrf[n:n + 1, :], (8, 128)) for n in range(NM)]
    for n in range(NM):
        x_s[n] = x0[n]
    mean0, rstd0 = _stats(x0)
    ones8 = jnp.ones((8, 128), f32)
    zero8 = jnp.zeros((8, 128), f32)

    def a_body(kt, carry):
        raw, cs = carry
        s = pl.multiple_of(kt * 128, 128)
        wait_dyn(("q", 0), kt, lambda i: [(wq_hbm.at[pl.ds(s, 128)], lq.at[pl.ds(s, 128)])])
        t = jnp.swapaxes(lq[pl.ds(s, 128)], 0, 1)
        s2 = pl.multiple_of(kt * 64, 64)
        for h in range(H):
            wq[h, pl.ds(s2, 64), :] = pltpu.bitcast(t[h], u32)
        for j, (ktv, h0) in enumerate(sorted(QV.items())):
            @pl.when(kt == ktv)
            def _():
                for h in range(h0, H):
                    w = wq[h, pl.ds(s2, 64), :]
                    q32[h, pl.ds(j * 128, 128), :] = pltpu.bitcast(w, bf16).astype(f32)
        lhs = jnp.concatenate([x_s[kt], ones8], axis=0)
        raw, cs = list(raw), list(cs)
        for h in range(H):
            g, r = divmod(h, 8)
            out = _dot(lhs, pltpu.bitcast(wq[h, pl.ds(s2, 64), :], bf16))
            raw[g] = jnp.where(masks[r], raw[g] + out[0:8], raw[g])
            cs[g] = jnp.where(masks[r], cs[g] + out[8:16], cs[g])
        return tuple(raw), tuple(cs)

    raw, cs = lax.fori_loop(0, NM, a_body, ((zero8,) * 4, (zero8,) * 4))
    for g in range(4):
        csq[g] = cs[g]
    q = [rstd0 * (raw[g] - mean0 * cs[g]) for g in range(4)]

    def b_body(ct, _):
        s = pl.multiple_of(ct * 128, 128)
        wait_dyn(("uk", 0), ct, lambda i: [(wuk_hbm.at[pl.ds(s, 128)], luk.at[pl.ds(s, 128)])])
        t = jnp.swapaxes(luk[pl.ds(s, 128)], 0, 1)
        for h in range(H):
            th = t[h].T
            wukt[h, ct] = pltpu.bitcast(th, u32)
            if h < BV:
                b32[h, ct] = th.astype(f32)
        qa = [zero8] * 4
        for h in range(H):
            g, r = divmod(h, 8)
            out = _dot(q[g], pltpu.bitcast(wukt[h, ct], bf16))
            qa[g] = jnp.where(masks[r], out, qa[g])
        qa_s[ct] = jnp.concatenate(qa, axis=0)
        return _

    lax.fori_loop(0, NC, b_body, 0)

    def cd_body(b, carry):
        m, l, acc = carry
        s = pl.multiple_of(b * 1024, 1024)
        wait_dyn(("ckv", 0), b, lambda i: [(ckv2.at[pl.ds(s, 1024), pl.ds(ct * 128, 128)],
                                            lckv.at[ct, pl.ds(s, 1024)]) for ct in range(NC)])
        ss = []
        for j in range(KB):
            kt = b * KB + j
            sk = pl.multiple_of(s + j * 128, 128)
            sc = None
            for ct in range(NC):
                t = lckv[ct, pl.ds(sk, 128), :]
                ckvn[kt, ct] = pltpu.bitcast(t, u32)
                t = t.T
                ckvt[kt, ct] = pltpu.bitcast(t, u32)
                o = _dot(qa_s[ct], t)
                sc = o if sc is None else sc + o
            ss.append(sc * SCALE)
        mb = ss[0]
        for j in range(1, KB):
            mb = jnp.maximum(mb, ss[j])
        m_new = jnp.maximum(m, jnp.max(mb, axis=1, keepdims=True))
        alpha = jnp.exp(m - m_new)
        ps = [jnp.exp(sj - m_new) for sj in ss]
        lb = ps[0]
        for j in range(1, KB):
            lb = lb + ps[j]
        l = l * alpha + lb
        acc = [a * alpha for a in acc]
        for j in range(KB):
            sk = pl.multiple_of(s + j * 128, 128)
            for ct in range(NC):
                acc[ct] = acc[ct] + _dot(ps[j], lckv[ct, pl.ds(sk, 128), :])
        return m_new, l, acc

    m_init = jnp.full((H, 128), -jnp.inf, f32)
    _, l, acc = lax.fori_loop(0, NB, cd_body,
                              (m_init, jnp.zeros((H, 128), f32),
                               [jnp.zeros((H, 128), f32)] * NC))
    linv = 1.0 / jnp.sum(l, axis=1, keepdims=True)
    for ct in range(NC):
        cc_s[ct] = acc[ct]

    def transpose_ffn(land, dst, dst32, fam):
        def body(ft, _):
            s = pl.multiple_of(ft * 128, 128)
            for kt in range(NM):
                t = land[pl.ds(s, 128), pl.ds(kt * 128, 128)].T
                dst[ft, kt] = pltpu.bitcast(t, u32)
                if kt < 2:
                    dst32[ft, pl.ds(kt * 128, 128), :] = t.astype(f32)
            return _
        wait((fam, 0))
        lax.fori_loop(0, 7, body, 0)
        wait((fam, 1))
        lax.fori_loop(7, 13, body, 0)

    transpose_ffn(lg, gt, g32, "g")
    transpose_ffn(lu, ut, u32s, "u")
    for kt in range(NM):
        t = jnp.concatenate([lg[pl.ds(13 * 128, 64), pl.ds(kt * 128, 128)],
                             lu[pl.ds(13 * 128, 64), pl.ds(kt * 128, 128)]], axis=0).T
        gt[13, kt] = pltpu.bitcast(t, u32)
        if kt < 2:
            g32[13, pl.ds(kt * 128, 128), :] = t.astype(f32)

    def e_body(ct, ctx):
        s = pl.multiple_of(ct * 128, 128)
        wait_dyn(("uv", 0), ct, lambda i: [(wuv_hbm.at[pl.ds(s, 128)], luv.at[pl.ds(s, 128)])])
        t = jnp.swapaxes(luv[pl.ds(s, 128)], 0, 1)
        s2 = pl.multiple_of(ct * 64, 64)
        for h in range(H):
            wuv[h, pl.ds(s2, 64), :] = pltpu.bitcast(t[h], u32)
        ctx = list(ctx)
        cc = cc_s[ct]
        for h in range(H):
            g, r = divmod(h, 8)
            out = _dot(cc[g * 8:(g + 1) * 8], pltpu.bitcast(wuv[h, pl.ds(s2, 64), :], bf16))
            ctx[g] = jnp.where(masks[r], ctx[g] + out, ctx[g])
        return tuple(ctx)

    ctx = lax.fori_loop(0, NC, e_body, (zero8,) * 4)
    for g in range(4):
        ctx_s[g] = ctx[g] * linv[g * 8:(g + 1) * 8]

    def f_body(g, acc):
        s = pl.multiple_of(g * 8, 8)
        wait_dyn(("o", 0), g, lambda i: [(wo_hbm.at[pl.ds(s, 8)], lo.at[pl.ds(s, 8)])])
        acc = list(acc)
        cg = ctx_s[g]
        for r in range(8):
            lhs = jnp.where(masks[r], cg, 0.0)
            for n in range(NM):
                t = lo[s + r, :, pl.ds(n * 128, 128)]
                wo2[s + r, n] = pltpu.bitcast(t, u32)
                acc[n] = acc[n] + _dot(lhs, t)
        for r in range(8):
            @pl.when(s + r < OV)
            def _():
                o32[jnp.minimum(s + r, OV - 1)] = lo[s + r].astype(f32)
        return tuple(acc)

    acc = lax.fori_loop(0, 4, f_body, (zero8,) * NM)
    x1 = [_rbf(x0[n] + _rbf(_rowsum(acc[n]))) for n in range(NM)]

    mean1, rstd1 = _stats(x1)
    ln1 = [(x - mean1) * rstd1 for x in x1]
    sig1 = _router(ln1, wr)
    lhs1 = [jnp.concatenate([x1[kt], ones8], axis=0) for kt in range(NM)]

    hh1 = []
    for ft in range(NF):
        og = ou = None
        for kt in range(NM):
            a = _dot(lhs1[kt], _tile(gt, ft, kt))
            og = a if og is None else og + a
            if ft < 13:
                b = _dot(lhs1[kt], _tile(ut, ft, kt))
                ou = b if ou is None else ou + b
        csg[ft] = og[8:16]
        g = rstd1 * (og[0:8] - mean1 * og[8:16])
        if ft < 13:
            csu[ft] = ou[8:16]
            u = rstd1 * (ou[0:8] - mean1 * ou[8:16])
        else:
            u = pltpu.roll(g, 64, 1)
        hh1.append(_silu(g) * u)
        if ft < NE:
            hh_s[ft] = hh1[ft]


    def wd_tile(ft, n):
        return ld[pl.ds(ft * 128, min(128, F - ft * 128)), pl.ds(n * 128, 128)]

    def down2(ft, n, hh):
        return _dot(hh if ft < 13 else hh[:, :64], wd_tile(ft, n))

    def wd_f32(ft, s, n):
        if ft < NE or n < 4:
            return d32[pl.ds(ft * 128 + s * 8, 8), pl.ds(n * 128, 128)]
        return wd_tile(ft, n).astype(f32)[s * 8:(s + 1) * 8]

    FPC = DRC // 128

    def h_body(i, y):
        s = pl.multiple_of(i * DRC, 128)
        wait_dyn(("d", 0), i, lambda _: [(wd_hbm.at[pl.ds(s, DRC)], ld.at[pl.ds(s, DRC)])])
        y = list(y)
        for j in range(FPC):
            ft = i * FPC + j
            sf = pl.multiple_of(s + j * 128, 128)
            hh = hh_s[ft]
            for n in range(NM):
                t = ld[pl.ds(sf, 128), pl.ds(n * 128, 128)]
                y[n] = y[n] + _dot(hh, t)
        for j in range(FPC):
            ft = i * FPC + j
            sf = pl.multiple_of(s + j * 128, 128)
            sd = pl.multiple_of(ft * 128, 128)
            d32[pl.ds(sd, 128), :] = ld[pl.ds(sf, 128), :].astype(f32)
        return tuple(y)

    y = list(lax.fori_loop(0, DR0 // DRC, h_body, (zero8,) * NM))

    x2 = [None] * NM
    racc = [None] * 4

    def h_late(n):
        for ft in range(NE, NF):
            y[n] = y[n] + down2(ft, n, hh1[ft])
        x2[n] = _rbf(x1[n] + _rbf(ln1[n] + _rbf(y[n] * sig1)))
        if n < 4:
            for ft in range(NE, DV):
                d32[pl.ds(ft * 128, 128), pl.ds(n * 128, 128)] = wd_tile(ft, n).astype(f32)

    def a_pass(kt, heads=range(H)):
        for h in heads:
            g, r = divmod(h, 8)
            o = _dot(jnp.where(masks[r], x2[kt], 0.0), _tile(wq, h, pl.ds(kt * 64, 64)))
            racc[g] = o if racc[g] is None else racc[g] + o

    def a_mxu(kt, heads=range(H)):
        a_pass(kt, [h for h in heads if h < QV.get(kt, H)])

    wait(("dc", 0))
    h_late(0)
    h_late(1)
    a_mxu(0)
    a_mxu(1)
    wait(("dc", 1))
    h_late(2)
    h_late(3)
    a_mxu(2)
    wait(("dc", 2))
    av = {}
    for j, (kt, h0) in enumerate(sorted(QV.items())):
        xb = _xb_gather(x2[kt])
        for h in range(h0, H):
            a = None
            for s in range(16):
                p = xb[s] * q32[h, pl.ds(j * 128 + s * 8, 8), :]
                a = p if a is None else a + p
            av[h] = a if h not in av else av[h] + a
    h_late(4)
    a_mxu(3, range(0, 16))
    mean2, rstd2 = _stats(x2)
    raw = {}
    KL = DGROUPS[-1][-1]
    last = {}
    for h in range(BV):
        last[h] = _dot(x2[KL], _tile(wq, h, pl.ds(KL * 64, 64)))
    a_mxu(3, range(16, H))
    for h in range(BV, H):
        last[h] = _dot(x2[KL], _tile(wq, h, pl.ds(KL * 64, 64)))
    for h in range(H):
        raw[h] = racc[h // 8] + last[h]
        if h in av:
            raw[h] = raw[h] + _rowsum(av[h])
    qv = {}
    for i in range(0, BV, 3):
        hs = list(range(i, min(i + 3, BV)))
        xbs = []
        for h in hs:
            g, r = divmod(h, 8)
            qh = raw[h][r:r + 1] - mean2[0:1] * csq[g, pl.ds(r, 1), :]
            xbs.append(_xb(qh))
        accs = _vmac3([[None] * NC for _ in hs], xbs,
                      lambda j, s, ct: b32[hs[j], ct, pl.ds(s * 8, 8), :])
        for j, h in enumerate(hs):
            for ct in range(NC):
                qv[h, ct] = _rowsum(accs[j][ct]) * rstd2
    q = {}
    for g in range(BV // 8, 4):
        rawg = zero8
        for r in range(8):
            if g * 8 + r >= BV:
                rawg = jnp.where(masks[r], raw[g * 8 + r], rawg)
        q[g] = rstd2 * (rawg - mean2 * csq[g])
    qm = {}
    g1 = BV // 8
    early = [h for h in range(BV, H) if h // 8 == g1] if BORD else []
    for h in early:
        for ct in range(NC):
            qm[h, ct] = _dot(q[h // 8], _tile(wukt, h, ct))
    for ct in range(NC):
        for h in range(BV, H):
            if h not in early:
                qm[h, ct] = _dot(q[h // 8], _tile(wukt, h, ct))
    qa = []
    for ct in range(NC):
        qg = [zero8] * 4
        for h in range(H):
            g, r = divmod(h, 8)
            o = qv[h, ct] if h < BV else qm[h, ct]
            qg[g] = jnp.where(masks[r], o, qg[g])
        qa.append(jnp.concatenate(qg, axis=0))

    def scores(b):
        sc = {}
        first = CFIRST if b == 0 else 0
        seq = [(j, ct) for ct in range(NC) for j in range(first)]
        seq += [(j, ct) for j in range(first, KB) for ct in range(NC)]
        for j, ct in seq:
            o = _dot(qa[ct], _tile(ckvt, b * KB + j, ct))
            sc[j] = o if j not in sc else sc[j] + o
        return [sc[j] * SCALE for j in range(KB)]

    def soft(ss, m, l):
        mb = ss[0]
        for j in range(1, KB):
            mb = jnp.maximum(mb, ss[j])
        mb = jnp.max(mb, axis=1, keepdims=True)
        m_new = mb if m is None else jnp.maximum(m, mb)
        ps = [jnp.exp(sj - m_new) for sj in ss]
        lb = ps[0]
        for j in range(1, KB):
            lb = lb + ps[j]
        if m is None:
            return ps, m_new, lb, None
        alpha = jnp.exp(m - m_new)
        return ps, m_new, l * alpha + lb, alpha

    def ctxc(b, ps, alpha, acc):
        if acc is not None:
            acc = [a * alpha for a in acc]
        else:
            acc = [None] * NC
        acc = list(acc)
        last = b == NB - 1
        seq = ([(j, ct) for ct in range(NC) for j in range(KB)] if last
               else [(j, ct) for j in range(KB) for ct in range(NC)])
        for j, ct in seq:
            kt = b * KB + j
            o = _dot(ps[j], _tile(ckvn, kt, ct))
            acc[ct] = o if acc[ct] is None else acc[ct] + o
        return acc

    s0 = scores(0)
    s1 = scores(1)
    p0, m, l, al0 = soft(s0, None, None)
    acc = ctxc(0, p0, None, None)
    s2 = scores(2)
    p1, m, l, al1 = soft(s1, m, l)
    acc = ctxc(1, p1, al1, acc)
    s3 = scores(3)
    p2, m, l, al2 = soft(s2, m, l)
    acc = ctxc(2, p2, al2, acc)
    p3, m, l, al3 = soft(s3, m, l)
    acc = ctxc(3, p3, al3, acc)
    linv = 1.0 / jnp.sum(l, axis=1, keepdims=True)

    accv = [[None] * NM for _ in range(3)]
    accm = [None] * NM

    def e_tiles(hs, cts, part):
        for ct in cts:
            for h in hs:
                g = h // 8
                o = _dot(acc[ct][g * 8:(g + 1) * 8], _tile(wuv, h, pl.ds(ct * 64, 64)))
                part[h] = o if h not in part else part[h] + o

    def head_ctx(h, part):
        g, r = divmod(h, 8)
        return part.pop(h)[r:r + 1] * linv[h:h + 1]

    def f_vpu(hs, part, accv):
        xbs = [_xb(head_ctx(h, part)) for h in hs]
        return _vmac3(accv, xbs, lambda j, s, n: o32[hs[j], pl.ds(s * 8, 8), pl.ds(n * 128, 128)])

    part = {}
    trip = [list(range(i, min(i + 3, OV))) for i in range(0, OV, 3)]
    e_tiles(trip[0], range(3), part)
    e_tiles(trip[1], range(3), part)
    e_tiles(trip[0], [3], part)
    accv = f_vpu(trip[0], part, accv)
    e_tiles(trip[1], [3], part)
    accv = f_vpu(trip[1], part, accv)
    for hs in trip[2:]:
        e_tiles(hs, range(NC), part)
        accv = f_vpu(hs, part, accv)
    lhs_m = {}
    for h in range(OV, H):
        e_tiles([h], range(NC), part)
        g, r = divmod(h, 8)
        lhs_m[h] = jnp.where(masks[r], part.pop(h) * linv[g * 8:(g + 1) * 8], 0.0)
    for n in range(NM):
        for h in range(OV, H):
            o = _dot(lhs_m[h], _tile(wo2, h, n))
            accm[n] = o if accm[n] is None else accm[n] + o
    x3 = [_rbf(x2[n] + _rbf(_rowsum(accm[n] + _fold3(accv, n)))) for n in range(NM)]
    mean3, rstd3 = _stats(x3)
    ln3 = [(x - mean3) * rstd3 for x in x3]
    sig3 = _router(ln3, wr)
    xb3 = list(enumerate(_xb_gather(x3[0])))
    KM = 128 - GX
    if GX:
        sub = lax.broadcasted_iota(i32, (8, 128), 0)
        for s in range(KM // 8, 16):
            xb3.append((16 + s, jnp.take_along_axis(x3[1], sub + 8 * s, axis=1,
                                                    mode="promise_in_bounds")))
    hh = {}
    for ft in GORD:
        srcs = (("g", g32, gt), ("u", u32s, ut)) if ft < 13 else (("g", g32, gt),)
        val = {}
        for nm, ref, mref in srcs:
            av_ = None
            for s, xs in xb3:
                p = xs * ref[ft, pl.ds(s * 8, 8), :]
                av_ = p if av_ is None else av_ + p
            om = None
            for kt in range(1, NM):
                if kt == 1 and GX:
                    a = _dot(x3[1][:, :KM], _tile(mref, ft, 1, pl.ds(0, KM // 2)))
                else:
                    a = _dot(x3[kt], _tile(mref, ft, kt))
                om = a if om is None else om + a
            cs_ = csg[ft] if nm == "g" else csu[ft]
            val[nm] = rstd3 * (om + _rowsum(av_) - mean3 * cs_)
        u = val["u"] if ft < 13 else pltpu.roll(val["g"], 64, 1)
        hh[ft] = _silu(val["g"]) * u
    y = [None] * NM
    for ft in range(DV, NF):
        for n in range(NM):
            o = down2(ft, n, hh[ft])
            y[n] = o if y[n] is None else y[n] + o
    yv = [[None] * NM for _ in range(3)]
    for i in range(0, DV, 3):
        fs = list(range(i, min(i + 3, DV)))
        yv = _vmac3(yv, [_xb(hh[ft][0:1]) for ft in fs],
                    lambda j, s, n: wd_f32(fs[j], s, n))
    y = [y[n] + _rowsum(_fold3(yv, n)) for n in range(NM)]
    x4 = [x3[n] + _rbf(ln3[n] + _rbf(y[n] * sig3)) for n in range(NM)]
    out = jnp.concatenate([x[0:1, :] for x in x4], axis=1)
    o_ref[0] = out.astype(bf16)


@jax.jit
def pallas_interleave_layers__compressed_kv_cla__moe_arch_mod__decode_kernel(
    A_x: jax.Array,
    A_c_kv: jax.Array,
    A_w_q: jax.Array,
    A_w_uk: jax.Array,
    A_w_uv: jax.Array,
    A_w_o: jax.Array,
    B_x: jax.Array,
    B_w_r: jax.Array,
    B_w_gate: jax.Array,
    B_w_up: jax.Array,
    B_w_down: jax.Array,
):
    del B_x
    any_spec = pl.BlockSpec(memory_space=pl.ANY)
    V = pltpu.VMEM
    scratch = [
        V((1, 1, M), bf16),
        V((NM, 128), bf16),
        V((M, H, D), bf16),
        V((DC, H, D), bf16),
        V((DC, H, D), bf16),
        V((NC, SK, 128), bf16),
        V((H, D, M), bf16),
        V((F, M), bf16),
        V((F, M), bf16),
        V((F, M), bf16),
        V((H, M // 2, D), u32),
        V((H, NC, D // 2, 128), u32),
        V((H, DC // 2, D), u32),
        V((NK, NC, 64, 128), u32),
        V((NK, NC, 64, 128), u32),
        V((NF, NM, 64, 128), u32),
        V((NF, NM, 64, 128), u32),
        V((NF, 256, 128), f32),
        V((NF, 256, 128), f32),
        V((DV * 128, M), f32),
        V((OV, D, M), f32),
        V((BV, NC, D, 128), f32),
        V((H, len(QV) * 128, D), f32),
        V((H, NM, 64, 128), u32),
        V((4, 8, 128), f32),
        V((NF, 8, 128), f32),
        V((NF, 8, 128), f32),
        V((NC, H, 128), f32),
        V((NC, H, 128), f32),
        V((4, 8, 128), f32),
        V((NF, 8, 128), f32),
        V((NM, 8, 128), f32),
        pltpu.SemaphoreType.DMA((40,)),
    ]
    return pl.pallas_call(
        _kernel,
        out_shape=jax.ShapeDtypeStruct((1, 1, M), bf16),
        in_specs=[any_spec] * 10,
        out_specs=pl.BlockSpec(memory_space=pltpu.VMEM),
        scratch_shapes=scratch,
        compiler_params=pltpu.CompilerParams(
            vmem_limit_bytes=100 * 1024 * 1024,
            disable_semaphore_checks=True,
        ),
    )(A_x, A_c_kv, A_w_q, A_w_uk, A_w_uv, A_w_o, B_w_r.reshape(NM, 128),
      B_w_gate.T, B_w_up.T, B_w_down)
```

```python
import functools

import jax
import jax.numpy as jnp
from jax import lax
import jax.experimental.pallas as pl
import jax.experimental.pallas.tpu as pltpu

f32 = jnp.float32
bf16 = jnp.bfloat16
u32 = jnp.uint32
i32 = jnp.int32

M = 640
H = 32
D = 128
DC = 512
SK = 4096
F = 1728
NM = M // 128
NC = DC // 128
NK = SK // 128
NF = 14
EPS = 1e-5
SCALE = float(D) ** -0.5
KB = 8
NB = NK // KB

QV = {2: 24, 3: 16}
BV = 12
OV = 21
DV = 8
GX = 32
CFIRST = 3
DRC = 384
DR0 = 768
DGROUPS = ((0, 1), (2, 3), (4,))
NE = DR0 // 128
GORD = list(range(10)) + [13, 10, 11, 12]


def _dot(a, b):
    return jnp.dot(a, b, preferred_element_type=f32)


def _rbf(x):
    return x.astype(bf16).astype(f32)


def _tile(ref, *idx):
    return pltpu.bitcast(ref[idx], bf16)


def _stats(xs):
    s = xs[0] + xs[1] + xs[2] + xs[3] + xs[4]
    mean = jnp.sum(s, axis=1, keepdims=True) * (1.0 / M)
    ds = [x - mean for x in xs]
    q = ds[0] * ds[0] + ds[1] * ds[1] + ds[2] * ds[2] + ds[3] * ds[3] + ds[4] * ds[4]
    var = jnp.sum(q, axis=1, keepdims=True) * (1.0 / M)
    rstd = 1.0 / jnp.sqrt(var + EPS)
    return mean, rstd


def _router(lns, wr):
    s = lns[0] * wr[0] + lns[1] * wr[1] + lns[2] * wr[2] + lns[3] * wr[3] + lns[4] * wr[4]
    r = jnp.sum(s, axis=1, keepdims=True)
    return jax.nn.sigmoid(r)


def _rowsum(x):
    return jnp.broadcast_to(jnp.sum(x, axis=0, keepdims=True), x.shape)


def _xb(row):
    t = jnp.broadcast_to(row, (128, 128)).T
    return [t[s * 8:(s + 1) * 8] for s in range(16)]


def _xb_gather(rows):
    sub = lax.broadcasted_iota(i32, (8, 128), 0)
    return [jnp.take_along_axis(rows, sub + 8 * s, axis=1, mode="promise_in_bounds")
            for s in range(16)]


def _vmac3(accs, xbs, load):
    accs = [list(a) for a in accs]
    for s in range(16):
        for j, xb in enumerate(xbs):
            for i in range(len(accs[j])):
                p = xb[s] * load(j, s, i)
                accs[j][i] = p if accs[j][i] is None else accs[j][i] + p
    return accs


def _fold3(accs, i):
    t = [a[i] for a in accs if a[i] is not None]
    return functools.reduce(lambda a, b: a + b, t)


def _silu(g):
    return g * jax.nn.sigmoid(g)


def _kernel(x_hbm, ckv_hbm, wq_hbm, wuk_hbm, wuv_hbm, wo_hbm, wr_hbm, wg_hbm, wu_hbm, wd_hbm,
            o_ref,
            x_v, wr_v, lq, luk, luv, lckv, lo, lg, lu, ld,
            wq, wukt, wuv, ckvt, ckvn, gt, ut, g32, u32s, d32, o32, b32, q32, wo2,
            csq, csg, csu, qa_s, cc_s, ctx_s, hh_s, x_s,
            sems):
    row8 = lax.broadcasted_iota(i32, (8, 128), 0)
    masks = [row8 == r for r in range(8)]

    copies = {}
    order = []

    def add(name, pairs):
        sem = sems.at[len(copies)]
        cs = [pltpu.make_async_copy(s, d, sem) for s, d in pairs]
        copies[name] = cs
        order.append(name)

    add("x", [(x_hbm, x_v)])
    add("wr", [(wr_hbm, wr_v)])
    for i in range(NM):
        add(("q", i), [(wq_hbm.at[pl.ds(i * 128, 128)], lq.at[pl.ds(i * 128, 128)])])
    for i in range(NC):
        add(("uk", i), [(wuk_hbm.at[pl.ds(i * 128, 128)], luk.at[pl.ds(i * 128, 128)])])
    ckv2 = ckv_hbm.at[0]
    for b in range(NB):
        add(("ckv", b), [(ckv2.at[pl.ds(b * 1024, 1024), pl.ds(ct * 128, 128)],
                          lckv.at[ct, pl.ds(b * 1024, 1024)]) for ct in range(NC)])
    FS = [(0, 896), (896, F - 896)]
    for i, (s, n) in enumerate(FS):
        add(("g", i), [(wg_hbm.at[pl.ds(s, n)], lg.at[pl.ds(s, n)])])
    for i, (s, n) in enumerate(FS):
        add(("u", i), [(wu_hbm.at[pl.ds(s, n)], lu.at[pl.ds(s, n)])])
    for i in range(NC):
        add(("uv", i), [(wuv_hbm.at[pl.ds(i * 128, 128)], luv.at[pl.ds(i * 128, 128)])])
    for g in range(4):
        add(("o", g), [(wo_hbm.at[pl.ds(g * 8, 8)], lo.at[pl.ds(g * 8, 8)])])
    for i in range(DR0 // DRC):
        add(("d", i), [(wd_hbm.at[pl.ds(i * DRC, DRC)], ld.at[pl.ds(i * DRC, DRC)])])
    for i, cols in enumerate(DGROUPS):
        c0, nc = cols[0] * 128, len(cols) * 128
        add(("dc", i), [(wd_hbm.at[pl.ds(DR0, F - DR0), pl.ds(c0, nc)],
                         ld.at[pl.ds(DR0, F - DR0), pl.ds(c0, nc)])])

    order = [("q", 0), "x", "wr"] + [n for n in order if n not in (("q", 0), "x", "wr")]
    for name in order:
        for c in copies[name]:
            c.start()

    def wait(name):
        for c in copies[name]:
            c.wait()

    names = list(copies)

    def wait_dyn(first_name, i, pairs_fn):
        base = names.index(first_name)
        for s, d in pairs_fn(i):
            pltpu.make_async_copy(s, d, sems.at[base + i]).wait()

    wait("x")
    wait("wr")
    xr = x_v[0].astype(f32)
    x0 = [jnp.broadcast_to(xr[:, n * 128:(n + 1) * 128], (8, 128)) for n in range(NM)]
    wrf = wr_v[...].astype(f32)
    wr = [jnp.broadcast_to(wrf[n:n + 1, :], (8, 128)) for n in range(NM)]
    for n in range(NM):
        x_s[n] = x0[n]
    mean0, rstd0 = _stats(x0)
    ones8 = jnp.ones((8, 128), f32)
    zero8 = jnp.zeros((8, 128), f32)

    def a_body(kt, carry):
        raw, cs = carry
        s = pl.multiple_of(kt * 128, 128)
        wait_dyn(("q", 0), kt, lambda i: [(wq_hbm.at[pl.ds(s, 128)], lq.at[pl.ds(s, 128)])])
        t = jnp.swapaxes(lq[pl.ds(s, 128)], 0, 1)
        s2 = pl.multiple_of(kt * 64, 64)
        for h in range(H):
            wq[h, pl.ds(s2, 64), :] = pltpu.bitcast(t[h], u32)
        for j, (ktv, h0) in enumerate(sorted(QV.items())):
            @pl.when(kt == ktv)
            def _():
                for h in range(h0, H):
                    w = wq[h, pl.ds(s2, 64), :]
                    q32[h, pl.ds(j * 128, 128), :] = pltpu.bitcast(w, bf16).astype(f32)
        lhs = jnp.concatenate([x_s[kt], ones8], axis=0)
        raw, cs = list(raw), list(cs)
        for h in range(H):
            g, r = divmod(h, 8)
            out = _dot(lhs, pltpu.bitcast(wq[h, pl.ds(s2, 64), :], bf16))
            raw[g] = jnp.where(masks[r], raw[g] + out[0:8], raw[g])
            cs[g] = jnp.where(masks[r], cs[g] + out[8:16], cs[g])
        return tuple(raw), tuple(cs)

    raw, cs = lax.fori_loop(0, NM, a_body, ((zero8,) * 4, (zero8,) * 4))
    for g in range(4):
        csq[g] = cs[g]
    q = [rstd0 * (raw[g] - mean0 * cs[g]) for g in range(4)]

    def b_body(ct, _):
        s = pl.multiple_of(ct * 128, 128)
        wait_dyn(("uk", 0), ct, lambda i: [(wuk_hbm.at[pl.ds(s, 128)], luk.at[pl.ds(s, 128)])])
        t = jnp.swapaxes(luk[pl.ds(s, 128)], 0, 1)
        for h in range(H):
            th = t[h].T
            wukt[h, ct] = pltpu.bitcast(th, u32)
            if h < BV:
                b32[h, ct] = th.astype(f32)
        qa = [zero8] * 4
        for h in range(H):
            g, r = divmod(h, 8)
            out = _dot(q[g], pltpu.bitcast(wukt[h, ct], bf16))
            qa[g] = jnp.where(masks[r], out, qa[g])
        qa_s[ct] = jnp.concatenate(qa, axis=0)
        return _

    lax.fori_loop(0, NC, b_body, 0)

    def cd_body(b, carry):
        m, l, acc = carry
        s = pl.multiple_of(b * 1024, 1024)
        wait_dyn(("ckv", 0), b, lambda i: [(ckv2.at[pl.ds(s, 1024), pl.ds(ct * 128, 128)],
                                            lckv.at[ct, pl.ds(s, 1024)]) for ct in range(NC)])
        ss = []
        for j in range(KB):
            kt = b * KB + j
            sk = pl.multiple_of(s + j * 128, 128)
            sc = None
            for ct in range(NC):
                t = lckv[ct, pl.ds(sk, 128), :]
                ckvn[kt, ct] = pltpu.bitcast(t, u32)
                t = t.T
                ckvt[kt, ct] = pltpu.bitcast(t, u32)
                o = _dot(qa_s[ct], t)
                sc = o if sc is None else sc + o
            ss.append(sc * SCALE)
        mb = ss[0]
        for j in range(1, KB):
            mb = jnp.maximum(mb, ss[j])
        m_new = jnp.maximum(m, jnp.max(mb, axis=1, keepdims=True))
        alpha = jnp.exp(m - m_new)
        ps = [jnp.exp(sj - m_new) for sj in ss]
        lb = ps[0]
        for j in range(1, KB):
            lb = lb + ps[j]
        l = l * alpha + lb
        acc = [a * alpha for a in acc]
        for j in range(KB):
            sk = pl.multiple_of(s + j * 128, 128)
            for ct in range(NC):
                acc[ct] = acc[ct] + _dot(ps[j], lckv[ct, pl.ds(sk, 128), :])
        return m_new, l, acc

    m_init = jnp.full((H, 128), -jnp.inf, f32)
    _, l, acc = lax.fori_loop(0, NB, cd_body,
                              (m_init, jnp.zeros((H, 128), f32),
                               [jnp.zeros((H, 128), f32)] * NC))
    linv = 1.0 / jnp.sum(l, axis=1, keepdims=True)
    for ct in range(NC):
        cc_s[ct] = acc[ct]

    def transpose_ffn(land, dst, dst32, fam):
        def body(ft, _):
            s = pl.multiple_of(ft * 128, 128)
            for kt in range(NM):
                t = land[pl.ds(s, 128), pl.ds(kt * 128, 128)].T
                dst[ft, kt] = pltpu.bitcast(t, u32)
                if kt < 2:
                    dst32[ft, pl.ds(kt * 128, 128), :] = t.astype(f32)
            return _
        wait((fam, 0))
        lax.fori_loop(0, 7, body, 0)
        wait((fam, 1))
        lax.fori_loop(7, 13, body, 0)

    transpose_ffn(lg, gt, g32, "g")
    transpose_ffn(lu, ut, u32s, "u")
    for kt in range(NM):
        t = jnp.concatenate([lg[pl.ds(13 * 128, 64), pl.ds(kt * 128, 128)],
                             lu[pl.ds(13 * 128, 64), pl.ds(kt * 128, 128)]], axis=0).T
        gt[13, kt] = pltpu.bitcast(t, u32)
        if kt < 2:
            g32[13, pl.ds(kt * 128, 128), :] = t.astype(f32)

    def e_body(ct, ctx):
        s = pl.multiple_of(ct * 128, 128)
        wait_dyn(("uv", 0), ct, lambda i: [(wuv_hbm.at[pl.ds(s, 128)], luv.at[pl.ds(s, 128)])])
        t = jnp.swapaxes(luv[pl.ds(s, 128)], 0, 1)
        s2 = pl.multiple_of(ct * 64, 64)
        for h in range(H):
            wuv[h, pl.ds(s2, 64), :] = pltpu.bitcast(t[h], u32)
        ctx = list(ctx)
        cc = cc_s[ct]
        for h in range(H):
            g, r = divmod(h, 8)
            out = _dot(cc[g * 8:(g + 1) * 8], pltpu.bitcast(wuv[h, pl.ds(s2, 64), :], bf16))
            ctx[g] = jnp.where(masks[r], ctx[g] + out, ctx[g])
        return tuple(ctx)

    ctx = lax.fori_loop(0, NC, e_body, (zero8,) * 4)
    for g in range(4):
        ctx_s[g] = ctx[g] * linv[g * 8:(g + 1) * 8]

    def f_body(g, acc):
        s = pl.multiple_of(g * 8, 8)
        wait_dyn(("o", 0), g, lambda i: [(wo_hbm.at[pl.ds(s, 8)], lo.at[pl.ds(s, 8)])])
        acc = list(acc)
        cg = ctx_s[g]
        for r in range(8):
            lhs = jnp.where(masks[r], cg, 0.0)
            for n in range(NM):
                t = lo[s + r, :, pl.ds(n * 128, 128)]
                wo2[s + r, n] = pltpu.bitcast(t, u32)
                acc[n] = acc[n] + _dot(lhs, t)
        for r in range(8):
            @pl.when(s + r < OV)
            def _():
                o32[jnp.minimum(s + r, OV - 1)] = lo[s + r].astype(f32)
        return tuple(acc)

    acc = lax.fori_loop(0, 4, f_body, (zero8,) * NM)
    x1 = [_rbf(x0[n] + _rbf(_rowsum(acc[n]))) for n in range(NM)]

    mean1, rstd1 = _stats(x1)
    ln1 = [(x - mean1) * rstd1 for x in x1]
    sig1 = _router(ln1, wr)
    lhs1 = [jnp.concatenate([x1[kt], ones8], axis=0) for kt in range(NM)]

    hh1 = []
    for ft in range(NF):
        og = ou = None
        for kt in range(NM):
            a = _dot(lhs1[kt], _tile(gt, ft, kt))
            og = a if og is None else og + a
            if ft < 13:
                b = _dot(lhs1[kt], _tile(ut, ft, kt))
                ou = b if ou is None else ou + b
        csg[ft] = og[8:16]
        g = rstd1 * (og[0:8] - mean1 * og[8:16])
        if ft < 13:
            csu[ft] = ou[8:16]
            u = rstd1 * (ou[0:8] - mean1 * ou[8:16])
        else:
            u = pltpu.roll(g, 64, 1)
        hh1.append(_silu(g) * u)
        if ft < NE:
            hh_s[ft] = hh1[ft]


    def wd_tile(ft, n):
        return ld[pl.ds(ft * 128, min(128, F - ft * 128)), pl.ds(n * 128, 128)]

    def down2(ft, n, hh):
        return _dot(hh if ft < 13 else hh[:, :64], wd_tile(ft, n))

    def wd_f32(ft, s, n):
        if ft < NE or n < 4:
            return d32[pl.ds(ft * 128 + s * 8, 8), pl.ds(n * 128, 128)]
        return wd_tile(ft, n).astype(f32)[s * 8:(s + 1) * 8]

    FPC = DRC // 128

    def h_body(i, y):
        s = pl.multiple_of(i * DRC, 128)
        wait_dyn(("d", 0), i, lambda _: [(wd_hbm.at[pl.ds(s, DRC)], ld.at[pl.ds(s, DRC)])])
        y = list(y)
        for j in range(FPC):
            ft = i * FPC + j
            sf = pl.multiple_of(s + j * 128, 128)
            hh = hh_s[ft]
            for n in range(NM):
                t = ld[pl.ds(sf, 128), pl.ds(n * 128, 128)]
                y[n] = y[n] + _dot(hh, t)
        for j in range(FPC):
            ft = i * FPC + j
            sf = pl.multiple_of(s + j * 128, 128)
            sd = pl.multiple_of(ft * 128, 128)
            d32[pl.ds(sd, 128), :] = ld[pl.ds(sf, 128), :].astype(f32)
        return tuple(y)

    y = list(lax.fori_loop(0, DR0 // DRC, h_body, (zero8,) * NM))

    x2 = [None] * NM
    racc = [None] * 4

    def h_late(n):
        for ft in range(NE, NF):
            y[n] = y[n] + down2(ft, n, hh1[ft])
        x2[n] = _rbf(x1[n] + _rbf(ln1[n] + _rbf(y[n] * sig1)))
        if n < 4:
            for ft in range(NE, DV):
                d32[pl.ds(ft * 128, 128), pl.ds(n * 128, 128)] = wd_tile(ft, n).astype(f32)

    def a_pass(kt, heads=range(H)):
        for h in heads:
            g, r = divmod(h, 8)
            o = _dot(jnp.where(masks[r], x2[kt], 0.0), _tile(wq, h, pl.ds(kt * 64, 64)))
            racc[g] = o if racc[g] is None else racc[g] + o

    def a_mxu(kt, heads=range(H)):
        a_pass(kt, [h for h in heads if h < QV.get(kt, H)])

    wait(("dc", 0))
    h_late(0)
    h_late(1)
    a_mxu(0)
    a_mxu(1)
    wait(("dc", 1))
    h_late(2)
    h_late(3)
    a_mxu(2)
    wait(("dc", 2))
    av = {}
    for j, (kt, h0) in enumerate(sorted(QV.items())):
        xb = _xb_gather(x2[kt])
        for h in range(h0, H):
            a = None
            for s in range(16):
                p = xb[s] * q32[h, pl.ds(j * 128 + s * 8, 8), :]
                a = p if a is None else a + p
            av[h] = a if h not in av else av[h] + a
    h_late(4)
    a_mxu(3, range(0, 16))
    mean2, rstd2 = _stats(x2)
    raw = {}
    KL = DGROUPS[-1][-1]
    last = {}
    for h in range(BV):
        last[h] = _dot(x2[KL], _tile(wq, h, pl.ds(KL * 64, 64)))
    a_mxu(3, range(16, H))
    for h in range(BV, H):
        last[h] = _dot(x2[KL], _tile(wq, h, pl.ds(KL * 64, 64)))
    for h in range(H):
        raw[h] = racc[h // 8] + last[h]
        if h in av:
            raw[h] = raw[h] + _rowsum(av[h])
    qv = {}
    for i in range(0, BV, 3):
        hs = list(range(i, min(i + 3, BV)))
        xbs = []
        for h in hs:
            g, r = divmod(h, 8)
            qh = raw[h][r:r + 1] - mean2[0:1] * csq[g, pl.ds(r, 1), :]
            xbs.append(_xb(qh))
        accs = _vmac3([[None] * NC for _ in hs], xbs,
                      lambda j, s, ct: b32[hs[j], ct, pl.ds(s * 8, 8), :])
        for j, h in enumerate(hs):
            for ct in range(NC):
                qv[h, ct] = _rowsum(accs[j][ct]) * rstd2
    q = {}
    for g in range(BV // 8, 4):
        rawg = zero8
        for r in range(8):
            if g * 8 + r >= BV:
                rawg = jnp.where(masks[r], raw[g * 8 + r], rawg)
        q[g] = rstd2 * (rawg - mean2 * csq[g])
    qa = []
    for ct in range(NC):
        qg = [zero8] * 4
        for h in range(H):
            g, r = divmod(h, 8)
            o = qv[h, ct] if h < BV else _dot(q[g], _tile(wukt, h, ct))
            qg[g] = jnp.where(masks[r], o, qg[g])
        qa.append(jnp.concatenate(qg, axis=0))

    def scores(b):
        sc = {}
        first = CFIRST if b == 0 else 0
        seq = [(j, ct) for ct in range(NC) for j in range(first)]
        seq += [(j, ct) for j in range(first, KB) for ct in range(NC)]
        for j, ct in seq:
            o = _dot(qa[ct], _tile(ckvt, b * KB + j, ct))
            sc[j] = o if j not in sc else sc[j] + o
        return [sc[j] * SCALE for j in range(KB)]

    def soft(ss, m, l):
        mb = ss[0]
        for j in range(1, KB):
            mb = jnp.maximum(mb, ss[j])
        mb = jnp.max(mb, axis=1, keepdims=True)
        m_new = mb if m is None else jnp.maximum(m, mb)
        ps = [jnp.exp(sj - m_new) for sj in ss]
        lb = ps[0]
        for j in range(1, KB):
            lb = lb + ps[j]
        if m is None:
            return ps, m_new, lb, None
        alpha = jnp.exp(m - m_new)
        return ps, m_new, l * alpha + lb, alpha

    def ctxc(b, ps, alpha, acc):
        if acc is not None:
            acc = [a * alpha for a in acc]
        else:
            acc = [None] * NC
        acc = list(acc)
        last = b == NB - 1
        seq = ([(j, ct) for ct in range(NC) for j in range(KB)] if last
               else [(j, ct) for j in range(KB) for ct in range(NC)])
        for j, ct in seq:
            kt = b * KB + j
            o = _dot(ps[j], _tile(ckvn, kt, ct))
            acc[ct] = o if acc[ct] is None else acc[ct] + o
        return acc

    s0 = scores(0)
    s1 = scores(1)
    p0, m, l, al0 = soft(s0, None, None)
    acc = ctxc(0, p0, None, None)
    s2 = scores(2)
    p1, m, l, al1 = soft(s1, m, l)
    acc = ctxc(1, p1, al1, acc)
    s3 = scores(3)
    p2, m, l, al2 = soft(s2, m, l)
    acc = ctxc(2, p2, al2, acc)
    p3, m, l, al3 = soft(s3, m, l)
    acc = ctxc(3, p3, al3, acc)
    linv = 1.0 / jnp.sum(l, axis=1, keepdims=True)

    accv = [[None] * NM for _ in range(3)]
    accm = [None] * NM

    def e_tiles(hs, cts, part):
        for ct in cts:
            for h in hs:
                g = h // 8
                o = _dot(acc[ct][g * 8:(g + 1) * 8], _tile(wuv, h, pl.ds(ct * 64, 64)))
                part[h] = o if h not in part else part[h] + o

    def head_ctx(h, part):
        g, r = divmod(h, 8)
        return part.pop(h)[r:r + 1] * linv[h:h + 1]

    def f_vpu(hs, part, accv):
        xbs = [_xb(head_ctx(h, part)) for h in hs]
        return _vmac3(accv, xbs, lambda j, s, n: o32[hs[j], pl.ds(s * 8, 8), pl.ds(n * 128, 128)])

    part = {}
    trip = [list(range(i, min(i + 3, OV))) for i in range(0, OV, 3)]
    e_tiles(trip[0], range(3), part)
    e_tiles(trip[1], range(3), part)
    e_tiles(trip[0], [3], part)
    accv = f_vpu(trip[0], part, accv)
    e_tiles(trip[1], [3], part)
    accv = f_vpu(trip[1], part, accv)
    for hs in trip[2:]:
        e_tiles(hs, range(NC), part)
        accv = f_vpu(hs, part, accv)
    lhs_m = {}
    for h in range(OV, H):
        e_tiles([h], range(NC), part)
        g, r = divmod(h, 8)
        lhs_m[h] = jnp.where(masks[r], part.pop(h) * linv[g * 8:(g + 1) * 8], 0.0)
    for n in range(NM):
        for h in range(OV, H):
            o = _dot(lhs_m[h], _tile(wo2, h, n))
            accm[n] = o if accm[n] is None else accm[n] + o
    x3 = [_rbf(x2[n] + _rbf(_rowsum(accm[n] + _fold3(accv, n)))) for n in range(NM)]
    mean3, rstd3 = _stats(x3)
    ln3 = [(x - mean3) * rstd3 for x in x3]
    sig3 = _router(ln3, wr)
    xb3 = list(enumerate(_xb_gather(x3[0])))
    KM = 128 - GX
    if GX:
        sub = lax.broadcasted_iota(i32, (8, 128), 0)
        for s in range(KM // 8, 16):
            xb3.append((16 + s, jnp.take_along_axis(x3[1], sub + 8 * s, axis=1,
                                                    mode="promise_in_bounds")))
    hh = {}
    for ft in GORD:
        srcs = (("g", g32, gt), ("u", u32s, ut)) if ft < 13 else (("g", g32, gt),)
        val = {}
        for nm, ref, mref in srcs:
            av_ = None
            for s, xs in xb3:
                p = xs * ref[ft, pl.ds(s * 8, 8), :]
                av_ = p if av_ is None else av_ + p
            om = None
            for kt in range(1, NM):
                if kt == 1 and GX:
                    a = _dot(x3[1][:, :KM], _tile(mref, ft, 1, pl.ds(0, KM // 2)))
                else:
                    a = _dot(x3[kt], _tile(mref, ft, kt))
                om = a if om is None else om + a
            cs_ = csg[ft] if nm == "g" else csu[ft]
            val[nm] = rstd3 * (om + _rowsum(av_) - mean3 * cs_)
        u = val["u"] if ft < 13 else pltpu.roll(val["g"], 64, 1)
        hh[ft] = _silu(val["g"]) * u
    y = [None] * NM
    for ft in [t for t in GORD if t >= DV]:
        for n in range(NM):
            o = down2(ft, n, hh[ft])
            y[n] = o if y[n] is None else y[n] + o
    yv = [[None] * NM for _ in range(3)]
    for i in range(0, DV, 3):
        fs = list(range(i, min(i + 3, DV)))
        yv = _vmac3(yv, [_xb(hh[ft][0:1]) for ft in fs],
                    lambda j, s, n: wd_f32(fs[j], s, n))
    y = [y[n] + _rowsum(_fold3(yv, n)) for n in range(NM)]
    x4 = [x3[n] + _rbf(ln3[n] + _rbf(y[n] * sig3)) for n in range(NM)]
    out = jnp.concatenate([x[0:1, :] for x in x4], axis=1)
    o_ref[0] = out.astype(bf16)


@jax.jit
def pallas_interleave_layers__compressed_kv_cla__moe_arch_mod__decode_kernel(
    A_x: jax.Array,
    A_c_kv: jax.Array,
    A_w_q: jax.Array,
    A_w_uk: jax.Array,
    A_w_uv: jax.Array,
    A_w_o: jax.Array,
    B_x: jax.Array,
    B_w_r: jax.Array,
    B_w_gate: jax.Array,
    B_w_up: jax.Array,
    B_w_down: jax.Array,
):
    del B_x
    any_spec = pl.BlockSpec(memory_space=pl.ANY)
    V = pltpu.VMEM
    scratch = [
        V((1, 1, M), bf16),
        V((NM, 128), bf16),
        V((M, H, D), bf16),
        V((DC, H, D), bf16),
        V((DC, H, D), bf16),
        V((NC, SK, 128), bf16),
        V((H, D, M), bf16),
        V((F, M), bf16),
        V((F, M), bf16),
        V((F, M), bf16),
        V((H, M // 2, D), u32),
        V((H, NC, D // 2, 128), u32),
        V((H, DC // 2, D), u32),
        V((NK, NC, 64, 128), u32),
        V((NK, NC, 64, 128), u32),
        V((NF, NM, 64, 128), u32),
        V((NF, NM, 64, 128), u32),
        V((NF, 256, 128), f32),
        V((NF, 256, 128), f32),
        V((DV * 128, M), f32),
        V((OV, D, M), f32),
        V((BV, NC, D, 128), f32),
        V((H, len(QV) * 128, D), f32),
        V((H, NM, 64, 128), u32),
        V((4, 8, 128), f32),
        V((NF, 8, 128), f32),
        V((NF, 8, 128), f32),
        V((NC, H, 128), f32),
        V((NC, H, 128), f32),
        V((4, 8, 128), f32),
        V((NF, 8, 128), f32),
        V((NM, 8, 128), f32),
        pltpu.SemaphoreType.DMA((40,)),
    ]
    return pl.pallas_call(
        _kernel,
        out_shape=jax.ShapeDtypeStruct((1, 1, M), bf16),
        in_specs=[any_spec] * 10,
        out_specs=pl.BlockSpec(memory_space=pltpu.VMEM),
        scratch_shapes=scratch,
        compiler_params=pltpu.CompilerParams(
            vmem_limit_bytes=100 * 1024 * 1024,
            disable_semaphore_checks=True,
        ),
    )(A_x, A_c_kv, A_w_q, A_w_uk, A_w_uv, A_w_o, B_w_r.reshape(NM, 128),
      B_w_gate.T, B_w_up.T, B_w_down)
```

```python
import functools

import jax
import jax.numpy as jnp
from jax import lax
import jax.experimental.pallas as pl
import jax.experimental.pallas.tpu as pltpu

f32 = jnp.float32
bf16 = jnp.bfloat16
u32 = jnp.uint32
i32 = jnp.int32

M = 640
H = 32
D = 128
DC = 512
SK = 4096
F = 1728
NM = M // 128
NC = DC // 128
NK = SK // 128
NF = 14
EPS = 1e-5
SCALE = float(D) ** -0.5
KB = 8
NB = NK // KB

QV = {2: 20, 3: 16}
BV = 12
OV = 21
DV = 8
GX = 32
CFIRST = 3
DRC = 384
DR0 = 768
DGROUPS = ((0, 1), (2, 3), (4,))
NE = DR0 // 128
GORD = list(range(10)) + [13, 10, 11, 12]


def _dot(a, b):
    return jnp.dot(a, b, preferred_element_type=f32)


def _rbf(x):
    return x.astype(bf16).astype(f32)


def _tile(ref, *idx):
    return pltpu.bitcast(ref[idx], bf16)


def _stats(xs):
    s = xs[0] + xs[1] + xs[2] + xs[3] + xs[4]
    mean = jnp.sum(s, axis=1, keepdims=True) * (1.0 / M)
    ds = [x - mean for x in xs]
    q = ds[0] * ds[0] + ds[1] * ds[1] + ds[2] * ds[2] + ds[3] * ds[3] + ds[4] * ds[4]
    var = jnp.sum(q, axis=1, keepdims=True) * (1.0 / M)
    rstd = 1.0 / jnp.sqrt(var + EPS)
    return mean, rstd


def _router(lns, wr):
    s = lns[0] * wr[0] + lns[1] * wr[1] + lns[2] * wr[2] + lns[3] * wr[3] + lns[4] * wr[4]
    r = jnp.sum(s, axis=1, keepdims=True)
    return jax.nn.sigmoid(r)


def _rowsum(x):
    return jnp.broadcast_to(jnp.sum(x, axis=0, keepdims=True), x.shape)


def _xb(row):
    t = jnp.broadcast_to(row, (128, 128)).T
    return [t[s * 8:(s + 1) * 8] for s in range(16)]


def _xb_gather(rows):
    sub = lax.broadcasted_iota(i32, (8, 128), 0)
    return [jnp.take_along_axis(rows, sub + 8 * s, axis=1, mode="promise_in_bounds")
            for s in range(16)]


def _vmac3(accs, xbs, load):
    accs = [list(a) for a in accs]
    for s in range(16):
        for j, xb in enumerate(xbs):
            for i in range(len(accs[j])):
                p = xb[s] * load(j, s, i)
                accs[j][i] = p if accs[j][i] is None else accs[j][i] + p
    return accs


def _fold3(accs, i):
    t = [a[i] for a in accs if a[i] is not None]
    return functools.reduce(lambda a, b: a + b, t)


def _silu(g):
    return g * jax.nn.sigmoid(g)


def _kernel(x_hbm, ckv_hbm, wq_hbm, wuk_hbm, wuv_hbm, wo_hbm, wr_hbm, wg_hbm, wu_hbm, wd_hbm,
            o_ref,
            x_v, wr_v, lq, luk, luv, lckv, lo, lg, lu, ld,
            wq, wukt, wuv, ckvt, ckvn, gt, ut, g32, u32s, d32, o32, b32, q32, wo2,
            csq, csg, csu, qa_s, cc_s, ctx_s, hh_s, x_s,
            sems):
    row8 = lax.broadcasted_iota(i32, (8, 128), 0)
    masks = [row8 == r for r in range(8)]

    copies = {}
    order = []

    def add(name, pairs):
        sem = sems.at[len(copies)]
        cs = [pltpu.make_async_copy(s, d, sem) for s, d in pairs]
        copies[name] = cs
        order.append(name)

    add("x", [(x_hbm, x_v)])
    add("wr", [(wr_hbm, wr_v)])
    for i in range(NM):
        add(("q", i), [(wq_hbm.at[pl.ds(i * 128, 128)], lq.at[pl.ds(i * 128, 128)])])
    for i in range(NC):
        add(("uk", i), [(wuk_hbm.at[pl.ds(i * 128, 128)], luk.at[pl.ds(i * 128, 128)])])
    ckv2 = ckv_hbm.at[0]
    for b in range(NB):
        add(("ckv", b), [(ckv2.at[pl.ds(b * 1024, 1024), pl.ds(ct * 128, 128)],
                          lckv.at[ct, pl.ds(b * 1024, 1024)]) for ct in range(NC)])
    FS = [(0, 896), (896, F - 896)]
    for i, (s, n) in enumerate(FS):
        add(("g", i), [(wg_hbm.at[pl.ds(s, n)], lg.at[pl.ds(s, n)])])
    for i, (s, n) in enumerate(FS):
        add(("u", i), [(wu_hbm.at[pl.ds(s, n)], lu.at[pl.ds(s, n)])])
    for i in range(NC):
        add(("uv", i), [(wuv_hbm.at[pl.ds(i * 128, 128)], luv.at[pl.ds(i * 128, 128)])])
    for g in range(4):
        add(("o", g), [(wo_hbm.at[pl.ds(g * 8, 8)], lo.at[pl.ds(g * 8, 8)])])
    for i in range(DR0 // DRC):
        add(("d", i), [(wd_hbm.at[pl.ds(i * DRC, DRC)], ld.at[pl.ds(i * DRC, DRC)])])
    for i, cols in enumerate(DGROUPS):
        c0, nc = cols[0] * 128, len(cols) * 128
        add(("dc", i), [(wd_hbm.at[pl.ds(DR0, F - DR0), pl.ds(c0, nc)],
                         ld.at[pl.ds(DR0, F - DR0), pl.ds(c0, nc)])])

    order = [("q", 0), "x", "wr"] + [n for n in order if n not in (("q", 0), "x", "wr")]
    for name in order:
        for c in copies[name]:
            c.start()

    def wait(name):
        for c in copies[name]:
            c.wait()

    names = list(copies)

    def wait_dyn(first_name, i, pairs_fn):
        base = names.index(first_name)
        for s, d in pairs_fn(i):
            pltpu.make_async_copy(s, d, sems.at[base + i]).wait()

    wait("x")
    wait("wr")
    xr = x_v[0].astype(f32)
    x0 = [jnp.broadcast_to(xr[:, n * 128:(n + 1) * 128], (8, 128)) for n in range(NM)]
    wrf = wr_v[...].astype(f32)
    wr = [jnp.broadcast_to(wrf[n:n + 1, :], (8, 128)) for n in range(NM)]
    for n in range(NM):
        x_s[n] = x0[n]
    mean0, rstd0 = _stats(x0)
    ones8 = jnp.ones((8, 128), f32)
    zero8 = jnp.zeros((8, 128), f32)

    def a_body(kt, carry):
        raw, cs = carry
        s = pl.multiple_of(kt * 128, 128)
        wait_dyn(("q", 0), kt, lambda i: [(wq_hbm.at[pl.ds(s, 128)], lq.at[pl.ds(s, 128)])])
        t = jnp.swapaxes(lq[pl.ds(s, 128)], 0, 1)
        s2 = pl.multiple_of(kt * 64, 64)
        for h in range(H):
            wq[h, pl.ds(s2, 64), :] = pltpu.bitcast(t[h], u32)
        for j, (ktv, h0) in enumerate(sorted(QV.items())):
            @pl.when(kt == ktv)
            def _():
                for h in range(h0, H):
                    w = wq[h, pl.ds(s2, 64), :]
                    q32[h, pl.ds(j * 128, 128), :] = pltpu.bitcast(w, bf16).astype(f32)
        lhs = jnp.concatenate([x_s[kt], ones8], axis=0)
        raw, cs = list(raw), list(cs)
        for h in range(H):
            g, r = divmod(h, 8)
            out = _dot(lhs, pltpu.bitcast(wq[h, pl.ds(s2, 64), :], bf16))
            raw[g] = jnp.where(masks[r], raw[g] + out[0:8], raw[g])
            cs[g] = jnp.where(masks[r], cs[g] + out[8:16], cs[g])
        return tuple(raw), tuple(cs)

    raw, cs = lax.fori_loop(0, NM, a_body, ((zero8,) * 4, (zero8,) * 4))
    for g in range(4):
        csq[g] = cs[g]
    q = [rstd0 * (raw[g] - mean0 * cs[g]) for g in range(4)]

    def b_body(ct, _):
        s = pl.multiple_of(ct * 128, 128)
        wait_dyn(("uk", 0), ct, lambda i: [(wuk_hbm.at[pl.ds(s, 128)], luk.at[pl.ds(s, 128)])])
        t = jnp.swapaxes(luk[pl.ds(s, 128)], 0, 1)
        for h in range(H):
            th = t[h].T
            wukt[h, ct] = pltpu.bitcast(th, u32)
            if h < BV:
                b32[h, ct] = th.astype(f32)
        qa = [zero8] * 4
        for h in range(H):
            g, r = divmod(h, 8)
            out = _dot(q[g], pltpu.bitcast(wukt[h, ct], bf16))
            qa[g] = jnp.where(masks[r], out, qa[g])
        qa_s[ct] = jnp.concatenate(qa, axis=0)
        return _

    lax.fori_loop(0, NC, b_body, 0)

    def cd_body(b, carry):
        m, l, acc = carry
        s = pl.multiple_of(b * 1024, 1024)
        wait_dyn(("ckv", 0), b, lambda i: [(ckv2.at[pl.ds(s, 1024), pl.ds(ct * 128, 128)],
                                            lckv.at[ct, pl.ds(s, 1024)]) for ct in range(NC)])
        ss = []
        for j in range(KB):
            kt = b * KB + j
            sk = pl.multiple_of(s + j * 128, 128)
            sc = None
            for ct in range(NC):
                t = lckv[ct, pl.ds(sk, 128), :]
                ckvn[kt, ct] = pltpu.bitcast(t, u32)
                t = t.T
                ckvt[kt, ct] = pltpu.bitcast(t, u32)
                o = _dot(qa_s[ct], t)
                sc = o if sc is None else sc + o
            ss.append(sc * SCALE)
        mb = ss[0]
        for j in range(1, KB):
            mb = jnp.maximum(mb, ss[j])
        m_new = jnp.maximum(m, jnp.max(mb, axis=1, keepdims=True))
        alpha = jnp.exp(m - m_new)
        ps = [jnp.exp(sj - m_new) for sj in ss]
        lb = ps[0]
        for j in range(1, KB):
            lb = lb + ps[j]
        l = l * alpha + lb
        acc = [a * alpha for a in acc]
        for j in range(KB):
            sk = pl.multiple_of(s + j * 128, 128)
            for ct in range(NC):
                acc[ct] = acc[ct] + _dot(ps[j], lckv[ct, pl.ds(sk, 128), :])
        return m_new, l, acc

    m_init = jnp.full((H, 128), -jnp.inf, f32)
    _, l, acc = lax.fori_loop(0, NB, cd_body,
                              (m_init, jnp.zeros((H, 128), f32),
                               [jnp.zeros((H, 128), f32)] * NC))
    linv = 1.0 / jnp.sum(l, axis=1, keepdims=True)
    for ct in range(NC):
        cc_s[ct] = acc[ct]

    def transpose_ffn(land, dst, dst32, fam):
        def body(ft, _):
            s = pl.multiple_of(ft * 128, 128)
            for kt in range(NM):
                t = land[pl.ds(s, 128), pl.ds(kt * 128, 128)].T
                dst[ft, kt] = pltpu.bitcast(t, u32)
                if kt < 2:
                    dst32[ft, pl.ds(kt * 128, 128), :] = t.astype(f32)
            return _
        wait((fam, 0))
        lax.fori_loop(0, 7, body, 0)
        wait((fam, 1))
        lax.fori_loop(7, 13, body, 0)

    transpose_ffn(lg, gt, g32, "g")
    transpose_ffn(lu, ut, u32s, "u")
    for kt in range(NM):
        t = jnp.concatenate([lg[pl.ds(13 * 128, 64), pl.ds(kt * 128, 128)],
                             lu[pl.ds(13 * 128, 64), pl.ds(kt * 128, 128)]], axis=0).T
        gt[13, kt] = pltpu.bitcast(t, u32)
        if kt < 2:
            g32[13, pl.ds(kt * 128, 128), :] = t.astype(f32)

    def e_body(ct, ctx):
        s = pl.multiple_of(ct * 128, 128)
        wait_dyn(("uv", 0), ct, lambda i: [(wuv_hbm.at[pl.ds(s, 128)], luv.at[pl.ds(s, 128)])])
        t = jnp.swapaxes(luv[pl.ds(s, 128)], 0, 1)
        s2 = pl.multiple_of(ct * 64, 64)
        for h in range(H):
            wuv[h, pl.ds(s2, 64), :] = pltpu.bitcast(t[h], u32)
        ctx = list(ctx)
        cc = cc_s[ct]
        for h in range(H):
            g, r = divmod(h, 8)
            out = _dot(cc[g * 8:(g + 1) * 8], pltpu.bitcast(wuv[h, pl.ds(s2, 64), :], bf16))
            ctx[g] = jnp.where(masks[r], ctx[g] + out, ctx[g])
        return tuple(ctx)

    ctx = lax.fori_loop(0, NC, e_body, (zero8,) * 4)
    for g in range(4):
        ctx_s[g] = ctx[g] * linv[g * 8:(g + 1) * 8]

    def f_body(g, acc):
        s = pl.multiple_of(g * 8, 8)
        wait_dyn(("o", 0), g, lambda i: [(wo_hbm.at[pl.ds(s, 8)], lo.at[pl.ds(s, 8)])])
        acc = list(acc)
        cg = ctx_s[g]
        for r in range(8):
            lhs = jnp.where(masks[r], cg, 0.0)
            for n in range(NM):
                t = lo[s + r, :, pl.ds(n * 128, 128)]
                wo2[s + r, n] = pltpu.bitcast(t, u32)
                acc[n] = acc[n] + _dot(lhs, t)
        for r in range(8):
            @pl.when(s + r < OV)
            def _():
                o32[jnp.minimum(s + r, OV - 1)] = lo[s + r].astype(f32)
        return tuple(acc)

    acc = lax.fori_loop(0, 4, f_body, (zero8,) * NM)
    x1 = [_rbf(x0[n] + _rbf(_rowsum(acc[n]))) for n in range(NM)]

    mean1, rstd1 = _stats(x1)
    ln1 = [(x - mean1) * rstd1 for x in x1]
    sig1 = _router(ln1, wr)
    lhs1 = [jnp.concatenate([x1[kt], ones8], axis=0) for kt in range(NM)]

    hh1 = []
    for ft in range(NF):
        og = ou = None
        for kt in range(NM):
            a = _dot(lhs1[kt], _tile(gt, ft, kt))
            og = a if og is None else og + a
            if ft < 13:
                b = _dot(lhs1[kt], _tile(ut, ft, kt))
                ou = b if ou is None else ou + b
        csg[ft] = og[8:16]
        g = rstd1 * (og[0:8] - mean1 * og[8:16])
        if ft < 13:
            csu[ft] = ou[8:16]
            u = rstd1 * (ou[0:8] - mean1 * ou[8:16])
        else:
            u = pltpu.roll(g, 64, 1)
        hh1.append(_silu(g) * u)
        if ft < NE:
            hh_s[ft] = hh1[ft]


    def wd_tile(ft, n):
        return ld[pl.ds(ft * 128, min(128, F - ft * 128)), pl.ds(n * 128, 128)]

    def down2(ft, n, hh):
        return _dot(hh if ft < 13 else hh[:, :64], wd_tile(ft, n))

    def wd_f32(ft, s, n):
        if ft < NE or n < 4:
            return d32[pl.ds(ft * 128 + s * 8, 8), pl.ds(n * 128, 128)]
        return wd_tile(ft, n).astype(f32)[s * 8:(s + 1) * 8]

    FPC = DRC // 128

    def h_body(i, y):
        s = pl.multiple_of(i * DRC, 128)
        wait_dyn(("d", 0), i, lambda _: [(wd_hbm.at[pl.ds(s, DRC)], ld.at[pl.ds(s, DRC)])])
        y = list(y)
        for j in range(FPC):
            ft = i * FPC + j
            sf = pl.multiple_of(s + j * 128, 128)
            hh = hh_s[ft]
            for n in range(NM):
                t = ld[pl.ds(sf, 128), pl.ds(n * 128, 128)]
                y[n] = y[n] + _dot(hh, t)
        for j in range(FPC):
            ft = i * FPC + j
            sf = pl.multiple_of(s + j * 128, 128)
            sd = pl.multiple_of(ft * 128, 128)
            d32[pl.ds(sd, 128), :] = ld[pl.ds(sf, 128), :].astype(f32)
        return tuple(y)

    y = list(lax.fori_loop(0, DR0 // DRC, h_body, (zero8,) * NM))

    x2 = [None] * NM
    racc = [None] * 4

    def h_late(n):
        for ft in range(NE, NF):
            y[n] = y[n] + down2(ft, n, hh1[ft])
        x2[n] = _rbf(x1[n] + _rbf(ln1[n] + _rbf(y[n] * sig1)))
        if n < 4:
            for ft in range(NE, DV):
                d32[pl.ds(ft * 128, 128), pl.ds(n * 128, 128)] = wd_tile(ft, n).astype(f32)

    def a_pass(kt, heads=range(H)):
        for h in heads:
            g, r = divmod(h, 8)
            o = _dot(jnp.where(masks[r], x2[kt], 0.0), _tile(wq, h, pl.ds(kt * 64, 64)))
            racc[g] = o if racc[g] is None else racc[g] + o

    def a_mxu(kt, heads=range(H)):
        a_pass(kt, [h for h in heads if h < QV.get(kt, H)])

    wait(("dc", 0))
    h_late(0)
    h_late(1)
    a_mxu(0)
    a_mxu(1)
    wait(("dc", 1))
    h_late(2)
    h_late(3)
    a_mxu(2)
    av = {}

    def a_vpu(j, kt, h0):
        xb = _xb_gather(x2[kt])
        for h in range(h0, H):
            a = None
            for s in range(16):
                p = xb[s] * q32[h, pl.ds(j * 128 + s * 8, 8), :]
                a = p if a is None else a + p
            av[h] = a if h not in av else av[h] + a

    a_vpu(0, 2, QV[2])
    wait(("dc", 2))
    a_vpu(1, 3, QV[3])
    h_late(4)
    a_mxu(3, range(0, 16))
    mean2, rstd2 = _stats(x2)
    raw = {}
    KL = DGROUPS[-1][-1]
    last = {}
    for h in range(BV):
        last[h] = _dot(x2[KL], _tile(wq, h, pl.ds(KL * 64, 64)))
    a_mxu(3, range(16, H))
    for h in range(BV, H):
        last[h] = _dot(x2[KL], _tile(wq, h, pl.ds(KL * 64, 64)))
    for h in range(H):
        raw[h] = racc[h // 8] + last[h]
        if h in av:
            raw[h] = raw[h] + _rowsum(av[h])
    qv = {}
    for i in range(0, BV, 3):
        hs = list(range(i, min(i + 3, BV)))
        xbs = []
        for h in hs:
            g, r = divmod(h, 8)
            qh = raw[h][r:r + 1] - mean2[0:1] * csq[g, pl.ds(r, 1), :]
            xbs.append(_xb(qh))
        accs = _vmac3([[None] * NC for _ in hs], xbs,
                      lambda j, s, ct: b32[hs[j], ct, pl.ds(s * 8, 8), :])
        for j, h in enumerate(hs):
            for ct in range(NC):
                qv[h, ct] = _rowsum(accs[j][ct]) * rstd2
    q = {}
    for g in range(BV // 8, 4):
        rawg = zero8
        for r in range(8):
            if g * 8 + r >= BV:
                rawg = jnp.where(masks[r], raw[g * 8 + r], rawg)
        q[g] = rstd2 * (rawg - mean2 * csq[g])
    qa = []
    for ct in range(NC):
        qg = [zero8] * 4
        for h in range(H):
            g, r = divmod(h, 8)
            o = qv[h, ct] if h < BV else _dot(q[g], _tile(wukt, h, ct))
            qg[g] = jnp.where(masks[r], o, qg[g])
        qa.append(jnp.concatenate(qg, axis=0))

    def scores(b):
        sc = {}
        first = CFIRST if b == 0 else 0
        seq = [(j, ct) for ct in range(NC) for j in range(first)]
        seq += [(j, ct) for j in range(first, KB) for ct in range(NC)]
        for j, ct in seq:
            o = _dot(qa[ct], _tile(ckvt, b * KB + j, ct))
            sc[j] = o if j not in sc else sc[j] + o
        return [sc[j] * SCALE for j in range(KB)]

    def soft(ss, m, l):
        mb = ss[0]
        for j in range(1, KB):
            mb = jnp.maximum(mb, ss[j])
        mb = jnp.max(mb, axis=1, keepdims=True)
        m_new = mb if m is None else jnp.maximum(m, mb)
        ps = [jnp.exp(sj - m_new) for sj in ss]
        lb = ps[0]
        for j in range(1, KB):
            lb = lb + ps[j]
        if m is None:
            return ps, m_new, lb, None
        alpha = jnp.exp(m - m_new)
        return ps, m_new, l * alpha + lb, alpha

    def ctxc(b, ps, alpha, acc):
        if acc is not None:
            acc = [a * alpha for a in acc]
        else:
            acc = [None] * NC
        acc = list(acc)
        last = b == NB - 1
        seq = ([(j, ct) for ct in range(NC) for j in range(KB)] if last
               else [(j, ct) for j in range(KB) for ct in range(NC)])
        for j, ct in seq:
            kt = b * KB + j
            o = _dot(ps[j], _tile(ckvn, kt, ct))
            acc[ct] = o if acc[ct] is None else acc[ct] + o
        return acc

    s0 = scores(0)
    s1 = scores(1)
    p0, m, l, al0 = soft(s0, None, None)
    acc = ctxc(0, p0, None, None)
    s2 = scores(2)
    p1, m, l, al1 = soft(s1, m, l)
    acc = ctxc(1, p1, al1, acc)
    s3 = scores(3)
    p2, m, l, al2 = soft(s2, m, l)
    acc = ctxc(2, p2, al2, acc)
    p3, m, l, al3 = soft(s3, m, l)
    acc = ctxc(3, p3, al3, acc)
    linv = 1.0 / jnp.sum(l, axis=1, keepdims=True)

    accv = [[None] * NM for _ in range(3)]
    accm = [None] * NM

    def e_tiles(hs, cts, part):
        for ct in cts:
            for h in hs:
                g = h // 8
                o = _dot(acc[ct][g * 8:(g + 1) * 8], _tile(wuv, h, pl.ds(ct * 64, 64)))
                part[h] = o if h not in part else part[h] + o

    def head_ctx(h, part):
        g, r = divmod(h, 8)
        return part.pop(h)[r:r + 1] * linv[h:h + 1]

    def f_vpu(hs, part, accv):
        xbs = [_xb(head_ctx(h, part)) for h in hs]
        return _vmac3(accv, xbs, lambda j, s, n: o32[hs[j], pl.ds(s * 8, 8), pl.ds(n * 128, 128)])

    part = {}
    trip = [list(range(i, min(i + 3, OV))) for i in range(0, OV, 3)]
    e_tiles(trip[0], range(3), part)
    e_tiles(trip[1], range(3), part)
    e_tiles(trip[0], [3], part)
    accv = f_vpu(trip[0], part, accv)
    e_tiles(trip[1], [3], part)
    accv = f_vpu(trip[1], part, accv)
    for hs in trip[2:]:
        e_tiles(hs, range(NC), part)
        accv = f_vpu(hs, part, accv)
    lhs_m = {}
    for h in range(OV, H):
        e_tiles([h], range(NC), part)
        g, r = divmod(h, 8)
        lhs_m[h] = jnp.where(masks[r], part.pop(h) * linv[g * 8:(g + 1) * 8], 0.0)
    for n in range(NM):
        for h in range(OV, H):
            o = _dot(lhs_m[h], _tile(wo2, h, n))
            accm[n] = o if accm[n] is None else accm[n] + o
    x3 = [_rbf(x2[n] + _rbf(_rowsum(accm[n] + _fold3(accv, n)))) for n in range(NM)]
    mean3, rstd3 = _stats(x3)
    ln3 = [(x - mean3) * rstd3 for x in x3]
    sig3 = _router(ln3, wr)
    xb3 = list(enumerate(_xb_gather(x3[0])))
    KM = 128 - GX
    if GX:
        sub = lax.broadcasted_iota(i32, (8, 128), 0)
        for s in range(KM // 8, 16):
            xb3.append((16 + s, jnp.take_along_axis(x3[1], sub + 8 * s, axis=1,
                                                    mode="promise_in_bounds")))
    hh = {}
    for ft in GORD:
        srcs = (("g", g32, gt), ("u", u32s, ut)) if ft < 13 else (("g", g32, gt),)
        val = {}
        for nm, ref, mref in srcs:
            av_ = None
            for s, xs in xb3:
                p = xs * ref[ft, pl.ds(s * 8, 8), :]
                av_ = p if av_ is None else av_ + p
            om = None
            for kt in range(1, NM):
                if kt == 1 and GX:
                    a = _dot(x3[1][:, :KM], _tile(mref, ft, 1, pl.ds(0, KM // 2)))
                else:
                    a = _dot(x3[kt], _tile(mref, ft, kt))
                om = a if om is None else om + a
            cs_ = csg[ft] if nm == "g" else csu[ft]
            val[nm] = rstd3 * (om + _rowsum(av_) - mean3 * cs_)
        u = val["u"] if ft < 13 else pltpu.roll(val["g"], 64, 1)
        hh[ft] = _silu(val["g"]) * u
    y = [None] * NM
    for ft in [t for t in GORD if t >= DV]:
        for n in range(NM):
            o = down2(ft, n, hh[ft])
            y[n] = o if y[n] is None else y[n] + o
    yv = [[None] * NM for _ in range(3)]
    for i in range(0, DV, 3):
        fs = list(range(i, min(i + 3, DV)))
        yv = _vmac3(yv, [_xb(hh[ft][0:1]) for ft in fs],
                    lambda j, s, n: wd_f32(fs[j], s, n))
    y = [y[n] + _rowsum(_fold3(yv, n)) for n in range(NM)]
    x4 = [x3[n] + _rbf(ln3[n] + _rbf(y[n] * sig3)) for n in range(NM)]
    out = jnp.concatenate([x[0:1, :] for x in x4], axis=1)
    o_ref[0] = out.astype(bf16)


@jax.jit
def pallas_interleave_layers__compressed_kv_cla__moe_arch_mod__decode_kernel(
    A_x: jax.Array,
    A_c_kv: jax.Array,
    A_w_q: jax.Array,
    A_w_uk: jax.Array,
    A_w_uv: jax.Array,
    A_w_o: jax.Array,
    B_x: jax.Array,
    B_w_r: jax.Array,
    B_w_gate: jax.Array,
    B_w_up: jax.Array,
    B_w_down: jax.Array,
):
    del B_x
    any_spec = pl.BlockSpec(memory_space=pl.ANY)
    V = pltpu.VMEM
    scratch = [
        V((1, 1, M), bf16),
        V((NM, 128), bf16),
        V((M, H, D), bf16),
        V((DC, H, D), bf16),
        V((DC, H, D), bf16),
        V((NC, SK, 128), bf16),
        V((H, D, M), bf16),
        V((F, M), bf16),
        V((F, M), bf16),
        V((F, M), bf16),
        V((H, M // 2, D), u32),
        V((H, NC, D // 2, 128), u32),
        V((H, DC // 2, D), u32),
        V((NK, NC, 64, 128), u32),
        V((NK, NC, 64, 128), u32),
        V((NF, NM, 64, 128), u32),
        V((NF, NM, 64, 128), u32),
        V((NF, 256, 128), f32),
        V((NF, 256, 128), f32),
        V((DV * 128, M), f32),
        V((OV, D, M), f32),
        V((BV, NC, D, 128), f32),
        V((H, len(QV) * 128, D), f32),
        V((H, NM, 64, 128), u32),
        V((4, 8, 128), f32),
        V((NF, 8, 128), f32),
        V((NF, 8, 128), f32),
        V((NC, H, 128), f32),
        V((NC, H, 128), f32),
        V((4, 8, 128), f32),
        V((NF, 8, 128), f32),
        V((NM, 8, 128), f32),
        pltpu.SemaphoreType.DMA((40,)),
    ]
    return pl.pallas_call(
        _kernel,
        out_shape=jax.ShapeDtypeStruct((1, 1, M), bf16),
        in_specs=[any_spec] * 10,
        out_specs=pl.BlockSpec(memory_space=pltpu.VMEM),
        scratch_shapes=scratch,
        compiler_params=pltpu.CompilerParams(
            vmem_limit_bytes=100 * 1024 * 1024,
            disable_semaphore_checks=True,
        ),
    )(A_x, A_c_kv, A_w_q, A_w_uk, A_w_uv, A_w_o, B_w_r.reshape(NM, 128),
      B_w_gate.T, B_w_up.T, B_w_down)
```
